```python
import jax
import jax.numpy as jnp

def _softmax(x, axis=-1):
    return jax.nn.softmax(x, axis=axis)
def _gelu(x):
    return jax.nn.gelu(x, approximate=True)
def _silu(x):
    return jax.nn.silu(x)
def _sigmoid(x):
    return jax.nn.sigmoid(x)
def _layernorm(x, axis=-1, eps=1e-5):
    m = jnp.mean(x, axis=axis, keepdims=True)
    v = jnp.var(x, axis=axis, keepdims=True)
    return (x - m) / jnp.sqrt(v + eps)
def _scatter_add(tgt, idx, src, axis=0):
    return tgt.at[idx].add(src)
def _segment_sum(src, seg, n):
    return jax.ops.segment_sum(src, seg, n)
class _Rng:
    def __init__(self, key):
        self._k = key
    def _next(self):
        self._k, sub = jax.random.split(self._k)
        return sub
    def normal(self, shape):
        return jax.random.normal(self._next(), shape, dtype=jnp.bfloat16)
    def randint(self, lo, hi, shape):
        return jax.random.randint(self._next(), shape, lo, hi, dtype=jnp.int32)
    def uniform(self, shape, lo=0.0, hi=1.0):
        return jax.random.uniform(self._next(), shape, jnp.bfloat16, lo, hi)
    def permutation(self, n):
        return jax.random.permutation(self._next(), n)


kernel_name = 'interleave_layers__sliding_block_cached__glu_gated_swiglu__decode'

def setup_inputs():
    _rng = _Rng(jax.random.key(int.from_bytes(__import__("os").urandom(4), "little")))
    _w = (lambda a: (lambda t: t.astype(jnp.bfloat16) if jnp.issubdtype(t.dtype, jnp.floating) else t)(jnp.asarray(a)))
    def _A_setup():
        B, Sq, D = 1, 1, 640
        Hq, Hkv, Sk, Dh = 32, 32, 32768, 192
        assert Hq % Hkv == 0, (Hq, Hkv)
        return {
            "x": _w((lambda *s: _rng.normal(s) * 0.05)(B, Sq, D)),
            "k_cache": _w((lambda *s: _rng.normal(s) * 0.05)(B, Hkv, Sk, Dh)),
            "v_cache": _w((lambda *s: _rng.normal(s) * 0.05)(B, Hkv, Sk, Dh)),
            "wq": _w((lambda *s: _rng.normal(s) * 0.05)(D, Hq * Dh) * (D ** -0.5)),
            "wo": _w((lambda *s: _rng.normal(s) * 0.05)(Hq * Dh, D) * ((Hq * Dh) ** -0.5)),
        }
    _A_in = _A_setup()

    def _B_setup():
        B, S, D, F = 1, 1, 640, 1536
        return {
            "x": _w((lambda *s: _rng.normal(s) * 0.05)(B, S, D)),
            "w1": _w((lambda *s: _rng.normal(s) * 0.05)(D, F) * (2.0 / D) ** 0.5),
            "w3": _w((lambda *s: _rng.normal(s) * 0.05)(D, F) * (2.0 / D) ** 0.5),
            "w2": _w((lambda *s: _rng.normal(s) * 0.05)(F, D) * (2.0 / F) ** 0.5),
        }
    _B_in = _B_setup()

    return {
        "A_x": _A_in["x"],
        "A_k_cache": _A_in["k_cache"],
        "A_v_cache": _A_in["v_cache"],
        "A_wq": _A_in["wq"],
        "A_wo": _A_in["wo"],
        "B_x": _B_in["x"],
        "B_w1": _B_in["w1"],
        "B_w3": _B_in["w3"],
        "B_w2": _B_in["w2"],
    }

def reference(A_x, A_k_cache, A_v_cache, A_wq, A_wo, B_x, B_w1, B_w3, B_w2):
    def _A_ref(x, k_cache, v_cache, wq, wo):
        B, Sq, D = x.shape
        Hq, Dh = 32, 192
        Hkv, Sk = k_cache.shape[1], k_cache.shape[2]
        W = min(4096, max(256, Sk // 4))
        rep = Hq // Hkv
        q = (lambda x, *d: x.transpose(*d))((x @ wq).reshape(B, Sq, Hq, Dh), 0, 2, 1, 3)
        k = jnp.repeat(k_cache[:, :, Sk - W:, :], rep, axis=1)
        v = jnp.repeat(v_cache[:, :, Sk - W:, :], rep, axis=1)
        scores = jnp.einsum("bhqd,bhkd->bhqk", q, k) * (Dh ** -0.5)
        p = _softmax(scores, axis=-1)
        o = jnp.einsum("bhqk,bhkd->bhqd", p, v)
        return (lambda x, *d: x.transpose(*d))(o, 0, 2, 1, 3).reshape(B, Sq, Hq * Dh) @ wo

    def _B_ref(x, w1, w3, w2):
        gate = jnp.einsum("bsd,df->bsf", x, w1)
        up = jnp.einsum("bsd,df->bsf", x, w3)
        h = _silu(gate) * up
        out = jnp.einsum("bsf,fd->bsd", h, w2)
        return out

    x = A_x
    x = x + _A_ref(_layernorm(x, axis=-1), A_k_cache, A_v_cache, A_wq, A_wo)
    x = x + _B_ref(_layernorm(x, axis=-1), B_w1, B_w3, B_w2)
    x = x + _A_ref(_layernorm(x, axis=-1), A_k_cache, A_v_cache, A_wq, A_wo)
    x = x + _B_ref(_layernorm(x, axis=-1), B_w1, B_w3, B_w2)
    return x
```

```python
import jax
import jax.numpy as jnp
from jax import lax
import jax.experimental.pallas as pl
import jax.experimental.pallas.tpu as pltpu

D = 640
H = 32
DH = 192
F = 1536
LANES = 128
EPS = 1e-5

NP = H // 2
PG = 2 * DH // 16
PW = 2 * DH


def _tile_view(w):
    r, c = w.shape
    return jnp.swapaxes(w.reshape(r // 16, 2, 8, c // LANES, LANES), 2, 3)


def _layernorm(x):
    m = jnp.mean(x, axis=-1, keepdims=True)
    xc = x - m
    v = jnp.mean(xc * xc, axis=-1, keepdims=True)
    return xc * lax.rsqrt(v + EPS)


def _rhs(w32, g0, ng, c):
    w = w32[pl.ds(g0, ng), c]
    return pltpu.bitcast(w.reshape(ng * 8, LANES), jnp.bfloat16)


def _make_kernel(n_tiles_total, n_tiles):
    c0 = n_tiles_total - n_tiles
    scale = DH ** -0.5

    def kernel(x_ref, k_hbm, v_hbm, wq_hbm, wo_hbm, w1_hbm, w3_hbm, w2_hbm,
               o_ref,
               kbuf, vbuf, wqbuf, wobuf, w1buf, w3buf, w2buf,
               q_ref, att_ref, ksem, vsem, wsem):
        def kv_copy(src, dst, sem, p, par):
            return pltpu.make_async_copy(
                src.at[pl.ds(p * PG, PG), par, pl.ds(c0, n_tiles)],
                dst.at[pl.ds(p * PG, PG), :, pl.ds(8 * par, 8), :],
                sem.at[2 * p + par])

        def w_copy(src, dst, idx, par):
            return pltpu.make_async_copy(
                src.at[:, par], dst.at[:, :, pl.ds(8 * par, 8), :],
                wsem.at[2 * idx + par])

        def start_kv(p):
            for par in range(2):
                kv_copy(k_hbm, kbuf, ksem, p, par).start()
            for par in range(2):
                kv_copy(v_hbm, vbuf, vsem, p, par).start()

        weights = [(wq_hbm, wqbuf), (wo_hbm, wobuf), (w1_hbm, w1buf),
                   (w3_hbm, w3buf), (w2_hbm, w2buf)]

        def start_w(i):
            for par in range(2):
                w_copy(*weights[i], i, par).start()

        def wait_w(i):
            for par in range(2):
                w_copy(*weights[i], i, par).wait()

        start_w(0)
        start_kv(0)
        start_kv(1)

        k32 = kbuf.bitcast(jnp.uint32)
        v32 = vbuf.bitcast(jnp.uint32)
        wq32 = wqbuf.bitcast(jnp.uint32)
        wo32 = wobuf.bitcast(jnp.uint32)
        w132 = w1buf.bitcast(jnp.uint32)
        w332 = w3buf.bitcast(jnp.uint32)
        w232 = w2buf.bitcast(jnp.uint32)

        row = lax.broadcasted_iota(jnp.int32, (16, PW), 0)
        lane = lax.broadcasted_iota(jnp.int32, (16, PW), 1)
        blockdiag = (row < 8) == (lane < DH)
        lane8 = lax.broadcasted_iota(jnp.int32, (8, PW), 1)

        def qproj(x):
            xn = jnp.broadcast_to(_layernorm(x), (16, D)).astype(jnp.bfloat16)
            for p in range(NP):
                rhs = jnp.concatenate(
                    [_rhs(wq32, 0, D // 16, 3 * p + t) for t in range(3)], axis=1)
                q = jnp.dot(xn, rhs, preferred_element_type=jnp.float32)
                q_ref[p] = jnp.where(blockdiag, q, 0.0).astype(jnp.bfloat16)

        def attend(p):
            kt = jnp.concatenate(
                [_rhs(k32, p * PG, PG, c) for c in range(n_tiles)], axis=1)
            s = jnp.dot(q_ref[p], kt, preferred_element_type=jnp.float32) * scale
            m = jnp.max(s, axis=-1, keepdims=True)
            e = jnp.exp(s - m)
            l = jnp.sum(e, axis=-1, keepdims=True)
            return e.astype(jnp.bfloat16), l

        def attend_v(p, e, l):
            vt = jnp.concatenate(
                [_rhs(v32, p * PG, PG, c) for c in range(n_tiles)], axis=1)
            o = lax.dot_general(e, vt, (((1,), (1,)), ((), ())),
                                preferred_element_type=jnp.float32)
            o = o / l
            att_ref[p] = jnp.where(lane8 < DH, o[0:8], o[8:16])

        def oproj():
            o = jnp.concatenate([att_ref[p] for p in range(NP)], axis=1)
            rhs = jnp.concatenate(
                [_rhs(wo32, 0, H * DH // 16, c) for c in range(D // LANES)], axis=1)
            y = jnp.dot(o.astype(jnp.bfloat16), rhs,
                        preferred_element_type=jnp.float32)
            return y[0:1]

        def ffn_up(x):
            xn = jnp.broadcast_to(_layernorm(x), (8, D)).astype(jnp.bfloat16)
            r1 = jnp.concatenate(
                [_rhs(w132, 0, D // 16, c) for c in range(F // LANES)], axis=1)
            r3 = jnp.concatenate(
                [_rhs(w332, 0, D // 16, c) for c in range(F // LANES)], axis=1)
            g = jnp.dot(xn, r1, preferred_element_type=jnp.float32)
            u = jnp.dot(xn, r3, preferred_element_type=jnp.float32)
            return (g * jax.nn.sigmoid(g) * u).astype(jnp.bfloat16)

        def ffn_down(hh):
            r2 = jnp.concatenate(
                [_rhs(w232, 0, F // 16, c) for c in range(D // LANES)], axis=1)
            y = jnp.dot(hh, r2, preferred_element_type=jnp.float32)
            return y[0:1]

        x = x_ref[...].astype(jnp.float32)

        wait_w(0)
        qproj(x)

        def body1(p, carry):
            @pl.when(p + 2 < NP)
            def _():
                start_kv(p + 2)

            @pl.when(p + 2 == NP)
            def _():
                for i in range(1, 5):
                    start_w(i)

            for par in range(2):
                kv_copy(k_hbm, kbuf, ksem, p, par).wait()
            e, l = attend(p)
            for par in range(2):
                kv_copy(v_hbm, vbuf, vsem, p, par).wait()
            attend_v(p, e, l)
            return carry

        lax.fori_loop(0, NP, body1, 0)
        wait_w(1)
        x = x + oproj()
        wait_w(2)
        wait_w(3)
        hh = ffn_up(x)
        wait_w(4)
        x = x + ffn_down(hh)
        qproj(x)

        def body2(p, carry):
            e, l = attend(p)
            attend_v(p, e, l)
            return carry

        lax.fori_loop(0, NP, body2, 0)
        x = x + oproj()
        x = x + ffn_down(ffn_up(x))
        o_ref[...] = x.astype(o_ref.dtype)

    return kernel


@jax.jit
def pallas_interleave_layers__sliding_block_cached__glu_gated_swiglu__decode_kernel(
    A_x: jax.Array,
    A_k_cache: jax.Array,
    A_v_cache: jax.Array,
    A_wq: jax.Array,
    A_wo: jax.Array,
    B_x: jax.Array,
    B_w1: jax.Array,
    B_w3: jax.Array,
    B_w2: jax.Array,
):
    sk = A_k_cache.shape[2]
    win = min(4096, max(256, sk // 4))
    nt_total, nt = sk // LANES, win // LANES

    def kv_view(a):
        return _tile_view(jnp.swapaxes(a, 2, 3).reshape(H * DH, sk))

    def wbuf(r, c):
        return pltpu.VMEM((r // 16, c // LANES, 16, LANES), jnp.bfloat16)

    any_spec = pl.BlockSpec(memory_space=pl.ANY)
    vmem_spec = pl.BlockSpec(memory_space=pltpu.VMEM)
    out = pl.pallas_call(
        _make_kernel(nt_total, nt),
        out_shape=jax.ShapeDtypeStruct((1, D), A_x.dtype),
        in_specs=[vmem_spec] + [any_spec] * 7,
        out_specs=vmem_spec,
        scratch_shapes=[
            wbuf(H * DH, win), wbuf(H * DH, win),
            wbuf(D, H * DH), wbuf(H * DH, D),
            wbuf(D, F), wbuf(D, F), wbuf(F, D),
            pltpu.VMEM((NP, 16, PW), jnp.bfloat16),
            pltpu.VMEM((NP, 8, PW), jnp.float32),
            pltpu.SemaphoreType.DMA((2 * NP,)),
            pltpu.SemaphoreType.DMA((2 * NP,)),
            pltpu.SemaphoreType.DMA((10,)),
        ],
        compiler_params=pltpu.CompilerParams(
            vmem_limit_bytes=126 * 1024 * 1024),
    )(A_x.reshape(1, D), kv_view(A_k_cache), kv_view(A_v_cache),
      _tile_view(A_wq), _tile_view(A_wo),
      _tile_view(B_w1), _tile_view(B_w3), _tile_view(B_w2))
    return out.reshape(A_x.shape)
```

```python
import functools
import math

import jax
import jax.numpy as jnp
from jax import lax
import jax.experimental.pallas as pl
import jax.experimental.pallas.tpu as pltpu

D = 640
H = 32
DH = 192
F = 1536
LANES = 128
EPS = 1e-5

NP = H // 2
PG = 2 * DH // 16
HG = DH // 16
PW = 2 * DH
NQC = H * DH // LANES
DT = D // LANES
FT = F // LANES

GP = 4
NGRP = NP // GP
W2_SPLIT = (0, 40, 72, 88, 96)

SPLIT = 17
PAD = 3

U32 = jnp.uint32
BF = jnp.bfloat16
F32 = jnp.float32


def _tile_view(w):
    r, c = w.shape
    return jnp.swapaxes(w.reshape(r // 16, 2, 8, c // LANES, LANES), 2, 3)


def _layernorm(x):
    m = jnp.mean(x, axis=-1, keepdims=True)
    xc = x - m
    v = jnp.mean(xc * xc, axis=-1, keepdims=True)
    return xc * lax.rsqrt(v + EPS)


def _rhs(w32, g0, ng, c):
    w = w32[pl.ds(g0, ng), c]
    return pltpu.bitcast(w.reshape(ng * 8, LANES), BF)


def _pack2(lo, hi):
    return pltpu.bitcast(jnp.concatenate([lo, hi], axis=0).astype(BF), U32)


def _make_kernel(n_tiles_total, nc):
    c0 = n_tiles_total - nc
    qscale = DH ** -0.5 * math.log2(math.e)
    prow = 2 * nc

    def kernel(x_hbm, k_hbm, v_hbm, wq_hbm, wo_hbm, w1_hbm, w3_hbm, w2_hbm,
               o_ref,
               kbuf, vbuf, wqbuf, wobuf, w1buf, w3buf, w2buf,
               t_ref, lhs_ref, s_ref, p_ref, linv_ref, ob_ref, mask_ref,
               xn_ref, y_ref, xbuf, ksem, vsem, wsem):
        def kv_copies(src, dst, sem, g):
            return [pltpu.make_async_copy(
                src.at[pl.ds(g * GP * PG, GP * PG), par, pl.ds(c0, nc)],
                dst.at[pl.ds(g * GP * PG, GP * PG), :, pl.ds(8 * par, 8), :],
                sem.at[g]) for par in range(2)]

        def w_copies(src, dst, idx, g0=0, g1=None):
            g1 = src.shape[0] if g1 is None else g1
            return [pltpu.make_async_copy(
                src.at[pl.ds(g0, g1 - g0), par],
                dst.at[pl.ds(g0, g1 - g0), :, pl.ds(8 * par, 8), :],
                wsem.at[idx]) for par in range(2)]

        x_copy = [pltpu.make_async_copy(x_hbm, xbuf, wsem.at[0])]
        wq_copy = w_copies(wq_hbm, wqbuf, 1)
        wo_copy = w_copies(wo_hbm, wobuf, 2)
        w1_copy = w_copies(w1_hbm, w1buf, 3)
        w3_copy = w_copies(w3_hbm, w3buf, 4)
        w2_copy = [w_copies(w2_hbm, w2buf, 5 + i, W2_SPLIT[i], W2_SPLIT[i + 1])
                   for i in range(len(W2_SPLIT) - 1)]

        def start(copies):
            for cp in copies:
                cp.start()

        def wait(copies):
            for cp in copies:
                cp.wait()

        start(wq_copy)
        start(x_copy)
        for g in range(NGRP):
            start(kv_copies(k_hbm, kbuf, ksem, g))
            start(kv_copies(v_hbm, vbuf, vsem, g))
        start(wo_copy)
        start(w1_copy)
        start(w3_copy)
        for cps in w2_copy:
            start(cps)

        k32 = kbuf.bitcast(U32)
        v32 = vbuf.bitcast(U32)
        wq32 = wqbuf.bitcast(U32)
        wo32 = wobuf.bitcast(U32)
        w132 = w1buf.bitcast(U32)
        w332 = w3buf.bitcast(U32)
        w232 = w2buf.bitcast(U32)

        sub = lax.broadcasted_iota(jnp.int32, (8, LANES), 0)
        lane = lax.broadcasted_iota(jnp.int32, (8, LANES), 1)
        lane3 = lax.broadcasted_iota(jnp.int32, (8, PW), 1)

        for r in range(8):
            half = U32(0x0000FFFF if r % 2 == 0 else 0xFFFF0000)
            lo = jnp.where(sub == r // 2, half, U32(0))
            hi = jnp.where(sub == 4 + r // 2, half, U32(0))
            mask_ref[r] = lo
            mask_ref[8 + r] = jnp.where(lane < DH - LANES, lo, hi)
            mask_ref[16 + r] = hi
        for i in range(PAD):
            t_ref[i] = jnp.zeros(t_ref.shape[1:], F32)
            linv_ref[i] = jnp.zeros(linv_ref.shape[1:], F32)
            ob_ref[i] = jnp.zeros(ob_ref.shape[1:], U32)
        p_ref[pl.ds(NP * prow, 32), :] = jnp.zeros((32, LANES), F32)

        def dot(l32, r):
            return jnp.dot(pltpu.bitcast(l32, BF), r, preferred_element_type=F32)

        def plain_dot(l32, r, free):
            del free
            return dot(l32, r)

        def stage_q(col, mm=plain_dot):
            acc = None
            for kk in range(DT):
                d = mm(xn_ref[:, pl.ds(kk * LANES, LANES)],
                       _rhs(wq32, 8 * kk, 8, col), True)[0:8]
                acc = d if acc is None else acc + d
            acc = acc * qscale
            q = _pack2(acc, acc)
            t = col % 3
            for r in range(8):
                lhs_ref[8 * col + r] = q & mask_ref[8 * t + r]

        def stage_qk(p, mm=plain_dot):
            for k in range(nc // 8):
                sa = sb = None
                for r in range(8):
                    c = 8 * k + r
                    r0 = mm(lhs_ref[PG * p + r], _rhs(k32, p * PG, 8, c), True)
                    r1 = mm(lhs_ref[PG * p + 8 + r], _rhs(k32, p * PG + 8, 8, c), None)
                    r2 = mm(lhs_ref[PG * p + 16 + r], _rhs(k32, p * PG + 16, 8, c), False)
                    a = r0[0:8] + r1[0:8]
                    b = r1[8:16] + r2[8:16]
                    sa = a if sa is None else sa + a
                    sb = b if sb is None else sb + b
                s_ref[p, pl.ds(8 * k, 8), :] = sa
                s_ref[p, pl.ds(nc + 8 * k, 8), :] = sb

        def prow_of(p, off):
            r = p * prow + off
            return r if isinstance(r, int) else pl.multiple_of(r, 8)

        def stage_softmax(p):
            ls = []
            for hd in range(2):
                s = s_ref[p, pl.ds(hd * nc, nc), :]
                m = jnp.max(jnp.max(s, axis=0, keepdims=True), axis=1, keepdims=True)
                e = jnp.exp2(s - m)
                p_ref[pl.ds(prow_of(p, hd * nc), nc), :] = e
                ls.append(jnp.sum(jnp.sum(e, axis=0, keepdims=True),
                                  axis=1, keepdims=True))
            linv_ref[PAD + p, :, 0:PW] = jnp.where(lane3 < DH, 1.0 / ls[0], 1.0 / ls[1])

        def p_bcast(p, hd, c):
            return p_ref[pl.ds(p * prow + hd * nc + c, 8, stride=0), :]

        def pv_chain(p, g):
            lo = hi = None
            for c in range(nc):
                w = pltpu.bitcast(v32[p * PG + g, c], BF).astype(F32)
                pb = p_bcast(p, g // HG, c)
                tl = w[0:8] * pb
                th = w[8:16] * pb
                lo = tl if lo is None else lo + tl
                hi = th if hi is None else hi + th
            t_ref[PAD + p, pl.ds(16 * g, 8), :] = lo
            t_ref[PAD + p, pl.ds(16 * g + 8, 8), :] = hi
            return lo, hi

        def pv_mxu(p):
            acc = [None] * 4
            for c in range(nc):
                l = pltpu.bitcast(_pack2(p_bcast(p, 0, c), p_bcast(p, 1, c)), BF)
                rs = [lax.dot_general(l, _rhs(v32, p * PG + 8 * t, 8, c),
                                      (((1,), (1,)), ((), ())),
                                      preferred_element_type=F32) for t in range(3)]
                parts = (rs[0][0:8], rs[1][0:8], rs[1][8:16], rs[2][8:16])
                acc = [x if a is None else a + x for a, x in zip(acc, parts)]
            o = jnp.concatenate(
                [acc[0], jnp.where(lane < DH - LANES, acc[1], acc[2]), acc[3]], axis=1)
            o = o * linv_ref[PAD + p, :, 0:PW]
            ob_ref[PAD + p, :, 0:PW] = _pack2(o, o)

        def stage_reduce(p):
            o = jnp.sum(t_ref[PAD + p].T, axis=0, keepdims=True)
            o = o * linv_ref[PAD + p, :, 0:PW]
            ob_ref[PAD + p, :, 0:PW] = _pack2(o, o)

        def stage_wo(p, pw, mm=plain_dot):
            for c in range(DT):
                acc = y_ref[:, pl.ds(c * LANES, LANES)]
                for t in range(3):
                    acc = acc + mm(ob_ref[PAD + p, :, pl.ds(t * LANES, LANES)],
                                   _rhs(wo32, pw * PG + 8 * t, 8, c), True)[0:8]
                y_ref[:, pl.ds(c * LANES, LANES)] = acc

        def set_xn(x):
            xn = _layernorm(x)
            xn_ref[:, 0:D] = _pack2(xn, xn)

        def ffn_up():
            hs = []
            for c in range(FT):
                g = u = None
                for kk in range(DT):
                    l = xn_ref[:, pl.ds(kk * LANES, LANES)]
                    dg = dot(l, _rhs(w132, 8 * kk, 8, c))[0:8]
                    du = dot(l, _rhs(w332, 8 * kk, 8, c))[0:8]
                    g = dg if g is None else g + dg
                    u = du if u is None else u + du
                hh = g * jax.nn.sigmoid(g) * u
                hs.append(_pack2(hh, hh))
            return hs

        def ffn_down(x, hs, k0, k1):
            cols = []
            for c in range(DT):
                acc = x[:, c * LANES:(c + 1) * LANES]
                for kk in range(k0, k1):
                    acc = acc + dot(hs[kk], _rhs(w232, 8 * kk, 8, c))[0:8]
                cols.append(acc)
            return jnp.concatenate(cols, axis=1)

        wait(x_copy)
        x = jnp.broadcast_to(xbuf[...].astype(F32), (8, D))
        set_xn(x)
        y_ref[:, 0:D] = x
        wait(wq_copy)

        def qloop(i, carry):
            for t in range(4):
                stage_q(4 * i + t)
            return carry

        lax.fori_loop(0, NQC // 4, qloop, 0)

        def group1(g, fence_row):
            wait(kv_copies(k_hbm, kbuf, ksem, g))

            def scores(j, carry):
                p = g * GP + j
                stage_qk(p)
                stage_softmax(p)
                return carry

            lax.fori_loop(0, GP, scores, 0)
            wait(kv_copies(v_hbm, vbuf, vsem, g))

            def values(j, carry):
                pv_mxu(g * GP + j)
                return carry

            lax.fori_loop(0, GP, values, 0)
            return fence_row + GP * prow

        fence_row = lax.fori_loop(0, NGRP, group1, 8)
        fence_row = pl.multiple_of(fence_row, 8)
        wait(wo_copy)

        def woloop(p, carry):
            stage_wo(p, p)
            return carry

        lax.fori_loop(0, NP, woloop, 0)
        x = y_ref[:, 0:D]
        set_xn(x)
        wait(w1_copy)
        wait(w3_copy)
        hs = ffn_up()
        for i in range(len(W2_SPLIT) - 1):
            wait(w2_copy[i])
            x = ffn_down(x, hs, W2_SPLIT[i] // 8, W2_SPLIT[i + 1] // 8)

        set_xn(x)
        y_ref[:, 0:D] = x

        def step(chains, mxu_stages, softmax_p, n_link, softmax_at, last_off):
            accs = [pv_chain(*ch) for ch in chains[:n_link]]
            pops = []
            linked = [0]

            def mm(l32, r, free):
                j = linked[0]
                if free is not None and j < n_link and len(pops) >= 4 + 5 * j:
                    linked[0] += 1
                    dep = (pltpu.bitcast(accs[j][0], U32)
                           | pltpu.bitcast(accs[j][1], U32))
                    l32 = jnp.where((sub < 4) if free else (sub >= 4), l32, dep)
                res = dot(l32, r)
                pops.append(res)
                return res

            for st in mxu_stages:
                st(mm)
            rest = chains[n_link:]
            last = len(pops) - last_off
            for n, ch in enumerate(rest):
                if n + n_link == softmax_at:
                    stage_softmax(softmax_p)
                ti = (n * last) // max(len(rest) - 1, 1)
                p_ref[pl.ds(fence_row, 8), :] = pops[ti][0:8]
                pv_chain(*ch)

        for col in range(8):
            stage_q(col)
        stage_qk(0)
        step([(0, g) for g in range(SPLIT)],
             [functools.partial(stage_qk, 1)], 0, 0, 0, 6)

        def body(j, carry):
            i = j + 1
            qcol = jnp.minimum(4 * j + 8, NQC - 4)
            stage_reduce(j - 1)
            stages = [functools.partial(stage_q, qcol + t) for t in range(4)]
            stages.append(functools.partial(stage_wo, j - 2, jnp.maximum(j - 2, 0)))
            stages.append(functools.partial(stage_qk, j + 2))
            step([(j, g) for g in range(SPLIT, PG)] + [(i, g) for g in range(SPLIT)],
                 stages, i, 4, 6, 6)
            return carry

        lax.fori_loop(0, NP - 2, body, 0)

        stage_reduce(NP - 3)
        stage_softmax(NP - 1)
        for g in range(SPLIT, PG):
            pv_chain(NP - 2, g)
        stage_reduce(NP - 2)
        for g in range(PG):
            pv_chain(NP - 1, g)
        stage_reduce(NP - 1)
        for p in range(NP - 4, NP):
            stage_wo(p, p)
        x = y_ref[:, 0:D]
        set_xn(x)
        x = ffn_down(x, ffn_up(), 0, FT)
        o_ref[...] = x[0:1].astype(o_ref.dtype)

    return kernel


@jax.jit
def pallas_interleave_layers__sliding_block_cached__glu_gated_swiglu__decode_kernel(
    A_x: jax.Array,
    A_k_cache: jax.Array,
    A_v_cache: jax.Array,
    A_wq: jax.Array,
    A_wo: jax.Array,
    B_x: jax.Array,
    B_w1: jax.Array,
    B_w3: jax.Array,
    B_w2: jax.Array,
):
    sk = A_k_cache.shape[2]
    win = min(4096, max(256, sk // 4))
    nt_total, nc = sk // LANES, win // LANES

    def kv_view(a):
        return _tile_view(jnp.swapaxes(a, 2, 3).reshape(H * DH, sk))

    def wbuf(r, c):
        return pltpu.VMEM((r // 16, c // LANES, 16, LANES), BF)

    any_spec = pl.BlockSpec(memory_space=pl.ANY)
    out = pl.pallas_call(
        _make_kernel(nt_total, nc),
        out_shape=jax.ShapeDtypeStruct((1, D), A_x.dtype),
        in_specs=[any_spec] * 8,
        out_specs=pl.BlockSpec(memory_space=pltpu.VMEM),
        scratch_shapes=[
            wbuf(H * DH, win), wbuf(H * DH, win),
            wbuf(D, H * DH), wbuf(H * DH, D),
            wbuf(D, F), wbuf(D, F), wbuf(F, D),
            pltpu.VMEM((PAD + NP, PW, LANES), F32),
            pltpu.VMEM((NQC * 8, 8, LANES), U32),
            pltpu.VMEM((NP, 2 * nc, LANES), F32),
            pltpu.VMEM((NP * 2 * nc + 32, LANES), F32),
            pltpu.VMEM((PAD + NP, 8, 512), F32),
            pltpu.VMEM((PAD + NP, 8, 512), U32),
            pltpu.VMEM((PG, 8, LANES), U32),
            pltpu.VMEM((8, 1024), U32),
            pltpu.VMEM((8, 1024), F32),
            pltpu.VMEM((1, D), BF),
            pltpu.SemaphoreType.DMA((NGRP,)),
            pltpu.SemaphoreType.DMA((NGRP,)),
            pltpu.SemaphoreType.DMA((4 + len(W2_SPLIT),)),
        ],
        compiler_params=pltpu.CompilerParams(
            vmem_limit_bytes=127 * 1024 * 1024),
    )(A_x.reshape(1, D), kv_view(A_k_cache), kv_view(A_v_cache),
      _tile_view(A_wq), _tile_view(A_wo),
      _tile_view(B_w1), _tile_view(B_w3), _tile_view(B_w2))
    return out.reshape(A_x.shape)
```

```python
import functools
import math

import jax
import jax.numpy as jnp
from jax import lax
import jax.experimental.pallas as pl
import jax.experimental.pallas.tpu as pltpu

D = 640
H = 32
DH = 192
F = 1536
LANES = 128
EPS = 1e-5

NP = H // 2
PG = 2 * DH // 16
HG = DH // 16
PW = 2 * DH
DT = D // LANES
FT = F // LANES

GP = 4
NGRP = NP // GP
W2_SPLIT = (0, 56, 88, 96)

SPLIT = 17
MCOLS = 2
NLINK = 4
LINK0 = 4
LINKSTEP = 5
SMAX_AT = 6
LAST_OFF = 6
ORDER = 0
PRO_FIRST = 100
PRO_LAST_OFF = 6
EPI_FIRST = 0
EPI_LAST = 40
PAD = 2

U32 = jnp.uint32
BF = jnp.bfloat16
F32 = jnp.float32


def _tile_view(w):
    r, c = w.shape
    return jnp.swapaxes(w.reshape(r // 16, 2, 8, c // LANES, LANES), 2, 3)


def _as_rhs(w):
    return pltpu.bitcast(w.reshape(8 * 8, LANES), BF)


def _rhs(w32, g0, c):
    return _as_rhs(w32[pl.ds(g0, 8), c])


def _pack2(lo, hi):
    return pltpu.bitcast(jnp.concatenate([lo, hi], axis=0).astype(BF), U32)


def _make_kernel(n_tiles_total, nc):
    c0 = n_tiles_total - nc
    qscale = DH ** -0.5 * math.log2(math.e)
    prow = 2 * nc
    nk = nc // 8

    def kernel(x_hbm, k_hbm, v_hbm, wq_hbm, wo_hbm, w1_hbm, w3_hbm, w2_hbm,
               o_ref,
               kbuf, vbuf, wqbuf, wobuf, w3buf, w2buf,
               t_ref, lhs_ref, s_ref, p_ref, pk_ref, linv_ref, om_ref, ob_ref,
               mask_ref, xn_ref, y_ref, xbuf, kvsem, wsem):
        def kv_copies(g):
            return [pltpu.make_async_copy(
                src.at[pl.ds(g * GP * PG, GP * PG), par, pl.ds(c0, nc)],
                dst.at[pl.ds(g * GP * PG, GP * PG), :, pl.ds(8 * par, 8), :],
                kvsem.at[g])
                for src, dst in ((k_hbm, kbuf), (v_hbm, vbuf)) for par in range(2)]

        def w_copies(src, dst, idx, g0=0, g1=None):
            g1 = src.shape[0] if g1 is None else g1
            return [pltpu.make_async_copy(
                src.at[pl.ds(g0, g1 - g0), par],
                dst.at[pl.ds(g0, g1 - g0), :, pl.ds(8 * par, 8), :],
                wsem.at[idx]) for par in range(2)]

        wq_copy = [pltpu.make_async_copy(
            wq_hbm.at[:, par],
            wqbuf.at[:, :, pl.ds(0, 3), pl.ds(8 * par, 8), :],
            wsem.at[0]) for par in range(2)]
        wq_copy.append(pltpu.make_async_copy(x_hbm, xbuf, wsem.at[0]))
        wo_copy = w_copies(wo_hbm, wobuf, 1)
        w13_copy = [pltpu.make_async_copy(
            w1_hbm.at[:, par],
            wqbuf.at[:, pl.ds(0, FT), 3, pl.ds(8 * par, 8), :],
            wsem.at[2]) for par in range(2)]
        w13_copy += w_copies(w3_hbm, w3buf, 2)
        w2_copy = [w_copies(w2_hbm, w2buf, 3 + i, W2_SPLIT[i], W2_SPLIT[i + 1])
                   for i in range(len(W2_SPLIT) - 1)]

        def start(copies):
            for cp in copies:
                cp.start()

        def wait(copies):
            for cp in copies:
                cp.wait()

        start(wq_copy)
        for g in range(NGRP):
            start(kv_copies(NGRP - 1 - g))
        start(wo_copy)
        start(w13_copy)
        for cps in w2_copy:
            start(cps)

        k32 = kbuf.bitcast(U32)
        v32 = vbuf.bitcast(U32)
        wq32 = wqbuf.bitcast(U32)
        wo32 = wobuf.bitcast(U32)
        w332 = w3buf.bitcast(U32)
        w232 = w2buf.bitcast(U32)

        sub = lax.broadcasted_iota(jnp.int32, (8, LANES), 0)
        lane = lax.broadcasted_iota(jnp.int32, (8, LANES), 1)
        lane3 = lax.broadcasted_iota(jnp.int32, (8, PW), 1)

        for r in range(8):
            half = U32(0x0000FFFF if r % 2 == 0 else 0xFFFF0000)
            lo = jnp.where(sub == r // 2, half, U32(0))
            hi = jnp.where(sub == 4 + r // 2, half, U32(0))
            mask_ref[r] = lo
            mask_ref[8 + r] = jnp.where(lane < DH - LANES, lo, hi)
            mask_ref[16 + r] = hi
            mask_ref[24 + r] = lo | hi
        t_ref[0] = jnp.zeros(t_ref.shape[1:], F32)
        for i in range(PAD):
            linv_ref[i] = jnp.zeros(linv_ref.shape[1:], F32)
            om_ref[i] = jnp.zeros(om_ref.shape[1:], F32)
            ob_ref[i] = jnp.zeros(ob_ref.shape[1:], U32)
        p_ref[pl.ds(NP * prow, 32), :] = jnp.zeros((32, LANES), F32)

        def dot(l32, r):
            return jnp.dot(pltpu.bitcast(l32, BF), r, preferred_element_type=F32)

        def plain_dot(l32, r, free):
            del free
            return dot(l32, r)

        def ln_stats(x):
            xb = x.astype(BF).astype(F32)
            m = jnp.mean(xb, axis=-1, keepdims=True)
            xc = xb - m
            v = jnp.mean(xc * xc, axis=-1, keepdims=True)
            return xb, m, lax.rsqrt(v + EPS)

        def ln_lhs(xb):
            l = _pack2(xb, jnp.ones_like(xb))
            return [l[:, kk * LANES:(kk + 1) * LANES] for kk in range(DT)]

        def ln_proj(lhs, m, r, tile, mm=plain_dot):
            acc = None
            for kk in range(DT):
                d = mm(lhs[kk], tile(kk), None)
                acc = d if acc is None else acc + d
            return (acc[0:8] - m * acc[8:16]) * r

        def store_q(p, t, q):
            q = _pack2(q, q)
            for r in range(8):
                lhs_ref[PG * p + 8 * t + r] = q & mask_ref[8 * t + r]

        def stage_q(p, pw, mm=plain_dot):
            for t in range(3):
                acc = None
                for kk in range(DT):
                    d = mm(xn_ref[:, pl.ds(kk * LANES, LANES)],
                           _as_rhs(wq32[pl.ds(8 * kk, 8), pw, t]), True)[0:8]
                    acc = d if acc is None else acc + d
                store_q(p, t, acc * qscale)

        def stage_qk(p, mm=plain_dot):
            for k in range(nk):
                sa = sb = None
                for r in range(8):
                    c = 8 * k + r
                    r0 = mm(lhs_ref[PG * p + r], _rhs(k32, p * PG, c), True)
                    r1 = mm(lhs_ref[PG * p + 8 + r], _rhs(k32, p * PG + 8, c), None)
                    r2 = mm(lhs_ref[PG * p + 16 + r], _rhs(k32, p * PG + 16, c), False)
                    a = r0[0:8] + r1[0:8]
                    b = r1[8:16] + r2[8:16]
                    sa = a if sa is None else sa + a
                    sb = b if sb is None else sb + b
                s_ref[p, pl.ds(8 * k, 8), :] = sa
                s_ref[p, pl.ds(nc + 8 * k, 8), :] = sb

        def stage_qk_split(p, mm):
            for k in range(nk):
                sa = sb = None
                for r in range(8):
                    c = 8 * k + r
                    r0 = mm(lhs_ref[PG * p + r], _rhs(k32, p * PG, c), True)
                    r1 = mm(lhs_ref[PG * p + 8 + r], _rhs(k32, p * PG + 8, c), None)
                    a = r0[0:8] + r1[0:8]
                    sa = a if sa is None else sa + a
                    sb = r1[8:16] if sb is None else sb + r1[8:16]
                s_ref[p, pl.ds(8 * k, 8), :] = sa
                s_ref[p, pl.ds(nc + 8 * k, 8), :] = sb
            for k in range(nk):
                sb = s_ref[p, pl.ds(nc + 8 * k, 8), :]
                for r in range(8):
                    c = 8 * k + r
                    r2 = mm(lhs_ref[PG * p + 16 + r], _rhs(k32, p * PG + 16, c), False)
                    sb = sb + r2[8:16]
                s_ref[p, pl.ds(nc + 8 * k, 8), :] = sb

        def prow_of(p, off):
            r = p * prow + off
            return r if isinstance(r, int) else pl.multiple_of(r, 8)

        def softmax_head(p, hd, store_p=True):
            s = s_ref[p, pl.ds(hd * nc, nc), :]
            m = jnp.max(jnp.max(s, axis=0, keepdims=True), axis=1, keepdims=True)
            e = jnp.exp2(s - m)
            if store_p:
                p_ref[pl.ds(prow_of(p, hd * nc), nc), :] = e
            l = jnp.sum(jnp.sum(e, axis=0, keepdims=True), axis=1, keepdims=True)
            return e, l

        def softmax_finish(p, ea, la, eb, lb, k0):
            for k in range(k0, nk):
                pk_ref[p, k] = _pack2(ea[8 * k:8 * k + 8], eb[8 * k:8 * k + 8])
            linv_ref[PAD + p, :, 0:PW] = jnp.where(lane3 < DH, 1.0 / la, 1.0 / lb)

        def stage_softmax(p, k0, store_p=True):
            softmax_finish(p, *softmax_head(p, 0, store_p),
                           *softmax_head(p, 1, store_p), k0)

        def pv_chain(p, g):
            lo = hi = None
            for c in range(nc - MCOLS):
                w = pltpu.bitcast(v32[p * PG + g, c], BF).astype(F32)
                pb = p_ref[pl.ds(p * prow + (g // HG) * nc + c, 8, stride=0), :]
                tl = w[0:8] * pb
                th = w[8:16] * pb
                lo = tl if lo is None else lo + tl
                hi = th if hi is None else hi + th
            t_ref[1 + p, pl.ds(16 * g, 8), :] = lo
            t_ref[1 + p, pl.ds(16 * g + 8, 8), :] = hi
            return lo, hi

        def pv_mxu(p, cols, transposed, mm=plain_dot):
            acc = [None] * 4
            for c in cols:
                l = pk_ref[p, c // 8] & mask_ref[24 + c % 8]
                rs = []
                for t in range(3):
                    tile = _rhs(v32, p * PG + 8 * t, c)
                    if transposed:
                        rs.append(mm(l, tile, (True, None, False)[t]))
                    else:
                        rs.append(lax.dot_general(
                            pltpu.bitcast(l, BF), tile, (((1,), (1,)), ((), ())),
                            preferred_element_type=F32))
                parts = (rs[0][0:8], rs[1][0:8], rs[1][8:16], rs[2][8:16])
                acc = [x if a is None else a + x for a, x in zip(acc, parts)]
            return jnp.concatenate(
                [acc[0], jnp.where(lane < DH - LANES, acc[1], acc[2]), acc[3]], axis=1)

        def stage_pvm(p, mm=plain_dot):
            om_ref[PAD + p, :, 0:PW] = pv_mxu(p, range(nc - MCOLS, nc), True, mm)

        def finish_o(p, o):
            o = jnp.sum(o, axis=0, keepdims=True) * linv_ref[PAD + p, :, 0:PW]
            ob_ref[PAD + p, :, 0:PW] = _pack2(o, o)

        def stage_reduce(p):
            tt = t_ref[1 + p].T
            o = jnp.sum(tt.reshape(LANES // 8, 8, PW), axis=0)
            if MCOLS:
                o = o + om_ref[PAD + p, :, 0:PW]
            finish_o(p, o)

        def transpose_v(p, c):
            for t in range(3):
                tile = _rhs(v32, p * PG + 8 * t, c)
                v32[pl.ds(p * PG + 8 * t, 8), c] = pltpu.bitcast(
                    tile.T, U32).reshape(8, 8, LANES)

        def stage_wo(p, pw, mm=plain_dot):
            for c in range(DT):
                acc = y_ref[:, pl.ds(c * LANES, LANES)]
                for t in range(3):
                    acc = acc + mm(ob_ref[PAD + p, :, pl.ds(t * LANES, LANES)],
                                   _rhs(wo32, pw * PG + 8 * t, c), True)[0:8]
                y_ref[:, pl.ds(c * LANES, LANES)] = acc

        def ffn_up(x):
            xb, m, r = ln_stats(x)
            lhs = ln_lhs(xb)
            hs = []
            for c in range(FT):
                g = ln_proj(lhs, m, r, lambda kk: _as_rhs(wq32[pl.ds(8 * kk, 8), c, 3]))
                u = ln_proj(lhs, m, r, lambda kk: _rhs(w332, 8 * kk, c))
                hh = g * jax.nn.sigmoid(g) * u
                hs.append(_pack2(hh, hh))
            return hs

        def ffn_down(x, hs, k0, k1):
            cols = [x[:, c * LANES:(c + 1) * LANES] for c in range(DT)]
            for kk in range(k0, k1):
                for c in range(DT):
                    cols[c] = cols[c] + dot(hs[kk], _rhs(w232, 8 * kk, c))[0:8]
            return jnp.concatenate(cols, axis=1)

        wait(wq_copy)
        x = jnp.broadcast_to(xbuf[...].astype(F32), (8, D))
        xb, m, r = ln_stats(x)
        xn = (xb - m) * r
        xn_ref[:, 0:D] = _pack2(xn, xn)
        y_ref[:, 0:D] = x

        def qloop(p, carry):
            stage_q(p, p)
            return carry

        lax.fori_loop(0, NP, qloop, 0)

        def group1(gi, fence_row):
            g = NGRP - 1 - gi
            wait(kv_copies(g))

            def pair(j, carry):
                p = g * GP + j
                stage_qk(p)
                stage_softmax(p, 0, store_p=False)
                finish_o(p, pv_mxu(p, range(nc), False))
                for c in range(nc - MCOLS, nc):
                    transpose_v(p, c)
                return carry

            lax.fori_loop(0, GP, pair, 0)

            @pl.when(gi == 0)
            def _():
                def tr(c2, carry):
                    transpose_v(NP - 1, 2 * c2)
                    transpose_v(NP - 1, 2 * c2 + 1)
                    return carry

                lax.fori_loop(0, (nc - MCOLS) // 2, tr, 0)
                if (nc - MCOLS) % 2:
                    transpose_v(NP - 1, nc - MCOLS - 1)

            return fence_row + GP * prow

        fence_row = lax.fori_loop(0, NGRP, group1, 8)
        fence_row = pl.multiple_of(fence_row, 8)
        wait(wo_copy)

        def woloop(p2, carry):
            stage_wo(2 * p2, 2 * p2)
            stage_wo(2 * p2 + 1, 2 * p2 + 1)
            return carry

        lax.fori_loop(0, NP // 2, woloop, 0)
        x = y_ref[:, 0:D]
        wait(w13_copy)
        hs = ffn_up(x)
        for i in range(len(W2_SPLIT) - 1):
            wait(w2_copy[i])
            x = ffn_down(x, hs, W2_SPLIT[i] // 8, W2_SPLIT[i + 1] // 8)

        def step(chains, mxu_stages, hooks, n_link, first, last_off):
            accs = [pv_chain(*ch) for ch in chains[:n_link]]
            pops = []
            linked = [0]

            def mm(l32, r, free):
                j = linked[0]
                if (free is not None and j < n_link
                        and len(pops) >= LINK0 + LINKSTEP * j):
                    linked[0] += 1
                    dep = (pltpu.bitcast(accs[j][0], U32)
                           | pltpu.bitcast(accs[j][1], U32))
                    l32 = jnp.where((sub < 4) if free else (sub >= 4), l32, dep)
                res = dot(l32, r)
                pops.append(res)
                return res

            for st in mxu_stages:
                st(mm)
            rest = chains[n_link:]
            last = len(pops) - last_off
            for n, ch in enumerate(rest):
                if n + n_link in hooks:
                    hooks[n + n_link]()
                ti = first + (n * (last - first)) // max(len(rest) - 1, 1)
                p_ref[pl.ds(fence_row, 8), :] = pops[ti][0:8]
                pv_chain(*ch)

        k0 = (nc - MCOLS) // 8
        y_ref[:, 0:D] = x
        xb, m, r = ln_stats(x)
        xn = (xb - m) * r
        xn_ref[:, 0:D] = _pack2(xn, xn)
        lhs0 = ln_lhs(xb)

        def first_q(p, mm):
            for t in range(3):
                store_q(p, t, ln_proj(
                    lhs0, m, r * qscale,
                    lambda kk: _as_rhs(wq32[pl.ds(8 * kk, 8), p, t]), mm))

        sm = {}

        def sm_a():
            sm['a'] = softmax_head(0, 0)

        def sm_b():
            softmax_finish(0, *sm['a'], *softmax_head(0, 1), k0)

        step([(0, g) for g in range(SPLIT)],
             [functools.partial(first_q, 0), functools.partial(first_q, 1),
              functools.partial(stage_qk_split, 0),
              functools.partial(stage_q, 2, 2),
              functools.partial(stage_qk, 1)],
             {0: sm_a, 8: sm_b}, 0, PRO_FIRST, PRO_LAST_OFF)

        def body(j, carry):
            i = j + 1
            stage_reduce(j - 1)
            sq = functools.partial(stage_q, j + 3, jnp.minimum(j + 3, NP - 1))
            sw = functools.partial(stage_wo, j - 2, jnp.maximum(j - 2, 0))
            sk = functools.partial(stage_qk, j + 2)
            sv = functools.partial(stage_pvm, j)
            stages = {0: [sq, sw, sv, sk], 1: [sk, sq, sw, sv], 2: [sw, sv, sk, sq]}[ORDER]
            if not MCOLS:
                stages.remove(sv)
            step([(j, g) for g in range(SPLIT, PG)] + [(i, g) for g in range(SPLIT)],
                 stages, {SMAX_AT: functools.partial(stage_softmax, i, k0)},
                 NLINK, 0, LAST_OFF)
            return carry

        lax.fori_loop(0, NP - 2, body, 0)

        stage_softmax(NP - 1, 0, store_p=False)
        stage_reduce(NP - 3)

        def last_pv(mm):
            finish_o(NP - 1, pv_mxu(NP - 1, range(nc), True, mm))

        stages = [functools.partial(stage_wo, NP - 4, NP - 4)]
        if MCOLS:
            stages.append(functools.partial(stage_pvm, NP - 2))
        stages += [last_pv, functools.partial(stage_wo, NP - 3, NP - 3)]
        step([(NP - 2, g) for g in range(SPLIT, PG)], stages, {},
             PG - SPLIT, EPI_FIRST, EPI_LAST)
        stage_reduce(NP - 2)
        stage_wo(NP - 2, NP - 2)
        stage_wo(NP - 1, NP - 1)
        x = y_ref[:, 0:D]
        x = ffn_down(x, ffn_up(x), 0, FT)
        o_ref[...] = x[0:1].astype(o_ref.dtype)

    return kernel


@jax.jit
def pallas_interleave_layers__sliding_block_cached__glu_gated_swiglu__decode_kernel(
    A_x: jax.Array,
    A_k_cache: jax.Array,
    A_v_cache: jax.Array,
    A_wq: jax.Array,
    A_wo: jax.Array,
    B_x: jax.Array,
    B_w1: jax.Array,
    B_w3: jax.Array,
    B_w2: jax.Array,
):
    sk = A_k_cache.shape[2]
    win = min(4096, max(256, sk // 4))
    nt_total, nc = sk // LANES, win // LANES

    def kv_view(a):
        return _tile_view(jnp.swapaxes(a, 2, 3).reshape(H * DH, sk))

    def wbuf(r, c):
        return pltpu.VMEM((r // 16, c // LANES, 16, LANES), BF)

    any_spec = pl.BlockSpec(memory_space=pl.ANY)
    out = pl.pallas_call(
        _make_kernel(nt_total, nc),
        out_shape=jax.ShapeDtypeStruct((1, D), A_x.dtype),
        in_specs=[any_spec] * 8,
        out_specs=pl.BlockSpec(memory_space=pltpu.VMEM),
        scratch_shapes=[
            wbuf(H * DH, win), wbuf(H * DH, win),
            pltpu.VMEM((D // 16, NP, 4, 16, LANES), BF),
            wbuf(H * DH, D), wbuf(D, F), wbuf(F, D),
            pltpu.VMEM((NP, PW, LANES), F32),
            pltpu.VMEM(((NP + 1) * PG, 8, LANES), U32),
            pltpu.VMEM((NP, 2 * nc, LANES), F32),
            pltpu.VMEM((NP * 2 * nc + 32, LANES), F32),
            pltpu.VMEM((NP, nc // 8, 8, LANES), U32),
            pltpu.VMEM((PAD + NP, 8, 512), F32),
            pltpu.VMEM((PAD + NP, 8, 512), F32),
            pltpu.VMEM((PAD + NP, 8, 512), U32),
            pltpu.VMEM((32, 8, LANES), U32),
            pltpu.VMEM((8, 1024), U32),
            pltpu.VMEM((8, 1024), F32),
            pltpu.VMEM((1, D), BF),
            pltpu.SemaphoreType.DMA((NGRP,)),
            pltpu.SemaphoreType.DMA((2 + len(W2_SPLIT),)),
        ],
        compiler_params=pltpu.CompilerParams(
            vmem_limit_bytes=127 * 1024 * 1024),
    )(A_x.reshape(1, D), kv_view(A_k_cache), kv_view(A_v_cache),
      _tile_view(A_wq).reshape(D // 16, 2, NP, 3, 8, LANES), _tile_view(A_wo),
      _tile_view(B_w1), _tile_view(B_w3), _tile_view(B_w2))
    return out.reshape(A_x.shape)
```

```python
import functools
import math

import jax
import jax.numpy as jnp
from jax import lax
import jax.experimental.pallas as pl
import jax.experimental.pallas.tpu as pltpu

D = 640
H = 32
DH = 192
F = 1536
LANES = 128
EPS = 1e-5

NP = H // 2
PG = 2 * DH // 16
HG = DH // 16
PW = 2 * DH
DT = D // LANES
FT = F // LANES

GP = 4
NGRP = NP // GP
W2_SPLIT = (0, 56, 88, 96)

SPLIT = 17
MCOLS = 2
LAST_VPU = 0
UNROLL = 1
NLINK = 3
LINK0 = 4
LINKSTEP = 5
SMAX_AT = 4
LAST_OFF = 12
ORDER = 0
WO_LAG = 2
Q_LEAD = 3
PRO_FIRST = 100
PRO_LAST_OFF = 6
PRO_SMB = 8
EPI_LINK = 7
EPI_FIRST = 10
EPI_LAST = 60
PAD = 2
NSEM = 3

U32 = jnp.uint32
BF = jnp.bfloat16
F32 = jnp.float32


def _tile_view(w):
    r, c = w.shape
    return jnp.swapaxes(w.reshape(r // 16, 2, 8, c // LANES, LANES), 2, 3)


def _as_rhs(w):
    return pltpu.bitcast(w.reshape(8 * 8, LANES), BF)


def _rhs(w32, g0, c):
    return _as_rhs(w32[pl.ds(g0, 8), c])


def _rhs4(w32, tile, c):
    return _as_rhs(w32[pl.ds(2 * tile, 2), :, c])


def _pack2(lo, hi):
    return pltpu.bitcast(jnp.concatenate([lo, hi], axis=0).astype(BF), U32)


def _make_kernel(n_tiles_total, nc):
    c0 = n_tiles_total - nc
    qscale = DH ** -0.5 * math.log2(math.e)
    prow = 2 * nc
    nk = nc // 8

    def kernel(x_hbm, k_hbm, v_hbm, wq_hbm, wo_hbm, w1_hbm, w3_hbm, w2_hbm,
               o_ref,
               kbuf, vbuf, wqbuf, wobuf, w3buf, w2buf,
               t_ref, lhs_ref, s_ref, p_ref, pk_ref, linv_ref, om_ref, ob_ref,
               mask_ref, xn_ref, y_ref, xbuf, sem):
        def halves(src, dst):
            return [(src(par), dst(pl.ds(8 * par, 8))) for par in range(2)]

        def kv_group(g):
            kr = pl.ds(g * GP * PG, GP * PG)
            vr = pl.ds(g * GP * PG // 4, GP * PG // 4)
            return (halves(lambda p: k_hbm.at[kr, p, pl.ds(c0, nc)],
                           lambda h: kbuf.at[kr, :, h, :])
                    + halves(lambda p: v_hbm.at[vr, p, :, pl.ds(c0, nc)],
                             lambda h: vbuf.at[vr, :, :, h, :]))

        def w2_group(i):
            rows = pl.ds(W2_SPLIT[i], W2_SPLIT[i + 1] - W2_SPLIT[i])
            return halves(lambda p: w2_hbm.at[rows, p], lambda h: w2buf.at[rows, :, h, :])

        wq_group = halves(lambda p: wq_hbm.at[:, p],
                          lambda h: wqbuf.at[:, :, pl.ds(0, 3), h, :]) + [(x_hbm, xbuf)]
        wo_group = halves(lambda p: wo_hbm.at[:, p], lambda h: wobuf.at[:, :, :, h, :])
        w13_group = (halves(lambda p: w1_hbm.at[:, p],
                            lambda h: wqbuf.at[:, pl.ds(0, FT), 3, h, :])
                     + halves(lambda p: w3_hbm.at[:, p], lambda h: w3buf.at[:, :, h, :]))
        groups = ([wq_group] + [kv_group(NGRP - 1 - g) for g in range(NGRP)]
                  + [wo_group, w13_group]
                  + [w2_group(i) for i in range(len(W2_SPLIT) - 1)])

        def copies(i):
            return [pltpu.make_async_copy(src, dst, sem.at[i % NSEM])
                    for src, dst in groups[i]]

        def start(i):
            for cp in copies(i):
                cp.start()

        def wait(i):
            for cp in copies(i):
                cp.wait()
            if i + NSEM < len(groups):
                start(i + NSEM)

        for i in range(NSEM):
            start(i)

        k32 = kbuf.bitcast(U32)
        v32 = vbuf.bitcast(U32)
        wq32 = wqbuf.bitcast(U32)
        wo32 = wobuf.bitcast(U32)
        w332 = w3buf.bitcast(U32)
        w232 = w2buf.bitcast(U32)

        sub = lax.broadcasted_iota(jnp.int32, (8, LANES), 0)
        lane = lax.broadcasted_iota(jnp.int32, (8, LANES), 1)
        lane3 = lax.broadcasted_iota(jnp.int32, (8, PW), 1)

        for r in range(8):
            half = U32(0x0000FFFF if r % 2 == 0 else 0xFFFF0000)
            lo = jnp.where(sub == r // 2, half, U32(0))
            hi = jnp.where(sub == 4 + r // 2, half, U32(0))
            mask_ref[r] = lo
            mask_ref[8 + r] = jnp.where(lane < DH - LANES, lo, hi)
            mask_ref[16 + r] = hi
            mask_ref[24 + r] = lo | hi
        t_ref[0] = jnp.zeros(t_ref.shape[1:], F32)
        for i in range(PAD):
            linv_ref[i] = jnp.zeros(linv_ref.shape[1:], F32)
            om_ref[i] = jnp.zeros(om_ref.shape[1:], F32)
            ob_ref[i] = jnp.zeros(ob_ref.shape[1:], U32)
        p_ref[pl.ds(NP * prow, 32), :] = jnp.zeros((32, LANES), F32)

        def dot(l32, r):
            return jnp.dot(pltpu.bitcast(l32, BF), r, preferred_element_type=F32)

        def plain_dot(l32, r, free):
            del free
            return dot(l32, r)

        def ln_stats(x):
            xb = x.astype(BF).astype(F32)
            m = jnp.mean(xb, axis=-1, keepdims=True)
            xc = xb - m
            v = jnp.mean(xc * xc, axis=-1, keepdims=True)
            return xb, m, lax.rsqrt(v + EPS)

        def ln_lhs(xb):
            l = _pack2(xb, jnp.ones_like(xb))
            return [l[:, kk * LANES:(kk + 1) * LANES] for kk in range(DT)]

        def ln_proj(lhs, m, r, tile, mm=plain_dot):
            acc = None
            for kk in range(DT):
                d = mm(lhs[kk], tile(kk), None)
                acc = d if acc is None else acc + d
            c = acc[0:8] - m * acc[8:16]
            return c if r is None else c * r

        def store_q(p, t, q):
            q = _pack2(q, q)
            for r in range(8):
                lhs_ref[PG * p + 8 * t + r] = q & mask_ref[8 * t + r]

        def stage_q(p, pw, mm=plain_dot):
            acc = [None] * 3
            for kk in range(DT):
                for t in range(3):
                    d = mm(xn_ref[:, pl.ds(kk * LANES, LANES)],
                           _as_rhs(wq32[pl.ds(8 * kk, 8), pw, t]), True)[0:8]
                    acc[t] = d if acc[t] is None else acc[t] + d
            for t in range(3):
                store_q(p, t, acc[t] * qscale)

        def qk_tiles(p, k, ts, sa, sb, mm):
            def add(a, x):
                return x if a is None else a + x

            for r0 in range(0, 8, 4):
                for t in ts:
                    for r in range(r0, r0 + 4):
                        res = mm(lhs_ref[PG * p + 8 * t + r],
                                 _rhs(k32, p * PG + 8 * t, 8 * k + r),
                                 (True, None, False)[t])
                        if t < 2:
                            sa = add(sa, res[0:8])
                        if t > 0:
                            sb = add(sb, res[8:16])
            return sa, sb

        def stage_qk(p, mm=plain_dot):
            for k in range(nk):
                sa, sb = qk_tiles(p, k, (0, 1, 2), None, None, mm)
                s_ref[p, pl.ds(8 * k, 8), :] = sa
                s_ref[p, pl.ds(nc + 8 * k, 8), :] = sb

        def stage_qk_split(p, scale, mm):
            for k in range(nk):
                sa, sb = qk_tiles(p, k, (0, 1), None, None, mm)
                s_ref[p, pl.ds(8 * k, 8), :] = sa * scale
                s_ref[p, pl.ds(nc + 8 * k, 8), :] = sb
            for k in range(nk):
                _, sb = qk_tiles(p, k, (2,), None,
                                 s_ref[p, pl.ds(nc + 8 * k, 8), :], mm)
                s_ref[p, pl.ds(nc + 8 * k, 8), :] = sb * scale

        def prow_of(p, off):
            r = p * prow + off
            return r if isinstance(r, int) else pl.multiple_of(r, 8)

        def softmax_head(p, hd, store_p=True):
            s = s_ref[p, pl.ds(hd * nc, nc), :]
            m = jnp.max(jnp.max(s, axis=0, keepdims=True), axis=1, keepdims=True)
            e = jnp.exp2(s - m)
            if store_p:
                p_ref[pl.ds(prow_of(p, hd * nc), nc), :] = e
            l = jnp.sum(jnp.sum(e, axis=0, keepdims=True), axis=1, keepdims=True)
            return e, l

        def softmax_finish(p, ea, la, eb, lb, k0):
            for k in range(k0, nk):
                pk_ref[p, k] = _pack2(ea[8 * k:8 * k + 8], eb[8 * k:8 * k + 8])
            linv_ref[PAD + p, :, 0:PW] = jnp.where(lane3 < DH, 1.0 / la, 1.0 / lb)

        def stage_softmax(p, k0, store_p=True):
            softmax_finish(p, *softmax_head(p, 0, store_p),
                           *softmax_head(p, 1, store_p), k0)

        def pv_chain(p, g, ncols=nc - MCOLS):
            lo = hi = None
            for c in range(ncols):
                w = pltpu.bitcast(v32[p * (PG // 4) + g // 4, g % 4, c], BF).astype(F32)
                pb = p_ref[pl.ds(p * prow + (g // HG) * nc + c, 8, stride=0), :]
                tl = w[0:8] * pb
                th = w[8:16] * pb
                lo = tl if lo is None else lo + tl
                hi = th if hi is None else hi + th
            t_ref[1 + p, pl.ds(16 * g, 8), :] = lo
            t_ref[1 + p, pl.ds(16 * g + 8, 8), :] = hi
            return lo, hi

        def pv_mxu(p, cols, transposed, mm=plain_dot):
            acc = [None] * 4
            cols = list(cols)
            for i0 in range(0, len(cols), 4):
                ls = {c: pk_ref[p, c // 8] & mask_ref[24 + c % 8]
                      for c in cols[i0:i0 + 4]}
                for t in range(3):
                    for c, l in ls.items():
                        tile = _rhs4(v32, 3 * p + t, c)
                        if transposed:
                            res = mm(l, tile, (True, None, False)[t])
                        else:
                            res = lax.dot_general(
                                pltpu.bitcast(l, BF), tile, (((1,), (1,)), ((), ())),
                                preferred_element_type=F32)
                        if t < 2:
                            acc[t] = res[0:8] if acc[t] is None else acc[t] + res[0:8]
                        if t > 0:
                            acc[t + 1] = (res[8:16] if acc[t + 1] is None
                                          else acc[t + 1] + res[8:16])
            return jnp.concatenate(
                [acc[0], jnp.where(lane < DH - LANES, acc[1], acc[2]), acc[3]], axis=1)

        def stage_pvm(p, mm=plain_dot, c_first=nc - MCOLS):
            om_ref[PAD + p, :, 0:PW] = pv_mxu(p, range(c_first, nc), True, mm)

        def finish_o(p, o):
            o = jnp.sum(o, axis=0, keepdims=True) * linv_ref[PAD + p, :, 0:PW]
            ob_ref[PAD + p, :, 0:PW] = _pack2(o, o)

        def stage_reduce(p):
            tt = t_ref[1 + p].T
            o = jnp.sum(tt.reshape(LANES // 8, 8, PW), axis=0)
            if MCOLS:
                o = o + om_ref[PAD + p, :, 0:PW]
            finish_o(p, o)

        def transpose_v(p, c):
            for t in range(3):
                tile = _rhs4(v32, 3 * p + t, c)
                v32[pl.ds(2 * (3 * p + t), 2), :, c] = pltpu.bitcast(
                    tile.T, U32).reshape(2, 4, 8, LANES)

        def stage_wo(p, pw, mm=plain_dot):
            for c in range(DT):
                acc = y_ref[:, pl.ds(c * LANES, LANES)]
                for t in range(3):
                    acc = acc + mm(ob_ref[PAD + p, :, pl.ds(t * LANES, LANES)],
                                   _rhs4(wo32, 3 * pw + t, c), True)[0:8]
                y_ref[:, pl.ds(c * LANES, LANES)] = acc

        def ffn_up(x):
            xb, m, r = ln_stats(x)
            lhs = ln_lhs(xb)
            hs = []
            for c in range(FT):
                g = ln_proj(lhs, m, r, lambda kk: _as_rhs(wq32[pl.ds(8 * kk, 8), c, 3]))
                u = ln_proj(lhs, m, r, lambda kk: _rhs(w332, 8 * kk, c))
                hh = g * jax.nn.sigmoid(g) * u
                hs.append(_pack2(hh, hh))
            return hs

        def ffn_down(x, hs, k0, k1):
            cols = [x[:, c * LANES:(c + 1) * LANES] for c in range(DT)]
            for kk in range(k0, k1):
                for c in range(DT):
                    cols[c] = cols[c] + dot(hs[kk], _rhs(w232, 8 * kk, c))[0:8]
            return jnp.concatenate(cols, axis=1)

        wait(0)
        x = jnp.broadcast_to(xbuf[...].astype(F32), (8, D))
        xb, m, r = ln_stats(x)
        xn = (xb - m) * r
        xn_ref[:, 0:D] = _pack2(xn, xn)
        y_ref[:, 0:D] = x

        def qloop(p, carry):
            stage_q(p, p)
            return carry

        lax.fori_loop(0, NP, qloop, 0)

        def group1(gi, fence_row):
            g = NGRP - 1 - gi
            for i in range(NGRP):
                pl.when(gi == i)(functools.partial(wait, 1 + i))

            def pair(j, carry):
                p = g * GP + j
                stage_qk(p)
                stage_softmax(p, 0, store_p=False)
                finish_o(p, pv_mxu(p, range(nc), False))
                for c in range(nc - MCOLS, nc):
                    transpose_v(p, c)
                return carry

            lax.fori_loop(0, GP, pair, 0)

            @pl.when(gi == 0)
            def _():
                def tr(c, carry):
                    transpose_v(NP - 1, c)
                    return carry

                lax.fori_loop(LAST_VPU, nc - MCOLS, tr, 0)

            return fence_row + GP * prow

        fence_row = lax.fori_loop(0, NGRP, group1, 8)
        fence_row = pl.multiple_of(fence_row, 8)
        wait(1 + NGRP)

        def woloop(p2, carry):
            stage_wo(2 * p2, 2 * p2)
            stage_wo(2 * p2 + 1, 2 * p2 + 1)
            return carry

        lax.fori_loop(0, NP // 2, woloop, 0)
        x = y_ref[:, 0:D]
        wait(2 + NGRP)
        hs = ffn_up(x)
        for i in range(len(W2_SPLIT) - 1):
            wait(3 + NGRP + i)
            x = ffn_down(x, hs, W2_SPLIT[i] // 8, W2_SPLIT[i + 1] // 8)

        def steps(subs, n_link, first, last_off):
            accs = [pv_chain(*ch) for ch in subs[0][0][:n_link]]
            pops = []
            linked = [0]

            def mm(l32, r, free):
                j = linked[0]
                if (free is not None and j < n_link
                        and len(pops) >= LINK0 + LINKSTEP * j):
                    linked[0] += 1
                    dep = (pltpu.bitcast(accs[j][0], U32)
                           | pltpu.bitcast(accs[j][1], U32))
                    l32 = jnp.where((sub < 4) if free else (sub >= 4), l32, dep)
                res = dot(l32, r)
                pops.append(res)
                return res

            n_rest = sum(len(sb_[0]) for sb_ in subs) - n_link
            n = 0
            for si, (chains, mxu_stages, hooks) in enumerate(subs):
                for st in mxu_stages:
                    st(mm)
                last = len(pops) * len(subs) // (si + 1) - last_off
                for ci, ch in enumerate(chains):
                    if si == 0 and ci < n_link:
                        continue
                    if ci in hooks:
                        hooks[ci]()
                    ti = first + (n * (last - first)) // max(n_rest - 1, 1)
                    p_ref[pl.ds(fence_row, 8), :] = pops[ti][0:8]
                    pv_chain(*ch)
                    n += 1

        k0 = (nc - MCOLS) // 8
        y_ref[:, 0:D] = x
        xb, m, r = ln_stats(x)
        xn = (xb - m) * r
        xn_ref[:, 0:D] = _pack2(xn, xn)
        lhs0 = ln_lhs(xb)

        def first_q(p, scale, mm):
            for t in range(3):
                store_q(p, t, ln_proj(
                    lhs0, m, scale,
                    lambda kk: _as_rhs(wq32[pl.ds(8 * kk, 8), p, t]), mm))

        sm = {}

        def sm_a():
            sm['a'] = softmax_head(0, 0)

        def sm_b():
            softmax_finish(0, *sm['a'], *softmax_head(0, 1), k0)

        stages = [functools.partial(first_q, 0, None),
                  functools.partial(first_q, 1, r * qscale),
                  functools.partial(stage_qk_split, 0, r * qscale)]
        if Q_LEAD == 3:
            stages.append(functools.partial(stage_q, 2, 2))
        stages.append(functools.partial(stage_qk, 1))
        steps([([(0, g) for g in range(SPLIT)], stages, {0: sm_a, PRO_SMB: sm_b})],
              0, PRO_FIRST, PRO_LAST_OFF)

        def substep(j):
            i = j + 1
            sr = lambda mm: stage_reduce(j - 1)
            sq = functools.partial(stage_q, j + Q_LEAD, jnp.minimum(j + Q_LEAD, NP - 1))
            sw = functools.partial(stage_wo, j - WO_LAG, jnp.maximum(j - WO_LAG, 0))
            sk = functools.partial(stage_qk, j + 2)
            sv = functools.partial(stage_pvm, j)
            stages = {0: [sr, sq, sw, sv, sk], 1: [sr, sq, sv, sk, sw],
                      2: [sr, sw, sv, sk, sq]}[ORDER]
            if not MCOLS:
                stages.remove(sv)
            return ([(j, g) for g in range(SPLIT, PG)] + [(i, g) for g in range(SPLIT)],
                    stages, {SMAX_AT: functools.partial(stage_softmax, i, k0)})

        def body(jj, carry):
            steps([substep(jj * UNROLL + u) for u in range(UNROLL)], NLINK, 0, LAST_OFF)
            return carry

        lax.fori_loop(0, (NP - 2) // UNROLL, body, 0)

        stage_softmax(NP - 1, LAST_VPU // 8, store_p=LAST_VPU > 0)
        stage_reduce(NP - 3)

        def last_pv(mm):
            if LAST_VPU:
                stage_pvm(NP - 1, mm, LAST_VPU)
            else:
                finish_o(NP - 1, pv_mxu(NP - 1, range(nc), True, mm))

        stages = [functools.partial(stage_wo, p, p) for p in range(NP - 2 - WO_LAG, NP - 3)]
        if MCOLS:
            stages.append(functools.partial(stage_pvm, NP - 2))
        stages += [last_pv, functools.partial(stage_wo, NP - 3, NP - 3)]
        chains = [(NP - 2, g) for g in range(SPLIT, PG)]
        if LAST_VPU:
            chains += [(NP - 1, g, LAST_VPU) for g in range(PG)]
        steps([(chains, stages, {})], EPI_LINK, EPI_FIRST, EPI_LAST)
        stage_reduce(NP - 2)
        stage_wo(NP - 2, NP - 2)
        if LAST_VPU:
            stage_reduce(NP - 1)
        stage_wo(NP - 1, NP - 1)
        x = y_ref[:, 0:D]
        x = ffn_down(x, ffn_up(x), 0, FT)
        o_ref[...] = x[0:1].astype(o_ref.dtype)

    return kernel


@jax.jit
def pallas_interleave_layers__sliding_block_cached__glu_gated_swiglu__decode_kernel(
    A_x: jax.Array,
    A_k_cache: jax.Array,
    A_v_cache: jax.Array,
    A_wq: jax.Array,
    A_wo: jax.Array,
    B_x: jax.Array,
    B_w1: jax.Array,
    B_w3: jax.Array,
    B_w2: jax.Array,
):
    sk = A_k_cache.shape[2]
    win = min(4096, max(256, sk // 4))
    nt_total, nc = sk // LANES, win // LANES

    def kv_view(a):
        return _tile_view(jnp.swapaxes(a, 2, 3).reshape(H * DH, sk))

    def wbuf(r, c):
        return pltpu.VMEM((r // 16, c // LANES, 16, LANES), BF)

    def wbuf4(r, c):
        return pltpu.VMEM((r // 64, 4, c // LANES, 16, LANES), BF)

    def view4(t):
        return t.reshape(t.shape[0] // 4, 2, 4, t.shape[2], 8, LANES)

    any_spec = pl.BlockSpec(memory_space=pl.ANY)
    out = pl.pallas_call(
        _make_kernel(nt_total, nc),
        out_shape=jax.ShapeDtypeStruct((1, D), A_x.dtype),
        in_specs=[any_spec] * 8,
        out_specs=pl.BlockSpec(memory_space=pltpu.VMEM),
        scratch_shapes=[
            wbuf(H * DH, win), wbuf4(H * DH, win),
            pltpu.VMEM((D // 16, NP, 4, 16, LANES), BF),
            wbuf4(H * DH, D), wbuf(D, F), wbuf(F, D),
            pltpu.VMEM((NP + 1, PW, LANES), F32),
            pltpu.VMEM(((NP + 1) * PG, 8, LANES), U32),
            pltpu.VMEM((NP, 2 * nc, LANES), F32),
            pltpu.VMEM((NP * 2 * nc + 32, LANES), F32),
            pltpu.VMEM((NP, nc // 8, 8, LANES), U32),
            pltpu.VMEM((PAD + NP, 8, 512), F32),
            pltpu.VMEM((PAD + NP, 8, 512), F32),
            pltpu.VMEM((PAD + NP, 8, 512), U32),
            pltpu.VMEM((32, 8, LANES), U32),
            pltpu.VMEM((8, 1024), U32),
            pltpu.VMEM((8, 1024), F32),
            pltpu.VMEM((1, D), BF),
            pltpu.SemaphoreType.DMA((NSEM,)),
        ],
        compiler_params=pltpu.CompilerParams(
            vmem_limit_bytes=127 * 1024 * 1024),
    )(A_x.reshape(1, D), kv_view(A_k_cache), view4(kv_view(A_v_cache)),
      _tile_view(A_wq).reshape(D // 16, 2, NP, 3, 8, LANES), view4(_tile_view(A_wo)),
      _tile_view(B_w1), _tile_view(B_w3), _tile_view(B_w2))
    return out.reshape(A_x.shape)
```

```python
import functools
import math

import jax
import jax.numpy as jnp
from jax import lax
import jax.experimental.pallas as pl
import jax.experimental.pallas.tpu as pltpu

D = 640
H = 32
DH = 192
F = 1536
LANES = 128
EPS = 1e-5

NP = H // 2
PG = 2 * DH // 16
HG = DH // 16
PW = 2 * DH
DT = D // LANES
FT = F // LANES

GP = 4
NGRP = NP // GP
W2_SPLIT = (0, 56, 88, 96)

NSEM = 3

MC = (0, 0, 3, 3, 3, 3, 3, 3, 3, 3, 4, 4, 4, 4, 4)
NSPLIT = 2
V_END = (168, 288, 351)
TILES = (1110, 670, 340)
PVM_AFTER = 1
WO_START = (0, 60, 60, 44)
WO_GAP = (0, 70, 48, 12)
WO_KEEP = 3
SM_LAG = 38
NLINK = 3
LINK0 = 4
LINKSTEP = 5
FSTEP = 4
FIRST = (116, 0, 0)
LAST_OFF = (8, 8, 8)

U32 = jnp.uint32
BF = jnp.bfloat16
F32 = jnp.float32


def _tile_view(w):
    r, c = w.shape
    return jnp.swapaxes(w.reshape(r // 16, 2, 8, c // LANES, LANES), 2, 3)


def _as_rhs(w):
    return pltpu.bitcast(w.reshape(8 * 8, LANES), BF)


def _rhs(w32, g0, c):
    return _as_rhs(w32[pl.ds(g0, 8), c])


def _rhs4(w32, tile, c):
    return _as_rhs(w32[pl.ds(2 * tile, 2), :, c])


def _pack2(lo, hi):
    return pltpu.bitcast(jnp.concatenate([lo, hi], axis=0).astype(BF), U32)


_LOG = []


def _plan(nc):
    nk = nc // 8
    seq = [('fq', 0), ('fq', 1)]
    for p in range(NP):
        prev = []
        if p > 0 and MC[p - 1]:
            prev.append(('pvm', p - 1, nc - MC[p - 1], nc, False))
        nxt = [('q', p + 1)] if 1 <= p < NP - 1 else []
        if p < NSPLIT:
            seq += [('qka', p), ('sm', p, (0,))] + nxt + prev
            seq += [('qkb', p), ('sm', p, (1,))]
        else:
            seq += nxt
            for k in range(nk):
                if k == PVM_AFTER:
                    seq += prev
                seq.append(('qk', p, k))
            seq.append(('sm', p, (0, 1)))
    seq += [('pvm', NP - 1, c, c + 4, c > 0) for c in range(0, nc, 4)]
    last_pv = seq[-nc // 4]

    def tiles(it):
        if it[0] == 'pvm':
            return 3 * (it[3] - it[2])
        return dict(fq=15, q=15, wo=15, qk=24, qka=64, qkb=32, sm=0, red=0)[it[0]]

    chains = [(p, g) for p in range(NP - 1) for g in range(PG)]
    blocks = []
    v0 = done = 0
    for b in range(len(V_END) + 1):
        final = b == len(V_END)
        v1 = len(chains) if final else V_END[b]
        todo = list(range(done, v0 // PG))
        done = v0 // PG
        budget = 10 ** 9 if final else TILES[b] - 15 * len(todo)
        body = []
        used = 0
        while seq and used + tiles(seq[0]) // 2 <= budget:
            body.append(seq.pop(0))
            used += tiles(body[-1])
        if body[-1][0] == 'sm':
            seq.insert(0, body.pop())
        keep = WO_KEEP if last_pv in body else 0
        items = [('red', p) for p in todo]
        used = 0
        nxt = WO_START[b]
        for it in body:
            if it == last_pv:
                while todo:
                    items.append(('wo', todo.pop(0)))
            if len(todo) > keep and used >= nxt:
                items.append(('wo', todo.pop(0)))
                nxt = used + WO_GAP[b]
            items.append(it)
            used += tiles(it)
        items += [('wo', p) for p in todo]
        if final:
            for p in (NP - 1, NP - 2):
                items += [('red', p), ('wo', p)]
            blocks.append((chains[v0:v1], items, v1 - v0, 0, 0))
        else:
            blocks.append((chains[v0:v1], items, NLINK if b else 0, FIRST[b], LAST_OFF[b]))
        v0 = v1
    return blocks


def _make_kernel(n_tiles_total, nc):
    c0 = n_tiles_total - nc
    qscale = DH ** -0.5 * math.log2(math.e)
    prow = 2 * nc
    nk = nc // 8

    def kernel(x_hbm, k_hbm, v_hbm, wq_hbm, wo_hbm, w1_hbm, w3_hbm, w2_hbm,
               o_ref,
               kbuf, vbuf, wqbuf, wobuf, w3buf, w2buf,
               t_ref, lhs_ref, s_ref, p_ref, p2_ref, pk_ref, lsum_ref, om_ref, ob_ref,
               mask_ref, xn_ref, y_ref, xbuf, sem):
        def halves(src, dst):
            return [(src(par), dst(pl.ds(8 * par, 8))) for par in range(2)]

        def kv_group(g):
            kr = pl.ds(g * GP * PG, GP * PG)
            vr = pl.ds(g * GP * PG // 4, GP * PG // 4)
            return (halves(lambda p: k_hbm.at[kr, p, pl.ds(c0, nc)],
                           lambda h: kbuf.at[kr, :, h, :])
                    + halves(lambda p: v_hbm.at[vr, p, :, pl.ds(c0, nc)],
                             lambda h: vbuf.at[vr, :, :, h, :]))

        def w2_group(i):
            rows = pl.ds(W2_SPLIT[i], W2_SPLIT[i + 1] - W2_SPLIT[i])
            return halves(lambda p: w2_hbm.at[rows, p], lambda h: w2buf.at[rows, :, h, :])

        wq_group = halves(lambda p: wq_hbm.at[:, p],
                          lambda h: wqbuf.at[:, :, pl.ds(0, 3), h, :]) + [(x_hbm, xbuf)]
        wo_group = halves(lambda p: wo_hbm.at[:, p], lambda h: wobuf.at[:, :, :, h, :])
        w13_group = (halves(lambda p: w1_hbm.at[:, p],
                            lambda h: wqbuf.at[:, pl.ds(0, FT), 3, h, :])
                     + halves(lambda p: w3_hbm.at[:, p], lambda h: w3buf.at[:, :, h, :]))
        groups = ([wq_group] + [kv_group(NGRP - 1 - g) for g in range(NGRP)]
                  + [wo_group, w13_group]
                  + [w2_group(i) for i in range(len(W2_SPLIT) - 1)])

        def copies(i):
            return [pltpu.make_async_copy(src, dst, sem.at[i % NSEM])
                    for src, dst in groups[i]]

        def start(i):
            for cp in copies(i):
                cp.start()

        def wait(i):
            for cp in copies(i):
                cp.wait()
            if i + NSEM < len(groups):
                start(i + NSEM)

        for i in range(NSEM):
            start(i)

        k32 = kbuf.bitcast(U32)
        v32 = vbuf.bitcast(U32)
        wq32 = wqbuf.bitcast(U32)
        wo32 = wobuf.bitcast(U32)
        w332 = w3buf.bitcast(U32)
        w232 = w2buf.bitcast(U32)

        sub = lax.broadcasted_iota(jnp.int32, (8, LANES), 0)
        lane = lax.broadcasted_iota(jnp.int32, (8, LANES), 1)
        lane3 = lax.broadcasted_iota(jnp.int32, (8, PW), 1)

        for r in range(8):
            half = U32(0x0000FFFF if r % 2 == 0 else 0xFFFF0000)
            lo = jnp.where(sub == r // 2, half, U32(0))
            hi = jnp.where(sub == 4 + r // 2, half, U32(0))
            mask_ref[r] = lo
            mask_ref[8 + r] = jnp.where(lane < DH - LANES, lo, hi)
            mask_ref[16 + r] = hi
            mask_ref[24 + r] = lo | hi
        p_refs = (p_ref, p2_ref)
        for pr in p_refs:
            pr[pl.ds(NP * prow, 32), :] = jnp.zeros((32, LANES), F32)

        def dot(l32, r):
            return jnp.dot(pltpu.bitcast(l32, BF), r, preferred_element_type=F32)

        def plain_dot(l32, r, free):
            del free
            return dot(l32, r)

        def ln_stats(x):
            xb = x.astype(BF).astype(F32)
            m = jnp.mean(xb, axis=-1, keepdims=True)
            xc = xb - m
            v = jnp.mean(xc * xc, axis=-1, keepdims=True)
            return xb, m, lax.rsqrt(v + EPS)

        def ln_lhs(xb):
            l = _pack2(xb, jnp.ones_like(xb))
            return [l[:, kk * LANES:(kk + 1) * LANES] for kk in range(DT)]

        def ln_proj(lhs, m, r, tile, mm=plain_dot):
            acc = None
            for kk in range(DT):
                d = mm(lhs[kk], tile(kk), None)
                acc = d if acc is None else acc + d
            c = acc[0:8] - m * acc[8:16]
            return c if r is None else c * r

        def store_q(p, t, q):
            q = _pack2(q, q)
            for r in range(8):
                lhs_ref[PG * p + 8 * t + r] = q & mask_ref[8 * t + r]

        def stage_q(p, mm=plain_dot):
            acc = [None] * 3
            for kk in range(DT):
                for t in range(3):
                    d = mm(xn_ref[:, pl.ds(kk * LANES, LANES)],
                           _as_rhs(wq32[pl.ds(8 * kk, 8), p, t]), True)[0:8]
                    acc[t] = d if acc[t] is None else acc[t] + d
            for t in range(3):
                store_q(p, t, acc[t] * qscale)

        def qk_tiles(p, k, ts, sa, sb, mm):
            def add(a, x):
                return x if a is None else a + x

            for r0 in range(0, 8, 4):
                for t in ts:
                    for r in range(r0, r0 + 4):
                        res = mm(lhs_ref[PG * p + 8 * t + r],
                                 _rhs(k32, p * PG + 8 * t, 8 * k + r),
                                 (True, None, False)[t])
                        if t < 2:
                            sa = add(sa, res[0:8])
                        if t > 0:
                            sb = add(sb, res[8:16])
            return sa, sb

        def stage_qk(p, k, mm=plain_dot):
            sa, sb = qk_tiles(p, k, (0, 1, 2), None, None, mm)
            s_ref[p, pl.ds(8 * k, 8), :] = sa
            s_ref[p, pl.ds(nc + 8 * k, 8), :] = sb

        def stage_qk_a(p, scale, mm):
            for k in range(nk):
                sa, sb = qk_tiles(p, k, (0, 1), None, None, mm)
                s_ref[p, pl.ds(8 * k, 8), :] = sa if scale is None else sa * scale
                s_ref[p, pl.ds(nc + 8 * k, 8), :] = sb

        def stage_qk_b(p, scale, mm):
            for k in range(nk):
                _, sb = qk_tiles(p, k, (2,), None,
                                 s_ref[p, pl.ds(nc + 8 * k, 8), :], mm)
                s_ref[p, pl.ds(nc + 8 * k, 8), :] = sb if scale is None else sb * scale

        def softmax(p, hd):
            s = s_ref[p, pl.ds(hd * nc, nc), :]
            m = jnp.max(jnp.max(s, axis=0, keepdims=True), axis=1, keepdims=True)
            e = jnp.exp2(s - m)
            l = jnp.sum(e.reshape(nk, 8, LANES), axis=0)
            lsum_ref[p, hd] = l
            return e, l

        def pack_probs(p, ea, eb, k0):
            for k in range(k0, nk):
                pk_ref[p, k] = _pack2(ea[8 * k:8 * k + 8], eb[8 * k:8 * k + 8])

        def pv_chain(p, g, gate):
            lo = hi = None
            for c in range(nc - MC[p]):
                w = pltpu.bitcast(v32[p * (PG // 4) + g // 4, g % 4, c], BF).astype(F32)
                pb = gate()[pl.ds(p * prow + (g // HG) * nc + c, 8, stride=0), :]
                tl = w[0:8] * pb
                th = w[8:16] * pb
                lo = tl if lo is None else lo + tl
                hi = th if hi is None else hi + th
            t_ref[p, pl.ds(16 * g, 8), :] = lo
            t_ref[p, pl.ds(16 * g + 8, 8), :] = hi
            return lo, hi

        def pv_mxu(p, cols, transposed, mm=plain_dot):
            acc = [None] * 4
            cols = list(cols)
            for i0 in range(0, len(cols), 4):
                ls = {c: pk_ref[p, c // 8] & mask_ref[24 + c % 8]
                      for c in cols[i0:i0 + 4]}
                for t in range(3):
                    for c, l in ls.items():
                        tile = _rhs4(v32, 3 * p + t, c)
                        if transposed:
                            res = mm(l, tile, (True, None, False)[t])
                        else:
                            res = lax.dot_general(
                                pltpu.bitcast(l, BF), tile, (((1,), (1,)), ((), ())),
                                preferred_element_type=F32)
                        if t < 2:
                            acc[t] = res[0:8] if acc[t] is None else acc[t] + res[0:8]
                        if t > 0:
                            acc[t + 1] = (res[8:16] if acc[t + 1] is None
                                          else acc[t + 1] + res[8:16])
            return jnp.concatenate(
                [acc[0], jnp.where(lane < DH - LANES, acc[1], acc[2]), acc[3]], axis=1)

        def stage_pvm(p, ca, cb, accumulate, mm):
            o = pv_mxu(p, range(ca, cb), True, mm)
            if accumulate:
                o = o + om_ref[p, :, 0:PW]
            om_ref[p, :, 0:PW] = o

        def finish_o(p, o):
            linv = [1.0 / jnp.sum(jnp.sum(lsum_ref[p, hd], axis=0, keepdims=True),
                                  axis=1, keepdims=True) for hd in range(2)]
            o = jnp.sum(o, axis=0, keepdims=True) * jnp.where(lane3 < DH, *linv)
            ob_ref[p, :, 0:PW] = _pack2(o, o)

        def stage_reduce(p):
            if p == NP - 1:
                o = om_ref[p, :, 0:PW]
            else:
                o = jnp.sum(t_ref[p].T.reshape(LANES // 8, 8, PW), axis=0)
                if MC[p]:
                    o = o + om_ref[p, :, 0:PW]
            finish_o(p, o)

        def transpose_v(p, c):
            for t in range(3):
                tile = _rhs4(v32, 3 * p + t, c)
                v32[pl.ds(2 * (3 * p + t), 2), :, c] = pltpu.bitcast(
                    tile.T, U32).reshape(2, 4, 8, LANES)

        def stage_wo(p, mm=plain_dot):
            for c in range(DT):
                acc = y_ref[:, pl.ds(c * LANES, LANES)]
                for t in range(3):
                    acc = acc + mm(ob_ref[p, :, pl.ds(t * LANES, LANES)],
                                   _rhs4(wo32, 3 * p + t, c), True)[0:8]
                y_ref[:, pl.ds(c * LANES, LANES)] = acc

        def ffn_up(x):
            xb, m, r = ln_stats(x)
            lhs = ln_lhs(xb)
            hs = []
            for c in range(FT):
                g = ln_proj(lhs, m, r, lambda kk: _as_rhs(wq32[pl.ds(8 * kk, 8), c, 3]))
                u = ln_proj(lhs, m, r, lambda kk: _rhs(w332, 8 * kk, c))
                hh = g * jax.nn.sigmoid(g) * u
                hs.append(_pack2(hh, hh))
            return hs

        def ffn_down(x, hs, k0, k1):
            cols = [x[:, c * LANES:(c + 1) * LANES] for c in range(DT)]
            for kk in range(k0, k1):
                for c in range(DT):
                    cols[c] = cols[c] + dot(hs[kk], _rhs(w232, 8 * kk, c))[0:8]
            return jnp.concatenate(cols, axis=1)

        wait(0)
        x = jnp.broadcast_to(xbuf[...].astype(F32), (8, D))
        xb, m, r = ln_stats(x)
        xn = (xb - m) * r
        xn_ref[:, 0:D] = _pack2(xn, xn)
        y_ref[:, 0:D] = x

        def qloop(p, carry):
            stage_q(p)
            return carry

        lax.fori_loop(0, NP, qloop, 0)

        def group1(gi, fence_row):
            g = NGRP - 1 - gi
            for i in range(NGRP):
                pl.when(gi == i)(functools.partial(wait, 1 + i))

            def pair(j, carry):
                p = g * GP + j
                for k in range(nk):
                    stage_qk(p, k)
                pack_probs(p, softmax(p, 0)[0], softmax(p, 1)[0], 0)
                finish_o(p, pv_mxu(p, range(nc), False))
                first = 0
                for pp in range(NP - 1):
                    first = jnp.where(p == pp, nc - MC[pp], first)

                def tr(c, carry2):
                    transpose_v(p, c)
                    return carry2

                lax.fori_loop(first, nc, tr, 0)
                return carry

            lax.fori_loop(0, GP, pair, 0)
            return fence_row + GP * prow

        fence_row = lax.fori_loop(0, NGRP, group1, 8)
        fence_row = pl.multiple_of(fence_row, 8)
        wait(1 + NGRP)

        def woloop(p2, carry):
            stage_wo(2 * p2)
            stage_wo(2 * p2 + 1)
            return carry

        lax.fori_loop(0, NP // 2, woloop, 0)
        x = y_ref[:, 0:D]
        wait(2 + NGRP)
        hs = ffn_up(x)
        for i in range(len(W2_SPLIT) - 1):
            wait(3 + NGRP + i)
            x = ffn_down(x, hs, W2_SPLIT[i] // 8, W2_SPLIT[i + 1] // 8)

        y_ref[:, 0:D] = x
        xb, m, r = ln_stats(x)
        xn = (xb - m) * r
        xn_ref[:, 0:D] = _pack2(xn, xn)
        lhs0 = ln_lhs(xb)

        def first_q(p, scale, mm):
            for t in range(3):
                store_q(p, t, ln_proj(
                    lhs0, m, scale,
                    lambda kk: _as_rhs(wq32[pl.ds(8 * kk, 8), p, t]), mm))

        def run_block(chains, items, n_link, first, last_off):
            links = []
            for j, (p, g) in enumerate(chains[:n_link]):
                lo, hi = pv_chain(p, g, lambda: p_refs[g % 2])
                links.append((LINK0 + LINKSTEP * j,
                              pltpu.bitcast(lo, U32) | pltpu.bitcast(hi, U32)))
            pops = []
            probs = {}
            ready = {}

            def mm(l32, rr, free):
                links.sort(key=lambda lk: lk[0])
                if free is not None and links and len(pops) >= links[0][0]:
                    l32 = jnp.where((sub < 4) if free else (sub >= 4), l32,
                                    links.pop(0)[1])
                res = dot(l32, rr)
                pops.append(res)
                return res

            for it in items:
                kind, p = it[0], it[1]
                scale = r * qscale if p == 0 else None
                if kind == 'fq':
                    first_q(p, None if p == 0 else r * qscale, mm)
                elif kind == 'qka':
                    stage_qk_a(p, scale, mm)
                    ready[p] = len(pops)
                elif kind == 'qkb':
                    stage_qk_b(p, scale, mm)
                elif kind == 'q':
                    stage_q(p, mm)
                elif kind == 'qk':
                    stage_qk(p, it[2], mm)
                    ready[p] = len(pops)
                elif kind == 'sm':
                    for hd in it[2]:
                        probs[p, hd], l = softmax(p, hd)
                        links.append((len(pops) + (SM_LAG if pops else SM_LAG - 14),
                                      pltpu.bitcast(l, U32)))
                    if p == NP - 1:
                        pack_probs(p, probs.pop((p, 0)), probs.pop((p, 1)), 0)
                    elif MC[p] and hd == 1:
                        pack_probs(p, probs[p, 0], probs[p, 1], (nc - MC[p]) // 8)
                elif kind == 'pvm':
                    stage_pvm(p, *it[2:], mm)
                elif kind == 'red':
                    stage_reduce(p)
                elif kind == 'wo':
                    stage_wo(p, mm)

            def store_probs(p, hd):
                e = probs.pop((p, hd))
                for pr in p_refs:
                    pr[pl.ds(p * prow + hd * nc, nc), :] = e

            rest = chains[n_link:]
            n_items = sum(nc - MC[p] for p, _ in rest)
            n_units = (len(pops) - last_off - first) // FSTEP + 1
            state = [0, -1]

            def gate():
                u = state[0] * n_units // n_items
                state[0] += 1
                if u != state[1]:
                    state[1] = u
                    p_refs[u % 2][pl.ds(fence_row, 8), :] = pops[first + u * FSTEP][0:8]
                return p_refs[u % 2]

            for p, g in rest:
                if (p, g // HG) in probs:
                    if g == 0 and p in ready:
                        _LOG.append((p, first + state[1] * FSTEP - ready[p]))
                    store_probs(p, g // HG)
                pv_chain(p, g, gate)
            for key in list(probs):
                store_probs(*key)

        blocks = _plan(nc)
        for b, blk in enumerate(blocks):
            if b == 0 or b == len(blocks) - 1:
                run_block(*blk)
            else:
                pl.when(fence_row > b)(functools.partial(run_block, *blk))
        x = y_ref[:, 0:D]
        x = ffn_down(x, ffn_up(x), 0, FT)
        o_ref[...] = x[0:1].astype(o_ref.dtype)

    return kernel


@jax.jit
def pallas_interleave_layers__sliding_block_cached__glu_gated_swiglu__decode_kernel(
    A_x: jax.Array,
    A_k_cache: jax.Array,
    A_v_cache: jax.Array,
    A_wq: jax.Array,
    A_wo: jax.Array,
    B_x: jax.Array,
    B_w1: jax.Array,
    B_w3: jax.Array,
    B_w2: jax.Array,
):
    sk = A_k_cache.shape[2]
    win = min(4096, max(256, sk // 4))
    nt_total, nc = sk // LANES, win // LANES

    def kv_view(a):
        return _tile_view(jnp.swapaxes(a, 2, 3).reshape(H * DH, sk))

    def wbuf(r, c):
        return pltpu.VMEM((r // 16, c // LANES, 16, LANES), BF)

    def wbuf4(r, c):
        return pltpu.VMEM((r // 64, 4, c // LANES, 16, LANES), BF)

    def view4(t):
        return t.reshape(t.shape[0] // 4, 2, 4, t.shape[2], 8, LANES)

    any_spec = pl.BlockSpec(memory_space=pl.ANY)
    out = pl.pallas_call(
        _make_kernel(nt_total, nc),
        out_shape=jax.ShapeDtypeStruct((1, D), A_x.dtype),
        in_specs=[any_spec] * 8,
        out_specs=pl.BlockSpec(memory_space=pltpu.VMEM),
        scratch_shapes=[
            wbuf(H * DH, win), wbuf4(H * DH, win),
            pltpu.VMEM((D // 16, NP, 4, 16, LANES), BF),
            wbuf4(H * DH, D), wbuf(D, F), wbuf(F, D),
            pltpu.VMEM((NP - 1, PW, LANES), F32),
            pltpu.VMEM((NP * PG, 8, LANES), U32),
            pltpu.VMEM((NP, 2 * nc, LANES), F32),
            pltpu.VMEM((NP * 2 * nc + 32, LANES), F32),
            pltpu.VMEM((NP * 2 * nc + 32, LANES), F32),
            pltpu.VMEM((NP, nc // 8, 8, LANES), U32),
            pltpu.VMEM((NP, 4, 8, LANES), F32),
            pltpu.VMEM((NP, 8, 512), F32),
            pltpu.VMEM((NP, 8, 512), U32),
            pltpu.VMEM((32, 8, LANES), U32),
            pltpu.VMEM((8, 1024), U32),
            pltpu.VMEM((8, 1024), F32),
            pltpu.VMEM((1, D), BF),
            pltpu.SemaphoreType.DMA((NSEM,)),
        ],
        compiler_params=pltpu.CompilerParams(
            vmem_limit_bytes=127 * 1024 * 1024),
    )(A_x.reshape(1, D), kv_view(A_k_cache), view4(kv_view(A_v_cache)),
      _tile_view(A_wq).reshape(D // 16, 2, NP, 3, 8, LANES), view4(_tile_view(A_wo)),
      _tile_view(B_w1), _tile_view(B_w3), _tile_view(B_w2))
    return out.reshape(A_x.shape)
```

```python
import functools
import math

import jax
import jax.numpy as jnp
from jax import lax
import jax.experimental.pallas as pl
import jax.experimental.pallas.tpu as pltpu

D = 640
H = 32
DH = 192
F = 1536
LANES = 128
EPS = 1e-5

NP = H // 2
PG = 2 * DH // 16
HG = DH // 16
PW = 2 * DH
DT = D // LANES
FT = F // LANES

GP = 4
NGRP = NP // GP
W2_SPLIT = (0, 56, 88, 96)

NSEM = 3

MC = (4, 4, 4, 4, 4, 4, 4, 4, 4, 4, 4, 4, 4, 4, 4)
NSPLIT = 1
V_END = (168, 288, 351)
TILES = (1080, 670, 350)
PVM_AFTER = 2
WO_START = (0, 60, 60, 44)
WO_GAP = (0, 70, 48, 12)
WO_KEEP = 3
SM_LAG = 60
SM_LAG0 = 42
SM_REP = 1
XC_REP = 4
NVQ = 4
VQ_FIRST = 30
XC_LINK = 46
XC_PUT = (0, 0, 0, 0, 0)
UP_K = 3
UP_COLS = 5
UP_LINK0 = 46
UP_LINKSTEP = 4.8
DOWN_K = 3
NLINK = 3
LINK0 = 4
LINKSTEP = 5
FSTEP = 2
FIRST = (136, 0, 0)
LAST_OFF = (8, 8, 8)

U32 = jnp.uint32
BF = jnp.bfloat16
F32 = jnp.float32


def _tile_view(w):
    r, c = w.shape
    return jnp.swapaxes(w.reshape(r // 16, 2, 8, c // LANES, LANES), 2, 3)


def _as_rhs(w):
    return pltpu.bitcast(w.reshape(8 * 8, LANES), BF)


def _rhs(w32, g0, c):
    return _as_rhs(w32[pl.ds(g0, 8), c])


def _rhs4(w32, tile, c):
    return _as_rhs(w32[pl.ds(2 * tile, 2), :, c])


def _swiglu(g, u):
    hg = 0.5 * g
    return hg * (1.0 + jnp.tanh(hg)) * u


def _pack2(lo, hi):
    return pltpu.bitcast(jnp.concatenate([lo, hi], axis=0).astype(BF), U32)


_LOG = []


def _plan(nc):
    nk = nc // 8
    seq = [('fq', 0), ('fq', 1)]
    for p in range(NP):
        prev = []
        if p > 0 and MC[p - 1]:
            prev.append(('pvm', p - 1, nc - MC[p - 1], nc, False))
        nxt = [('q' if p + 1 < NP - NVQ else 'qx', p + 1)] if 1 <= p < NP - 1 else []
        if p < NSPLIT:
            seq += [('qka', p), ('sm', p, (0,))] + nxt + prev
            seq += [('qkb', p), ('sm', p, (1,))]
        else:
            seq += nxt
            for k in range(nk):
                if k == PVM_AFTER:
                    seq += prev
                seq.append(('qk', p, k))
            seq.append(('sm', p, (0, 1)))
    seq += [('pvm', NP - 1, c, c + 4, c > 0) for c in range(0, nc, 4)]
    last_pv = seq[-nc // 4]

    def tiles(it):
        if it[0] == 'pvm':
            return 3 * (it[3] - it[2])
        return dict(fq=15, q=15, wo=15, qk=24, qka=64, qkb=32, sm=0, red=0, qx=0)[it[0]]

    chains = [(p, g) for p in range(NP - 1) for g in range(PG)]
    blocks = []
    v0 = done = 0
    for b in range(len(V_END) + 1):
        final = b == len(V_END)
        v1 = len(chains) if final else V_END[b]
        todo = list(range(done, v0 // PG))
        done = v0 // PG
        budget = 10 ** 9 if final else TILES[b] - 15 * len(todo)
        body = []
        used = 0
        while seq and used + tiles(seq[0]) // 2 <= budget:
            body.append(seq.pop(0))
            used += tiles(body[-1])
        if body[-1][0] == 'sm':
            seq.insert(0, body.pop())
        keep = WO_KEEP if last_pv in body else 0
        items = [('red', p) for p in todo]
        used = 0
        nxt = WO_START[b]
        for it in body:
            if it == last_pv:
                while todo:
                    items.append(('wo', todo.pop(0)))
            if len(todo) > keep and used >= nxt:
                items.append(('wo', todo.pop(0)))
                nxt = used + WO_GAP[b]
            items.append(it)
            used += tiles(it)
        items += [('wo', p) for p in todo]
        if final:
            for p in (NP - 1, NP - 2):
                items += [('red', p), ('wo', p)]
            blocks.append((chains[v0:v1], items, v1 - v0, 0, 0))
        else:
            blocks.append((chains[v0:v1], items, NLINK if b else 0, FIRST[b], LAST_OFF[b]))
        v0 = v1
    return blocks


def _make_kernel(n_tiles_total, nc):
    c0 = n_tiles_total - nc
    qscale = DH ** -0.5 * math.log2(math.e)
    prow = 2 * nc
    nk = nc // 8

    def kernel(x_hbm, k_hbm, v_hbm, wq_hbm, wo_hbm, w1_hbm, w3_hbm, w2_hbm,
               o_ref,
               kbuf, vbuf, wqbuf, wobuf, w3buf, w2buf,
               t_ref, lhs_ref, s_ref, p_ref, p2_ref, pk_ref, lsum_ref, om_ref, ob_ref,
               mask_ref, cs_ref, qpk_ref, xn_ref, y_ref, xbuf, sem):
        def halves(src, dst):
            return [(src(par), dst(pl.ds(8 * par, 8))) for par in range(2)]

        def kv_group(g):
            kr = pl.ds(g * GP * PG, GP * PG)
            vr = pl.ds(g * GP * PG // 4, GP * PG // 4)
            return (halves(lambda p: k_hbm.at[kr, p, pl.ds(c0, nc)],
                           lambda h: kbuf.at[kr, :, h, :])
                    + halves(lambda p: v_hbm.at[vr, p, :, pl.ds(c0, nc)],
                             lambda h: vbuf.at[vr, :, :, h, :]))

        def w2_group(i):
            rows = pl.ds(W2_SPLIT[i], W2_SPLIT[i + 1] - W2_SPLIT[i])
            return halves(lambda p: w2_hbm.at[rows, p], lambda h: w2buf.at[rows, :, h, :])

        wq_group = halves(lambda p: wq_hbm.at[:, p],
                          lambda h: wqbuf.at[:, :, pl.ds(0, 3), h, :]) + [(x_hbm, xbuf)]
        wo_group = halves(lambda p: wo_hbm.at[:, p], lambda h: wobuf.at[:, :, :, h, :])
        w13_group = (halves(lambda p: w1_hbm.at[:, p],
                            lambda h: wqbuf.at[:, pl.ds(0, FT), 3, h, :])
                     + halves(lambda p: w3_hbm.at[:, p], lambda h: w3buf.at[:, :, h, :]))
        groups = ([wq_group] + [kv_group(NGRP - 1 - g) for g in range(NGRP)]
                  + [wo_group, w13_group]
                  + [w2_group(i) for i in range(len(W2_SPLIT) - 1)])

        def copies(i):
            return [pltpu.make_async_copy(src, dst, sem.at[i % NSEM])
                    for src, dst in groups[i]]

        def start(i):
            for cp in copies(i):
                cp.start()

        def wait(i):
            for cp in copies(i):
                cp.wait()
            if i + NSEM < len(groups):
                start(i + NSEM)

        for i in range(NSEM):
            start(i)

        k32 = kbuf.bitcast(U32)
        v32 = vbuf.bitcast(U32)
        wq32 = wqbuf.bitcast(U32)
        wo32 = wobuf.bitcast(U32)
        w332 = w3buf.bitcast(U32)
        w232 = w2buf.bitcast(U32)

        sub = lax.broadcasted_iota(jnp.int32, (8, LANES), 0)
        lane = lax.broadcasted_iota(jnp.int32, (8, LANES), 1)
        lane3 = lax.broadcasted_iota(jnp.int32, (8, PW), 1)

        for r in range(8):
            half = U32(0x0000FFFF if r % 2 == 0 else 0xFFFF0000)
            lo = jnp.where(sub == r // 2, half, U32(0))
            hi = jnp.where(sub == 4 + r // 2, half, U32(0))
            mask_ref[r] = lo
            mask_ref[8 + r] = jnp.where(lane < DH - LANES, lo, hi)
            mask_ref[16 + r] = hi
            mask_ref[24 + r] = lo | hi
        p_refs = (p_ref, p2_ref)
        for pr in p_refs:
            pr[...] = jnp.zeros(pr.shape, F32)

        def dot(l32, r):
            return jnp.dot(pltpu.bitcast(l32, BF), r, preferred_element_type=F32)

        def plain_dot(l32, r, free):
            del free
            return dot(l32, r)

        def ln_stats(x):
            xb = x.astype(BF).astype(F32)
            m = jnp.mean(xb, axis=-1, keepdims=True)
            xc = xb - m
            v = jnp.mean(xc * xc, axis=-1, keepdims=True)
            return xb, m, lax.rsqrt(v + EPS)

        def ln_lhs(xb):
            l = _pack2(xb, jnp.ones_like(xb))
            return [l[:, kk * LANES:(kk + 1) * LANES] for kk in range(DT)]

        def ln_proj(lhs, m, r, tile, mm=plain_dot):
            acc = None
            for kk in range(DT):
                d = mm(lhs[kk], tile(kk), None)
                acc = d if acc is None else acc + d
            c = acc[0:8] - m * acc[8:16]
            return c if r is None else c * r

        def store_q(p, t, q):
            expand_q(p, t, _pack2(q, q))

        def expand_q(p, t, q):
            for r in range(8):
                lhs_ref[PG * p + 8 * t + r] = q & mask_ref[8 * t + r]

        def stage_q(p, mm=plain_dot):
            acc = [None] * 3
            for kk in range(DT):
                for t in range(3):
                    d = mm(xn_ref[:, pl.ds(kk * LANES, LANES)],
                           _as_rhs(wq32[pl.ds(8 * kk, 8), p, t]), True)[0:8]
                    acc[t] = d if acc[t] is None else acc[t] + d
            for t in range(3):
                store_q(p, t, acc[t] * qscale)

        def qk_tiles(p, k, ts, sa, sb, mm):
            def add(a, x):
                return x if a is None else a + x

            for r0 in range(0, 8, 4):
                for t in ts:
                    for r in range(r0, r0 + 4):
                        res = mm(lhs_ref[PG * p + 8 * t + r],
                                 _rhs(k32, p * PG + 8 * t, 8 * k + r),
                                 (True, None, False)[t])
                        if t < 2:
                            sa = add(sa, res[0:8])
                        if t > 0:
                            sb = add(sb, res[8:16])
            return sa, sb

        def stage_qk(p, k, mm=plain_dot):
            sa, sb = qk_tiles(p, k, (0, 1, 2), None, None, mm)
            s_ref[p, pl.ds(8 * k, 8), :] = sa
            s_ref[p, pl.ds(nc + 8 * k, 8), :] = sb

        def stage_qk_a(p, scale, mm):
            for k in range(nk):
                sa, sb = qk_tiles(p, k, (0, 1), None, None, mm)
                s_ref[p, pl.ds(8 * k, 8), :] = sa if scale is None else sa * scale
                s_ref[p, pl.ds(nc + 8 * k, 8), :] = sb

        def stage_qk_b(p, scale, mm):
            for k in range(nk):
                _, sb = qk_tiles(p, k, (2,), None,
                                 s_ref[p, pl.ds(nc + 8 * k, 8), :], mm)
                s_ref[p, pl.ds(nc + 8 * k, 8), :] = sb if scale is None else sb * scale

        def softmax(p, hd):
            s = s_ref[p, pl.ds(hd * nc, nc), :]
            m = jnp.max(jnp.max(s, axis=0, keepdims=True), axis=1, keepdims=True)
            e = jnp.exp2(s - m)
            l = jnp.sum(e.reshape(nk, 8, LANES), axis=0)
            lsum_ref[p, hd] = l
            return e, l

        def pack_probs(p, ea, eb, k0):
            for k in range(k0, nk):
                pk_ref[p, k] = _pack2(ea[8 * k:8 * k + 8], eb[8 * k:8 * k + 8])

        def pv_chain(p, g, gate):
            lo = hi = None
            for c in range(nc - MC[p]):
                w = pltpu.bitcast(v32[p * (PG // 4) + g // 4, g % 4, c], BF).astype(F32)
                pb = gate()[pl.ds(p * prow + (g // HG) * nc + c, 8, stride=0), :]
                tl = w[0:8] * pb
                th = w[8:16] * pb
                lo = tl if lo is None else lo + tl
                hi = th if hi is None else hi + th
            t_ref[p, pl.ds(16 * g, 8), :] = lo
            t_ref[p, pl.ds(16 * g + 8, 8), :] = hi
            return lo, hi

        def pv_mxu(p, cols, transposed, mm=plain_dot):
            acc = [None] * 4
            cols = list(cols)
            for i0 in range(0, len(cols), 4):
                ls = {c: pk_ref[p, c // 8] & mask_ref[24 + c % 8]
                      for c in cols[i0:i0 + 4]}
                for t in range(3):
                    for c, l in ls.items():
                        tile = _rhs4(v32, 3 * p + t, c)
                        if transposed:
                            res = mm(l, tile, (True, None, False)[t])
                        else:
                            res = lax.dot_general(
                                pltpu.bitcast(l, BF), tile, (((1,), (1,)), ((), ())),
                                preferred_element_type=F32)
                        if t < 2:
                            acc[t] = res[0:8] if acc[t] is None else acc[t] + res[0:8]
                        if t > 0:
                            acc[t + 1] = (res[8:16] if acc[t + 1] is None
                                          else acc[t + 1] + res[8:16])
            return jnp.concatenate(
                [acc[0], jnp.where(lane < DH - LANES, acc[1], acc[2]), acc[3]], axis=1)

        def stage_pvm(p, ca, cb, accumulate, mm):
            o = pv_mxu(p, range(ca, cb), True, mm)
            if accumulate:
                o = o + om_ref[p, :, 0:PW]
            om_ref[p, :, 0:PW] = o

        def finish_o(p, o):
            linv = [1.0 / jnp.sum(jnp.sum(lsum_ref[p, hd], axis=0, keepdims=True),
                                  axis=1, keepdims=True) for hd in range(2)]
            o = jnp.sum(o, axis=0, keepdims=True) * jnp.where(lane3 < DH, *linv)
            ob_ref[p, :, 0:PW] = _pack2(o, o)

        def stage_reduce(p):
            if p == NP - 1:
                o = om_ref[p, :, 0:PW]
            else:
                o = jnp.sum(t_ref[p].T.reshape(LANES // 8, 8, PW), axis=0)
                if MC[p]:
                    o = o + om_ref[p, :, 0:PW]
            finish_o(p, o)

        def transpose_v(p, c):
            for t in range(3):
                tile = _rhs4(v32, 3 * p + t, c)
                v32[pl.ds(2 * (3 * p + t), 2), :, c] = pltpu.bitcast(
                    tile.T, U32).reshape(2, 4, 8, LANES)

        def stage_wo(p, mm=plain_dot):
            for c in range(DT):
                acc = y_ref[:, pl.ds(c * LANES, LANES)]
                for t in range(3):
                    acc = acc + mm(ob_ref[p, :, pl.ds(t * LANES, LANES)],
                                   _rhs4(wo32, 3 * p + t, c), True)[0:8]
                y_ref[:, pl.ds(c * LANES, LANES)] = acc

        def w13(j, kg, n):
            rows = kg if n == 1 else pl.ds(kg, n)
            return wq32[rows, j // 2, 3] if j % 2 == 0 else w332[rows, j // 2]

        def ffn_up(x):
            xb, m, r = ln_stats(x)
            lhs = ln_lhs(xb)
            gu = []
            for j in range(2 * FT):
                acc = None
                for kk in range(DT):
                    d = dot(lhs[kk], _as_rhs(w13(j, 8 * kk, 8)))
                    acc = d if acc is None else acc + d
                cs_ref[j] = acc[8:16]
                gu.append((acc[0:8] - m * acc[8:16]) * r)
            hs = [_swiglu(g, u) for g, u in zip(gu[0::2], gu[1::2])]
            return [_pack2(hh, hh) for hh in hs]

        def col_bcast(v):
            return jnp.concatenate([v] * (LANES // 8), axis=0).T

        def vpu_fma(acc, w, xlo, xhi):
            w = pltpu.bitcast(w, BF).astype(F32)
            t = w[0:8] * xlo + w[8:16] * xhi
            return t if acc is None else acc + t

        def sub_sum(a):
            return jnp.broadcast_to(jnp.sum(a, axis=0, keepdims=True), a.shape)

        def ffn_down(x, hs, k0, k1):
            cols = [x[:, c * LANES:(c + 1) * LANES] for c in range(DT)]
            for kk in range(k0, k1):
                for c in range(DT):
                    cols[c] = cols[c] + dot(hs[kk], _rhs(w232, 8 * kk, c))[0:8]
            return jnp.concatenate(cols, axis=1)

        wait(0)
        x = jnp.broadcast_to(xbuf[...].astype(F32), (8, D))
        xb, m, r = ln_stats(x)
        xn = (xb - m) * r
        xn_ref[:, 0:D] = _pack2(xn, xn)
        y_ref[:, 0:D] = x

        def qloop(p, carry):
            stage_q(p)
            return carry

        lax.fori_loop(0, NP, qloop, 0)

        def group1(gi, fence_row):
            g = NGRP - 1 - gi
            for i in range(NGRP):
                pl.when(gi == i)(functools.partial(wait, 1 + i))

            def pair(j, carry):
                p = g * GP + j
                for k in range(nk):
                    stage_qk(p, k)
                pack_probs(p, softmax(p, 0)[0], softmax(p, 1)[0], 0)
                finish_o(p, pv_mxu(p, range(nc), False))
                first = 0
                for pp in range(NP - 1):
                    first = jnp.where(p == pp, nc - MC[pp], first)

                def tr(c, carry2):
                    transpose_v(p, c)
                    return carry2

                lax.fori_loop(first, nc, tr, 0)
                return carry

            lax.fori_loop(0, GP, pair, 0)
            return fence_row + GP * prow

        fence_row = lax.fori_loop(0, NGRP, group1, 8)
        fence_row = pl.multiple_of(fence_row, 8)
        wait(1 + NGRP)

        def woloop(p2, carry):
            stage_wo(2 * p2)
            stage_wo(2 * p2 + 1)
            return carry

        lax.fori_loop(0, NP // 2, woloop, 0)
        x = y_ref[:, 0:D]
        wait(2 + NGRP)
        hs = ffn_up(x)
        for i in range(len(W2_SPLIT) - 1):
            wait(3 + NGRP + i)
            x = ffn_down(x, hs, W2_SPLIT[i] // 8, W2_SPLIT[i + 1] // 8)

        y_ref[:, 0:D] = x
        xb, m, r = ln_stats(x)
        xn = (xb - m) * r
        xn_ref[:, 0:D] = _pack2(xn, xn)
        lhs0 = ln_lhs(xb)

        def first_q(p, scale, mm):
            for t in range(3):
                store_q(p, t, ln_proj(
                    lhs0, m, scale,
                    lambda kk: _as_rhs(wq32[pl.ds(8 * kk, 8), p, t]), mm))

        def run_block(chains, items, n_link, first, last_off, start=False, end=False):
            links = []
            for j, (p, g) in enumerate(chains[:n_link]):
                lo, hi = pv_chain(p, g, lambda: p_refs[g % 2])
                links.append((LINK0 + LINKSTEP * j,
                              pltpu.bitcast(lo, U32) | pltpu.bitcast(hi, U32)))
            pops = []
            probs = {}
            ready = {}
            if start and NVQ:
                xcol = []
                for kk in range(DT):
                    xt = col_bcast(xb[:, kk * LANES:(kk + 1) * LANES])
                    xcol.append(xt - m[0:1])
                dep = functools.reduce(
                    lambda a, b: a | b,
                    [pltpu.bitcast(xc[LANES - 8:], U32) for xc in xcol])
                links.extend([(XC_LINK, dep)] * XC_REP)

            def mm(l32, rr, free):
                links.sort(key=lambda lk: lk[0])
                if free is not None and links and len(pops) >= links[0][0]:
                    l32 = jnp.where((sub < 4) if free else (sub >= 4), l32,
                                    links.pop(0)[1])
                res = dot(l32, rr)
                pops.append(res)
                return res

            for it in items:
                kind, p = it[0], it[1]
                scale = r * qscale if p == 0 else None
                if kind == 'fq':
                    first_q(p, None if p == 0 else r * qscale, mm)
                elif kind == 'qka':
                    stage_qk_a(p, scale, mm)
                    ready[p] = len(pops)
                elif kind == 'qkb':
                    stage_qk_b(p, scale, mm)
                elif kind == 'q':
                    stage_q(p, mm)
                elif kind == 'qx':
                    for t in range(3):
                        expand_q(p, t, qpk_ref[3 * (NP - 1 - p) + t])
                elif kind == 'qk':
                    stage_qk(p, it[2], mm)
                    ready[p] = len(pops)
                elif kind == 'sm':
                    dep = None
                    for hd in it[2]:
                        probs[p, hd], l = softmax(p, hd)
                        dep = l if dep is None else dep + l
                    lag = SM_LAG0 if p < NSPLIT else SM_LAG
                    links.extend([(len(pops) + (lag if pops else lag - 14),
                                   pltpu.bitcast(dep, U32))] * SM_REP)
                    if p == NP - 1:
                        pack_probs(p, probs.pop((p, 0)), probs.pop((p, 1)), 0)
                    elif MC[p] and hd == 1:
                        pack_probs(p, probs[p, 0], probs[p, 1], (nc - MC[p]) // 8)
                elif kind == 'pvm':
                    stage_pvm(p, *it[2:], mm)
                elif kind == 'red':
                    stage_reduce(p)
                elif kind == 'wo':
                    stage_wo(p, mm)

            def store_probs(p, hd):
                e = probs.pop((p, hd))
                for pr in p_refs:
                    pr[pl.ds(p * prow + hd * nc, nc), :] = e

            def make_gate(n_items, a0, a1, phase):
                n_units = (a1 - a0) // FSTEP
                state = [0, -1]

                def gate():
                    u = state[0] * n_units // n_items
                    state[0] += 1
                    buf = p_refs[(u + phase) % 2]
                    if u != state[1]:
                        state[1] = u
                        buf[pl.ds(fence_row, 8), :] = pops[a0 + u * FSTEP][0:8]
                    return buf

                return gate, state, n_units

            if start and NVQ:
                xc0 = NP * prow + 32
                nkg = D // 16
                cols = [(p, t) for p in range(NP - NVQ, NP) for t in range(3)]

                def put(kk):
                    for i in range(8):
                        p_refs[i % 2][pl.ds(xc0 + LANES * kk + 16 * i, 16), :] = (
                            xcol[kk][16 * i:16 * i + 16])

                acc = [None] * len(cols)
                for kg in range(nkg):
                    for kk in range(DT):
                        if XC_PUT[kk] == kg:
                            put(kk)
                    buf = p_refs[kg % 2]
                    buf[pl.ds(fence_row, 8), :] = pops[
                        VQ_FIRST + kg * (first - VQ_FIRST) // nkg][0:8]
                    xlo = buf[pl.ds(xc0 + 16 * kg, 8), :]
                    xhi = buf[pl.ds(xc0 + 16 * kg + 8, 8), :]
                    for i, (p, t) in enumerate(cols):
                        acc[i] = vpu_fma(acc[i], wq32[kg, p, t], xlo, xhi)
                for i, (p, t) in enumerate(cols):
                    q = sub_sum(acc[i]) * (r * qscale)
                    qpk_ref[3 * (NP - 1 - p) + t] = _pack2(q, q)

            rest = chains[n_link:]
            if rest:
                gate, state, _ = make_gate(sum(nc - MC[p] for p, _ in rest), first,
                                           len(pops) - last_off + FSTEP, 0)
            for p, g in rest:
                if (p, g // HG) in probs:
                    if g == 0 and p in ready:
                        _LOG.append((p, first + state[1] * FSTEP - ready[p]))
                    store_probs(p, g // HG)
                pv_chain(p, g, gate)
            for key in list(probs):
                store_probs(*key)

            if end:
                last_ffn(mm, pops, links)

        def last_ffn(mm, pops, links):
            x = y_ref[:, 0:D]
            xb, m, r = ln_stats(x)
            lhs = _pack2(xb, xb)
            base = len(pops)
            xcol = [col_bcast(xb[:, kk * LANES:(kk + 1) * LANES]) for kk in range(UP_K)]
            j0 = 2 * (FT - UP_COLS)
            part = {}
            for j in range(j0, 2 * FT):
                acc = None
                for kg in range(8 * UP_K):
                    xc = xcol[kg // 8][16 * (kg % 8):16 * (kg % 8) + 16]
                    acc = vpu_fma(acc, w13(j, kg, 1), xc[0:8], xc[8:16])
                part[j] = sub_sum(acc)
                links.append((base + int(UP_LINK0 + UP_LINKSTEP * (j - j0)),
                              pltpu.bitcast(part[j], U32)))
            gu = []
            for j in range(2 * FT):
                acc = part.get(j)
                for kk in range(UP_K if j in part else 0, DT):
                    d = mm(lhs[:, kk * LANES:(kk + 1) * LANES],
                           _as_rhs(w13(j, 8 * kk, 8)), True)[0:8]
                    acc = d if acc is None else acc + d
                gu.append((acc - m * cs_ref[j]) * r)
            hs = [_swiglu(g, u) for g, u in zip(gu[0::2], gu[1::2])]
            cols = [x[:, c * LANES:(c + 1) * LANES] for c in range(DT)]
            for kk in range(DOWN_K, FT):
                hh = _pack2(hs[kk], hs[kk])
                for c in range(DT):
                    cols[c] = cols[c] + mm(hh, _rhs(w232, 8 * kk, c), True)[0:8]
            if DOWN_K:
                acc = [None] * DT
                for kk in range(DOWN_K):
                    hcol = col_bcast(hs[kk].astype(BF).astype(F32))
                    for i in range(8):
                        for c in range(DT):
                            acc[c] = vpu_fma(acc[c], w232[8 * kk + i, c],
                                             hcol[16 * i:16 * i + 8],
                                             hcol[16 * i + 8:16 * i + 16])
                cols = [cc + sub_sum(a) for cc, a in zip(cols, acc)]
            o_ref[...] = jnp.concatenate(cols, axis=1)[0:1].astype(o_ref.dtype)

        blocks = _plan(nc)
        for b, blk in enumerate(blocks):
            if b == 0 or b == len(blocks) - 1:
                run_block(*blk, start=b == 0, end=b > 0)
            else:
                pl.when(fence_row > b)(functools.partial(run_block, *blk))

    return kernel


@jax.jit
def pallas_interleave_layers__sliding_block_cached__glu_gated_swiglu__decode_kernel(
    A_x: jax.Array,
    A_k_cache: jax.Array,
    A_v_cache: jax.Array,
    A_wq: jax.Array,
    A_wo: jax.Array,
    B_x: jax.Array,
    B_w1: jax.Array,
    B_w3: jax.Array,
    B_w2: jax.Array,
):
    sk = A_k_cache.shape[2]
    win = min(4096, max(256, sk // 4))
    nt_total, nc = sk // LANES, win // LANES

    def kv_view(a):
        return _tile_view(jnp.swapaxes(a, 2, 3).reshape(H * DH, sk))

    def wbuf(r, c):
        return pltpu.VMEM((r // 16, c // LANES, 16, LANES), BF)

    def wbuf4(r, c):
        return pltpu.VMEM((r // 64, 4, c // LANES, 16, LANES), BF)

    def view4(t):
        return t.reshape(t.shape[0] // 4, 2, 4, t.shape[2], 8, LANES)

    any_spec = pl.BlockSpec(memory_space=pl.ANY)
    out = pl.pallas_call(
        _make_kernel(nt_total, nc),
        out_shape=jax.ShapeDtypeStruct((1, D), A_x.dtype),
        in_specs=[any_spec] * 8,
        out_specs=pl.BlockSpec(memory_space=pltpu.VMEM),
        scratch_shapes=[
            wbuf(H * DH, win), wbuf4(H * DH, win),
            pltpu.VMEM((D // 16, NP, 4, 16, LANES), BF),
            wbuf4(H * DH, D), wbuf(D, F), wbuf(F, D),
            pltpu.VMEM((NP - 1, PW, LANES), F32),
            pltpu.VMEM((NP * PG, 8, LANES), U32),
            pltpu.VMEM((NP, 2 * nc, LANES), F32),
            pltpu.VMEM((NP * 2 * nc + 32 + D, LANES), F32),
            pltpu.VMEM((NP * 2 * nc + 32 + D, LANES), F32),
            pltpu.VMEM((NP, nc // 8, 8, LANES), U32),
            pltpu.VMEM((NP, 4, 8, LANES), F32),
            pltpu.VMEM((NP, 8, 512), F32),
            pltpu.VMEM((NP, 8, 512), U32),
            pltpu.VMEM((32, 8, LANES), U32),
            pltpu.VMEM((2 * FT, 8, LANES), F32),
            pltpu.VMEM((24, 8, LANES), U32),
            pltpu.VMEM((8, 1024), U32),
            pltpu.VMEM((8, 1024), F32),
            pltpu.VMEM((1, D), BF),
            pltpu.SemaphoreType.DMA((NSEM,)),
        ],
        compiler_params=pltpu.CompilerParams(
            vmem_limit_bytes=127 * 1024 * 1024),
    )(A_x.reshape(1, D), kv_view(A_k_cache), view4(kv_view(A_v_cache)),
      _tile_view(A_wq).reshape(D // 16, 2, NP, 3, 8, LANES), view4(_tile_view(A_wo)),
      _tile_view(B_w1), _tile_view(B_w3), _tile_view(B_w2))
    return out.reshape(A_x.shape)
```

```python
import functools
import math

import jax
import jax.numpy as jnp
from jax import lax
import jax.experimental.pallas as pl
import jax.experimental.pallas.tpu as pltpu

D = 640
H = 32
DH = 192
F = 1536
LANES = 128
EPS = 1e-5

NP = H // 2
PG = 2 * DH // 16
HG = DH // 16
PW = 2 * DH
DT = D // LANES
FT = F // LANES

GP = 4
NGRP = NP // GP
W2_SPLIT = (0, 56, 88, 96)

NSEM = 3

MC = (4, 4, 4, 4, 4, 4, 4, 4, 4, 4, 5, 5, 4, 4, 4)
VQ = (11, 12, 13, 14, 15)
ORDER = tuple(range(NP))
V_END = (174, 290, 351)
TILES = (1100, 650, 345)
PVM_AFTER = 2
WO_START = (0, 60, 60, 999)
WO_GAP = (0, 70, 48, 12)
WO_KEEP = 3
NVW = 0
VW_LINK = 62
VW_STEP = 4.5
UP_REP = 1
FIN_REP = 1
HC_REP = 4
DN_FIRST = 0
DN_LAST = 6
UX_LINK = 999
SPLIT_MODE = 1
FIN_ORDER = (NP - 1, NP - 2)
SM_LAG = 60
SM_LAG0 = 42
VQ_FIRST = 28
VQ_UNIT = 4
XC_LINK = 46
UP_K = 3
UP_COLS = 5
UP_LINK0 = 50
UP_LINKSTEP = 4.5
DOWN_K = 3
HC_LINK = (999, 999, 999, 999, 999, 999)
NLINK = 3
LINK0 = 8
LINKSTEP = 4
LINK_REP = 4
FIN_LINK0 = 4
FIN_LINKSTEP = 6
FSTEP = 2
FIRST = (150, 0, 0)
LAST_OFF = (8, 6, 4)

U32 = jnp.uint32
BF = jnp.bfloat16
F32 = jnp.float32


def _tile_view(w):
    r, c = w.shape
    return jnp.swapaxes(w.reshape(r // 16, 2, 8, c // LANES, LANES), 2, 3)


def _as_rhs(w):
    return pltpu.bitcast(w.reshape(8 * 8, LANES), BF)


def _rhs(w32, g0, c):
    return _as_rhs(w32[pl.ds(g0, 8), c])


def _rhs4(w32, tile, c):
    return _as_rhs(w32[pl.ds(2 * tile, 2), :, c])


def _swiglu(g, u):
    hg = 0.5 * g
    return hg * (1.0 + jnp.tanh(hg)) * u


def _pack2(lo, hi):
    return pltpu.bitcast(jnp.concatenate([lo, hi], axis=0).astype(BF), U32)


_LOG = []
ONLY = None


def _plan(nc):
    nk = nc // 8
    seq = [('fq', 0), ('fq', 1)]
    for i, p in enumerate(ORDER):
        if 1 <= i < NP - 1:
            seq.append(('qx' if ORDER[i + 1] in VQ else 'q', ORDER[i + 1]))
        for k in range(nk):
            pp = ORDER[i - 1]
            if k == PVM_AFTER and i > 0 and pp < NP - 1 and MC[pp]:
                seq.append(('pvm', pp, nc - MC[pp], nc, False))
            seq.append(('qk', p, k))
        seq.append(('sm', p))
    tail = [('pvm', NP - 1, c, c + 4, c > 0) for c in range(0, nc, 4)]
    last_pv = tail[0] if ORDER[-1] == NP - 1 else None
    if last_pv is None:
        tail.insert(4, ('pvm', ORDER[-1], nc - MC[ORDER[-1]], nc, False))
    seq += tail

    def tiles(it):
        if it[0] == 'pvm':
            return 3 * (it[3] - it[2])
        return dict(fq=15, q=15, wo=15, qk=24, sm=0, red=0, qx=0)[it[0]]

    chains = [(p, g) for p in range(NP - 1) for g in range(PG)]
    blocks = []
    v0 = done = 0
    for b in range(len(V_END) + 1):
        final = b == len(V_END)
        v1 = len(chains) if final else V_END[b]
        todo = list(range(done, v0 // PG))
        done = v0 // PG
        reds = [('red', p) for p in todo]
        if b == len(V_END) - 1 and NVW:
            vpu_wo, todo = todo[-NVW:], todo[:-NVW]
        budget = 10 ** 9 if final else TILES[b] - 15 * len(todo)
        body = []
        used = 0
        while seq and used + tiles(seq[0]) // 2 <= budget:
            body.append(seq.pop(0))
            used += tiles(body[-1])
        if body[-1][0] == 'sm':
            seq.insert(0, body.pop())
        keep = WO_KEEP if last_pv in body else 0
        items = reds + ([('vwo', p) for p in vpu_wo] if final and NVW else [])
        used = 0
        nxt = WO_START[b]
        for it in body:
            if it == last_pv:
                while todo:
                    items.append(('wo', todo.pop(0)))
            if len(todo) > keep and used >= nxt:
                items.append(('wo', todo.pop(0)))
                nxt = used + WO_GAP[b]
            items.append(it)
            used += tiles(it)
        items += [('wo', p) for p in todo]
        if final:
            for p in FIN_ORDER:
                items += [('red', p), ('wo', p)]
            blocks.append((chains[v0:v1], items, v1 - v0, 0, 0))
        else:
            blocks.append((chains[v0:v1], items, NLINK if b else 0, FIRST[b], LAST_OFF[b]))
        v0 = v1
    return blocks


def _make_kernel(n_tiles_total, nc):
    c0 = n_tiles_total - nc
    qscale = DH ** -0.5 * math.log2(math.e)
    prow = 2 * nc
    nk = nc // 8

    def kernel(x_hbm, k_hbm, v_hbm, wq_hbm, wo_hbm, w1_hbm, w3_hbm, w2_hbm,
               o_ref,
               kbuf, vbuf, wqbuf, wobuf, w3buf, w2buf,
               t_ref, lhs_ref, s_ref, p_ref, p2_ref, pk_ref, lsum_ref, om_ref, ob_ref,
               mask_ref, cs_ref, qpk_ref, xn_ref, y_ref, xbuf, sem):
        def halves(src, dst):
            return [(src(par), dst(pl.ds(8 * par, 8))) for par in range(2)]

        def kv_group(g):
            kr = pl.ds(g * GP * PG, GP * PG)
            vr = pl.ds(g * GP * PG // 4, GP * PG // 4)
            return (halves(lambda p: k_hbm.at[kr, p, pl.ds(c0, nc)],
                           lambda h: kbuf.at[kr, :, h, :])
                    + halves(lambda p: v_hbm.at[vr, p, :, pl.ds(c0, nc)],
                             lambda h: vbuf.at[vr, :, :, h, :]))

        def w2_group(i):
            rows = pl.ds(W2_SPLIT[i], W2_SPLIT[i + 1] - W2_SPLIT[i])
            return halves(lambda p: w2_hbm.at[rows, p], lambda h: w2buf.at[rows, :, h, :])

        wq_group = halves(lambda p: wq_hbm.at[:, p],
                          lambda h: wqbuf.at[:, :, pl.ds(0, 3), h, :]) + [(x_hbm, xbuf)]
        wo_group = halves(lambda p: wo_hbm.at[:, p], lambda h: wobuf.at[:, :, :, h, :])
        w13_group = (halves(lambda p: w1_hbm.at[:, p],
                            lambda h: wqbuf.at[:, pl.ds(0, FT), 3, h, :])
                     + halves(lambda p: w3_hbm.at[:, p], lambda h: w3buf.at[:, :, h, :]))
        groups = ([wq_group] + [kv_group(NGRP - 1 - g) for g in range(NGRP)]
                  + [wo_group, w13_group]
                  + [w2_group(i) for i in range(len(W2_SPLIT) - 1)])
        n_real = len(groups)
        if SPLIT_MODE and ONLY is None:
            groups.append([(x_hbm, xbuf)])

        def copies(i):
            return [pltpu.make_async_copy(src, dst, sem.at[i % NSEM])
                    for src, dst in groups[i]]

        def start(i):
            for cp in copies(i):
                cp.start()

        def wait(i):
            for cp in copies(i):
                cp.wait()
            if i + NSEM < len(groups):
                start(i + NSEM)

        for i in range(NSEM):
            start(i)

        k32 = kbuf.bitcast(U32)
        v32 = vbuf.bitcast(U32)
        wq32 = wqbuf.bitcast(U32)
        wo32 = wobuf.bitcast(U32)
        w332 = w3buf.bitcast(U32)
        w232 = w2buf.bitcast(U32)

        sub = lax.broadcasted_iota(jnp.int32, (8, LANES), 0)
        lane = lax.broadcasted_iota(jnp.int32, (8, LANES), 1)
        lane3 = lax.broadcasted_iota(jnp.int32, (8, PW), 1)

        for r in range(4):
            half = U32(0x0000FFFF if r % 2 == 0 else 0xFFFF0000)
            lo = jnp.where(sub == r // 2, half, U32(0))
            hi = jnp.where(sub == 2 + r // 2, half, U32(0))
            mask_ref[r] = lo
            mask_ref[4 + r] = jnp.where(lane < DH - LANES, lo, hi)
            mask_ref[8 + r] = hi
            mask_ref[12 + r] = lo | hi
        p_refs = (p_ref, p2_ref)
        for pr in p_refs:
            pr[...] = jnp.zeros(pr.shape, F32)

        def dot(l32, r):
            return jnp.dot(pltpu.bitcast(l32, BF), r, preferred_element_type=F32)

        def plain_dot(l32, r, free):
            del free
            return dot(l32, r)

        def ln_stats(x):
            xb = x.astype(BF).astype(F32)
            m = jnp.mean(xb, axis=-1, keepdims=True)
            xc = xb - m
            v = jnp.mean(xc * xc, axis=-1, keepdims=True)
            return xb, m, lax.rsqrt(v + EPS)

        def ln_lhs(xb):
            l = _pack2(xb, jnp.ones_like(xb))
            return [l[:, kk * LANES:(kk + 1) * LANES] for kk in range(DT)]

        def ln_proj(lhs, m, r, tile, mm=plain_dot):
            acc = None
            for kk in range(DT):
                d = mm(lhs[kk], tile(kk), None)
                acc = d if acc is None else acc + d
            c = acc[0:8] - m * acc[8:16]
            return c if r is None else c * r

        def store_q(p, t, q):
            expand_q(p, t, _pack2(q, q))

        def expand_q(p, t, q):
            for r in range(4):
                lhs_ref[12 * p + 4 * t + r] = q & mask_ref[4 * t + r]

        def stage_q(p, mm=plain_dot):
            acc = [None] * 3
            for kk in range(DT):
                for t in range(3):
                    d = mm(xn_ref[:, pl.ds(kk * LANES, LANES)],
                           _as_rhs(wq32[pl.ds(8 * kk, 8), p, t]), True)[0:8]
                    acc[t] = d if acc[t] is None else acc[t] + d
            for t in range(3):
                store_q(p, t, acc[t] * qscale)

        def stage_qk(p, k, mm=plain_dot, scale=None):
            for j in range(2 * k, 2 * k + 2):
                acc = None
                for t in range(3):
                    for r in range(4):
                        d = mm(lhs_ref[12 * p + 4 * t + r],
                               _rhs(k32, p * PG + 8 * t, 4 * j + r), True)[0:8]
                        acc = d if acc is None else acc + d
                s_ref[p, pl.ds(8 * j, 8), :] = acc if scale is None else acc * scale

        def head_reduce(v, op, lane_op):
            for d in (1, 2):
                up = pltpu.roll(v, d, 0)
                down = pltpu.roll(v, 8 - d, 0)
                v = op(v, jnp.where(sub % (2 * d) >= d, up, down))
            return lane_op(v, axis=1, keepdims=True)

        def softmax(p, j0):
            s = s_ref[p].reshape(nc // 4, 8, LANES)
            m = head_reduce(jnp.max(s, axis=0), jnp.maximum, jnp.max)
            e = jnp.exp2(s - m)
            l = jnp.sum(e, axis=0)
            lsum_ref[p] = l
            for j in range(j0, nc // 4):
                pk_ref[p, j] = _pack2(e[j], e[j])
            return e.reshape(prow, LANES), l

        def pv_chain(p, g, gate):
            lo = hi = None
            for c in range(nc - MC[p]):
                w = pltpu.bitcast(v32[p * (PG // 4) + g // 4, g % 4, c], BF).astype(F32)
                row = p * prow + 8 * (c // 4) + 4 * (g // HG) + c % 4
                pb = gate()[pl.ds(row, 8, stride=0), :]
                tl = w[0:8] * pb
                th = w[8:16] * pb
                lo = tl if lo is None else lo + tl
                hi = th if hi is None else hi + th
            t_ref[p, pl.ds(16 * g, 8), :] = lo
            t_ref[p, pl.ds(16 * g + 8, 8), :] = hi
            return lo, hi

        def pv_mxu(p, cols, transposed, mm=plain_dot):
            acc = [None] * 3
            cols = list(cols)
            for i0 in range(0, len(cols), 4):
                ls = {c: pk_ref[p, c // 4] & mask_ref[12 + c % 4]
                      for c in cols[i0:i0 + 4]}
                for t in range(3):
                    for c, l in ls.items():
                        tile = _rhs4(v32, 3 * p + t, c)
                        if transposed:
                            res = mm(l, tile, True)
                        else:
                            res = lax.dot_general(
                                pltpu.bitcast(l, BF), tile, (((1,), (1,)), ((), ())),
                                preferred_element_type=F32)
                        acc[t] = res[0:8] if acc[t] is None else acc[t] + res[0:8]
            return jnp.concatenate(acc, axis=1)

        def stage_pvm(p, ca, cb, accumulate, mm):
            o = pv_mxu(p, range(ca, cb), True, mm)
            if accumulate:
                o = o + om_ref[p, :, 0:PW]
            om_ref[p, :, 0:PW] = o

        def own_head(o):
            sub3 = lax.broadcasted_iota(jnp.int32, (8, PW), 0)
            return jnp.where((sub3 < 4) == (lane3 < DH), o, 0.0)

        def finish_o(p, o):
            linv = 1.0 / head_reduce(lsum_ref[p], jnp.add, jnp.sum)
            o = (jnp.sum(o, axis=0, keepdims=True)
                 * jnp.where(lane3 < DH, linv[0:1], linv[4:5]))
            ob_ref[p, :, 0:PW] = _pack2(o, o)

        def stage_reduce(p):
            if p == NP - 1:
                o = own_head(om_ref[p, :, 0:PW])
            else:
                o = jnp.sum(t_ref[p].T.reshape(LANES // 8, 8, PW), axis=0)
                if MC[p]:
                    o = o + own_head(om_ref[p, :, 0:PW])
            finish_o(p, o)

        def transpose_v(p, c):
            for t in range(3):
                tile = _rhs4(v32, 3 * p + t, c)
                v32[pl.ds(2 * (3 * p + t), 2), :, c] = pltpu.bitcast(
                    tile.T, U32).reshape(2, 4, 8, LANES)

        def stage_wo(p, mm=plain_dot):
            for c in range(DT):
                acc = y_ref[:, pl.ds(c * LANES, LANES)]
                for t in range(3):
                    acc = acc + mm(ob_ref[p, :, pl.ds(t * LANES, LANES)],
                                   _rhs4(wo32, 3 * p + t, c), True)[0:8]
                y_ref[:, pl.ds(c * LANES, LANES)] = acc

        def w13(j, kg, n):
            rows = kg if n == 1 else pl.ds(kg, n)
            return wq32[rows, j // 2, 3] if j % 2 == 0 else w332[rows, j // 2]

        def ffn_up(x):
            xb, m, r = ln_stats(x)
            lhs = ln_lhs(xb)
            gu = []
            for j in range(2 * FT):
                acc = None
                for kk in range(DT):
                    d = dot(lhs[kk], _as_rhs(w13(j, 8 * kk, 8)))
                    acc = d if acc is None else acc + d
                cs_ref[j] = acc[8:16]
                gu.append((acc[0:8] - m * acc[8:16]) * r)
            hs = [_swiglu(g, u) for g, u in zip(gu[0::2], gu[1::2])]
            return [_pack2(hh, hh) for hh in hs]

        def col_bcast(v):
            return jnp.concatenate([v] * (LANES // 8), axis=0).T

        def vpu_fma(acc, w, xlo, xhi):
            w = pltpu.bitcast(w, BF).astype(F32)
            t = w[0:8] * xlo + w[8:16] * xhi
            return t if acc is None else acc + t

        def sub_sum(a):
            return jnp.broadcast_to(jnp.sum(a, axis=0, keepdims=True), a.shape)

        def ffn_down(x, hs, k0, k1):
            cols = [x[:, c * LANES:(c + 1) * LANES] for c in range(DT)]
            for kk in range(k0, k1):
                for c in range(DT):
                    cols[c] = cols[c] + dot(hs[kk], _rhs(w232, 8 * kk, c))[0:8]
            return jnp.concatenate(cols, axis=1)

        wait(0)
        x = jnp.broadcast_to(xbuf[...].astype(F32), (8, D))
        xb, m, r = ln_stats(x)
        xn = (xb - m) * r
        xn_ref[:, 0:D] = _pack2(xn, xn)
        y_ref[:, 0:D] = x

        def qloop(p, carry):
            stage_q(p)
            t_ref[jnp.minimum(p, NP - 2), 0:8, :] = jnp.zeros((8, LANES), F32)
            om_ref[p] = jnp.zeros(om_ref.shape[1:], F32)
            qpk_ref[p] = jnp.zeros((8, LANES), U32)
            cs_ref[p] = jnp.zeros((8, LANES), F32)
            return carry

        lax.fori_loop(0, NP, qloop, 0)

        def group1(gi, fence_row):
            g = NGRP - 1 - gi
            for i in range(NGRP):
                pl.when(gi == i)(functools.partial(wait, 1 + i))

            def pair(j, carry):
                p = g * GP + j
                for k in range(nk):
                    stage_qk(p, k)
                softmax(p, 0)
                finish_o(p, own_head(pv_mxu(p, range(nc), False)))
                first = 0
                for pp in range(NP - 1):
                    first = jnp.where(p == pp, nc - MC[pp], first)

                def tr(c, carry2):
                    transpose_v(p, c)
                    return carry2

                lax.fori_loop(first, nc, tr, 0)
                return carry

            lax.fori_loop(0, GP, pair, 0)
            return fence_row + GP * prow

        fence_row = lax.fori_loop(0, NGRP, group1, 0)
        fence_row = pl.multiple_of(fence_row, 8)
        wait(1 + NGRP)

        def woloop(p2, carry):
            stage_wo(2 * p2)
            stage_wo(2 * p2 + 1)
            return carry

        lax.fori_loop(0, NP // 2, woloop, 0)
        x = y_ref[:, 0:D]
        wait(2 + NGRP)
        hs = ffn_up(x)
        for i in range(len(W2_SPLIT) - 1):
            wait(3 + NGRP + i)
            x = ffn_down(x, hs, W2_SPLIT[i] // 8, W2_SPLIT[i + 1] // 8)

        y_ref[:, 0:D] = x
        xb, m, r = ln_stats(x)
        xn = (xb - m) * r
        xn_ref[:, 0:D] = _pack2(xn, xn)
        lhs0 = ln_lhs(xb)

        def first_q(p, scale, mm):
            for t in range(3):
                store_q(p, t, ln_proj(
                    lhs0, m, scale,
                    lambda kk: _as_rhs(wq32[pl.ds(8 * kk, 8), p, t]), mm))

        def run_block(chains, items, n_link, first, last_off, start=False, end=False):
            links = []
            for j, (p, g) in enumerate(chains[:n_link]):
                lo, hi = pv_chain(p, g, lambda: p_refs[g % 2])
                pos = FIN_LINK0 + FIN_LINKSTEP * j if end else LINK0 + LINKSTEP * j
                links.extend([(pos, pltpu.bitcast(lo, U32) | pltpu.bitcast(hi, U32))]
                             * (FIN_REP if end else LINK_REP))
            pops = []
            probs = {}
            ready = {}
            if start:
                xcol = []
                for kk in range(DT):
                    xt = col_bcast(xb[:, kk * LANES:(kk + 1) * LANES])
                    xcol.append(xt - m[0:1])
                dep = functools.reduce(
                    lambda a, b: a | b,
                    [pltpu.bitcast(xc[LANES - 8:], U32) for xc in xcol])
                links.extend([(XC_LINK, dep)] * 4)

            def mm(l32, rr, free):
                links.sort(key=lambda lk: lk[0])
                if free is not None and links and len(pops) >= links[0][0]:
                    l32 = jnp.where(sub < 4, l32, links.pop(0)[1])
                res = dot(l32, rr)
                pops.append(res)
                return res

            y_vpu = [None] * DT
            n_vw = 0
            for it in items:
                kind, p = it[0], it[1]
                if kind == 'fq':
                    first_q(p, None if p == 0 else r * qscale, mm)
                elif kind == 'q':
                    stage_q(p, mm)
                elif kind == 'qx':
                    for t in range(3):
                        expand_q(p, t, qpk_ref[3 * VQ.index(p) + t])
                elif kind == 'qk':
                    stage_qk(p, it[2], mm, r * qscale if p == 0 else None)
                    ready[p] = len(pops)
                elif kind == 'sm':
                    e, l = softmax(p, 0 if p == NP - 1 else (nc - MC[p]) // 4)
                    lag = SM_LAG0 if p == 0 else SM_LAG
                    links.append((len(pops) + (lag if pops else lag - 14),
                                  pltpu.bitcast(l, U32)))
                    if p < NP - 1:
                        probs[p] = e
                elif kind == 'pvm':
                    stage_pvm(p, *it[2:], mm)
                elif kind == 'red':
                    stage_reduce(p)
                elif kind == 'wo':
                    stage_wo(p, mm)
                elif kind == 'vwo':
                    ocol = []
                    for t in range(3):
                        o = pltpu.bitcast(ob_ref[p, :, pl.ds(t * LANES, LANES)], BF)
                        ocol.append(col_bcast(o[0:8].astype(F32)))
                    for c in range(DT):
                        for g in range(PG):
                            oc = ocol[g // 8][16 * (g % 8):16 * (g % 8) + 16]
                            y_vpu[c] = vpu_fma(y_vpu[c], wo32[6 * p + g // 4, g % 4, c],
                                               oc[0:8], oc[8:16])
                        links.extend([(int(VW_LINK + VW_STEP * n_vw),
                                       pltpu.bitcast(y_vpu[c], U32))] * FIN_REP)
                        n_vw += 1

            def store_probs(p):
                e = probs.pop(p)
                n = 8 * ((nc - MC[p] + 3) // 4)
                for pr in p_refs:
                    pr[pl.ds(p * prow, n), :] = e[0:n]

            def make_gate(n_items, a0, a1, phase):
                n_units = (a1 - a0) // FSTEP
                state = [0, -1]

                def gate():
                    u = state[0] * n_units // n_items
                    state[0] += 1
                    buf = p_refs[(u + phase) % 2]
                    if u != state[1]:
                        state[1] = u
                        buf[pl.ds(fence_row, 8), :] = pops[a0 + u * FSTEP][0:8]
                    return buf

                return gate, state, n_units

            if start:
                xc0 = NP * prow + 32
                nkg = D // 16
                for kg in range(nkg):
                    p_refs[(kg // VQ_UNIT) % 2][pl.ds(xc0 + 16 * kg, 16), :] = (
                        xcol[kg // 8][16 * (kg % 8):16 * (kg % 8) + 16])
                for i, p in enumerate(VQ):
                    acc = [None] * 3
                    for kg in range(nkg):
                        buf = p_refs[(kg // VQ_UNIT) % 2]
                        if kg % VQ_UNIT == 0:
                            a = (i * nkg + kg) * (first - VQ_FIRST) // (len(VQ) * nkg)
                            buf[pl.ds(fence_row, 8), :] = pops[VQ_FIRST + a // 2 * 2][0:8]
                        xlo = buf[pl.ds(xc0 + 16 * kg, 8), :]
                        xhi = buf[pl.ds(xc0 + 16 * kg + 8, 8), :]
                        for t in range(3):
                            acc[t] = vpu_fma(acc[t], wq32[kg, p, t], xlo, xhi)
                    for t in range(3):
                        q = sub_sum(acc[t]) * (r * qscale)
                        qpk_ref[3 * i + t] = _pack2(q, q)

            rest = chains[n_link:]
            if rest:
                gate, state, _ = make_gate(sum(nc - MC[p] for p, _ in rest), first,
                                           len(pops) - last_off + FSTEP, 0)
            for p, g in rest:
                if p in probs:
                    if p in ready:
                        _LOG.append((p, first + state[1] * FSTEP - ready[p]))
                    store_probs(p)
                pv_chain(p, g, gate)
            for key in list(probs):
                store_probs(key)

            if end:
                x = y_ref[:, 0:D]
                if NVW:
                    x = x + jnp.concatenate([sub_sum(a) for a in y_vpu], axis=1)
                last_ffn(x, mm, pops, links)

        def last_ffn(x, mm, pops, links):
            xb, m, r = ln_stats(x)
            lhs = _pack2(xb, xb)
            base = len(pops)
            xcol = [col_bcast(xb[:, kk * LANES:(kk + 1) * LANES]) for kk in range(UP_K)]
            dep = functools.reduce(
                lambda a, b: a | b, [pltpu.bitcast(xc[LANES - 8:], U32) for xc in xcol])
            links.extend([(base + UX_LINK, dep)] * 4)
            j0 = 2 * (FT - UP_COLS)
            part = {}
            for j in range(j0, 2 * FT):
                acc = None
                for kg in range(8 * UP_K):
                    xc = xcol[kg // 8][16 * (kg % 8):16 * (kg % 8) + 16]
                    acc = vpu_fma(acc, w13(j, kg, 1), xc[0:8], xc[8:16])
                part[j] = sub_sum(acc)
                links.extend([(base + int(UP_LINK0 + UP_LINKSTEP * (j - j0)),
                               pltpu.bitcast(part[j], U32))] * UP_REP)
            gu, hs, hcol = [], [], []
            for j in range(2 * FT):
                acc = part.get(j)
                for kk in range(UP_K if j in part else 0, DT):
                    d = mm(lhs[:, kk * LANES:(kk + 1) * LANES],
                           _as_rhs(w13(j, 8 * kk, 8)), True)[0:8]
                    acc = d if acc is None else acc + d
                gu.append((acc - m * cs_ref[j]) * r)
                if j % 2:
                    hs.append(_swiglu(gu[-2], gu[-1]))
                    if j // 2 < DOWN_K:
                        hcol.append(col_bcast(hs[-1].astype(BF).astype(F32)))
                        links.extend([(base + HC_LINK[j // 2],
                                       pltpu.bitcast(hcol[-1][LANES - 8:], U32))] * HC_REP)
            cols = [x[:, c * LANES:(c + 1) * LANES] for c in range(DT)]
            for kk in range(DOWN_K, FT):
                hh = _pack2(hs[kk], hs[kk])
                for c in range(DT):
                    cols[c] = cols[c] + mm(hh, _rhs(w232, 8 * kk, c), True)[0:8]
            acc = [None] * DT
            xc0 = NP * prow + 32
            for kk in range(DOWN_K):
                if DN_FIRST and kk % 2 == 0:
                    for k2 in range(kk, min(kk + 2, DOWN_K)):
                        for i in range(8):
                            p_refs[(i // 2) % 2][pl.ds(xc0 + LANES * k2 + 16 * i, 16), :] = (
                                hcol[k2][16 * i:16 * i + 16])
                for i in range(8):
                    if DN_FIRST:
                        buf = p_refs[(i // 2) % 2]
                        if i % 2 == 0:
                            span = len(pops) - DN_LAST - base - DN_FIRST
                            a = base + DN_FIRST + (8 * kk + i) * span // (8 * DOWN_K - 2)
                            buf[pl.ds(fence_row, 8), :] = pops[a][0:8]
                        hc = buf[pl.ds(xc0 + LANES * kk + 16 * i, 16), :]
                    else:
                        hc = hcol[kk][16 * i:16 * i + 16]
                    for c in range(DT):
                        acc[c] = vpu_fma(acc[c], w232[8 * kk + i, c], hc[0:8], hc[8:16])
            cols = [cc + sub_sum(a) for cc, a in zip(cols, acc)]
            o_ref[...] = jnp.concatenate(cols, axis=1)[0:1].astype(o_ref.dtype)

        blocks = _plan(nc)
        for b, blk in enumerate(blocks):
            if ONLY is not None and b not in ONLY and b < len(blocks) - 1:
                if b == 1:
                    @pl.when(fence_row > b)
                    def _():
                        for pp in range(NP - 1):
                            stage_reduce(pp)
                            expand_q(pp, 0, qpk_ref[pp])
                continue
            if SPLIT_MODE and ONLY is None:
                if b > 0:
                    wait(n_real)
                    if b < len(blocks) - 1:
                        start(n_real)
                run_block(*blk, start=b == 0, end=b == len(blocks) - 1)
            elif b == 0 or b == len(blocks) - 1:
                run_block(*blk, start=b == 0, end=b > 0)
            else:
                pl.when(fence_row > b)(functools.partial(run_block, *blk))

    return kernel


@jax.jit
def pallas_interleave_layers__sliding_block_cached__glu_gated_swiglu__decode_kernel(
    A_x: jax.Array,
    A_k_cache: jax.Array,
    A_v_cache: jax.Array,
    A_wq: jax.Array,
    A_wo: jax.Array,
    B_x: jax.Array,
    B_w1: jax.Array,
    B_w3: jax.Array,
    B_w2: jax.Array,
):
    sk = A_k_cache.shape[2]
    win = min(4096, max(256, sk // 4))
    nt_total, nc = sk // LANES, win // LANES

    def kv_view(a):
        return _tile_view(jnp.swapaxes(a, 2, 3).reshape(H * DH, sk))

    def wbuf(r, c):
        return pltpu.VMEM((r // 16, c // LANES, 16, LANES), BF)

    def wbuf4(r, c):
        return pltpu.VMEM((r // 64, 4, c // LANES, 16, LANES), BF)

    def view4(t):
        return t.reshape(t.shape[0] // 4, 2, 4, t.shape[2], 8, LANES)

    any_spec = pl.BlockSpec(memory_space=pl.ANY)
    out = pl.pallas_call(
        _make_kernel(nt_total, nc),
        out_shape=jax.ShapeDtypeStruct((1, D), A_x.dtype),
        in_specs=[any_spec] * 8,
        out_specs=pl.BlockSpec(memory_space=pltpu.VMEM),
        scratch_shapes=[
            wbuf(H * DH, win), wbuf4(H * DH, win),
            pltpu.VMEM((D // 16, NP, 4, 16, LANES), BF),
            wbuf4(H * DH, D), wbuf(D, F), wbuf(F, D),
            pltpu.VMEM((NP - 1, PW, LANES), F32),
            pltpu.VMEM((NP * 12, 8, LANES), U32),
            pltpu.VMEM((NP, 2 * nc, LANES), F32),
            pltpu.VMEM((NP * 2 * nc + 32 + D, LANES), F32),
            pltpu.VMEM((NP * 2 * nc + 32 + D, LANES), F32),
            pltpu.VMEM((NP, nc // 4, 8, LANES), U32),
            pltpu.VMEM((NP, 8, LANES), F32),
            pltpu.VMEM((NP, 8, 512), F32),
            pltpu.VMEM((NP, 8, 512), U32),
            pltpu.VMEM((16, 8, LANES), U32),
            pltpu.VMEM((2 * FT, 8, LANES), F32),
            pltpu.VMEM((24, 8, LANES), U32),
            pltpu.VMEM((8, 1024), U32),
            pltpu.VMEM((8, 1024), F32),
            pltpu.VMEM((1, D), BF),
            pltpu.SemaphoreType.DMA((NSEM,)),
        ],
        compiler_params=pltpu.CompilerParams(
            vmem_limit_bytes=127 * 1024 * 1024),
    )(A_x.reshape(1, D), kv_view(A_k_cache), view4(kv_view(A_v_cache)),
      _tile_view(A_wq).reshape(D // 16, 2, NP, 3, 8, LANES), view4(_tile_view(A_wo)),
      _tile_view(B_w1), _tile_view(B_w3), _tile_view(B_w2))
    return out.reshape(A_x.shape)
```

```python
import functools
import math

import jax
import jax.numpy as jnp
from jax import lax
import jax.experimental.pallas as pl
import jax.experimental.pallas.tpu as pltpu

D = 640
H = 32
DH = 192
F = 1536
LANES = 128
EPS = 1e-5

NP = H // 2
PG = 2 * DH // 16
HG = DH // 16
PW = 2 * DH
DT = D // LANES
FT = F // LANES

GP = 4
NGRP = NP // GP
W2_SPLIT = (0, 56, 80, 92, 96)
W2_MXU = 80
NSEM = 3
RING = 4
PRING = 6

MC = (3, 2, 3, 3, 2, 3, 3, 2, 3, 3, 2, 3, 3, 2, 3)
XCOLS = (2, 7, 12, 17, 22, 27)
VQ = (11, 12, 13, 14, 15)
V_END = (172, 288, 351)
TILES = (1075, 620, 340)
GSHARE = 2
PVM_AFTER = 2
WO_START = (0, 60, 60, 999)
WO_GAP = (0, 60, 48, 12)
WO_KEEP = 3
FSTEP = 2
FIRST = (156, 2, 0)
LAST_OFF = (8, 6, 4)
VQ_FIRST = 30
VQ_UNIT = 4
XC_LINK = 50
SM_LAG = 54
SM_LAG0 = 42
RED_W = 12
RED_A = 44
RED_B = 16
SM_W = 4
SM_A = 30
SM_B = 16
NLINK = 3
LINK0 = 8
LINKSTEP = 4
LINK_REP = 4
FIN_LINK0 = 4
FIN_LINKSTEP = 6
FIN_REP = 1
UP_K = 3
UP_COLS = 5
UP_LINK0 = 50
UP_LINKSTEP = 4.5
UX_LINK = 999
DOWN_K = 3

U32 = jnp.uint32
BF = jnp.bfloat16
F32 = jnp.float32

_LOG = []
ONLY = None


def _tile_view(w):
    r, c = w.shape
    return jnp.swapaxes(w.reshape(r // 16, 2, 8, c // LANES, LANES), 2, 3)


def _rhs(w32, g0, c):
    return pltpu.bitcast(w32[pl.ds(g0, 8), c].reshape(64, LANES), BF)


def _rhs4(w32, tile, c):
    return pltpu.bitcast(w32[pl.ds(2 * tile, 2), :, c].reshape(64, LANES), BF)


def _swiglu(g, u):
    hg = 0.5 * g
    return hg * (1.0 + jnp.tanh(hg)) * u


def _pack2(lo, hi):
    return pltpu.bitcast(jnp.concatenate([lo, hi], axis=0).astype(BF), U32)


def _add(a, b):
    return b if a is None else a + b


def _bits_or(vals):
    return functools.reduce(lambda a, b: a | b, [pltpu.bitcast(v, U32) for v in vals])


def _plan(nc):
    nk = nc // 8
    seq = [('fq', 0), ('fq', 1)]
    for p in range(NP):
        if 1 <= p < NP - 1:
            seq.append(('qx' if p + 1 in VQ else 'q', p + 1))
        for k in range(nk):
            if k == PVM_AFTER and p > 0 and MC[p - 1]:
                seq.append(('pvm', p - 1, nc - MC[p - 1], nc, False))
            seq.append(('qk', p, k))
        seq.append(('sm', p))
    seq += [('pvm', NP - 1, c, c + 4, c > 0) for c in range(0, nc, 4)]
    last_pv = seq[-nc // 4]

    def tiles(it):
        if it[0] == 'pvm':
            return 3 * (it[3] - it[2])
        return dict(fq=15, q=15, wo=15, qk=24, sm=0, qx=0)[it[0]]

    chains = [(p, g) for p in range(NP - 1) for g in range(PG)]
    blocks = []
    v0 = done = 0
    for b in range(len(V_END) + 1):
        final = b == len(V_END)
        v1 = len(chains) if final else V_END[b]
        todo = list(range(done, v0 // PG))
        done = v0 // PG
        budget = 10 ** 9 if final else TILES[b] - 15 * len(todo)
        body = []
        used = 0
        while seq and used + tiles(seq[0]) // 2 <= budget:
            body.append(seq.pop(0))
            used += tiles(body[-1])
        while body[-1][0] in ('sm', 'qx'):
            seq.insert(0, body.pop())
        assert b > 0 or not any(it[1] in VQ for it in body)
        keep = WO_KEEP if last_pv in body else 0
        items = [('red', p) for p in todo]
        used = 0
        nxt = WO_START[b]
        for it in body:
            if it == last_pv:
                while todo:
                    items.append(('wo', todo.pop(0)))
            if len(todo) > keep and used >= nxt:
                items.append(('wo', todo.pop(0)))
                nxt = used + WO_GAP[b]
            items.append(it)
            used += tiles(it)
        items += [('wo', p) for p in todo]
        if final:
            assert done == NP - 2
            for p in (NP - 1, NP - 2):
                items += [('red', p), ('wo', p)]
            blocks.append((chains[v0:v1], items, v1 - v0, 0, 0))
        else:
            blocks.append((chains[v0:v1], items, NLINK if b else 0, FIRST[b], LAST_OFF[b]))
        v0 = v1
    seen = set()
    for chs, items, n_link, _, _ in blocks:
        assert all(p in seen for p, _ in chs[:n_link])
        seen |= {it[1] for it in items if it[0] == 'sm'}
        assert all(p in seen for p, _ in chs)
        assert max(seen) - chs[-1][0] < PRING
    return blocks


def _make_kernel(n_tiles_total, nc):
    c0 = n_tiles_total - nc
    qscale = DH ** -0.5 * math.log2(math.e)
    prow = 2 * nc
    nk = nc // 8

    def kernel(x_hbm, k_hbm, v_hbm, wq_hbm, wo_hbm, w1_hbm, w3_hbm, w2_hbm,
               o_ref,
               kbuf, vbuf, wqbuf, wobuf, w1buf, w3buf, w2buf,
               vx_ref, lhs_ref, s_ref, p_ref, p2_ref, pk_ref, lsum_ref, om_ref,
               ob_ref, mask_ref, cs_ref, qpk_ref, xn_ref, y_ref, xbuf, sem):
        def halves(src, dst):
            return [(src(par), dst(pl.ds(8 * par, 8))) for par in range(2)]

        def whole(src, dst):
            return halves(lambda p: src.at[:, p], lambda h: dst.at[:, :, h, :])

        def kv_group(g):
            kr = pl.ds(g * GP * PG, GP * PG)
            vr = pl.ds(g * GP * PG // 4, GP * PG // 4)
            return (halves(lambda p: k_hbm.at[kr, p, pl.ds(c0, nc)],
                           lambda h: kbuf.at[kr, :, h, :])
                    + halves(lambda p: v_hbm.at[vr, p, :, pl.ds(c0, nc)],
                             lambda h: vbuf.at[vr, :, :, h, :]))

        def w2_group(i):
            rows = pl.ds(W2_SPLIT[i], W2_SPLIT[i + 1] - W2_SPLIT[i])
            return halves(lambda p: w2_hbm.at[rows, p], lambda h: w2buf.at[rows, :, h, :])

        groups = ([whole(wq_hbm, wqbuf) + [(x_hbm, xbuf)]]
                  + [kv_group(NGRP - 1 - g) for g in range(NGRP)]
                  + [halves(lambda p: wo_hbm.at[:, p], lambda h: wobuf.at[:, :, :, h, :]),
                     whole(w1_hbm, w1buf) + whole(w3_hbm, w3buf)]
                  + [w2_group(i) for i in range(len(W2_SPLIT) - 1)])
        marker = len(groups)
        groups.append([(x_hbm, xbuf)])

        def copies(i):
            return [pltpu.make_async_copy(src, dst, sem.at[i % NSEM])
                    for src, dst in groups[i]]

        def start(i):
            for cp in copies(i):
                cp.start()

        def wait(i):
            for cp in copies(i):
                cp.wait()
            if i + NSEM < len(groups):
                start(i + NSEM)

        for i in range(NSEM):
            start(i)

        k32 = kbuf.bitcast(U32)
        v32 = vbuf.bitcast(U32)
        wq32 = wqbuf.bitcast(U32)
        wo32 = wobuf.bitcast(U32)
        w13 = (w1buf.bitcast(U32), w3buf.bitcast(U32))
        w232 = w2buf.bitcast(U32)

        sub = lax.broadcasted_iota(jnp.int32, (8, LANES), 0)
        lane = lax.broadcasted_iota(jnp.int32, (8, LANES), 1)
        sub3 = lax.broadcasted_iota(jnp.int32, (8, PW), 0)
        lane3 = lax.broadcasted_iota(jnp.int32, (8, PW), 1)

        for r in range(4):
            half = U32(0x0000FFFF if r % 2 == 0 else 0xFFFF0000)
            lo = jnp.where(sub == r // 2, half, U32(0))
            hi = jnp.where(sub == 2 + r // 2, half, U32(0))
            mask_ref[r] = lo
            mask_ref[4 + r] = jnp.where(lane < DH - LANES, lo, hi)
            mask_ref[8 + r] = hi
            mask_ref[12 + r] = lo | hi
        p_refs = (p_ref, p2_ref)
        for pr in p_refs:
            pr[...] = jnp.zeros(pr.shape, F32)

        def dot(l32, r, free=True):
            del free
            return jnp.dot(pltpu.bitcast(l32, BF), r, preferred_element_type=F32)

        def tile_of(v, kk):
            return v[:, kk * LANES:(kk + 1) * LANES]

        def ln_stats(x):
            xb = x.astype(BF).astype(F32)
            m = jnp.mean(xb, axis=-1, keepdims=True)
            xc = xb - m
            v = jnp.mean(xc * xc, axis=-1, keepdims=True)
            return xb, m, lax.rsqrt(v + EPS)

        def raw_proj(xb, w32, c, mm=dot):
            lhs = _pack2(xb, jnp.ones_like(xb))
            acc = None
            for kk in range(DT):
                acc = _add(acc, mm(tile_of(lhs, kk), _rhs(w32, 8 * kk, c), False))
            return acc[0:8], acc[8:16]

        def col_bcast(v):
            return jnp.concatenate([v] * (LANES // 8), axis=0).T

        def vpu_fma(acc, w, xlo, xhi):
            w = pltpu.bitcast(w, BF).astype(F32)
            return _add(acc, w[0:8] * xlo + w[8:16] * xhi)

        def sub_sum(a):
            return jnp.broadcast_to(jnp.sum(a, axis=0, keepdims=True), a.shape)

        def expand_q(p, t, q):
            for r in range(4):
                lhs_ref[p % RING, 4 * t + r] = q & mask_ref[4 * t + r]

        def stage_q(p, mm=dot):
            acc = [None] * 3
            for kk in range(DT):
                for t in range(3):
                    acc[t] = _add(acc[t], mm(xn_ref[:, pl.ds(kk * LANES, LANES)],
                                             _rhs(wq32, 8 * kk, 3 * p + t))[0:8])
            for t in range(3):
                q = acc[t] * qscale
                expand_q(p, t, _pack2(q, q))

        def stage_qk(p, k, mm=dot, scale=None):
            for j in range(2 * k, 2 * k + 2):
                acc = None
                for t in range(3):
                    for r in range(4):
                        acc = _add(acc, mm(lhs_ref[p % RING, 4 * t + r],
                                           _rhs(k32, p * PG + 8 * t, 4 * j + r))[0:8])
                s_ref[p % RING, j] = acc if scale is None else acc * scale

        def head_reduce(v, op, lane_op):
            for d in (1, 2):
                up = pltpu.roll(v, d, 0)
                down = pltpu.roll(v, 8 - d, 0)
                v = op(v, jnp.where(sub % (2 * d) >= d, up, down))
            return lane_op(v, axis=1, keepdims=True)

        def softmax(p, j0):
            s = s_ref[p % RING]
            m = head_reduce(jnp.max(s, axis=0), jnp.maximum, jnp.max)
            e = jnp.exp2(s - m)
            l = jnp.sum(e, axis=0)
            lsum_ref[p] = l
            for j in range(j0, nc // 4):
                pk_ref[p % RING, j] = _pack2(e[j], e[j])
            return e.reshape(prow, LANES), l

        def v_idx(p, g, c):
            return p * (PG // 4) + g // 4, g % 4, c

        def pv_chain(p, g, gate, n=1):
            acc = [None] * (2 * n)
            for c in range(nc - MC[p]):
                row = (p % PRING) * prow + 8 * (c // 4) + 4 * (g // HG) + c % 4
                pb = gate()[pl.ds(row, 8, stride=0), :]
                for i in range(n):
                    if i:
                        gate()
                    w = v32[v_idx(p, g + i, c)]
                    if c in XCOLS:
                        w = (pltpu.bitcast(w, F32), vx_ref[p, g + i, XCOLS.index(c)])
                    else:
                        w = pltpu.bitcast(w, BF).astype(F32)
                        w = (w[0:8], w[8:16])
                    for h in range(2):
                        acc[2 * i + h] = _add(acc[2 * i + h], w[h] * pb)
            for i in range(2 * n):
                j = 2 * g + i
                k32[p * PG + j // nc, j % nc] = pltpu.bitcast(acc[i], U32)
            return acc

        def pv_mxu(p, cols, transposed, mm=dot):
            acc = [None] * 3
            cols = list(cols)
            for i0 in range(0, len(cols), 4):
                ls = {c: pk_ref[p % RING, c // 4] & mask_ref[12 + c % 4]
                      for c in cols[i0:i0 + 4]}
                for t in range(3):
                    for c, l in ls.items():
                        tile = _rhs4(v32, 3 * p + t, c)
                        if transposed:
                            res = mm(l, tile)
                        else:
                            res = lax.dot_general(
                                pltpu.bitcast(l, BF), tile, (((1,), (1,)), ((), ())),
                                preferred_element_type=F32)
                        acc[t] = _add(acc[t], res[0:8])
            return jnp.concatenate(acc, axis=1)

        def own_head(o):
            return jnp.where((sub3 < 4) == (lane3 < DH), o, 0.0)

        def finish_o(p, o):
            linv = 1.0 / head_reduce(lsum_ref[p], jnp.add, jnp.sum)
            o = (jnp.sum(o, axis=0, keepdims=True)
                 * jnp.where(lane3 < DH, linv[0:1], linv[4:5]))
            ob_ref[p] = _pack2(o, o)

        def stage_reduce(p):
            o = None
            if p < NP - 1:
                tt = jnp.concatenate([k32[p * PG], k32[p * PG + 1, 0:2 * PG - nc]])
                tt = pltpu.bitcast(tt.reshape(PW, LANES), F32)
                o = jnp.sum(tt.T.reshape(LANES // 8, 8, PW), axis=0)
            if p == NP - 1 or MC[p]:
                o = _add(o, own_head(om_ref[p]))
            finish_o(p, o)

        def stage_wo(p, mm=dot):
            for c in range(DT):
                acc = y_ref[:, pl.ds(c * LANES, LANES)]
                for t in range(3):
                    acc = acc + mm(ob_ref[p, :, pl.ds(t * LANES, LANES)],
                                   _rhs4(wo32, 3 * p + t, c))[0:8]
                y_ref[:, pl.ds(c * LANES, LANES)] = acc

        def begin_attention(x):
            y_ref[:, 0:D] = x
            xb, m, r = ln_stats(x)
            xn = (xb - m) * r
            xn_ref[:, 0:D] = _pack2(xn, xn)
            return xb, m, r

        wait(0)
        begin_attention(jnp.broadcast_to(xbuf[...].astype(F32), (8, D)))

        def pair1(p, carry):
            stage_q(p)
            for k in range(nk):
                stage_qk(p, k)
            softmax(p, 0)
            finish_o(p, own_head(pv_mxu(p, range(nc), False)))
            om_ref[p] = jnp.zeros(om_ref.shape[1:], F32)
            qpk_ref[p] = jnp.zeros((8, LANES), U32)
            cs_ref[p] = jnp.zeros((8, LANES), F32)

            first = 0
            for pp in range(NP - 1):
                first = jnp.where(p == pp, nc - MC[pp], first)

            def transpose_v(c, carry2):
                for t in range(3):
                    tile = _rhs4(v32, 3 * p + t, c)
                    v32[pl.ds(2 * (3 * p + t), 2), :, c] = pltpu.bitcast(
                        tile.T, U32).reshape(2, 4, 8, LANES)
                return carry2

            lax.fori_loop(first, nc, transpose_v, 0)

            @pl.when(p < NP - 1)
            def _():
                for g in range(PG):
                    for e, c in enumerate(XCOLS):
                        w = pltpu.bitcast(v32[v_idx(p, g, c)], BF).astype(F32)
                        v32[v_idx(p, g, c)] = pltpu.bitcast(w[0:8], U32)
                        vx_ref[p, g, e] = w[8:16]

            return carry

        def group1(gi, row):
            for i in range(NGRP):
                pl.when(gi == i)(functools.partial(wait, 1 + i))
            g = NGRP - 1 - gi
            lax.fori_loop(g * GP, (g + 1) * GP, pair1, 0)
            return row + PRING * prow // NGRP

        fence_row = pl.multiple_of(lax.fori_loop(0, NGRP, group1, 0), 8)
        wait(1 + NGRP)

        def woloop(p2, carry):
            stage_wo(2 * p2)
            stage_wo(2 * p2 + 1)
            return carry

        lax.fori_loop(0, NP // 2, woloop, 0)

        x = y_ref[:, 0:D]
        xb, m, r = ln_stats(x)
        wait(2 + NGRP)
        gu = []
        for j in range(2 * FT):
            raw, cs = raw_proj(xb, w13[j % 2], j // 2)
            cs_ref[j] = cs
            gu.append((raw - m * cs) * r)
        hs = [_swiglu(g, u) for g, u in zip(gu[0::2], gu[1::2])]
        for kk in range(W2_MXU // 8, FT):
            p_ref[pl.ds(LANES * kk - 16 * W2_MXU, LANES), :] = col_bcast(
                hs[kk].astype(BF).astype(F32))
        hs = [_pack2(hh, hh) for hh in hs[:W2_MXU // 8]]
        cols = [tile_of(x, c) for c in range(DT)]
        part = [None] * DT
        for i in range(len(W2_SPLIT) - 1):
            wait(3 + NGRP + i)
            g0, g1 = W2_SPLIT[i], W2_SPLIT[i + 1]
            for c in range(DT):
                if g1 <= W2_MXU:
                    for kk in range(g0 // 8, g1 // 8):
                        cols[c] = cols[c] + dot(hs[kk], _rhs(w232, 8 * kk, c))[0:8]
                else:
                    for g in range(g0, g1):
                        row = 16 * (g - W2_MXU)
                        part[c] = vpu_fma(part[c], w232[g, c], p_ref[pl.ds(row, 8), :],
                                          p_ref[pl.ds(row + 8, 8), :])
        x = jnp.concatenate([cc + sub_sum(a) for cc, a in zip(cols, part)], axis=1)

        xb, m, r = begin_attention(x)
        rq = r * qscale

        def run_block(chains, items, n_link, first, last_off, start, end):
            links = []
            for j, (p, g) in enumerate(chains[:n_link]):
                dep = _bits_or(pv_chain(p, g, lambda: p_refs[g % 2]))
                if end:
                    links.extend([(FIN_LINK0 + FIN_LINKSTEP * j, dep)] * FIN_REP)
                else:
                    links.extend([(LINK0 + LINKSTEP * j, dep)] * LINK_REP)
            if start:
                xcol = [col_bcast(tile_of(xb, kk)) - m[0:1] for kk in range(DT)]
                links.extend([(XC_LINK, _bits_or(xc[LANES - 8:] for xc in xcol))] * 4)
            pops = []
            probs = {}
            ready = {}
            busy = []

            def mm(l32, rr, free=True):
                links.sort(key=lambda lk: lk[0])
                if free and links and len(pops) >= links[0][0]:
                    l32 = jnp.where(sub < 4, l32, links.pop(0)[1])
                pops.append(dot(l32, rr))
                return pops[-1]

            for it in items:
                kind, p = it[0], it[1]
                if kind == 'fq':
                    for t in range(3):
                        raw, cs = raw_proj(xb, wq32, 3 * p + t, mm)
                        q = raw - m * cs
                        q = q if p == 0 else q * rq
                        expand_q(p, t, _pack2(q, q))
                elif kind == 'q':
                    stage_q(p, mm)
                elif kind == 'qx':
                    for t in range(3):
                        expand_q(p, t, qpk_ref[3 * VQ.index(p) + t])
                elif kind == 'qk':
                    stage_qk(p, it[2], mm, rq if p == 0 else None)
                    ready[p] = len(pops)
                elif kind == 'sm':
                    e, l = softmax(p, 0 if p == NP - 1 else (nc - MC[p]) // 4)
                    lag = SM_LAG0 if p == 0 else SM_LAG
                    pos = len(pops) + (lag if pops else lag - 14)
                    links.append((pos, pltpu.bitcast(l, U32)))
                    busy.append((pos - SM_A, pos - SM_B, SM_W))
                    if p < NP - 1:
                        probs[p] = e
                elif kind == 'pvm':
                    o = pv_mxu(p, range(it[2], it[3]), True, mm)
                    om_ref[p] = o + om_ref[p] if it[4] else o
                elif kind == 'red':
                    stage_reduce(p)
                elif kind == 'wo':
                    busy.append((len(pops) - RED_A, len(pops) - RED_B, RED_W))
                    stage_wo(p, mm)

            def fence(buf, a):
                buf[pl.ds(fence_row, 8), :] = pops[a][0:8]

            if start:
                nkg = D // 16

                def xslot(kg):
                    u = kg // VQ_UNIT
                    return p_refs[u % 2], 16 * (u // 2 * VQ_UNIT + kg % VQ_UNIT)

                for kg in range(nkg):
                    buf, row = xslot(kg)
                    buf[pl.ds(row, 16), :] = xcol[kg // 8][16 * (kg % 8):16 * (kg % 8) + 16]
                for i, p in enumerate(VQ):
                    acc = [None] * 3
                    for kg in range(nkg):
                        buf, row = xslot(kg)
                        if kg % VQ_UNIT == 0:
                            a = (i * nkg + kg) * (first - VQ_FIRST) // (len(VQ) * nkg)
                            fence(buf, VQ_FIRST + a // 2 * 2)
                        xlo = buf[pl.ds(row, 8), :]
                        xhi = buf[pl.ds(row + 8, 8), :]
                        for t in range(3):
                            acc[t] = vpu_fma(acc[t], wq32[kg, 3 * p + t], xlo, xhi)
                    for t in range(3):
                        q = sub_sum(acc[t]) * rq
                        qpk_ref[3 * i + t] = _pack2(q, q)

            def store_probs(p):
                e = probs.pop(p)
                n = 8 * ((nc - MC[p] + 3) // 4)
                for pr in p_refs:
                    pr[pl.ds((p % PRING) * prow, n), :] = e[0:n]

            rest = chains[n_link:]
            if rest:
                n_items = sum(nc - MC[p] for p, _ in rest)
                n_units = (len(pops) - last_off - first) // FSTEP + 1
                less = [0.0] * n_units
                for lo, hi, w in busy:
                    us = [u for u in range(n_units) if lo <= first + u * FSTEP < hi]
                    for u in us:
                        less[u] += w / len(us)
                per = (n_items + sum(less)) / n_units
                unit_of, total = [], 0.0
                for u in range(n_units):
                    total += per - less[u]
                    while len(unit_of) < min(total - 1e-6, n_items):
                        unit_of.append(u)
                state = [0, -1, 1]

                def gate():
                    u = unit_of[state[0]]
                    state[0] += 1
                    if u != state[1]:
                        state[1] = u
                        state[2] += 1
                        fence(p_refs[state[2] % 2], first + u * FSTEP)
                    return p_refs[state[2] % 2]

            while rest:
                p, g = rest[0]
                if p in probs:
                    if p in ready:
                        _LOG.append((p, first + state[1] * FSTEP - ready[p]))
                    store_probs(p)
                n = min(GSHARE - g % GSHARE, len(rest))
                pv_chain(p, g, gate, n)
                rest = rest[n:]
            for p in list(probs):
                store_probs(p)
            if end:
                last_ffn(y_ref[:, 0:D], mm, len(pops), links)

        def last_ffn(x, mm, base, links):
            xb, m, r = ln_stats(x)
            lhs = _pack2(xb, xb)
            xcol = [col_bcast(tile_of(xb, kk)) for kk in range(UP_K)]
            links.extend([(base + UX_LINK, _bits_or(xc[LANES - 8:] for xc in xcol))] * 4)
            j0 = 2 * (FT - UP_COLS)
            part = {}
            for j in range(j0, 2 * FT):
                acc = None
                for kg in range(8 * UP_K):
                    xc = xcol[kg // 8][16 * (kg % 8):16 * (kg % 8) + 16]
                    acc = vpu_fma(acc, w13[j % 2][kg, j // 2], xc[0:8], xc[8:16])
                part[j] = sub_sum(acc)
                links.append((base + int(UP_LINK0 + UP_LINKSTEP * (j - j0)),
                              pltpu.bitcast(part[j], U32)))
            gu = []
            for j in range(2 * FT):
                acc = part.get(j)
                for kk in range(UP_K if j in part else 0, DT):
                    acc = _add(acc, mm(tile_of(lhs, kk),
                                       _rhs(w13[j % 2], 8 * kk, j // 2))[0:8])
                gu.append((acc - m * cs_ref[j]) * r)
            hs = [_swiglu(g, u) for g, u in zip(gu[0::2], gu[1::2])]
            cols = [tile_of(x, c) for c in range(DT)]
            for kk in range(DOWN_K, FT):
                hh = _pack2(hs[kk], hs[kk])
                for c in range(DT):
                    cols[c] = cols[c] + mm(hh, _rhs(w232, 8 * kk, c))[0:8]
            acc = [None] * DT
            for kk in range(DOWN_K):
                hcol = col_bcast(hs[kk].astype(BF).astype(F32))
                for i in range(8):
                    for c in range(DT):
                        acc[c] = vpu_fma(acc[c], w232[8 * kk + i, c],
                                         hcol[16 * i:16 * i + 8],
                                         hcol[16 * i + 8:16 * i + 16])
            cols = [cc + sub_sum(a) for cc, a in zip(cols, acc)]
            o_ref[...] = jnp.concatenate(cols, axis=1)[0:1].astype(o_ref.dtype)

        blocks = _plan(nc)
        for b, blk in enumerate(blocks):
            end = b == len(blocks) - 1
            if b > 0:
                wait(marker)
                if not end:
                    start(marker)
            if ONLY is not None and b not in ONLY and not end:
                if b < 2:
                    expand_q(0, 0, _bits_or(qpk_ref[pp] for pp in range(NP - 1)))
                    for pp in range(2):
                        stage_reduce(pp)
                continue
            run_block(*blk, b == 0, end)

    return kernel


@jax.jit
def pallas_interleave_layers__sliding_block_cached__glu_gated_swiglu__decode_kernel(
    A_x: jax.Array,
    A_k_cache: jax.Array,
    A_v_cache: jax.Array,
    A_wq: jax.Array,
    A_wo: jax.Array,
    B_x: jax.Array,
    B_w1: jax.Array,
    B_w3: jax.Array,
    B_w2: jax.Array,
):
    sk = A_k_cache.shape[2]
    win = min(4096, max(256, sk // 4))
    nt_total, nc = sk // LANES, win // LANES

    def kv_view(a):
        return _tile_view(jnp.swapaxes(a, 2, 3).reshape(H * DH, sk))

    def view4(t):
        return t.reshape(t.shape[0] // 4, 2, 4, t.shape[2], 8, LANES)

    def wbuf(r, c):
        return pltpu.VMEM((r // 16, c // LANES, 16, LANES), BF)

    def wbuf4(r, c):
        return pltpu.VMEM((r // 64, 4, c // LANES, 16, LANES), BF)

    any_spec = pl.BlockSpec(memory_space=pl.ANY)
    out = pl.pallas_call(
        _make_kernel(nt_total, nc),
        out_shape=jax.ShapeDtypeStruct((1, D), A_x.dtype),
        in_specs=[any_spec] * 8,
        out_specs=pl.BlockSpec(memory_space=pltpu.VMEM),
        scratch_shapes=[
            wbuf(H * DH, win), wbuf4(H * DH, win),
            wbuf(D, H * DH), wbuf4(H * DH, D),
            wbuf(D, F), wbuf(D, F), wbuf(F, D),
            pltpu.VMEM((NP - 1, PG, len(XCOLS), 8, LANES), F32),
            pltpu.VMEM((RING, 12, 8, LANES), U32),
            pltpu.VMEM((RING, nc // 4, 8, LANES), F32),
            pltpu.VMEM((PRING * 2 * nc + 32, LANES), F32),
            pltpu.VMEM((PRING * 2 * nc + 32, LANES), F32),
            pltpu.VMEM((RING, nc // 4, 8, LANES), U32),
            pltpu.VMEM((NP, 8, LANES), F32),
            pltpu.VMEM((NP, 8, PW), F32),
            pltpu.VMEM((NP, 8, PW), U32),
            pltpu.VMEM((16, 8, LANES), U32),
            pltpu.VMEM((2 * FT, 8, LANES), F32),
            pltpu.VMEM((16, 8, LANES), U32),
            pltpu.VMEM((8, 1024), U32),
            pltpu.VMEM((8, 1024), F32),
            pltpu.VMEM((1, D), BF),
            pltpu.SemaphoreType.DMA((NSEM,)),
        ],
        compiler_params=pltpu.CompilerParams(
            vmem_limit_bytes=128 * 1024 * 1024),
    )(A_x.reshape(1, D), kv_view(A_k_cache), view4(kv_view(A_v_cache)),
      _tile_view(A_wq), view4(_tile_view(A_wo)),
      _tile_view(B_w1), _tile_view(B_w3), _tile_view(B_w2))
    return out.reshape(A_x.shape)
```

```python
import functools
import math

import jax
import jax.numpy as jnp
from jax import lax
import jax.experimental.pallas as pl
import jax.experimental.pallas.tpu as pltpu

D = 640
H = 32
DH = 192
F = 1536
LANES = 128
EPS = 1e-5

NP = H // 2
PG = 2 * DH // 16
HG = DH // 16
PW = 2 * DH
DT = D // LANES
FT = F // LANES

GP = 4
NGRP = NP // GP
W2_SPLIT = (0, 56, 80, 92, 96)
W2_MXU = 80
NSEM = 3
RING = 4
PRING = 6

MC = (3, 2, 3, 3, 2, 3, 3, 3, 3, 3, 3, 3, 3, 2, 3)
XCOLS = (3, 7, 11, 15, 19, 23)
VQ = (11, 12, 13, 14, 15)
V_END = (174, 290, 352)
TILES = (1075, 620, 340)
GSHARE = 2
PVM_AFTER = 2
WO_START = (0, 60, 60, 999)
WO_GAP = (0, 60, 48, 12)
WO_KEEP = 3
FSTEP = 2
FIRST = (156, 2, 0)
LAST_OFF = (8, 6, 4)
VQ_FIRST = 30
VQ_UNIT = 4
XC_LINK = 50
SM_LAG = 54
SM_LAG0 = 42
PST = 0
PST_OFF = 12
RED_W = 12
RED_A = 44
RED_B = 16
Q_W = 4
Q_A = 6
Q_B = -4
SM_W = 4
SM_A = 30
SM_B = 16
NLINK = 3
LINK0 = 8
LINKSTEP = 4
LINK_REP = 4
FIN_LINK0 = 4
FIN_LINKSTEP = 6
FIN_REP = 1
UP_K = 3
UP_COLS = 5
UP_LINK0 = 50
UP_LINKSTEP = 4.5
UX_LINK = 999
DOWN_K = 3

U32 = jnp.uint32
BF = jnp.bfloat16
F32 = jnp.float32

_LOG = []
ONLY = None


def _tile_view(w):
    r, c = w.shape
    return jnp.swapaxes(w.reshape(r // 16, 2, 8, c // LANES, LANES), 2, 3)


def _rhs(w32, g0, c):
    return pltpu.bitcast(w32[pl.ds(g0, 8), c].reshape(64, LANES), BF)


def _rhs4(w32, tile, c):
    return pltpu.bitcast(w32[pl.ds(2 * tile, 2), :, c].reshape(64, LANES), BF)


def _swiglu(g, u):
    hg = 0.5 * g
    return hg * (1.0 + jnp.tanh(hg)) * u


def _pack2(lo, hi):
    return pltpu.bitcast(jnp.concatenate([lo, hi], axis=0).astype(BF), U32)


def _add(a, b):
    return b if a is None else a + b


def _bits_or(vals):
    return functools.reduce(lambda a, b: a | b, [pltpu.bitcast(v, U32) for v in vals])


def _plan(nc):
    nk = nc // 8
    seq = [('fq', 0), ('fq', 1)]
    for p in range(NP):
        if 1 <= p < NP - 1:
            seq.append(('qx' if p + 1 in VQ else 'q', p + 1))
        for k in range(nk):
            if k == PVM_AFTER and p > 0 and MC[p - 1]:
                seq.append(('pvm', p - 1, nc - MC[p - 1], nc, False))
            seq.append(('qk', p, k))
        seq.append(('sm', p))
    seq += [('pvm', NP - 1, c, c + 4, c > 0) for c in range(0, nc, 4)]
    last_pv = seq[-nc // 4]

    def tiles(it):
        if it[0] == 'pvm':
            return 3 * (it[3] - it[2])
        return dict(fq=15, q=15, wo=15, qk=24, sm=0, qx=0)[it[0]]

    chains = [(p, g) for p in range(NP - 1) for g in range(PG)]
    blocks = []
    v0 = done = 0
    for b in range(len(V_END) + 1):
        final = b == len(V_END)
        v1 = len(chains) if final else V_END[b]
        todo = list(range(done, v0 // PG))
        done = v0 // PG
        budget = 10 ** 9 if final else TILES[b] - 15 * len(todo)
        body = []
        used = 0
        while seq and used + tiles(seq[0]) // 2 <= budget:
            body.append(seq.pop(0))
            used += tiles(body[-1])
        while body[-1][0] in ('sm', 'qx'):
            seq.insert(0, body.pop())
        assert b > 0 or not any(it[1] in VQ for it in body)
        keep = WO_KEEP if last_pv in body else 0
        items = [('red', p) for p in todo]
        used = 0
        nxt = WO_START[b]
        for it in body:
            if it == last_pv:
                while todo:
                    items.append(('wo', todo.pop(0)))
            if len(todo) > keep and used >= nxt:
                items.append(('wo', todo.pop(0)))
                nxt = used + WO_GAP[b]
            items.append(it)
            used += tiles(it)
        items += [('wo', p) for p in todo]
        if final:
            assert done == NP - 2
            for p in (NP - 1, NP - 2):
                items += [('red', p), ('wo', p)]
            blocks.append((chains[v0:v1], items, v1 - v0, 0, 0))
        else:
            blocks.append((chains[v0:v1], items, NLINK if b else 0, FIRST[b], LAST_OFF[b]))
        v0 = v1
    seen = set()
    for chs, items, n_link, _, _ in blocks:
        assert all(p in seen for p, _ in chs[:n_link])
        seen |= {it[1] for it in items if it[0] == 'sm'}
        assert all(p in seen for p, _ in chs)
    return blocks


def _make_kernel(n_tiles_total, nc):
    c0 = n_tiles_total - nc
    qscale = DH ** -0.5 * math.log2(math.e)
    prow = 2 * nc
    nk = nc // 8

    def kernel(x_hbm, k_hbm, v_hbm, wq_hbm, wo_hbm, w1_hbm, w3_hbm, w2_hbm,
               o_ref,
               kbuf, vbuf, wqbuf, wobuf, w1buf, w3buf, w2buf,
               vx_ref, lhs_ref, s_ref, p_ref, p2_ref, pk_ref, lsum_ref, om_ref,
               ob_ref, mask_ref, cs_ref, qpk_ref, xn_ref, y_ref, xbuf, sem):
        def halves(src, dst):
            return [(src(par), dst(pl.ds(8 * par, 8))) for par in range(2)]

        def whole(src, dst):
            return halves(lambda p: src.at[:, p], lambda h: dst.at[:, :, h, :])

        def kv_group(g):
            kr = pl.ds(g * GP * PG, GP * PG)
            vr = pl.ds(g * GP * PG // 4, GP * PG // 4)
            return (halves(lambda p: k_hbm.at[kr, p, pl.ds(c0, nc)],
                           lambda h: kbuf.at[kr, :, h, :])
                    + halves(lambda p: v_hbm.at[vr, p, :, pl.ds(c0, nc)],
                             lambda h: vbuf.at[vr, :, :, h, :]))

        def w2_group(i):
            rows = pl.ds(W2_SPLIT[i], W2_SPLIT[i + 1] - W2_SPLIT[i])
            return halves(lambda p: w2_hbm.at[rows, p], lambda h: w2buf.at[rows, :, h, :])

        groups = ([whole(wq_hbm, wqbuf) + [(x_hbm, xbuf)]]
                  + [kv_group(NGRP - 1 - g) for g in range(NGRP)]
                  + [halves(lambda p: wo_hbm.at[:, p], lambda h: wobuf.at[:, :, :, h, :]),
                     whole(w1_hbm, w1buf) + whole(w3_hbm, w3buf)]
                  + [w2_group(i) for i in range(len(W2_SPLIT) - 1)])
        marker = len(groups)
        groups.append([(x_hbm, xbuf)])

        def copies(i):
            return [pltpu.make_async_copy(src, dst, sem.at[i % NSEM])
                    for src, dst in groups[i]]

        def start(i):
            for cp in copies(i):
                cp.start()

        def wait(i):
            for cp in copies(i):
                cp.wait()
            if i + NSEM < len(groups):
                start(i + NSEM)

        for i in range(NSEM):
            start(i)

        k32 = kbuf.bitcast(U32)
        v32 = vbuf.bitcast(U32)
        wq32 = wqbuf.bitcast(U32)
        wo32 = wobuf.bitcast(U32)
        w13 = (w1buf.bitcast(U32), w3buf.bitcast(U32))
        w232 = w2buf.bitcast(U32)

        sub = lax.broadcasted_iota(jnp.int32, (8, LANES), 0)
        lane = lax.broadcasted_iota(jnp.int32, (8, LANES), 1)
        sub3 = lax.broadcasted_iota(jnp.int32, (8, PW), 0)
        lane3 = lax.broadcasted_iota(jnp.int32, (8, PW), 1)

        for r in range(4):
            half = U32(0x0000FFFF if r % 2 == 0 else 0xFFFF0000)
            lo = jnp.where(sub == r // 2, half, U32(0))
            hi = jnp.where(sub == 2 + r // 2, half, U32(0))
            mask_ref[r] = lo
            mask_ref[4 + r] = jnp.where(lane < DH - LANES, lo, hi)
            mask_ref[8 + r] = hi
            mask_ref[12 + r] = lo | hi
        p_refs = (p_ref, p2_ref)
        for pr in p_refs:
            pr[...] = jnp.zeros(pr.shape, F32)

        def dot(l32, r, free=True):
            del free
            return jnp.dot(pltpu.bitcast(l32, BF), r, preferred_element_type=F32)

        def tile_of(v, kk):
            return v[:, kk * LANES:(kk + 1) * LANES]

        def ln_stats(x):
            xb = x.astype(BF).astype(F32)
            m = jnp.mean(xb, axis=-1, keepdims=True)
            xc = xb - m
            v = jnp.mean(xc * xc, axis=-1, keepdims=True)
            return xb, m, lax.rsqrt(v + EPS)

        def raw_proj(xb, w32, c, mm=dot):
            lhs = _pack2(xb, jnp.ones_like(xb))
            acc = None
            for kk in range(DT):
                acc = _add(acc, mm(tile_of(lhs, kk), _rhs(w32, 8 * kk, c), False))
            return acc[0:8], acc[8:16]

        def col_bcast(v):
            return jnp.concatenate([v] * (LANES // 8), axis=0).T

        def vpu_fma(acc, w, xlo, xhi):
            w = pltpu.bitcast(w, BF).astype(F32)
            return _add(acc, w[0:8] * xlo + w[8:16] * xhi)

        def sub_sum(a):
            return jnp.broadcast_to(jnp.sum(a, axis=0, keepdims=True), a.shape)

        def expand_q(p, t, q):
            for r in range(4):
                lhs_ref[p % RING, 4 * t + r] = q & mask_ref[4 * t + r]

        def stage_q(p, mm=dot):
            acc = [None] * 3
            for kk in range(DT):
                for t in range(3):
                    acc[t] = _add(acc[t], mm(xn_ref[:, pl.ds(kk * LANES, LANES)],
                                             _rhs(wq32, 8 * kk, 3 * p + t))[0:8])
            for t in range(3):
                q = acc[t] * qscale
                expand_q(p, t, _pack2(q, q))

        def stage_qk(p, k, mm=dot, scale=None):
            for j in range(2 * k, 2 * k + 2):
                acc = None
                for t in range(3):
                    for r in range(4):
                        acc = _add(acc, mm(lhs_ref[p % RING, 4 * t + r],
                                           _rhs(k32, p * PG + 8 * t, 4 * j + r))[0:8])
                s_ref[p % RING, j] = acc if scale is None else acc * scale

        def head_reduce(v, op, lane_op):
            for d in (1, 2):
                up = pltpu.roll(v, d, 0)
                down = pltpu.roll(v, 8 - d, 0)
                v = op(v, jnp.where(sub % (2 * d) >= d, up, down))
            return lane_op(v, axis=1, keepdims=True)

        def softmax(p, j0):
            s = s_ref[p % RING]
            m = head_reduce(jnp.max(s, axis=0), jnp.maximum, jnp.max)
            e = jnp.exp2(s - m)
            l = jnp.sum(e, axis=0)
            lsum_ref[p] = l
            for j in range(j0, nc // 4):
                pk_ref[p % RING, j] = _pack2(e[j], e[j])
            return e, l

        def v_idx(p, g, c):
            return p * (PG // 4) + g // 4, g % 4, c

        def pv_chain(p, g, gate, n=1):
            acc = [None] * (2 * n)
            for c in range(nc - MC[p]):
                row = (p % PRING) * prow + 8 * (c // 4) + 4 * (g // HG) + c % 4
                pb = gate()[pl.ds(row, 8, stride=0), :]
                for i in range(n):
                    if i:
                        gate()
                    w = v32[v_idx(p, g + i, c)]
                    if c in XCOLS:
                        w = (pltpu.bitcast(w, F32), vx_ref[p, g + i, XCOLS.index(c)])
                    else:
                        w = pltpu.bitcast(w, BF).astype(F32)
                        w = (w[0:8], w[8:16])
                    for h in range(2):
                        acc[2 * i + h] = _add(acc[2 * i + h], w[h] * pb)
            for i in range(2 * n):
                j = 2 * g + i
                k32[p * PG + j // nc, j % nc] = pltpu.bitcast(acc[i], U32)
            return acc

        def pv_mxu(p, cols, transposed, mm=dot):
            acc = [None] * 3
            cols = list(cols)
            for i0 in range(0, len(cols), 4):
                ls = {c: pk_ref[p % RING, c // 4] & mask_ref[12 + c % 4]
                      for c in cols[i0:i0 + 4]}
                for t in range(3):
                    for c, l in ls.items():
                        tile = _rhs4(v32, 3 * p + t, c)
                        if transposed:
                            res = mm(l, tile)
                        else:
                            res = lax.dot_general(
                                pltpu.bitcast(l, BF), tile, (((1,), (1,)), ((), ())),
                                preferred_element_type=F32)
                        acc[t] = _add(acc[t], res[0:8])
            return jnp.concatenate(acc, axis=1)

        def own_head(o):
            return jnp.where((sub3 < 4) == (lane3 < DH), o, 0.0)

        def finish_o(p, o):
            linv = 1.0 / head_reduce(lsum_ref[p], jnp.add, jnp.sum)
            o = (jnp.sum(o, axis=0, keepdims=True)
                 * jnp.where(lane3 < DH, linv[0:1], linv[4:5]))
            ob_ref[p] = _pack2(o, o)

        def stage_reduce(p):
            o = None
            if p < NP - 1:
                tt = jnp.concatenate([k32[p * PG], k32[p * PG + 1, 0:2 * PG - nc]])
                tt = pltpu.bitcast(tt.reshape(PW, LANES), F32)
                o = jnp.sum(tt.T.reshape(LANES // 8, 8, PW), axis=0)
            if p == NP - 1 or MC[p]:
                o = _add(o, own_head(om_ref[p]))
            finish_o(p, o)

        def stage_wo(p, mm=dot):
            for c in range(DT):
                acc = y_ref[:, pl.ds(c * LANES, LANES)]
                for t in range(3):
                    acc = acc + mm(ob_ref[p, :, pl.ds(t * LANES, LANES)],
                                   _rhs4(wo32, 3 * p + t, c))[0:8]
                y_ref[:, pl.ds(c * LANES, LANES)] = acc

        def begin_attention(x):
            y_ref[:, 0:D] = x
            xb, m, r = ln_stats(x)
            xn = (xb - m) * r
            xn_ref[:, 0:D] = _pack2(xn, xn)
            return xb, m, r

        wait(0)
        begin_attention(jnp.broadcast_to(xbuf[...].astype(F32), (8, D)))

        def pair1(p, carry):
            stage_q(p)
            for k in range(nk):
                stage_qk(p, k)
            softmax(p, 0)
            finish_o(p, own_head(pv_mxu(p, range(nc), False)))
            om_ref[p] = jnp.zeros(om_ref.shape[1:], F32)
            qpk_ref[p] = jnp.zeros((8, LANES), U32)
            cs_ref[p] = jnp.zeros((8, LANES), F32)

            first = 0
            for pp in range(NP - 1):
                first = jnp.where(p == pp, nc - MC[pp], first)

            def transpose_v(c, carry2):
                for t in range(3):
                    tile = _rhs4(v32, 3 * p + t, c)
                    v32[pl.ds(2 * (3 * p + t), 2), :, c] = pltpu.bitcast(
                        tile.T, U32).reshape(2, 4, 8, LANES)
                return carry2

            lax.fori_loop(first, nc, transpose_v, 0)

            @pl.when(p < NP - 1)
            def _():
                for g in range(PG):
                    for e, c in enumerate(XCOLS):
                        w = pltpu.bitcast(v32[v_idx(p, g, c)], BF).astype(F32)
                        v32[v_idx(p, g, c)] = pltpu.bitcast(w[0:8], U32)
                        vx_ref[p, g, e] = w[8:16]

            return carry

        def group1(gi, row):
            for i in range(NGRP):
                pl.when(gi == i)(functools.partial(wait, 1 + i))
            g = NGRP - 1 - gi
            lax.fori_loop(g * GP, (g + 1) * GP, pair1, 0)
            return row + PRING * prow // NGRP

        fence_row = pl.multiple_of(lax.fori_loop(0, NGRP, group1, 0), 8)
        wait(1 + NGRP)

        def woloop(p2, carry):
            stage_wo(2 * p2)
            stage_wo(2 * p2 + 1)
            return carry

        lax.fori_loop(0, NP // 2, woloop, 0)

        x = y_ref[:, 0:D]
        xb, m, r = ln_stats(x)
        wait(2 + NGRP)
        gu = []
        for j in range(2 * FT):
            raw, cs = raw_proj(xb, w13[j % 2], j // 2)
            cs_ref[j] = cs
            gu.append((raw - m * cs) * r)
        hs = [_swiglu(g, u) for g, u in zip(gu[0::2], gu[1::2])]
        for kk in range(W2_MXU // 8, FT):
            p_ref[pl.ds(LANES * kk - 16 * W2_MXU, LANES), :] = col_bcast(
                hs[kk].astype(BF).astype(F32))
        hs = [_pack2(hh, hh) for hh in hs[:W2_MXU // 8]]
        cols = [tile_of(x, c) for c in range(DT)]
        part = [None] * DT
        for i in range(len(W2_SPLIT) - 1):
            wait(3 + NGRP + i)
            g0, g1 = W2_SPLIT[i], W2_SPLIT[i + 1]
            for c in range(DT):
                if g1 <= W2_MXU:
                    for kk in range(g0 // 8, g1 // 8):
                        cols[c] = cols[c] + dot(hs[kk], _rhs(w232, 8 * kk, c))[0:8]
                else:
                    for g in range(g0, g1):
                        row = 16 * (g - W2_MXU)
                        part[c] = vpu_fma(part[c], w232[g, c], p_ref[pl.ds(row, 8), :],
                                          p_ref[pl.ds(row + 8, 8), :])
        x = jnp.concatenate([cc + sub_sum(a) for cc, a in zip(cols, part)], axis=1)

        xb, m, r = begin_attention(x)
        rq = r * qscale

        def run_block(chains, items, n_link, first, last_off, start, end):
            links = []
            for j, (p, g) in enumerate(chains[:n_link]):
                dep = _bits_or(pv_chain(p, g, lambda: p_refs[g % 2]))
                if end:
                    links.extend([(FIN_LINK0 + FIN_LINKSTEP * j, dep)] * FIN_REP)
                else:
                    links.extend([(LINK0 + LINKSTEP * j, dep)] * LINK_REP)
            if start:
                xcol = [col_bcast(tile_of(xb, kk)) - m[0:1] for kk in range(DT)]
                links.extend([(XC_LINK, _bits_or(xc[LANES - 8:] for xc in xcol))] * 4)
            pops = []
            probs = ([], [])
            ready = {}
            busy = []

            def mm(l32, rr, free=True):
                links.sort(key=lambda lk: lk[0])
                if free and links and len(pops) >= links[0][0]:
                    l32 = jnp.where(sub < 4, l32, links.pop(0)[1])
                pops.append(dot(l32, rr))
                return pops[-1]

            for it in items:
                kind, p = it[0], it[1]
                if kind == 'fq':
                    for t in range(3):
                        raw, cs = raw_proj(xb, wq32, 3 * p + t, mm)
                        q = raw - m * cs
                        q = q if p == 0 else q * rq
                        expand_q(p, t, _pack2(q, q))
                elif kind == 'q':
                    stage_q(p, mm)
                    busy.append((len(pops) - Q_A, len(pops) - Q_B, Q_W))
                elif kind == 'qx':
                    for t in range(3):
                        expand_q(p, t, qpk_ref[3 * VQ.index(p) + t])
                elif kind == 'qk':
                    stage_qk(p, it[2], mm, rq if p == 0 else None)
                    ready[p] = len(pops)
                elif kind == 'sm':
                    e, l = softmax(p, 0 if p == NP - 1 else (nc - MC[p]) // 4)
                    lag = SM_LAG0 if p == 0 else SM_LAG
                    pos = len(pops) + (lag if pops else lag - 14)
                    links.append((pos, pltpu.bitcast(l, U32)))
                    busy.append((pos - SM_A, pos - SM_B, SM_W))
                    if p < NP - 1:
                        for j in range((nc - MC[p] + 3) // 4):
                            for pend in probs:
                                pend.append((p, pos - PST_OFF, j, e[j]))
                elif kind == 'pvm':
                    o = pv_mxu(p, range(it[2], it[3]), True, mm)
                    om_ref[p] = o + om_ref[p] if it[4] else o
                elif kind == 'red':
                    stage_reduce(p)
                elif kind == 'wo':
                    busy.append((len(pops) - RED_A, len(pops) - RED_B, RED_W))
                    stage_wo(p, mm)

            def fence(buf, a):
                buf[pl.ds(fence_row, 8), :] = pops[a][0:8]

            if start:
                nkg = D // 16

                def xslot(kg):
                    u = kg // VQ_UNIT
                    return p_refs[u % 2], 16 * (u // 2 * VQ_UNIT + kg % VQ_UNIT)

                for kg in range(nkg):
                    buf, row = xslot(kg)
                    buf[pl.ds(row, 16), :] = xcol[kg // 8][16 * (kg % 8):16 * (kg % 8) + 16]
                for i, p in enumerate(VQ):
                    acc = [None] * 3
                    for kg in range(nkg):
                        buf, row = xslot(kg)
                        if kg % VQ_UNIT == 0:
                            a = (i * nkg + kg) * (first - VQ_FIRST) // (len(VQ) * nkg)
                            fence(buf, VQ_FIRST + a // 2 * 2)
                        xlo = buf[pl.ds(row, 8), :]
                        xhi = buf[pl.ds(row + 8, 8), :]
                        for t in range(3):
                            acc[t] = vpu_fma(acc[t], wq32[kg, 3 * p + t], xlo, xhi)
                    for t in range(3):
                        q = sub_sum(acc[t]) * rq
                        qpk_ref[3 * i + t] = _pack2(q, q)

            def store_probs(b, due, limit=10 ** 9):
                while probs[b] and due(probs[b][0]) and limit:
                    p, _, j, e = probs[b].pop(0)
                    assert p - current[0] < PRING
                    p_refs[b][pl.ds((p % PRING) * prow + 8 * j, 8), :] = e
                    limit -= 1

            rest = chains[n_link:]
            current = [chains[0][0]]
            if rest:
                n_items = sum(nc - MC[p] for p, _ in rest)
                n_units = (len(pops) - last_off - first) // FSTEP + 1
                less = [0.0] * n_units
                for lo, hi, w in busy:
                    us = [u for u in range(n_units) if lo <= first + u * FSTEP < hi]
                    for u in us:
                        less[u] += w / len(us)
                per = (n_items + sum(less)) / n_units
                unit_of, total = [], 0.0
                for u in range(n_units):
                    total += per - less[u]
                    while len(unit_of) < min(total - 1e-6, n_items):
                        unit_of.append(u)
                state = [0, -1, 1]

                def gate():
                    u = unit_of[state[0]]
                    state[0] += 1
                    if u != state[1]:
                        state[1] = u
                        state[2] += 1
                        a = first + u * FSTEP
                        fence(p_refs[state[2] % 2], a)
                        store_probs(state[2] % 2, lambda it: it[1] <= a, PST)
                    return p_refs[state[2] % 2]

            while rest:
                p, g = rest[0]
                current[0] = p
                if g == 0 and p in ready:
                    _LOG.append((p, first + state[1] * FSTEP - ready[p]))
                if g == 0:
                    for i in range(state[0], n_items):
                        if unit_of[i] != state[1] or state[1] + 1 == n_units:
                            break
                        unit_of[i] += 1
                for b in range(2):
                    store_probs(b, lambda it: it[0] <= p)
                n = min(GSHARE - g % GSHARE, len(rest))
                pv_chain(p, g, gate, n)
                rest = rest[n:]
            for b in range(2):
                store_probs(b, lambda it: True)
            if end:
                last_ffn(y_ref[:, 0:D], mm, len(pops), links)

        def last_ffn(x, mm, base, links):
            xb, m, r = ln_stats(x)
            lhs = _pack2(xb, xb)
            xcol = [col_bcast(tile_of(xb, kk)) for kk in range(UP_K)]
            links.extend([(base + UX_LINK, _bits_or(xc[LANES - 8:] for xc in xcol))] * 4)
            j0 = 2 * (FT - UP_COLS)
            part = {}
            for j in range(j0, 2 * FT):
                acc = None
                for kg in range(8 * UP_K):
                    xc = xcol[kg // 8][16 * (kg % 8):16 * (kg % 8) + 16]
                    acc = vpu_fma(acc, w13[j % 2][kg, j // 2], xc[0:8], xc[8:16])
                part[j] = sub_sum(acc)
                links.append((base + int(UP_LINK0 + UP_LINKSTEP * (j - j0)),
                              pltpu.bitcast(part[j], U32)))
            gu = []
            for j in range(2 * FT):
                acc = part.get(j)
                for kk in range(UP_K if j in part else 0, DT):
                    acc = _add(acc, mm(tile_of(lhs, kk),
                                       _rhs(w13[j % 2], 8 * kk, j // 2))[0:8])
                gu.append((acc - m * cs_ref[j]) * r)
            hs = [_swiglu(g, u) for g, u in zip(gu[0::2], gu[1::2])]
            cols = [tile_of(x, c) for c in range(DT)]
            for kk in range(DOWN_K, FT):
                hh = _pack2(hs[kk], hs[kk])
                for c in range(DT):
                    cols[c] = cols[c] + mm(hh, _rhs(w232, 8 * kk, c))[0:8]
            acc = [None] * DT
            for kk in range(DOWN_K):
                hcol = col_bcast(hs[kk].astype(BF).astype(F32))
                for i in range(8):
                    for c in range(DT):
                        acc[c] = vpu_fma(acc[c], w232[8 * kk + i, c],
                                         hcol[16 * i:16 * i + 8],
                                         hcol[16 * i + 8:16 * i + 16])
            cols = [cc + sub_sum(a) for cc, a in zip(cols, acc)]
            o_ref[...] = jnp.concatenate(cols, axis=1)[0:1].astype(o_ref.dtype)

        blocks = _plan(nc)
        for b, blk in enumerate(blocks):
            end = b == len(blocks) - 1
            if b > 0:
                wait(marker)
                if not end:
                    start(marker)
            if ONLY is not None and b not in ONLY and not end:
                if b < 2:
                    expand_q(0, 0, _bits_or(qpk_ref[pp] for pp in range(NP - 1)))
                    for pp in range(2):
                        stage_reduce(pp)
                continue
            run_block(*blk, b == 0, end)

    return kernel


@jax.jit
def pallas_interleave_layers__sliding_block_cached__glu_gated_swiglu__decode_kernel(
    A_x: jax.Array,
    A_k_cache: jax.Array,
    A_v_cache: jax.Array,
    A_wq: jax.Array,
    A_wo: jax.Array,
    B_x: jax.Array,
    B_w1: jax.Array,
    B_w3: jax.Array,
    B_w2: jax.Array,
):
    sk = A_k_cache.shape[2]
    win = min(4096, max(256, sk // 4))
    nt_total, nc = sk // LANES, win // LANES

    def kv_view(a):
        return _tile_view(jnp.swapaxes(a, 2, 3).reshape(H * DH, sk))

    def view4(t):
        return t.reshape(t.shape[0] // 4, 2, 4, t.shape[2], 8, LANES)

    def wbuf(r, c):
        return pltpu.VMEM((r // 16, c // LANES, 16, LANES), BF)

    def wbuf4(r, c):
        return pltpu.VMEM((r // 64, 4, c // LANES, 16, LANES), BF)

    any_spec = pl.BlockSpec(memory_space=pl.ANY)
    out = pl.pallas_call(
        _make_kernel(nt_total, nc),
        out_shape=jax.ShapeDtypeStruct((1, D), A_x.dtype),
        in_specs=[any_spec] * 8,
        out_specs=pl.BlockSpec(memory_space=pltpu.VMEM),
        scratch_shapes=[
            wbuf(H * DH, win), wbuf4(H * DH, win),
            wbuf(D, H * DH), wbuf4(H * DH, D),
            wbuf(D, F), wbuf(D, F), wbuf(F, D),
            pltpu.VMEM((NP - 1, PG, len(XCOLS), 8, LANES), F32),
            pltpu.VMEM((RING, 12, 8, LANES), U32),
            pltpu.VMEM((RING, nc // 4, 8, LANES), F32),
            pltpu.VMEM((PRING * 2 * nc + 32, LANES), F32),
            pltpu.VMEM((PRING * 2 * nc + 32, LANES), F32),
            pltpu.VMEM((RING, nc // 4, 8, LANES), U32),
            pltpu.VMEM((NP, 8, LANES), F32),
            pltpu.VMEM((NP, 8, PW), F32),
            pltpu.VMEM((NP, 8, PW), U32),
            pltpu.VMEM((16, 8, LANES), U32),
            pltpu.VMEM((2 * FT, 8, LANES), F32),
            pltpu.VMEM((16, 8, LANES), U32),
            pltpu.VMEM((8, 1024), U32),
            pltpu.VMEM((8, 1024), F32),
            pltpu.VMEM((1, D), BF),
            pltpu.SemaphoreType.DMA((NSEM,)),
        ],
        compiler_params=pltpu.CompilerParams(
            vmem_limit_bytes=128 * 1024 * 1024),
    )(A_x.reshape(1, D), kv_view(A_k_cache), view4(kv_view(A_v_cache)),
      _tile_view(A_wq), view4(_tile_view(A_wo)),
      _tile_view(B_w1), _tile_view(B_w3), _tile_view(B_w2))
    return out.reshape(A_x.shape)
```

```python
import functools
import math

import jax
import jax.numpy as jnp
from jax import lax
import jax.experimental.pallas as pl
import jax.experimental.pallas.tpu as pltpu

D = 640
H = 32
DH = 192
F = 1536
LANES = 128
EPS = 1e-5

NP = H // 2
PG = 2 * DH // 16
HG = DH // 16
PW = 2 * DH
DT = D // LANES
FT = F // LANES

GP = 4
NGRP = NP // GP
W2_SPLIT = (0, 56, 80, 92, 96)
W2_MXU = 80
RELOAD_ROWS = 8
NSEM = 3
RING = 4
PRING = 6

MC = (2, 2, 2, 2, 2, 2, 2, 2, 2, 2, 2, 2, 2, 2, 2)
XCOLS = (1, 7, 10, 16, 22, 25, 4, 13, 19, 28)
NVX = 6
VQ = (11, 12, 13, 14, 15)
V_END = (173, 298, 352)
TILES = (1060, 655, 290)
GSHARE = 2
PVM_AFTER = 2
WO_START = (0, 80, 50, 999)
WO_GAP = (0, 60, 48, 12)
WO_KEEP = 3
FSTEP = 2
FIRST = (156, 2, 0)
LAST_OFF = (8, 6, 4)
VQ_FIRST = 34
VQ_UNIT = 4
XC_LINK = 50
SM_LAG = 48
SM_LAG0 = 38
PST = 0
PST_OFF = 12
RED_W = 10
RED_A = 40
RED_B = 16
Q_W = 4
Q_A = 12
Q_B = -4
SM_W = 7
SM_A = 40
SM_B = 20
NLINK = 3
LINK0 = 8
LINKSTEP = 4
LINK_REP = 1
FIN_LINK0 = 4
FIN_LINKSTEP = 5
FIN_REP = 1
UP_K = 3
UP_COLS = 6
UP_LINK0 = 52
UP_LINKSTEP = 4.5
UX_LINK = 999
DOWN_K = 3

U32 = jnp.uint32
BF = jnp.bfloat16
F32 = jnp.float32

_LOG = []
ONLY = None


def _tile_view(w):
    r, c = w.shape
    return jnp.swapaxes(w.reshape(r // 16, 2, 8, c // LANES, LANES), 2, 3)


def _rhs(w32, g0, c):
    return pltpu.bitcast(w32[pl.ds(g0, 8), c].reshape(64, LANES), BF)


def _rhs4(w32, tile, c):
    return pltpu.bitcast(w32[pl.ds(2 * tile, 2), :, c].reshape(64, LANES), BF)


def _swiglu(g, u):
    hg = 0.5 * g
    return hg * (1.0 + jnp.tanh(hg)) * u


def _pack2(lo, hi):
    return pltpu.bitcast(jnp.concatenate([lo, hi], axis=0).astype(BF), U32)


def _add(a, b):
    return b if a is None else a + b


def _bits_or(vals):
    return functools.reduce(lambda a, b: a | b, [pltpu.bitcast(v, U32) for v in vals])


def _plan(nc):
    nk = nc // 8
    seq = [('fq', 0), ('fq', 1)]
    for p in range(NP):
        if 1 <= p < NP - 1:
            seq.append(('qx' if p + 1 in VQ else 'q', p + 1))
        for k in range(nk):
            if k == PVM_AFTER and p > 0 and MC[p - 1]:
                seq.append(('pvm', p - 1, nc - MC[p - 1], nc, False))
            seq.append(('qk', p, k))
        if p < 2:
            seq.append(('reload', p))
        seq.append(('sm', p))
    seq += [('pvm', NP - 1, c, c + 4, c > 0) for c in range(0, nc, 4)]
    last_pv = seq[-nc // 4]

    def tiles(it):
        if it[0] == 'pvm':
            return 3 * (it[3] - it[2])
        return dict(fq=15, q=15, wo=15, qk=24, sm=0, qx=0, reload=0)[it[0]]

    chains = [(p, g) for p in range(NP - 1) for g in range(PG)]
    blocks = []
    v0 = done = 0
    for b in range(len(V_END) + 1):
        final = b == len(V_END)
        v1 = len(chains) if final else V_END[b]
        todo = list(range(done, v0 // PG))
        done = v0 // PG
        budget = 10 ** 9 if final else TILES[b] - 15 * len(todo)
        body = []
        used = 0
        while seq and used + tiles(seq[0]) // 2 <= budget:
            body.append(seq.pop(0))
            used += tiles(body[-1])
        while body[-1][0] in ('sm', 'qx'):
            seq.insert(0, body.pop())
        assert b > 0 or not any(it[1] in VQ for it in body)
        keep = WO_KEEP if last_pv in body else 0
        items = [('red', p) for p in todo]
        used = 0
        nxt = WO_START[b]
        for it in body:
            if it == last_pv:
                while todo:
                    items.append(('wo', todo.pop(0)))
            if len(todo) > keep and used >= nxt:
                items.append(('wo', todo.pop(0)))
                nxt = used + WO_GAP[b]
            items.append(it)
            used += tiles(it)
        items += [('wo', p) for p in todo]
        if final:
            assert done == NP - 2
            for p in (NP - 1, NP - 2):
                items += [('red', p), ('wo', p)]
            blocks.append((chains[v0:v1], items, v1 - v0, 0, 0))
        else:
            blocks.append((chains[v0:v1], items, NLINK if b else 0, FIRST[b], LAST_OFF[b]))
        v0 = v1
    seen = set()
    for b, (chs, items, n_link, _, _) in enumerate(blocks):
        assert all(it[1] - (NP - 2) < b for it in items if it[0] == 'qk')
        assert all(p in seen for p, _ in chs[:n_link])
        seen |= {it[1] for it in items if it[0] == 'sm'}
        assert all(p in seen for p, _ in chs)
    return blocks


def _make_kernel(n_tiles_total, nc):
    c0 = n_tiles_total - nc
    qscale = DH ** -0.5 * math.log2(math.e)
    prow = 2 * nc
    nk = nc // 8

    def kernel(x_hbm, k_hbm, v_hbm, wq_hbm, wo_hbm, w1_hbm, w3_hbm, w2_hbm,
               o_ref,
               kbuf, vbuf, wqbuf, wobuf, w1buf, w3buf, w2buf,
               vx_ref, t0_ref, lhs_ref, s_ref, p_ref, p2_ref, pk_ref, lsum_ref, om_ref,
               ob_ref, mask_ref, cs_ref, qpk_ref, xn_ref, y_ref, xbuf, sem):
        def halves(src, dst):
            return [(src(par), dst(pl.ds(8 * par, 8))) for par in range(2)]

        def whole(src, dst):
            return halves(lambda p: src.at[:, p], lambda h: dst.at[:, :, h, :])

        def kv_group(g):
            kr = pl.ds(g * GP * PG, GP * PG)
            vr = pl.ds(g * GP * PG // 4, GP * PG // 4)
            return (halves(lambda p: k_hbm.at[kr, p, pl.ds(c0, nc)],
                           lambda h: kbuf.at[kr, :, h, :])
                    + halves(lambda p: v_hbm.at[vr, p, :, pl.ds(c0, nc)],
                             lambda h: vbuf.at[vr, :, :, h, :]))

        def w2_group(i):
            rows = pl.ds(W2_SPLIT[i], W2_SPLIT[i + 1] - W2_SPLIT[i])
            return halves(lambda p: w2_hbm.at[rows, p], lambda h: w2buf.at[rows, :, h, :])

        groups = ([whole(wq_hbm, wqbuf) + [(x_hbm, xbuf)]]
                  + [kv_group(NGRP - 1 - g) for g in range(NGRP)]
                  + [halves(lambda p: wo_hbm.at[:, p], lambda h: wobuf.at[:, :, :, h, :]),
                     whole(w1_hbm, w1buf) + whole(w3_hbm, w3buf)]
                  + [w2_group(i) for i in range(len(W2_SPLIT) - 1)])
        marker = len(groups)
        groups.append([(x_hbm, xbuf)])
        n_ring = len(groups)
        def k_rows(i, rows):
            return halves(lambda p: k_hbm.at[rows((NP - 2 + i) * PG), p, pl.ds(c0, nc)],
                          lambda h: kbuf.at[rows(i * PG), :, h, :])

        for i, n in enumerate((PG, RELOAD_ROWS)):
            groups.append([cp for g in range(n) for cp in k_rows(i, lambda r0: r0 + g)])
        late = n_ring + 1 + NSEM
        groups += [[]] * (late - len(groups))
        groups.append(k_rows(1, lambda r0: pl.ds(r0 + RELOAD_ROWS, PG - RELOAD_ROWS)))

        def copies(i):
            return [pltpu.make_async_copy(src, dst, sem.at[i % NSEM])
                    for src, dst in groups[i]]

        def start_dma(i):
            for cp in copies(i):
                cp.start()

        def wait(i):
            for cp in copies(i):
                cp.wait()
            if i + NSEM < n_ring:
                start_dma(i + NSEM)

        for i in range(NSEM):
            start_dma(i)

        k32 = kbuf.bitcast(U32)
        v32 = vbuf.bitcast(U32)
        wq32 = wqbuf.bitcast(U32)
        wo32 = wobuf.bitcast(U32)
        w13 = (w1buf.bitcast(U32), w3buf.bitcast(U32))
        w232 = w2buf.bitcast(U32)

        sub = lax.broadcasted_iota(jnp.int32, (8, LANES), 0)
        lane = lax.broadcasted_iota(jnp.int32, (8, LANES), 1)
        sub3 = lax.broadcasted_iota(jnp.int32, (8, PW), 0)
        lane3 = lax.broadcasted_iota(jnp.int32, (8, PW), 1)

        for r in range(4):
            half = U32(0x0000FFFF if r % 2 == 0 else 0xFFFF0000)
            lo = jnp.where(sub == r // 2, half, U32(0))
            hi = jnp.where(sub == 2 + r // 2, half, U32(0))
            mask_ref[r] = lo
            mask_ref[4 + r] = jnp.where(lane < DH - LANES, lo, hi)
            mask_ref[8 + r] = hi
            mask_ref[12 + r] = lo | hi
        p_refs = (p_ref, p2_ref)
        for pr in p_refs:
            pr[...] = jnp.zeros(pr.shape, F32)

        def dot(l32, r, free=True):
            del free
            return jnp.dot(pltpu.bitcast(l32, BF), r, preferred_element_type=F32)

        def tile_of(v, kk):
            return v[:, kk * LANES:(kk + 1) * LANES]

        def ln_stats(x):
            xb = x.astype(BF).astype(F32)
            m = jnp.mean(xb, axis=-1, keepdims=True)
            xc = xb - m
            v = jnp.mean(xc * xc, axis=-1, keepdims=True)
            return xb, m, lax.rsqrt(v + EPS)

        def raw_proj(xb, w32, c, mm=dot):
            lhs = _pack2(xb, jnp.ones_like(xb))
            acc = None
            for kk in range(DT):
                acc = _add(acc, mm(tile_of(lhs, kk), _rhs(w32, 8 * kk, c), False))
            return acc[0:8], acc[8:16]

        def col_bcast(v):
            return jnp.concatenate([v] * (LANES // 8), axis=0).T

        def vpu_fma(acc, w, xlo, xhi):
            w = pltpu.bitcast(w, BF).astype(F32)
            return _add(acc, w[0:8] * xlo + w[8:16] * xhi)

        def sub_sum(a):
            return jnp.broadcast_to(jnp.sum(a, axis=0, keepdims=True), a.shape)

        def expand_q(p, t, q):
            for r in range(4):
                lhs_ref[p % RING, 4 * t + r] = q & mask_ref[4 * t + r]

        def stage_q(p, mm=dot):
            acc = [None] * 3
            for kk in range(DT):
                for t in range(3):
                    acc[t] = _add(acc[t], mm(xn_ref[:, pl.ds(kk * LANES, LANES)],
                                             _rhs(wq32, 8 * kk, 3 * p + t))[0:8])
            for t in range(3):
                q = acc[t] * qscale
                expand_q(p, t, _pack2(q, q))

        def stage_qk(p, k, krow, mm=dot, scale=None):
            for j in range(2 * k, 2 * k + 2):
                acc = None
                for t in range(3):
                    for r in range(4):
                        acc = _add(acc, mm(lhs_ref[p % RING, 4 * t + r],
                                           _rhs(k32, krow + 8 * t, 4 * j + r))[0:8])
                s_ref[p % RING, j] = acc if scale is None else acc * scale

        def head_reduce(v, op, lane_op):
            for d in (1, 2):
                up = pltpu.roll(v, d, 0)
                down = pltpu.roll(v, 8 - d, 0)
                v = op(v, jnp.where(sub % (2 * d) >= d, up, down))
            return lane_op(v, axis=1, keepdims=True)

        def softmax(p, j0):
            s = s_ref[p % RING]
            m = head_reduce(jnp.max(s, axis=0), jnp.maximum, jnp.max)
            e = jnp.exp2(s - m)
            l = jnp.sum(e, axis=0)
            lsum_ref[p] = l
            for j in range(j0, nc // 4):
                pk_ref[p % RING, j] = _pack2(e[j], e[j])
            return e, l

        def v_idx(p, g, c):
            return p * (PG // 4) + g // 4, g % 4, c

        def vx_slot(p, g, e):
            return (NP - 2) * PG + 3 * p + g // 8, g % 8 * 4 + e - NVX

        def t_slot(p, j):
            if p == 0:
                return t0_ref, j
            row = (NP - 2) * PG if p == 1 else p * PG if p < NP - 2 else 2 * PG + 2
            return k32, (row + j // nc, j % nc)

        def pv_chain(p, g, gate, n=1):
            acc = [None] * (2 * n)
            for c in range(nc - MC[p]):
                row = (p % PRING) * prow + 8 * (c // 4) + 4 * (g // HG) + c % 4
                pb = gate()[pl.ds(row, 8, stride=0), :]
                for i in range(n):
                    if i:
                        gate()
                    w = v32[v_idx(p, g + i, c)]
                    if c in (XCOLS if p else XCOLS[:NVX]):
                        e = XCOLS.index(c)
                        w = (pltpu.bitcast(w, F32),
                             vx_ref[p, g + i, e] if e < NVX else
                             pltpu.bitcast(k32[vx_slot(p, g + i, e)], F32))
                    else:
                        w = pltpu.bitcast(w, BF).astype(F32)
                        w = (w[0:8], w[8:16])
                    for h in range(2):
                        acc[2 * i + h] = _add(acc[2 * i + h], w[h] * pb)
            for i in range(2 * n):
                ref, idx = t_slot(p, 2 * g + i)
                ref[idx] = pltpu.bitcast(acc[i], U32)
            return acc

        def pv_mxu(p, cols, transposed, mm=dot):
            acc = [None] * 3
            cols = list(cols)
            for i0 in range(0, len(cols), 4):
                ls = {c: pk_ref[p % RING, c // 4] & mask_ref[12 + c % 4]
                      for c in cols[i0:i0 + 4]}
                for t in range(3):
                    for c, l in ls.items():
                        tile = _rhs4(v32, 3 * p + t, c)
                        if transposed:
                            res = mm(l, tile)
                        else:
                            res = lax.dot_general(
                                pltpu.bitcast(l, BF), tile, (((1,), (1,)), ((), ())),
                                preferred_element_type=F32)
                        acc[t] = _add(acc[t], res[0:8])
            return jnp.concatenate(acc, axis=1)

        def own_head(o):
            return jnp.where((sub3 < 4) == (lane3 < DH), o, 0.0)

        def finish_o(p, o):
            linv = 1.0 / head_reduce(lsum_ref[p], jnp.add, jnp.sum)
            o = (jnp.sum(o, axis=0, keepdims=True)
                 * jnp.where(lane3 < DH, linv[0:1], linv[4:5]))
            ob_ref[p] = _pack2(o, o)

        def stage_reduce(p):
            o = None
            if p < NP - 1:
                slots = [t_slot(p, j) for j in range(2 * PG)]
                tt = pltpu.bitcast(jnp.concatenate([ref[idx] for ref, idx in slots]), F32)
                o = jnp.sum(tt.T.reshape(LANES // 8, 8, PW), axis=0)
            if p == NP - 1 or MC[p]:
                o = _add(o, own_head(om_ref[p]))
            finish_o(p, o)

        def stage_wo(p, mm=dot):
            for c in range(DT):
                acc = y_ref[:, pl.ds(c * LANES, LANES)]
                for t in range(3):
                    acc = acc + mm(ob_ref[p, :, pl.ds(t * LANES, LANES)],
                                   _rhs4(wo32, 3 * p + t, c))[0:8]
                y_ref[:, pl.ds(c * LANES, LANES)] = acc

        def begin_attention(x):
            y_ref[:, 0:D] = x
            xb, m, r = ln_stats(x)
            xn = (xb - m) * r
            xn_ref[:, 0:D] = _pack2(xn, xn)
            return xb, m, r

        wait(0)
        begin_attention(jnp.broadcast_to(xbuf[...].astype(F32), (8, D)))

        def pair1(i, carry):
            p = NP - 1 - i
            stage_q(p)
            for k in range(nk):
                stage_qk(p, k, p * PG)
            softmax(p, 0)
            finish_o(p, own_head(pv_mxu(p, range(nc), False)))
            om_ref[p] = jnp.zeros(om_ref.shape[1:], F32)
            qpk_ref[p] = jnp.zeros((8, LANES), U32)
            t0_ref[p] = jnp.zeros((8, LANES), U32)
            cs_ref[p] = jnp.zeros((8, LANES), F32)

            first = 0
            for pp in range(NP - 1):
                first = jnp.where(p == pp, nc - MC[pp], first)

            def transpose_v(c, carry2):
                for t in range(3):
                    tile = _rhs4(v32, 3 * p + t, c)
                    v32[pl.ds(2 * (3 * p + t), 2), :, c] = pltpu.bitcast(
                        tile.T, U32).reshape(2, 4, 8, LANES)
                return carry2

            lax.fori_loop(first, nc, transpose_v, 0)

            def widen(es):
                for g in range(PG):
                    for e in es:
                        idx = v_idx(p, g, XCOLS[e])
                        w = pltpu.bitcast(v32[idx], BF).astype(F32)
                        v32[idx] = pltpu.bitcast(w[0:8], U32)
                        if e < NVX:
                            vx_ref[p, g, e] = w[8:16]
                        else:
                            k32[vx_slot(p, g, e)] = pltpu.bitcast(w[8:16], U32)

            pl.when(p < NP - 1)(functools.partial(widen, range(NVX)))
            pl.when((p < NP - 1) & (p > 0))(
                functools.partial(widen, range(NVX, len(XCOLS))))
            return carry

        def group1(gi, row):
            for i in range(NGRP):
                pl.when(gi == i)(functools.partial(wait, 1 + i))
            lax.fori_loop(gi * GP, (gi + 1) * GP, pair1, 0)
            return row + PRING * prow // NGRP

        fence_row = pl.multiple_of(lax.fori_loop(0, NGRP, group1, 0), 8)
        wait(1 + NGRP)

        def woloop(p2, carry):
            stage_wo(2 * p2)
            stage_wo(2 * p2 + 1)
            return carry

        lax.fori_loop(0, NP // 2, woloop, 0)

        x = y_ref[:, 0:D]
        xb, m, r = ln_stats(x)
        wait(2 + NGRP)
        gu = []
        for j in range(2 * FT):
            raw, cs = raw_proj(xb, w13[j % 2], j // 2)
            cs_ref[j] = cs
            gu.append((raw - m * cs) * r)
        hs = [_swiglu(g, u) for g, u in zip(gu[0::2], gu[1::2])]
        for kk in range(W2_MXU // 8, FT):
            p_ref[pl.ds(LANES * kk - 16 * W2_MXU, LANES), :] = col_bcast(
                hs[kk].astype(BF).astype(F32))
        hs = [_pack2(hh, hh) for hh in hs[:W2_MXU // 8]]
        cols = [tile_of(x, c) for c in range(DT)]
        part = [None] * DT
        for i in range(len(W2_SPLIT) - 1):
            wait(3 + NGRP + i)
            g0, g1 = W2_SPLIT[i], W2_SPLIT[i + 1]
            for c in range(DT):
                if g1 <= W2_MXU:
                    for kk in range(g0 // 8, g1 // 8):
                        cols[c] = cols[c] + dot(hs[kk], _rhs(w232, 8 * kk, c))[0:8]
                else:
                    for g in range(g0, g1):
                        row = 16 * (g - W2_MXU)
                        part[c] = vpu_fma(part[c], w232[g, c], p_ref[pl.ds(row, 8), :],
                                          p_ref[pl.ds(row + 8, 8), :])
        x = jnp.concatenate([cc + sub_sum(a) for cc, a in zip(cols, part)], axis=1)

        xb, m, r = begin_attention(x)
        rq = r * qscale

        def run_block(chains, items, n_link, first, last_off, start, end):
            links = []
            for j, (p, g) in enumerate(chains[:n_link]):
                dep = _bits_or(pv_chain(p, g, lambda: p_refs[g % 2]))
                if end:
                    links.extend([(FIN_LINK0 + FIN_LINKSTEP * j, dep)] * FIN_REP)
                else:
                    links.extend([(LINK0 + LINKSTEP * j, dep)] * LINK_REP)
            if start:
                xcol = [col_bcast(tile_of(xb, kk)) - m[0:1] for kk in range(DT)]
                links.extend([(XC_LINK, _bits_or(xc[LANES - 8:] for xc in xcol))] * 4)
            pops = []
            probs = ([], [])
            ready = {}
            busy = []

            def mm(l32, rr, free=True):
                links.sort(key=lambda lk: lk[0])
                if free and links and len(pops) >= links[0][0]:
                    l32 = jnp.where(sub < 4, l32, links.pop(0)[1])
                pops.append(dot(l32, rr))
                return pops[-1]

            for it in items:
                kind, p = it[0], it[1]
                if kind == 'fq':
                    for t in range(3):
                        raw, cs = raw_proj(xb, wq32, 3 * p + t, mm)
                        q = raw - m * cs
                        q = q if p == 0 else q * rq
                        expand_q(p, t, _pack2(q, q))
                elif kind == 'q':
                    stage_q(p, mm)
                    busy.append((len(pops) - Q_A, len(pops) - Q_B, Q_W))
                elif kind == 'qx':
                    for t in range(3):
                        expand_q(p, t, qpk_ref[3 * VQ.index(p) + t])
                elif kind == 'qk':
                    stage_qk(p, it[2], p % (NP - 2) * PG, mm, rq if p == 0 else None)
                    ready[p] = len(pops)
                elif kind == 'sm':
                    e, l = softmax(p, 0 if p == NP - 1 else (nc - MC[p]) // 4)
                    lag = SM_LAG0 if p == 0 else SM_LAG
                    pos = len(pops) + (lag if pops else lag - 14)
                    links.append((pos, pltpu.bitcast(l, U32)))
                    busy.append((pos - SM_A, pos - SM_B, SM_W))
                    if p < NP - 1:
                        for j in range((nc - MC[p] + 3) // 4):
                            for pend in probs:
                                pend.append((p, pos - PST_OFF, j, e[j]))
                elif kind == 'pvm':
                    o = pv_mxu(p, range(it[2], it[3]), True, mm)
                    om_ref[p] = o + om_ref[p] if it[4] else o
                elif kind == 'reload':
                    start_dma(n_ring + p)
                elif kind == 'red':
                    stage_reduce(p)
                elif kind == 'wo':
                    busy.append((len(pops) - RED_A, len(pops) - RED_B, RED_W))
                    stage_wo(p, mm)

            def fence(buf, a):
                buf[pl.ds(fence_row, 8), :] = pops[a][0:8]

            if start:
                nkg = D // 16

                def xslot(kg):
                    u = kg // VQ_UNIT
                    return p_refs[u % 2], 16 * (u // 2 * VQ_UNIT + kg % VQ_UNIT)

                for kg in range(nkg):
                    buf, row = xslot(kg)
                    buf[pl.ds(row, 16), :] = xcol[kg // 8][16 * (kg % 8):16 * (kg % 8) + 16]
                for i, p in enumerate(VQ):
                    acc = [None] * 3
                    for kg in range(nkg):
                        buf, row = xslot(kg)
                        if kg % VQ_UNIT == 0:
                            a = (i * nkg + kg) * (first - VQ_FIRST) // (len(VQ) * nkg)
                            fence(buf, VQ_FIRST + a // 2 * 2)
                        xlo = buf[pl.ds(row, 8), :]
                        xhi = buf[pl.ds(row + 8, 8), :]
                        for t in range(3):
                            acc[t] = vpu_fma(acc[t], wq32[kg, 3 * p + t], xlo, xhi)
                    for t in range(3):
                        q = sub_sum(acc[t]) * rq
                        qpk_ref[3 * i + t] = _pack2(q, q)

            def store_probs(b, due, limit=10 ** 9):
                while probs[b] and due(probs[b][0]) and limit:
                    p, _, j, e = probs[b].pop(0)
                    assert p - current[0] < PRING
                    p_refs[b][pl.ds((p % PRING) * prow + 8 * j, 8), :] = e
                    limit -= 1

            rest = chains[n_link:]
            current = [chains[0][0]]
            if rest:
                n_items = sum(nc - MC[p] for p, _ in rest)
                n_units = (len(pops) - last_off - first) // FSTEP + 1
                less = [0.0] * n_units
                for lo, hi, w in busy:
                    us = [u for u in range(n_units) if lo <= first + u * FSTEP < hi]
                    for u in us:
                        less[u] += w / len(us)
                per = (n_items + sum(less)) / n_units
                unit_of, total = [], 0.0
                for u in range(n_units):
                    total += per - less[u]
                    while len(unit_of) < min(total - 1e-6, n_items):
                        unit_of.append(u)
                state = [0, -1, 1]

                def gate():
                    u = unit_of[state[0]]
                    state[0] += 1
                    if u != state[1]:
                        state[1] = u
                        state[2] += 1
                        a = first + u * FSTEP
                        fence(p_refs[state[2] % 2], a)
                        store_probs(state[2] % 2, lambda it: it[1] <= a, PST)
                    return p_refs[state[2] % 2]

            while rest:
                p, g = rest[0]
                current[0] = p
                if g == 0 and p in ready:
                    _LOG.append((p, first + state[1] * FSTEP - ready[p]))
                if g == 0:
                    for i in range(state[0], n_items):
                        if unit_of[i] != state[1] or state[1] + 1 == n_units:
                            break
                        unit_of[i] += 1
                for b in range(2):
                    store_probs(b, lambda it: it[0] <= p)
                n = min(GSHARE - g % GSHARE, len(rest))
                pv_chain(p, g, gate, n)
                rest = rest[n:]
            for b in range(2):
                store_probs(b, lambda it: True)
            if end:
                last_ffn(y_ref[:, 0:D], mm, len(pops), links)

        def last_ffn(x, mm, base, links):
            xb, m, r = ln_stats(x)
            lhs = _pack2(xb, xb)
            xcol = [col_bcast(tile_of(xb, kk)) for kk in range(UP_K)]
            links.extend([(base + UX_LINK, _bits_or(xc[LANES - 8:] for xc in xcol))] * 4)
            j0 = 2 * (FT - UP_COLS)
            part = {}
            for j in range(j0, 2 * FT):
                acc = None
                for kg in range(8 * UP_K):
                    xc = xcol[kg // 8][16 * (kg % 8):16 * (kg % 8) + 16]
                    acc = vpu_fma(acc, w13[j % 2][kg, j // 2], xc[0:8], xc[8:16])
                part[j] = sub_sum(acc)
                links.append((base + int(UP_LINK0 + UP_LINKSTEP * (j - j0)),
                              pltpu.bitcast(part[j], U32)))
            gu = []
            for j in range(2 * FT):
                acc = part.get(j)
                for kk in range(UP_K if j in part else 0, DT):
                    acc = _add(acc, mm(tile_of(lhs, kk),
                                       _rhs(w13[j % 2], 8 * kk, j // 2))[0:8])
                gu.append((acc - m * cs_ref[j]) * r)
            hs = [_swiglu(g, u) for g, u in zip(gu[0::2], gu[1::2])]
            cols = [tile_of(x, c) for c in range(DT)]
            for kk in range(DOWN_K, FT):
                hh = _pack2(hs[kk], hs[kk])
                for c in range(DT):
                    cols[c] = cols[c] + mm(hh, _rhs(w232, 8 * kk, c))[0:8]
            acc = [None] * DT
            for kk in range(DOWN_K):
                hcol = col_bcast(hs[kk].astype(BF).astype(F32))
                for i in range(8):
                    for c in range(DT):
                        acc[c] = vpu_fma(acc[c], w232[8 * kk + i, c],
                                         hcol[16 * i:16 * i + 8],
                                         hcol[16 * i + 8:16 * i + 16])
            cols = [cc + sub_sum(a) for cc, a in zip(cols, acc)]
            o_ref[...] = jnp.concatenate(cols, axis=1)[0:1].astype(o_ref.dtype)

        blocks = _plan(nc)
        for b, blk in enumerate(blocks):
            end = b == len(blocks) - 1
            if b > 0:
                wait(marker if end else n_ring + b - 1)
            if b == 1:
                start_dma(late)
            if b == 2:
                wait(late)
            if ONLY is not None and b not in ONLY and not end:
                if b == 0:
                    start_dma(n_ring)
                    start_dma(n_ring + 1)
                if b < 2:
                    expand_q(0, 0, _bits_or(qpk_ref[pp] for pp in range(NP - 1)))
                    for pp in range(2):
                        stage_reduce(pp)
                continue
            run_block(*blk, b == 0, end)

    return kernel


@jax.jit
def pallas_interleave_layers__sliding_block_cached__glu_gated_swiglu__decode_kernel(
    A_x: jax.Array,
    A_k_cache: jax.Array,
    A_v_cache: jax.Array,
    A_wq: jax.Array,
    A_wo: jax.Array,
    B_x: jax.Array,
    B_w1: jax.Array,
    B_w3: jax.Array,
    B_w2: jax.Array,
):
    sk = A_k_cache.shape[2]
    win = min(4096, max(256, sk // 4))
    nt_total, nc = sk // LANES, win // LANES

    def kv_view(a):
        return _tile_view(jnp.swapaxes(a, 2, 3).reshape(H * DH, sk))

    def view4(t):
        return t.reshape(t.shape[0] // 4, 2, 4, t.shape[2], 8, LANES)

    def wbuf(r, c):
        return pltpu.VMEM((r // 16, c // LANES, 16, LANES), BF)

    def wbuf4(r, c):
        return pltpu.VMEM((r // 64, 4, c // LANES, 16, LANES), BF)

    any_spec = pl.BlockSpec(memory_space=pl.ANY)
    out = pl.pallas_call(
        _make_kernel(nt_total, nc),
        out_shape=jax.ShapeDtypeStruct((1, D), A_x.dtype),
        in_specs=[any_spec] * 8,
        out_specs=pl.BlockSpec(memory_space=pltpu.VMEM),
        scratch_shapes=[
            wbuf(H * DH, win), wbuf4(H * DH, win),
            wbuf(D, H * DH), wbuf4(H * DH, D),
            wbuf(D, F), wbuf(D, F), wbuf(F, D),
            pltpu.VMEM((NP - 1, PG, NVX, 8, LANES), F32),
            pltpu.VMEM((2 * PG, 8, LANES), U32),
            pltpu.VMEM((RING, 12, 8, LANES), U32),
            pltpu.VMEM((RING, nc // 4, 8, LANES), F32),
            pltpu.VMEM((PRING * 2 * nc + 32, LANES), F32),
            pltpu.VMEM((PRING * 2 * nc + 32, LANES), F32),
            pltpu.VMEM((RING, nc // 4, 8, LANES), U32),
            pltpu.VMEM((NP, 8, LANES), F32),
            pltpu.VMEM((NP, 8, PW), F32),
            pltpu.VMEM((NP, 8, PW), U32),
            pltpu.VMEM((16, 8, LANES), U32),
            pltpu.VMEM((2 * FT, 8, LANES), F32),
            pltpu.VMEM((16, 8, LANES), U32),
            pltpu.VMEM((8, 1024), U32),
            pltpu.VMEM((8, 1024), F32),
            pltpu.VMEM((1, D), BF),
            pltpu.SemaphoreType.DMA((NSEM,)),
        ],
        compiler_params=pltpu.CompilerParams(
            vmem_limit_bytes=128 * 1024 * 1024),
    )(A_x.reshape(1, D), kv_view(A_k_cache), view4(kv_view(A_v_cache)),
      _tile_view(A_wq), view4(_tile_view(A_wo)),
      _tile_view(B_w1), _tile_view(B_w3), _tile_view(B_w2))
    return out.reshape(A_x.shape)
```

```python
import functools
import math

import jax
import jax.numpy as jnp
from jax import lax
import jax.experimental.pallas as pl
import jax.experimental.pallas.tpu as pltpu

D = 640
H = 32
DH = 192
F = 1536
LANES = 128
EPS = 1e-5

NP = H // 2
PG = 2 * DH // 16
HG = DH // 16
PW = 2 * DH
DT = D // LANES
FT = F // LANES

GP = 4
NGRP = NP // GP
W2_SPLIT = (0, 56, 80, 92, 96)
W2_MXU = 80
RELOAD_ROWS = 8
NSEM = 3
RING = 4
PRING = 6

MC = (2, 2, 2, 2, 2, 2, 2, 2, 2, 2, 2, 2, 2, 2, 2)
XCOLS = (1, 7, 10, 16, 22, 25, 4, 13, 19, 28)
NVX = 6
VQ = (11, 12, 13, 14, 15)
V_END = (172, 297, 352)
TILES = (1060, 655, 290)
XCOST = (0.67, 0.77, 0.67, 0.67)
GSHARE = 2
PVM_AFTER = 2
WO_START = (0, 80, 65, 999)
WO_GAP = (0, 72, 60, 12)
WO_KEEP = 3
FSTEP = 2
FIRST = (160, 2, 0)
LAST_OFF = (8, 6, 6)
VQ_FIRST = 30
VQ_UNIT = 4
XC_LINK = 50
SM_LAG = (60, 64, 64, 64)
SM_LAG0 = 52
RED_W = (10, 10, 10, 10)
RED_A = (40, 40, 40, 40)
RED_B = (16, 20, 20, 16)
Q_W = (4, 4, 4, 4)
Q_A = (18, 12, 12, 12)
Q_B = (-4, -4, -4, -4)
SM_W = (4, 4, 7, 7)
SM_A = (56, 56, 56, 56)
SM_B = (30, 42, 30, 30)
NLINK = (0, 4, 3)
LINK0 = (8, 8, 8, 6)
LINKSTEP = (4, 5, 4, 6.0)
LINK_REP = (1, 1, 1, 4)
UP_K = 3
UP_COLS = 6
UP_LINK0 = 54
UP_LINKSTEP = 4.25
UX_LINK = 44
DOWN_K = 3

U32 = jnp.uint32
BF = jnp.bfloat16
F32 = jnp.float32

_LOG = []
ONLY = None


def _tile_view(w):
    r, c = w.shape
    return jnp.swapaxes(w.reshape(r // 16, 2, 8, c // LANES, LANES), 2, 3)


def _rhs(w32, g0, c):
    return pltpu.bitcast(w32[pl.ds(g0, 8), c].reshape(64, LANES), BF)


def _rhs4(w32, tile, c):
    return pltpu.bitcast(w32[pl.ds(2 * tile, 2), :, c].reshape(64, LANES), BF)


def _swiglu(g, u):
    hg = 0.5 * g
    return hg * (1.0 + jnp.tanh(hg)) * u


def _pack2(lo, hi):
    return pltpu.bitcast(jnp.concatenate([lo, hi], axis=0).astype(BF), U32)


def _add(a, b):
    return b if a is None else a + b


def _bits_or(vals):
    return functools.reduce(lambda a, b: a | b, [pltpu.bitcast(v, U32) for v in vals])


def _plan(nc):
    nk = nc // 8
    seq = [('fq', 0), ('fq', 1)]
    for p in range(NP):
        if 1 <= p < NP - 1:
            seq.append(('qx' if p + 1 in VQ else 'q', p + 1))
        for k in range(nk):
            if k == PVM_AFTER and p > 0 and MC[p - 1]:
                seq.append(('pvm', p - 1, nc - MC[p - 1], nc, False))
            seq.append(('qk', p, k))
        if p < 2:
            seq.append(('reload', p))
        seq.append(('sm', p))
    seq += [('pvm', NP - 1, c, c + 4, c > 0) for c in range(0, nc, 4)]
    last_pv = seq[-nc // 4]

    def tiles(it):
        if it[0] == 'pvm':
            return 3 * (it[3] - it[2])
        return dict(fq=15, q=15, wo=15, qk=24, sm=0, qx=0, reload=0)[it[0]]

    chains = [(p, g) for p in range(NP - 1) for g in range(PG)]
    blocks = []
    v0 = done = 0
    for b in range(len(V_END) + 1):
        final = b == len(V_END)
        v1 = len(chains) if final else V_END[b]
        todo = list(range(done, v0 // PG))
        done = v0 // PG
        budget = 10 ** 9 if final else TILES[b] - 15 * len(todo)
        body = []
        used = 0
        while seq and used + tiles(seq[0]) // 2 <= budget:
            body.append(seq.pop(0))
            used += tiles(body[-1])
        while body[-1][0] in ('sm', 'qx'):
            seq.insert(0, body.pop())
        assert b > 0 or not any(it[1] in VQ for it in body)
        keep = WO_KEEP if last_pv in body else 0
        items = [('red', p) for p in todo]
        used = 0
        nxt = WO_START[b]
        for it in body:
            if it == last_pv:
                while todo:
                    items.append(('wo', todo.pop(0)))
            if len(todo) > keep and used >= nxt:
                items.append(('wo', todo.pop(0)))
                nxt = used + WO_GAP[b]
            items.append(it)
            used += tiles(it)
        items += [('wo', p) for p in todo]
        if final:
            assert done == NP - 2
            for p in (NP - 1, NP - 2):
                items += [('red', p), ('wo', p)]
            blocks.append((chains[v0:v1], items, v1 - v0, 0, 0))
        else:
            blocks.append((chains[v0:v1], items, NLINK[b], FIRST[b], LAST_OFF[b]))
        v0 = v1
    seen = set()
    for b, (chs, items, n_link, _, _) in enumerate(blocks):
        assert all(it[1] - (NP - 2) < b for it in items if it[0] == 'qk')
        assert all(p in seen for p, _ in chs[:n_link])
        seen |= {it[1] for it in items if it[0] == 'sm'}
        assert all(p in seen for p, _ in chs)
        assert max(seen) - chs[-1][0] < PRING
    return blocks


def _make_kernel(n_tiles_total, nc):
    c0 = n_tiles_total - nc
    qscale = DH ** -0.5 * math.log2(math.e)
    prow = 2 * nc
    nk = nc // 8

    def kernel(x_hbm, k_hbm, v_hbm, wq_hbm, wo_hbm, w1_hbm, w3_hbm, w2_hbm,
               o_ref,
               kbuf, vbuf, wqbuf, wobuf, w1buf, w3buf, w2buf,
               vx_ref, t0_ref, lhs_ref, s_ref, p_ref, p2_ref, pk_ref, lsum_ref, om_ref,
               ob_ref, mask_ref, cs_ref, qpk_ref, xn_ref, y_ref, xbuf, sem):
        def halves(src, dst):
            return [(src(par), dst(pl.ds(8 * par, 8))) for par in range(2)]

        def whole(src, dst):
            return halves(lambda p: src.at[:, p], lambda h: dst.at[:, :, h, :])

        def kv_group(g):
            kr = pl.ds(g * GP * PG, GP * PG)
            vr = pl.ds(g * GP * PG // 4, GP * PG // 4)
            return (halves(lambda p: k_hbm.at[kr, p, pl.ds(c0, nc)],
                           lambda h: kbuf.at[kr, :, h, :])
                    + halves(lambda p: v_hbm.at[vr, p, :, pl.ds(c0, nc)],
                             lambda h: vbuf.at[vr, :, :, h, :]))

        def w2_group(i):
            rows = pl.ds(W2_SPLIT[i], W2_SPLIT[i + 1] - W2_SPLIT[i])
            return halves(lambda p: w2_hbm.at[rows, p], lambda h: w2buf.at[rows, :, h, :])

        groups = ([whole(wq_hbm, wqbuf) + [(x_hbm, xbuf)]]
                  + [kv_group(NGRP - 1 - g) for g in range(NGRP)]
                  + [halves(lambda p: wo_hbm.at[:, p], lambda h: wobuf.at[:, :, :, h, :]),
                     whole(w1_hbm, w1buf) + whole(w3_hbm, w3buf)]
                  + [w2_group(i) for i in range(len(W2_SPLIT) - 1)])
        marker = len(groups)
        groups.append([(x_hbm, xbuf)])
        n_ring = len(groups)
        def k_rows(i, rows):
            return halves(lambda p: k_hbm.at[rows((NP - 2 + i) * PG), p, pl.ds(c0, nc)],
                          lambda h: kbuf.at[rows(i * PG), :, h, :])

        for i, n in enumerate((PG, RELOAD_ROWS)):
            groups.append([cp for g in range(n) for cp in k_rows(i, lambda r0: r0 + g)])
        late = n_ring + 1 + NSEM
        groups += [[]] * (late - len(groups))
        groups.append(k_rows(1, lambda r0: pl.ds(r0 + RELOAD_ROWS, PG - RELOAD_ROWS)))

        def copies(i):
            return [pltpu.make_async_copy(src, dst, sem.at[i % NSEM])
                    for src, dst in groups[i]]

        def start_dma(i):
            for cp in copies(i):
                cp.start()

        def wait(i):
            for cp in copies(i):
                cp.wait()
            if i + NSEM < n_ring:
                start_dma(i + NSEM)

        for i in range(NSEM):
            start_dma(i)

        k32 = kbuf.bitcast(U32)
        v32 = vbuf.bitcast(U32)
        wq32 = wqbuf.bitcast(U32)
        wo32 = wobuf.bitcast(U32)
        w13 = (w1buf.bitcast(U32), w3buf.bitcast(U32))
        w232 = w2buf.bitcast(U32)

        sub = lax.broadcasted_iota(jnp.int32, (8, LANES), 0)
        lane = lax.broadcasted_iota(jnp.int32, (8, LANES), 1)
        sub3 = lax.broadcasted_iota(jnp.int32, (8, PW), 0)
        lane3 = lax.broadcasted_iota(jnp.int32, (8, PW), 1)

        for r in range(4):
            half = U32(0x0000FFFF if r % 2 == 0 else 0xFFFF0000)
            lo = jnp.where(sub == r // 2, half, U32(0))
            hi = jnp.where(sub == 2 + r // 2, half, U32(0))
            mask_ref[r] = lo
            mask_ref[4 + r] = jnp.where(lane < DH - LANES, lo, hi)
            mask_ref[8 + r] = hi
            mask_ref[12 + r] = lo | hi
        p_refs = (p_ref, p2_ref)
        for pr in p_refs:
            pr[...] = jnp.zeros(pr.shape, F32)

        def dot(l32, r, free=True):
            del free
            return jnp.dot(pltpu.bitcast(l32, BF), r, preferred_element_type=F32)

        def tile_of(v, kk):
            return v[:, kk * LANES:(kk + 1) * LANES]

        def ln_stats(x):
            xb = x.astype(BF).astype(F32)
            m = jnp.mean(xb, axis=-1, keepdims=True)
            xc = xb - m
            v = jnp.mean(xc * xc, axis=-1, keepdims=True)
            return xb, m, lax.rsqrt(v + EPS)

        def raw_proj(xb, w32, c, mm=dot):
            lhs = _pack2(xb, jnp.ones_like(xb))
            acc = None
            for kk in range(DT):
                acc = _add(acc, mm(tile_of(lhs, kk), _rhs(w32, 8 * kk, c), False))
            return acc[0:8], acc[8:16]

        def col_bcast(v):
            return jnp.concatenate([v] * (LANES // 8), axis=0).T

        def vpu_fma(acc, w, xlo, xhi):
            w = pltpu.bitcast(w, BF).astype(F32)
            return _add(acc, w[0:8] * xlo + w[8:16] * xhi)

        def sub_sum(a):
            return jnp.broadcast_to(jnp.sum(a, axis=0, keepdims=True), a.shape)

        def expand_q(p, t, q):
            for r in range(4):
                lhs_ref[p % RING, 4 * t + r] = q & mask_ref[4 * t + r]

        def stage_q(p, mm=dot):
            acc = [None] * 3
            for kk in range(DT):
                for t in range(3):
                    acc[t] = _add(acc[t], mm(xn_ref[:, pl.ds(kk * LANES, LANES)],
                                             _rhs(wq32, 8 * kk, 3 * p + t))[0:8])
            for t in range(3):
                q = acc[t] * qscale
                expand_q(p, t, _pack2(q, q))

        def stage_qk(p, k, krow, mm=dot, scale=None):
            for j in range(2 * k, 2 * k + 2):
                acc = None
                for t in range(3):
                    for r in range(4):
                        acc = _add(acc, mm(lhs_ref[p % RING, 4 * t + r],
                                           _rhs(k32, krow + 8 * t, 4 * j + r))[0:8])
                s_ref[p % RING, j] = acc if scale is None else acc * scale

        def head_reduce(v, op, lane_op):
            for d in (1, 2):
                up = pltpu.roll(v, d, 0)
                down = pltpu.roll(v, 8 - d, 0)
                v = op(v, jnp.where(sub % (2 * d) >= d, up, down))
            return lane_op(v, axis=1, keepdims=True)

        def softmax(p, j0):
            s = s_ref[p % RING]
            m = head_reduce(jnp.max(s, axis=0), jnp.maximum, jnp.max)
            e = jnp.exp2(s - m)
            l = jnp.sum(e, axis=0)
            l = jnp.broadcast_to(head_reduce(l, jnp.add, jnp.sum), l.shape)
            lsum_ref[p] = l
            for j in range(j0, nc // 4):
                pk_ref[p % RING, j] = _pack2(e[j], e[j])
            return e, l

        def v_idx(p, g, c):
            return p * (PG // 4) + g // 4, g % 4, c

        def widened(p):
            return XCOLS if p else XCOLS[:NVX]

        def vx_slot(p, g, e):
            return (NP - 2) * PG + 3 * p + g // 8, g % 8 * 4 + e - NVX

        def t_slot(p, j):
            if p == 0:
                return t0_ref, j
            row = (NP - 2) * PG if p == 1 else p * PG if p < NP - 2 else 2 * PG + 2
            return k32, (row + j // nc, j % nc)

        def pv_chain(p, g, gate, n=1):
            acc = [None] * (2 * n)
            for c in range(nc - MC[p]):
                row = (p % PRING) * prow + 8 * (c // 4) + 4 * (g // HG) + c % 4
                pb = gate()[pl.ds(row, 8, stride=0), :]
                for i in range(n):
                    w = v32[v_idx(p, g + i, c)]
                    if c in widened(p):
                        e = XCOLS.index(c)
                        w = (pltpu.bitcast(w, F32),
                             vx_ref[p, g + i, e] if e < NVX else
                             pltpu.bitcast(k32[vx_slot(p, g + i, e)], F32))
                    else:
                        w = pltpu.bitcast(w, BF).astype(F32)
                        w = (w[0:8], w[8:16])
                    for h in range(2):
                        acc[2 * i + h] = _add(acc[2 * i + h], w[h] * pb)
            for i in range(2 * n):
                ref, idx = t_slot(p, 2 * g + i)
                ref[idx] = pltpu.bitcast(acc[i], U32)
            return acc

        def pv_mxu(p, cols, transposed, mm=dot):
            acc = [None] * 3
            cols = list(cols)
            for i0 in range(0, len(cols), 4):
                ls = {c: pk_ref[p % RING, c // 4] & mask_ref[12 + c % 4]
                      for c in cols[i0:i0 + 4]}
                for t in range(3):
                    for c, l in ls.items():
                        tile = _rhs4(v32, 3 * p + t, c)
                        if transposed:
                            res = mm(l, tile)
                        else:
                            res = lax.dot_general(
                                pltpu.bitcast(l, BF), tile, (((1,), (1,)), ((), ())),
                                preferred_element_type=F32)
                        acc[t] = _add(acc[t], res[0:8])
            return jnp.concatenate(acc, axis=1)

        def own_head(o):
            return jnp.where((sub3 < 4) == (lane3 < DH), o, 0.0)

        def finish_o(p, o):
            linv = 1.0 / lsum_ref[p]
            la = jnp.broadcast_to(linv[0:1], linv.shape)
            lb = jnp.broadcast_to(linv[4:5], linv.shape)
            linv = jnp.concatenate([la, jnp.where(lane < DH - LANES, la, lb), lb], axis=1)
            o = jnp.sum(o, axis=0, keepdims=True) * linv
            ob_ref[p] = _pack2(o, o)

        def stage_reduce(p):
            o = None
            if p < NP - 1:
                slots = [t_slot(p, j) for j in range(2 * PG)]
                tt = pltpu.bitcast(jnp.concatenate([ref[idx] for ref, idx in slots]), F32)
                o = jnp.sum(tt.T.reshape(LANES // 8, 8, PW), axis=0)
            if p == NP - 1 or MC[p]:
                o = _add(o, own_head(om_ref[p]))
            finish_o(p, o)

        def stage_wo(p, mm=dot):
            for c in range(DT):
                acc = y_ref[:, pl.ds(c * LANES, LANES)]
                for t in range(3):
                    acc = acc + mm(ob_ref[p, :, pl.ds(t * LANES, LANES)],
                                   _rhs4(wo32, 3 * p + t, c))[0:8]
                y_ref[:, pl.ds(c * LANES, LANES)] = acc

        def begin_attention(x):
            y_ref[:, 0:D] = x
            xb, m, r = ln_stats(x)
            xn = (xb - m) * r
            xn_ref[:, 0:D] = _pack2(xn, xn)
            return xb, m, r

        wait(0)
        begin_attention(jnp.broadcast_to(xbuf[...].astype(F32), (8, D)))

        def pair1(i, carry):
            p = NP - 1 - i
            stage_q(p)
            for k in range(nk):
                stage_qk(p, k, p * PG)
            softmax(p, 0)
            finish_o(p, own_head(pv_mxu(p, range(nc), False)))
            om_ref[p] = jnp.zeros(om_ref.shape[1:], F32)
            qpk_ref[p] = jnp.zeros((8, LANES), U32)
            t0_ref[p] = jnp.zeros((8, LANES), U32)
            cs_ref[p] = jnp.zeros((8, LANES), F32)

            first = 0
            for pp in range(NP - 1):
                first = jnp.where(p == pp, nc - MC[pp], first)

            def transpose_v(c, carry2):
                for t in range(3):
                    tile = _rhs4(v32, 3 * p + t, c)
                    v32[pl.ds(2 * (3 * p + t), 2), :, c] = pltpu.bitcast(
                        tile.T, U32).reshape(2, 4, 8, LANES)
                return carry2

            lax.fori_loop(first, nc, transpose_v, 0)

            def widen(es):
                for g in range(PG):
                    for e in es:
                        idx = v_idx(p, g, XCOLS[e])
                        w = pltpu.bitcast(v32[idx], BF).astype(F32)
                        v32[idx] = pltpu.bitcast(w[0:8], U32)
                        if e < NVX:
                            vx_ref[p, g, e] = w[8:16]
                        else:
                            k32[vx_slot(p, g, e)] = pltpu.bitcast(w[8:16], U32)

            pl.when(p < NP - 1)(functools.partial(widen, range(NVX)))
            pl.when((p < NP - 1) & (p > 0))(
                functools.partial(widen, range(NVX, len(XCOLS))))
            return carry

        def group1(gi, row):
            for i in range(NGRP):
                pl.when(gi == i)(functools.partial(wait, 1 + i))
            lax.fori_loop(gi * GP, (gi + 1) * GP, pair1, 0)
            return row + PRING * prow // NGRP

        fence_row = pl.multiple_of(lax.fori_loop(0, NGRP, group1, 0), 8)
        wait(1 + NGRP)

        def woloop(p2, carry):
            stage_wo(2 * p2)
            stage_wo(2 * p2 + 1)
            return carry

        lax.fori_loop(0, NP // 2, woloop, 0)

        x = y_ref[:, 0:D]
        xb, m, r = ln_stats(x)
        wait(2 + NGRP)
        gu = []
        for j in range(2 * FT):
            raw, cs = raw_proj(xb, w13[j % 2], j // 2)
            cs_ref[j] = cs
            gu.append((raw - m * cs) * r)
        hs = [_swiglu(g, u) for g, u in zip(gu[0::2], gu[1::2])]
        for kk in range(W2_MXU // 8, FT):
            p_ref[pl.ds(LANES * kk - 16 * W2_MXU, LANES), :] = col_bcast(
                hs[kk].astype(BF).astype(F32))
        hs = [_pack2(hh, hh) for hh in hs[:W2_MXU // 8]]
        cols = [tile_of(x, c) for c in range(DT)]
        part = [None] * DT
        for i in range(len(W2_SPLIT) - 1):
            wait(3 + NGRP + i)
            g0, g1 = W2_SPLIT[i], W2_SPLIT[i + 1]
            for c in range(DT):
                if g1 <= W2_MXU:
                    for kk in range(g0 // 8, g1 // 8):
                        cols[c] = cols[c] + dot(hs[kk], _rhs(w232, 8 * kk, c))[0:8]
                else:
                    for g in range(g0, g1):
                        row = 16 * (g - W2_MXU)
                        part[c] = vpu_fma(part[c], w232[g, c], p_ref[pl.ds(row, 8), :],
                                          p_ref[pl.ds(row + 8, 8), :])
        x = jnp.concatenate([cc + sub_sum(a) for cc, a in zip(cols, part)], axis=1)

        xb, m, r = begin_attention(x)
        rq = r * qscale

        def run_block(blk, chains, items, n_link, first, last_off, start, end):
            links = []
            for j, (p, g) in enumerate(chains[:n_link]):
                dep = _bits_or(pv_chain(p, g, lambda: p_refs[g % 2]))
                links.extend([(LINK0[blk] + LINKSTEP[blk] * j, dep)] * LINK_REP[blk])
            if start:
                xcol = [col_bcast(tile_of(xb, kk)) - m[0:1] for kk in range(DT)]
                links.extend([(XC_LINK, _bits_or(xc[LANES - 8:] for xc in xcol))] * 4)
            pops = []
            probs = {}
            ready = {}
            busy = []

            def mm(l32, rr, free=True):
                links.sort(key=lambda lk: lk[0])
                if free and links and len(pops) >= links[0][0]:
                    l32 = jnp.where(sub < 4, l32, links.pop(0)[1])
                pops.append(dot(l32, rr))
                return pops[-1]

            for it in items:
                kind, p = it[0], it[1]
                if kind == 'fq':
                    for t in range(3):
                        raw, cs = raw_proj(xb, wq32, 3 * p + t, mm)
                        q = raw - m * cs
                        q = q if p == 0 else q * rq
                        expand_q(p, t, _pack2(q, q))
                elif kind == 'q':
                    stage_q(p, mm)
                    busy.append((len(pops) - Q_A[blk], len(pops) - Q_B[blk], Q_W[blk]))
                elif kind == 'qx':
                    for t in range(3):
                        expand_q(p, t, qpk_ref[3 * VQ.index(p) + t])
                elif kind == 'qk':
                    stage_qk(p, it[2], p % (NP - 2) * PG, mm, rq if p == 0 else None)
                    ready[p] = len(pops)
                elif kind == 'sm':
                    e, l = softmax(p, 0 if p == NP - 1 else (nc - MC[p]) // 4)
                    lag = SM_LAG0 if p == 0 else SM_LAG[blk]
                    pos = len(pops) + (lag if pops else lag - 14)
                    links.append((pos, pltpu.bitcast(l, U32)))
                    busy.append((pos - SM_A[blk], pos - SM_B[blk], SM_W[blk]))
                    if p < NP - 1:
                        probs[p] = e
                elif kind == 'pvm':
                    o = pv_mxu(p, range(it[2], it[3]), True, mm)
                    om_ref[p] = o + om_ref[p] if it[4] else o
                elif kind == 'reload':
                    start_dma(n_ring + p)
                elif kind == 'red':
                    stage_reduce(p)
                elif kind == 'wo':
                    busy.append((len(pops) - RED_A[blk], len(pops) - RED_B[blk], RED_W[blk]))
                    stage_wo(p, mm)

            def fence(buf, a):
                buf[pl.ds(fence_row, 8), :] = pops[a][0:8]

            if start:
                nkg = D // 16

                def xslot(kg):
                    u = kg // VQ_UNIT
                    return p_refs[u % 2], 16 * (u // 2 * VQ_UNIT + kg % VQ_UNIT)

                for kg in range(nkg):
                    buf, row = xslot(kg)
                    buf[pl.ds(row, 16), :] = xcol[kg // 8][16 * (kg % 8):16 * (kg % 8) + 16]
                for i, p in enumerate(VQ):
                    acc = [None] * 3
                    for kg in range(nkg):
                        buf, row = xslot(kg)
                        if kg % VQ_UNIT == 0:
                            a = (i * nkg + kg) * (first - VQ_FIRST) // (len(VQ) * nkg)
                            fence(buf, VQ_FIRST + a // 2 * 2)
                        xlo = buf[pl.ds(row, 8), :]
                        xhi = buf[pl.ds(row + 8, 8), :]
                        for t in range(3):
                            acc[t] = vpu_fma(acc[t], wq32[kg, 3 * p + t], xlo, xhi)
                    for t in range(3):
                        q = sub_sum(acc[t]) * rq
                        qpk_ref[3 * i + t] = _pack2(q, q)

            def store_probs(p):
                e = probs.pop(p)
                for pr in p_refs:
                    for j in range((nc - MC[p] + 3) // 4):
                        pr[pl.ds((p % PRING) * prow + 8 * j, 8), :] = e[j]

            rest = chains[n_link:]
            if rest:
                runs, i = [], 0
                while i < len(rest):
                    p, g = rest[i]
                    runs.append((p, g, min(GSHARE - g % GSHARE, len(rest) - i)))
                    i += runs[-1][2]
                cost = [n * (XCOST[blk] if c in widened(p) else 1.0)
                        for p, _, n in runs for c in range(nc - MC[p])]
                n_items = len(cost)
                n_units = (len(pops) - last_off - first) // FSTEP + 1
                less = [0.0] * n_units
                for lo, hi, w in busy:
                    us = [u for u in range(n_units) if lo <= first + u * FSTEP < hi]
                    for u in us:
                        less[u] += w / len(us)
                per = (sum(cost) + sum(less)) / n_units
                unit_of, total, used = [], 0.0, 0.0
                for u in range(n_units):
                    total += per - less[u]
                    while len(unit_of) < n_items and (
                            used + cost[len(unit_of)] / 2 < total or u + 1 == n_units):
                        used += cost[len(unit_of)]
                        unit_of.append(u)
                state = [0, -1, 1]

                def gate():
                    u = unit_of[state[0]]
                    state[0] += 1
                    if u != state[1]:
                        state[1] = u
                        state[2] += 1
                        fence(p_refs[state[2] % 2], first + u * FSTEP)
                    return p_refs[state[2] % 2]

            for p, g, n in runs if rest else []:
                if g == 0 and p in ready:
                    _LOG.append((p, first + state[1] * FSTEP - ready[p]))
                if g == 0:
                    for i in range(state[0], n_items):
                        if unit_of[i] != state[1] or state[1] + 1 == n_units:
                            break
                        unit_of[i] += 1
                if p in probs:
                    store_probs(p)
                pv_chain(p, g, gate, n)
            for p in list(probs):
                store_probs(p)
            if end:
                last_ffn(y_ref[:, 0:D], mm, len(pops), links)

        def last_ffn(x, mm, base, links):
            xb, m, r = ln_stats(x)
            lhs = _pack2(xb, xb)
            xcol = [col_bcast(tile_of(xb, kk)) for kk in range(UP_K)]
            links.extend([(base + UX_LINK, _bits_or(xc[LANES - 8:] for xc in xcol))] * 4)
            j0 = 2 * (FT - UP_COLS)
            part = {}
            for j in range(j0, 2 * FT):
                acc = None
                for kg in range(8 * UP_K):
                    xc = xcol[kg // 8][16 * (kg % 8):16 * (kg % 8) + 16]
                    acc = vpu_fma(acc, w13[j % 2][kg, j // 2], xc[0:8], xc[8:16])
                part[j] = sub_sum(acc)
                links.append((base + int(UP_LINK0 + UP_LINKSTEP * (j - j0)),
                              pltpu.bitcast(part[j], U32)))
            gu = []
            for j in range(2 * FT):
                acc = part.get(j)
                for kk in range(UP_K if j in part else 0, DT):
                    acc = _add(acc, mm(tile_of(lhs, kk),
                                       _rhs(w13[j % 2], 8 * kk, j // 2))[0:8])
                gu.append((acc - m * cs_ref[j]) * r)
            hs = [_swiglu(g, u) for g, u in zip(gu[0::2], gu[1::2])]
            cols = [tile_of(x, c) for c in range(DT)]
            for kk in range(DOWN_K, FT):
                hh = _pack2(hs[kk], hs[kk])
                for c in range(DT):
                    cols[c] = cols[c] + mm(hh, _rhs(w232, 8 * kk, c))[0:8]
            acc = [None] * DT
            for kk in range(DOWN_K):
                hcol = col_bcast(hs[kk].astype(BF).astype(F32))
                for i in range(8):
                    for c in range(DT):
                        acc[c] = vpu_fma(acc[c], w232[8 * kk + i, c],
                                         hcol[16 * i:16 * i + 8],
                                         hcol[16 * i + 8:16 * i + 16])
            cols = [cc + sub_sum(a) for cc, a in zip(cols, acc)]
            o_ref[...] = jnp.concatenate(cols, axis=1)[0:1].astype(o_ref.dtype)

        blocks = _plan(nc)
        for b, plan in enumerate(blocks):
            end = b == len(blocks) - 1
            if b > 0:
                wait(marker if end else n_ring + b - 1)
            if b == 1:
                start_dma(late)
            if b == 2:
                wait(late)
            if ONLY is not None and b not in ONLY and not end:
                if b == 0:
                    start_dma(n_ring)
                    start_dma(n_ring + 1)
                if b < 2:
                    expand_q(0, 0, _bits_or(qpk_ref[pp] for pp in range(NP - 1)))
                    for pp in range(2):
                        stage_reduce(pp)
                continue
            run_block(b, *plan, b == 0, end)

    return kernel


@jax.jit
def pallas_interleave_layers__sliding_block_cached__glu_gated_swiglu__decode_kernel(
    A_x: jax.Array,
    A_k_cache: jax.Array,
    A_v_cache: jax.Array,
    A_wq: jax.Array,
    A_wo: jax.Array,
    B_x: jax.Array,
    B_w1: jax.Array,
    B_w3: jax.Array,
    B_w2: jax.Array,
):
    sk = A_k_cache.shape[2]
    win = min(4096, max(256, sk // 4))
    nt_total, nc = sk // LANES, win // LANES

    def kv_view(a):
        return _tile_view(jnp.swapaxes(a, 2, 3).reshape(H * DH, sk))

    def view4(t):
        return t.reshape(t.shape[0] // 4, 2, 4, t.shape[2], 8, LANES)

    def wbuf(r, c):
        return pltpu.VMEM((r // 16, c // LANES, 16, LANES), BF)

    def wbuf4(r, c):
        return pltpu.VMEM((r // 64, 4, c // LANES, 16, LANES), BF)

    any_spec = pl.BlockSpec(memory_space=pl.ANY)
    out = pl.pallas_call(
        _make_kernel(nt_total, nc),
        out_shape=jax.ShapeDtypeStruct((1, D), A_x.dtype),
        in_specs=[any_spec] * 8,
        out_specs=pl.BlockSpec(memory_space=pltpu.VMEM),
        scratch_shapes=[
            wbuf(H * DH, win), wbuf4(H * DH, win),
            wbuf(D, H * DH), wbuf4(H * DH, D),
            wbuf(D, F), wbuf(D, F), wbuf(F, D),
            pltpu.VMEM((NP - 1, PG, NVX, 8, LANES), F32),
            pltpu.VMEM((2 * PG, 8, LANES), U32),
            pltpu.VMEM((RING, 12, 8, LANES), U32),
            pltpu.VMEM((RING, nc // 4, 8, LANES), F32),
            pltpu.VMEM((PRING * 2 * nc + 32, LANES), F32),
            pltpu.VMEM((PRING * 2 * nc + 32, LANES), F32),
            pltpu.VMEM((RING, nc // 4, 8, LANES), U32),
            pltpu.VMEM((NP, 8, LANES), F32),
            pltpu.VMEM((NP, 8, PW), F32),
            pltpu.VMEM((NP, 8, PW), U32),
            pltpu.VMEM((16, 8, LANES), U32),
            pltpu.VMEM((2 * FT, 8, LANES), F32),
            pltpu.VMEM((16, 8, LANES), U32),
            pltpu.VMEM((8, 1024), U32),
            pltpu.VMEM((8, 1024), F32),
            pltpu.VMEM((1, D), BF),
            pltpu.SemaphoreType.DMA((NSEM,)),
        ],
        compiler_params=pltpu.CompilerParams(
            vmem_limit_bytes=128 * 1024 * 1024),
    )(A_x.reshape(1, D), kv_view(A_k_cache), view4(kv_view(A_v_cache)),
      _tile_view(A_wq), view4(_tile_view(A_wo)),
      _tile_view(B_w1), _tile_view(B_w3), _tile_view(B_w2))
    return out.reshape(A_x.shape)
```

```python
import functools
import math

import jax
import jax.numpy as jnp
from jax import lax
import jax.experimental.pallas as pl
import jax.experimental.pallas.tpu as pltpu

D = 640
H = 32
DH = 192
F = 1536
LANES = 128
EPS = 1e-5

NP = H // 2
PG = 2 * DH // 16
HG = DH // 16
PW = 2 * DH
DT = D // LANES
FT = F // LANES

GP = 4
NGRP = NP // GP
W2_SPLIT = (0, 56, 80, 92, 96)
W2_MXU = 80
RELOAD_ROWS = 8
NSEM = 3
RING = 4
PRING = 6

MC = (2, 2, 2, 2, 2, 2, 2, 2, 2, 2, 2, 2, 2, 2, 2)
XCOLS = (1, 7, 10, 16, 22, 25, 4, 13, 19, 28)
NVX = 6
VQ = (11, 12, 13, 14, 15)
V_END = (172, 297, 352)
TILES = (1060, 655, 290)
XCOST = (0.67, 0.77, 0.77, 0.67)
GSHARE = 2
PVM_AFTER = 2
WO_START = (0, 80, 65, 999)
WO_GAP = (0, 72, 60, 12)
WO_KEEP = 3
FSTEP = 2
FIRST = (160, 2, 0)
LAST_OFF = (8, 6, 6)
VQ_FIRST = 30
VQ_UNIT = 4
XC_LINK = 50
SM_LAG = (60, 64, 64, 64)
SM_LAG0 = 52
RED_W = (10, 10, 10, 10)
RED_A = (40, 40, 40, 40)
RED_B = (16, 20, 20, 16)
Q_W = (4, 4, 4, 4)
Q_A = (18, 12, 12, 12)
Q_B = (-4, -4, -4, -4)
SM_W = (4, 4, 7, 7)
SM_A = (56, 56, 56, 56)
SM_B = (30, 42, 30, 30)
NLINK = (0, 4, 3)
LINK0 = (8, 8, 8, 10)
LINKSTEP = (4, 5, 4, 6.0)
LINK_REP = (1, 1, 4, 4)
UP_K = 3
UP_COLS = 6
UP_LINK0 = 54
UP_LINKSTEP = 4.75
UX_LINK = 44
DOWN_K = 3

U32 = jnp.uint32
BF = jnp.bfloat16
F32 = jnp.float32


def _tile_view(w):
    r, c = w.shape
    return jnp.swapaxes(w.reshape(r // 16, 2, 8, c // LANES, LANES), 2, 3)


def _rhs(w32, g0, c):
    return pltpu.bitcast(w32[pl.ds(g0, 8), c].reshape(64, LANES), BF)


def _rhs4(w32, tile, c):
    return pltpu.bitcast(w32[pl.ds(2 * tile, 2), :, c].reshape(64, LANES), BF)


def _swiglu(g, u):
    hg = 0.5 * g
    return hg * (1.0 + jnp.tanh(hg)) * u


def _pack2(lo, hi):
    return pltpu.bitcast(jnp.concatenate([lo, hi], axis=0).astype(BF), U32)


def _add(a, b):
    return b if a is None else a + b


def _bits_or(vals):
    return functools.reduce(lambda a, b: a | b, [pltpu.bitcast(v, U32) for v in vals])


def _plan(nc):
    nk = nc // 8
    seq = [('fq', 0), ('fq', 1)]
    for p in range(NP):
        if 1 <= p < NP - 1:
            seq.append(('qx' if p + 1 in VQ else 'q', p + 1))
        for k in range(nk):
            if k == PVM_AFTER and p > 0 and MC[p - 1]:
                seq.append(('pvm', p - 1, nc - MC[p - 1], nc, False))
            seq.append(('qk', p, k))
        if p < 2:
            seq.append(('reload', p))
        seq.append(('sm', p))
    seq += [('pvm', NP - 1, c, c + 4, c > 0) for c in range(0, nc, 4)]
    last_pv = seq[-nc // 4]

    def tiles(it):
        if it[0] == 'pvm':
            return 3 * (it[3] - it[2])
        return dict(fq=15, q=15, wo=15, qk=24, sm=0, qx=0, reload=0)[it[0]]

    chains = [(p, g) for p in range(NP - 1) for g in range(PG)]
    blocks = []
    v0 = done = 0
    for b in range(len(V_END) + 1):
        final = b == len(V_END)
        v1 = len(chains) if final else V_END[b]
        todo = list(range(done, v0 // PG))
        done = v0 // PG
        budget = 10 ** 9 if final else TILES[b] - 15 * len(todo)
        body = []
        used = 0
        while seq and used + tiles(seq[0]) // 2 <= budget:
            body.append(seq.pop(0))
            used += tiles(body[-1])
        while body[-1][0] in ('sm', 'qx'):
            seq.insert(0, body.pop())
        assert b > 0 or not any(it[1] in VQ for it in body)
        keep = WO_KEEP if last_pv in body else 0
        items = [('red', p) for p in todo]
        used = 0
        nxt = WO_START[b]
        for it in body:
            if it == last_pv:
                while todo:
                    items.append(('wo', todo.pop(0)))
            if len(todo) > keep and used >= nxt:
                items.append(('wo', todo.pop(0)))
                nxt = used + WO_GAP[b]
            items.append(it)
            used += tiles(it)
        items += [('wo', p) for p in todo]
        if final:
            assert done == NP - 2
            for p in (NP - 1, NP - 2):
                items += [('red', p), ('wo', p)]
            blocks.append((chains[v0:v1], items, v1 - v0, 0, 0))
        else:
            blocks.append((chains[v0:v1], items, NLINK[b], FIRST[b], LAST_OFF[b]))
        v0 = v1
    seen = set()
    for b, (chs, items, n_link, _, _) in enumerate(blocks):
        assert all(it[1] - (NP - 2) < b for it in items if it[0] == 'qk')
        assert all(p in seen for p, _ in chs[:n_link])
        seen |= {it[1] for it in items if it[0] == 'sm'}
        assert all(p in seen for p, _ in chs)
        assert max(seen) - chs[-1][0] < PRING
    return blocks


def _make_kernel(n_tiles_total, nc):
    c0 = n_tiles_total - nc
    qscale = DH ** -0.5 * math.log2(math.e)
    prow = 2 * nc
    nk = nc // 8

    def kernel(x_hbm, k_hbm, v_hbm, wq_hbm, wo_hbm, w1_hbm, w3_hbm, w2_hbm,
               o_ref,
               kbuf, vbuf, wqbuf, wobuf, w1buf, w3buf, w2buf,
               vx_ref, t0_ref, lhs_ref, s_ref, p_ref, p2_ref, pk_ref, lsum_ref, om_ref,
               ob_ref, mask_ref, cs_ref, qpk_ref, xn_ref, y_ref, xbuf, sem):
        def halves(src, dst):
            return [(src(par), dst(pl.ds(8 * par, 8))) for par in range(2)]

        def whole(src, dst):
            return halves(lambda p: src.at[:, p], lambda h: dst.at[:, :, h, :])

        def kv_group(g):
            kr = pl.ds(g * GP * PG, GP * PG)
            vr = pl.ds(g * GP * PG // 4, GP * PG // 4)
            return (halves(lambda p: k_hbm.at[kr, p, pl.ds(c0, nc)],
                           lambda h: kbuf.at[kr, :, h, :])
                    + halves(lambda p: v_hbm.at[vr, p, :, pl.ds(c0, nc)],
                             lambda h: vbuf.at[vr, :, :, h, :]))

        def w2_group(i):
            rows = pl.ds(W2_SPLIT[i], W2_SPLIT[i + 1] - W2_SPLIT[i])
            return halves(lambda p: w2_hbm.at[rows, p], lambda h: w2buf.at[rows, :, h, :])

        groups = ([whole(wq_hbm, wqbuf) + [(x_hbm, xbuf)]]
                  + [kv_group(NGRP - 1 - g) for g in range(NGRP)]
                  + [halves(lambda p: wo_hbm.at[:, p], lambda h: wobuf.at[:, :, :, h, :]),
                     whole(w1_hbm, w1buf) + whole(w3_hbm, w3buf)]
                  + [w2_group(i) for i in range(len(W2_SPLIT) - 1)])
        marker = len(groups)
        groups.append([(x_hbm, xbuf)])
        n_ring = len(groups)
        def k_rows(i, rows):
            return halves(lambda p: k_hbm.at[rows((NP - 2 + i) * PG), p, pl.ds(c0, nc)],
                          lambda h: kbuf.at[rows(i * PG), :, h, :])

        for i, n in enumerate((PG, RELOAD_ROWS)):
            groups.append([cp for g in range(n) for cp in k_rows(i, lambda r0: r0 + g)])
        late = n_ring + 1 + NSEM
        groups += [[]] * (late - len(groups))
        groups.append(k_rows(1, lambda r0: pl.ds(r0 + RELOAD_ROWS, PG - RELOAD_ROWS)))

        def copies(i):
            return [pltpu.make_async_copy(src, dst, sem.at[i % NSEM])
                    for src, dst in groups[i]]

        def start_dma(i):
            for cp in copies(i):
                cp.start()

        def wait(i):
            for cp in copies(i):
                cp.wait()
            if i + NSEM < n_ring:
                start_dma(i + NSEM)

        for i in range(NSEM):
            start_dma(i)

        k32 = kbuf.bitcast(U32)
        v32 = vbuf.bitcast(U32)
        wq32 = wqbuf.bitcast(U32)
        wo32 = wobuf.bitcast(U32)
        w13 = (w1buf.bitcast(U32), w3buf.bitcast(U32))
        w232 = w2buf.bitcast(U32)

        sub = lax.broadcasted_iota(jnp.int32, (8, LANES), 0)
        lane = lax.broadcasted_iota(jnp.int32, (8, LANES), 1)
        sub3 = lax.broadcasted_iota(jnp.int32, (8, PW), 0)
        lane3 = lax.broadcasted_iota(jnp.int32, (8, PW), 1)

        for r in range(4):
            half = U32(0x0000FFFF if r % 2 == 0 else 0xFFFF0000)
            lo = jnp.where(sub == r // 2, half, U32(0))
            hi = jnp.where(sub == 2 + r // 2, half, U32(0))
            mask_ref[r] = lo
            mask_ref[4 + r] = jnp.where(lane < DH - LANES, lo, hi)
            mask_ref[8 + r] = hi
            mask_ref[12 + r] = lo | hi
        p_refs = (p_ref, p2_ref)
        for pr in p_refs:
            pr[...] = jnp.zeros(pr.shape, F32)

        def dot(l32, r, free=True):
            del free
            return jnp.dot(pltpu.bitcast(l32, BF), r, preferred_element_type=F32)

        def tile_of(v, kk):
            return v[:, kk * LANES:(kk + 1) * LANES]

        def ln_stats(x):
            xb = x.astype(BF).astype(F32)
            m = jnp.mean(xb, axis=-1, keepdims=True)
            xc = xb - m
            v = jnp.mean(xc * xc, axis=-1, keepdims=True)
            return xb, m, lax.rsqrt(v + EPS)

        def raw_proj(xb, w32, c, mm=dot):
            lhs = _pack2(xb, jnp.ones_like(xb))
            acc = None
            for kk in range(DT):
                acc = _add(acc, mm(tile_of(lhs, kk), _rhs(w32, 8 * kk, c), False))
            return acc[0:8], acc[8:16]

        def col_bcast(v):
            return jnp.concatenate([v] * (LANES // 8), axis=0).T

        def vpu_fma(acc, w, xlo, xhi):
            w = pltpu.bitcast(w, BF).astype(F32)
            return _add(acc, w[0:8] * xlo + w[8:16] * xhi)

        def sub_sum(a):
            return jnp.broadcast_to(jnp.sum(a, axis=0, keepdims=True), a.shape)

        def expand_q(p, t, q):
            for r in range(4):
                lhs_ref[p % RING, 4 * t + r] = q & mask_ref[4 * t + r]

        def stage_q(p, mm=dot):
            acc = [None] * 3
            for kk in range(DT):
                for t in range(3):
                    acc[t] = _add(acc[t], mm(xn_ref[:, pl.ds(kk * LANES, LANES)],
                                             _rhs(wq32, 8 * kk, 3 * p + t))[0:8])
            for t in range(3):
                q = acc[t] * qscale
                expand_q(p, t, _pack2(q, q))

        def stage_qk(p, k, krow, mm=dot, scale=None):
            for j in range(2 * k, 2 * k + 2):
                acc = None
                for t in range(3):
                    for r in range(4):
                        acc = _add(acc, mm(lhs_ref[p % RING, 4 * t + r],
                                           _rhs(k32, krow + 8 * t, 4 * j + r))[0:8])
                s_ref[p % RING, j] = acc if scale is None else acc * scale

        def head_reduce(v, op, lane_op):
            for d in (1, 2):
                up = pltpu.roll(v, d, 0)
                down = pltpu.roll(v, 8 - d, 0)
                v = op(v, jnp.where(sub % (2 * d) >= d, up, down))
            return lane_op(v, axis=1, keepdims=True)

        def softmax(p, j0):
            s = s_ref[p % RING]
            m = head_reduce(jnp.max(s, axis=0), jnp.maximum, jnp.max)
            e = jnp.exp2(s - m)
            l = jnp.sum(e, axis=0)
            l = jnp.broadcast_to(head_reduce(l, jnp.add, jnp.sum), l.shape)
            lsum_ref[p] = l
            for j in range(j0, nc // 4):
                pk_ref[p % RING, j] = _pack2(e[j], e[j])
            return e, l

        def v_idx(p, g, c):
            return p * (PG // 4) + g // 4, g % 4, c

        def widened(p):
            return XCOLS if p else XCOLS[:NVX]

        def vx_slot(p, g, e):
            return (NP - 2) * PG + 3 * p + g // 8, g % 8 * 4 + e - NVX

        def t_slot(p, j):
            if p == 0:
                return t0_ref, j
            row = (NP - 2) * PG if p == 1 else p * PG if p < NP - 2 else 2 * PG + 2
            return k32, (row + j // nc, j % nc)

        def pv_chain(p, g, gate, n=1):
            acc = [None] * (2 * n)
            for c in range(nc - MC[p]):
                row = (p % PRING) * prow + 8 * (c // 4) + 4 * (g // HG) + c % 4
                pb = gate()[pl.ds(row, 8, stride=0), :]
                for i in range(n):
                    w = v32[v_idx(p, g + i, c)]
                    if c in widened(p):
                        e = XCOLS.index(c)
                        w = (pltpu.bitcast(w, F32),
                             vx_ref[p, g + i, e] if e < NVX else
                             pltpu.bitcast(k32[vx_slot(p, g + i, e)], F32))
                    else:
                        w = pltpu.bitcast(w, BF).astype(F32)
                        w = (w[0:8], w[8:16])
                    for h in range(2):
                        acc[2 * i + h] = _add(acc[2 * i + h], w[h] * pb)
            for i in range(2 * n):
                ref, idx = t_slot(p, 2 * g + i)
                ref[idx] = pltpu.bitcast(acc[i], U32)
            return acc

        def pv_mxu(p, cols, transposed, mm=dot):
            acc = [None] * 3
            cols = list(cols)
            for i0 in range(0, len(cols), 4):
                ls = {c: pk_ref[p % RING, c // 4] & mask_ref[12 + c % 4]
                      for c in cols[i0:i0 + 4]}
                for t in range(3):
                    for c, l in ls.items():
                        tile = _rhs4(v32, 3 * p + t, c)
                        if transposed:
                            res = mm(l, tile)
                        else:
                            res = lax.dot_general(
                                pltpu.bitcast(l, BF), tile, (((1,), (1,)), ((), ())),
                                preferred_element_type=F32)
                        acc[t] = _add(acc[t], res[0:8])
            return jnp.concatenate(acc, axis=1)

        def own_head(o):
            return jnp.where((sub3 < 4) == (lane3 < DH), o, 0.0)

        def finish_o(p, o):
            linv = 1.0 / lsum_ref[p]
            la = jnp.broadcast_to(linv[0:1], linv.shape)
            lb = jnp.broadcast_to(linv[4:5], linv.shape)
            linv = jnp.concatenate([la, jnp.where(lane < DH - LANES, la, lb), lb], axis=1)
            o = jnp.sum(o, axis=0, keepdims=True) * linv
            ob_ref[p] = _pack2(o, o)

        def stage_reduce(p):
            o = None
            if p < NP - 1:
                slots = [t_slot(p, j) for j in range(2 * PG)]
                tt = pltpu.bitcast(jnp.concatenate([ref[idx] for ref, idx in slots]), F32)
                o = jnp.sum(tt.T.reshape(LANES // 8, 8, PW), axis=0)
            if p == NP - 1 or MC[p]:
                o = _add(o, own_head(om_ref[p]))
            finish_o(p, o)

        def stage_wo(p, mm=dot):
            for c in range(DT):
                acc = y_ref[:, pl.ds(c * LANES, LANES)]
                for t in range(3):
                    acc = acc + mm(ob_ref[p, :, pl.ds(t * LANES, LANES)],
                                   _rhs4(wo32, 3 * p + t, c))[0:8]
                y_ref[:, pl.ds(c * LANES, LANES)] = acc

        def begin_attention(x):
            y_ref[:, 0:D] = x
            xb, m, r = ln_stats(x)
            xn = (xb - m) * r
            xn_ref[:, 0:D] = _pack2(xn, xn)
            return xb, m, r

        wait(0)
        begin_attention(jnp.broadcast_to(xbuf[...].astype(F32), (8, D)))

        def pair1(i, carry):
            p = NP - 1 - i
            stage_q(p)
            for k in range(nk):
                stage_qk(p, k, p * PG)
            softmax(p, 0)
            finish_o(p, own_head(pv_mxu(p, range(nc), False)))
            om_ref[p] = jnp.zeros(om_ref.shape[1:], F32)
            qpk_ref[p] = jnp.zeros((8, LANES), U32)
            t0_ref[p] = jnp.zeros((8, LANES), U32)
            cs_ref[p] = jnp.zeros((8, LANES), F32)

            first = 0
            for pp in range(NP - 1):
                first = jnp.where(p == pp, nc - MC[pp], first)

            def transpose_v(c, carry2):
                for t in range(3):
                    tile = _rhs4(v32, 3 * p + t, c)
                    v32[pl.ds(2 * (3 * p + t), 2), :, c] = pltpu.bitcast(
                        tile.T, U32).reshape(2, 4, 8, LANES)
                return carry2

            lax.fori_loop(first, nc, transpose_v, 0)

            def widen(es):
                for g in range(PG):
                    for e in es:
                        idx = v_idx(p, g, XCOLS[e])
                        w = pltpu.bitcast(v32[idx], BF).astype(F32)
                        v32[idx] = pltpu.bitcast(w[0:8], U32)
                        if e < NVX:
                            vx_ref[p, g, e] = w[8:16]
                        else:
                            k32[vx_slot(p, g, e)] = pltpu.bitcast(w[8:16], U32)

            pl.when(p < NP - 1)(functools.partial(widen, range(NVX)))
            pl.when((p < NP - 1) & (p > 0))(
                functools.partial(widen, range(NVX, len(XCOLS))))
            return carry

        def group1(gi, row):
            for i in range(NGRP):
                pl.when(gi == i)(functools.partial(wait, 1 + i))
            lax.fori_loop(gi * GP, (gi + 1) * GP, pair1, 0)
            return row + PRING * prow // NGRP

        fence_row = pl.multiple_of(lax.fori_loop(0, NGRP, group1, 0), 8)
        wait(1 + NGRP)

        def woloop(p2, carry):
            stage_wo(2 * p2)
            stage_wo(2 * p2 + 1)
            return carry

        lax.fori_loop(0, NP // 2, woloop, 0)

        x = y_ref[:, 0:D]
        xb, m, r = ln_stats(x)
        wait(2 + NGRP)
        gu = []
        for j in range(2 * FT):
            raw, cs = raw_proj(xb, w13[j % 2], j // 2)
            cs_ref[j] = cs
            gu.append((raw - m * cs) * r)
        hs = [_swiglu(g, u) for g, u in zip(gu[0::2], gu[1::2])]
        for kk in range(W2_MXU // 8, FT):
            p_ref[pl.ds(LANES * kk - 16 * W2_MXU, LANES), :] = col_bcast(
                hs[kk].astype(BF).astype(F32))
        hs = [_pack2(hh, hh) for hh in hs[:W2_MXU // 8]]
        cols = [tile_of(x, c) for c in range(DT)]
        part = [None] * DT
        for i in range(len(W2_SPLIT) - 1):
            wait(3 + NGRP + i)
            g0, g1 = W2_SPLIT[i], W2_SPLIT[i + 1]
            for c in range(DT):
                if g1 <= W2_MXU:
                    for kk in range(g0 // 8, g1 // 8):
                        cols[c] = cols[c] + dot(hs[kk], _rhs(w232, 8 * kk, c))[0:8]
                else:
                    for g in range(g0, g1):
                        row = 16 * (g - W2_MXU)
                        part[c] = vpu_fma(part[c], w232[g, c], p_ref[pl.ds(row, 8), :],
                                          p_ref[pl.ds(row + 8, 8), :])
        x = jnp.concatenate([cc + sub_sum(a) for cc, a in zip(cols, part)], axis=1)

        xb, m, r = begin_attention(x)
        rq = r * qscale

        def run_block(blk, chains, items, n_link, first, last_off, start, end):
            links = []
            for j, (p, g) in enumerate(chains[:n_link]):
                dep = _bits_or(pv_chain(p, g, lambda: p_refs[g % 2]))
                links.extend([(LINK0[blk] + LINKSTEP[blk] * j, dep)] * LINK_REP[blk])
            if start:
                xcol = [col_bcast(tile_of(xb, kk)) - m[0:1] for kk in range(DT)]
                links.extend([(XC_LINK, _bits_or(xc[LANES - 8:] for xc in xcol))] * 4)
            pops = []
            probs = {}
            busy = []

            def mm(l32, rr, free=True):
                links.sort(key=lambda lk: lk[0])
                if free and links and len(pops) >= links[0][0]:
                    l32 = jnp.where(sub < 4, l32, links.pop(0)[1])
                pops.append(dot(l32, rr))
                return pops[-1]

            for it in items:
                kind, p = it[0], it[1]
                if kind == 'fq':
                    for t in range(3):
                        raw, cs = raw_proj(xb, wq32, 3 * p + t, mm)
                        q = raw - m * cs
                        q = q if p == 0 else q * rq
                        expand_q(p, t, _pack2(q, q))
                elif kind == 'q':
                    stage_q(p, mm)
                    busy.append((len(pops) - Q_A[blk], len(pops) - Q_B[blk], Q_W[blk]))
                elif kind == 'qx':
                    for t in range(3):
                        expand_q(p, t, qpk_ref[3 * VQ.index(p) + t])
                elif kind == 'qk':
                    stage_qk(p, it[2], p % (NP - 2) * PG, mm, rq if p == 0 else None)
                elif kind == 'sm':
                    e, l = softmax(p, 0 if p == NP - 1 else (nc - MC[p]) // 4)
                    lag = SM_LAG0 if p == 0 else SM_LAG[blk]
                    pos = len(pops) + (lag if pops else lag - 14)
                    links.append((pos, pltpu.bitcast(l, U32)))
                    busy.append((pos - SM_A[blk], pos - SM_B[blk], SM_W[blk]))
                    if p < NP - 1:
                        probs[p] = e
                elif kind == 'pvm':
                    o = pv_mxu(p, range(it[2], it[3]), True, mm)
                    om_ref[p] = o + om_ref[p] if it[4] else o
                elif kind == 'reload':
                    start_dma(n_ring + p)
                elif kind == 'red':
                    stage_reduce(p)
                elif kind == 'wo':
                    busy.append((len(pops) - RED_A[blk], len(pops) - RED_B[blk], RED_W[blk]))
                    stage_wo(p, mm)

            def fence(buf, a):
                buf[pl.ds(fence_row, 8), :] = pops[a][0:8]

            if start:
                nkg = D // 16

                def xslot(kg):
                    u = kg // VQ_UNIT
                    return p_refs[u % 2], 16 * (u // 2 * VQ_UNIT + kg % VQ_UNIT)

                for kg in range(nkg):
                    buf, row = xslot(kg)
                    buf[pl.ds(row, 16), :] = xcol[kg // 8][16 * (kg % 8):16 * (kg % 8) + 16]
                for i, p in enumerate(VQ):
                    acc = [None] * 3
                    for kg in range(nkg):
                        buf, row = xslot(kg)
                        if kg % VQ_UNIT == 0:
                            a = (i * nkg + kg) * (first - VQ_FIRST) // (len(VQ) * nkg)
                            fence(buf, VQ_FIRST + a // 2 * 2)
                        xlo = buf[pl.ds(row, 8), :]
                        xhi = buf[pl.ds(row + 8, 8), :]
                        for t in range(3):
                            acc[t] = vpu_fma(acc[t], wq32[kg, 3 * p + t], xlo, xhi)
                    for t in range(3):
                        q = sub_sum(acc[t]) * rq
                        qpk_ref[3 * i + t] = _pack2(q, q)

            def store_probs(p):
                e = probs.pop(p)
                for pr in p_refs:
                    for j in range((nc - MC[p] + 3) // 4):
                        pr[pl.ds((p % PRING) * prow + 8 * j, 8), :] = e[j]

            rest = chains[n_link:]
            if rest:
                runs, i = [], 0
                while i < len(rest):
                    p, g = rest[i]
                    runs.append((p, g, min(GSHARE - g % GSHARE, len(rest) - i)))
                    i += runs[-1][2]
                cost = [n * (XCOST[blk] if c in widened(p) else 1.0)
                        for p, _, n in runs for c in range(nc - MC[p])]
                n_items = len(cost)
                n_units = (len(pops) - last_off - first) // FSTEP + 1
                less = [0.0] * n_units
                for lo, hi, w in busy:
                    us = [u for u in range(n_units) if lo <= first + u * FSTEP < hi]
                    for u in us:
                        less[u] += w / len(us)
                per = (sum(cost) + sum(less)) / n_units
                unit_of, total, used = [], 0.0, 0.0
                for u in range(n_units):
                    total += per - less[u]
                    while len(unit_of) < n_items and (
                            used + cost[len(unit_of)] / 2 < total or u + 1 == n_units):
                        used += cost[len(unit_of)]
                        unit_of.append(u)
                state = [0, -1, 1]

                def gate():
                    u = unit_of[state[0]]
                    state[0] += 1
                    if u != state[1]:
                        state[1] = u
                        state[2] += 1
                        fence(p_refs[state[2] % 2], first + u * FSTEP)
                    return p_refs[state[2] % 2]

            for p, g, n in runs if rest else []:
                if g == 0:
                    for i in range(state[0], n_items):
                        if unit_of[i] != state[1] or state[1] + 1 == n_units:
                            break
                        unit_of[i] += 1
                if p in probs:
                    store_probs(p)
                pv_chain(p, g, gate, n)
            for p in list(probs):
                store_probs(p)
            if end:
                last_ffn(y_ref[:, 0:D], mm, len(pops), links)

        def last_ffn(x, mm, base, links):
            xb, m, r = ln_stats(x)
            lhs = _pack2(xb, xb)
            xcol = [col_bcast(tile_of(xb, kk)) for kk in range(UP_K)]
            links.extend([(base + UX_LINK, _bits_or(xc[LANES - 8:] for xc in xcol))] * 4)
            j0 = 2 * (FT - UP_COLS)
            part = {}
            for j in range(j0, 2 * FT):
                acc = None
                for kg in range(8 * UP_K):
                    xc = xcol[kg // 8][16 * (kg % 8):16 * (kg % 8) + 16]
                    acc = vpu_fma(acc, w13[j % 2][kg, j // 2], xc[0:8], xc[8:16])
                part[j] = sub_sum(acc)
                links.append((base + int(UP_LINK0 + UP_LINKSTEP * (j - j0)),
                              pltpu.bitcast(part[j], U32)))
            gu = []
            for j in range(2 * FT):
                acc = part.get(j)
                for kk in range(UP_K if j in part else 0, DT):
                    acc = _add(acc, mm(tile_of(lhs, kk),
                                       _rhs(w13[j % 2], 8 * kk, j // 2))[0:8])
                gu.append((acc - m * cs_ref[j]) * r)
            hs = [_swiglu(g, u) for g, u in zip(gu[0::2], gu[1::2])]
            cols = [tile_of(x, c) for c in range(DT)]
            for kk in range(DOWN_K, FT):
                hh = _pack2(hs[kk], hs[kk])
                for c in range(DT):
                    cols[c] = cols[c] + mm(hh, _rhs(w232, 8 * kk, c))[0:8]
            acc = [None] * DT
            for kk in range(DOWN_K):
                hcol = col_bcast(hs[kk].astype(BF).astype(F32))
                for i in range(8):
                    for c in range(DT):
                        acc[c] = vpu_fma(acc[c], w232[8 * kk + i, c],
                                         hcol[16 * i:16 * i + 8],
                                         hcol[16 * i + 8:16 * i + 16])
            cols = [cc + sub_sum(a) for cc, a in zip(cols, acc)]
            o_ref[...] = jnp.concatenate(cols, axis=1)[0:1].astype(o_ref.dtype)

        blocks = _plan(nc)
        for b, plan in enumerate(blocks):
            end = b == len(blocks) - 1
            if b > 0:
                wait(marker if end else n_ring + b - 1)
            if b == 1:
                start_dma(late)
            if b == 2:
                wait(late)
            run_block(b, *plan, b == 0, end)

    return kernel


@jax.jit
def pallas_interleave_layers__sliding_block_cached__glu_gated_swiglu__decode_kernel(
    A_x: jax.Array,
    A_k_cache: jax.Array,
    A_v_cache: jax.Array,
    A_wq: jax.Array,
    A_wo: jax.Array,
    B_x: jax.Array,
    B_w1: jax.Array,
    B_w3: jax.Array,
    B_w2: jax.Array,
):
    sk = A_k_cache.shape[2]
    win = min(4096, max(256, sk // 4))
    nt_total, nc = sk // LANES, win // LANES

    def kv_view(a):
        return _tile_view(jnp.swapaxes(a, 2, 3).reshape(H * DH, sk))

    def view4(t):
        return t.reshape(t.shape[0] // 4, 2, 4, t.shape[2], 8, LANES)

    def wbuf(r, c):
        return pltpu.VMEM((r // 16, c // LANES, 16, LANES), BF)

    def wbuf4(r, c):
        return pltpu.VMEM((r // 64, 4, c // LANES, 16, LANES), BF)

    any_spec = pl.BlockSpec(memory_space=pl.ANY)
    out = pl.pallas_call(
        _make_kernel(nt_total, nc),
        out_shape=jax.ShapeDtypeStruct((1, D), A_x.dtype),
        in_specs=[any_spec] * 8,
        out_specs=pl.BlockSpec(memory_space=pltpu.VMEM),
        scratch_shapes=[
            wbuf(H * DH, win), wbuf4(H * DH, win),
            wbuf(D, H * DH), wbuf4(H * DH, D),
            wbuf(D, F), wbuf(D, F), wbuf(F, D),
            pltpu.VMEM((NP - 1, PG, NVX, 8, LANES), F32),
            pltpu.VMEM((2 * PG, 8, LANES), U32),
            pltpu.VMEM((RING, 12, 8, LANES), U32),
            pltpu.VMEM((RING, nc // 4, 8, LANES), F32),
            pltpu.VMEM((PRING * 2 * nc + 32, LANES), F32),
            pltpu.VMEM((PRING * 2 * nc + 32, LANES), F32),
            pltpu.VMEM((RING, nc // 4, 8, LANES), U32),
            pltpu.VMEM((NP, 8, LANES), F32),
            pltpu.VMEM((NP, 8, PW), F32),
            pltpu.VMEM((NP, 8, PW), U32),
            pltpu.VMEM((16, 8, LANES), U32),
            pltpu.VMEM((2 * FT, 8, LANES), F32),
            pltpu.VMEM((16, 8, LANES), U32),
            pltpu.VMEM((8, 1024), U32),
            pltpu.VMEM((8, 1024), F32),
            pltpu.VMEM((1, D), BF),
            pltpu.SemaphoreType.DMA((NSEM,)),
        ],
        compiler_params=pltpu.CompilerParams(
            vmem_limit_bytes=128 * 1024 * 1024),
    )(A_x.reshape(1, D), kv_view(A_k_cache), view4(kv_view(A_v_cache)),
      _tile_view(A_wq), view4(_tile_view(A_wo)),
      _tile_view(B_w1), _tile_view(B_w3), _tile_view(B_w2))
    return out.reshape(A_x.shape)
```

```python
import functools
import math

import jax
import jax.numpy as jnp
from jax import lax
import jax.experimental.pallas as pl
import jax.experimental.pallas.tpu as pltpu

D = 640
H = 32
DH = 192
F = 1536
LANES = 128
EPS = 1e-5

NP = H // 2
PG = 2 * DH // 16
HG = DH // 16
PW = 2 * DH
DT = D // LANES
FT = F // LANES

GP = 4
NGRP = NP // GP
W2_SPLIT = (0, 56, 80, 92, 96)
W2_MXU = 80
RELOAD_ROWS = 8
NSEM = 3
RING = 4
PRING = 6

MC = (2, 2, 2, 2, 2, 2, 2, 2, 2, 2, 2, 2, 2, 0, 0)
XCOLS = (1, 7, 10, 16, 22, 25, 4, 13, 19, 28)
NVX = 6
VQ = (11, 12, 13, 14, 15)
V_END = (172, 297, 349)
TILES = (1060, 655, 291)
XCOST = (0.67, 0.77, 0.77, 0.67)
GSHARE = 2
PVM_AFTER = 2
WO_START = (0, 80, 65, 999)
WO_GAP = (0, 72, 60, 12)
WO_KEEP = 4
FSTEP = 2
FIRST = (160, 2, 0)
LAST_OFF = (8, 6, 6)
VQ_FIRST = 30
VQ_UNIT = 4
XC_LINK = 50
SM_LAG = (60, 64, 64, 64)
SM_LAG0 = 52
RED_W = (10, 10, 10, 10)
RED_A = (40, 40, 32, 40)
RED_B = (16, 24, 20, 16)
Q_W = (4, 4, 4, 4)
Q_A = (18, 12, 12, 12)
Q_B = (-4, -4, -4, -4)
SM_W = (4, 4, 7, 7)
SM_A = (56, 56, 56, 56)
SM_B = (30, 42, 30, 30)
NLINK = (0, 4, 3)
LINK0 = (8, 8, 8, 10)
LINKSTEP = (4, 5, 4, 7)
LINK_REP = (1, 1, 4, 1)
TAIL_T = 2
FIN_ORDER = (NP - 1, NP - 2)
WO_JOINT = 2
UP_KM = 8
UP_IMAJ = 1
UP_G = 1
DN_MODE = 1
UP_REP = 1
UP_K = 3
UP_COLS = 6
UP_LINK0 = 60
UP_LINKSTEP = 4.75
UX_LINK = 44
DOWN_K = 4

U32 = jnp.uint32
BF = jnp.bfloat16
F32 = jnp.float32


def _tile_view(w):
    r, c = w.shape
    return jnp.swapaxes(w.reshape(r // 16, 2, 8, c // LANES, LANES), 2, 3)


def _rhs(w32, g0, c):
    return pltpu.bitcast(w32[pl.ds(g0, 8), c].reshape(64, LANES), BF)


def _rhs4(w32, tile, c):
    return pltpu.bitcast(w32[pl.ds(2 * tile, 2), :, c].reshape(64, LANES), BF)


def _swiglu(g, u):
    hg = 0.5 * g
    return hg * (1.0 + jnp.tanh(hg)) * u


def _pack2(lo, hi):
    return pltpu.bitcast(jnp.concatenate([lo, hi], axis=0).astype(BF), U32)


def _add(a, b):
    return b if a is None else a + b


def _bits_or(vals):
    return functools.reduce(lambda a, b: a | b, [pltpu.bitcast(v, U32) for v in vals])


def _plan(nc):
    nk = nc // 8
    seq = [('fq', 0), ('fq', 1)]
    for p in range(NP):
        if 1 <= p < NP - 1:
            seq.append(('qx' if p + 1 in VQ else 'q', p + 1))
        for k in range(nk):
            if k == PVM_AFTER and p > 0 and MC[p - 1]:
                seq.append(('pvm', p - 1, nc - MC[p - 1], nc, False))
            seq.append(('qk', p, k))
        if p < 2:
            seq.append(('reload', p))
        seq.append(('sm', p))
    seq += [('pvm', NP - 1, c, c + 4, c > 0) for c in range(0, nc, 4)]
    last_pv = seq[-nc // 4]

    def tiles(it):
        if it[0] == 'pvm':
            return 3 * (it[3] - it[2])
        return dict(fq=15, q=15, wo=15, qk=24, sm=0, qx=0, reload=0)[it[0]]

    chains = [(p, g) for p in range(NP - 1) for g in range(PG)]
    blocks = []
    v0 = done = 0
    for b in range(len(V_END) + 1):
        final = b == len(V_END)
        v1 = len(chains) if final else V_END[b]
        todo = list(range(done, v0 // PG))
        done = v0 // PG
        budget = 10 ** 9 if final else TILES[b] - 15 * len(todo)
        body = []
        used = 0
        while seq and used + tiles(seq[0]) // 2 <= budget:
            body.append(seq.pop(0))
            used += tiles(body[-1])
        while body[-1][0] in ('sm', 'qx'):
            seq.insert(0, body.pop())
        assert b > 0 or not any(it[1] in VQ for it in body)
        keep = WO_KEEP if last_pv in body else 0
        items = [('red', p) for p in todo]
        used = 0
        nxt = WO_START[b]
        for it in body:
            if it == last_pv:
                while todo:
                    items.append(('wo', todo.pop(0)))
            if len(todo) > keep and used >= nxt:
                items.append(('wo', todo.pop(0)))
                nxt = used + WO_GAP[b]
            items.append(it)
            used += tiles(it)
        items += [('wo', p) for p in todo]
        if final:
            assert done == NP - 2
            assert TAIL_T == 3 or (MC[NP - 2] == 0 and v0 % PG <= 8 * TAIL_T)
            for p in FIN_ORDER:
                items += [('red', p), ('wo', p)]
            joint = [it for it in items if it[0] == 'wo'][-WO_JOINT:]
            items = [it for it in items if it not in joint]
            items.append(('wo', *[it[1] for it in joint]))
            blocks.append((chains[v0:v1], items, v1 - v0, 0, 0))
        else:
            blocks.append((chains[v0:v1], items, NLINK[b], FIRST[b], LAST_OFF[b]))
        v0 = v1
    seen = set()
    for b, (chs, items, n_link, _, _) in enumerate(blocks):
        assert all(it[1] - (NP - 2) < b for it in items if it[0] == 'qk')
        assert all(p in seen for p, _ in chs[:n_link])
        seen |= {it[1] for it in items if it[0] == 'sm'}
        assert all(p in seen for p, _ in chs)
        assert max(seen) - chs[-1][0] < PRING
    return blocks


def _make_kernel(n_tiles_total, nc):
    c0 = n_tiles_total - nc
    qscale = DH ** -0.5 * math.log2(math.e)
    prow = 2 * nc
    nk = nc // 8

    def kernel(x_hbm, k_hbm, v_hbm, wq_hbm, wo_hbm, w1_hbm, w3_hbm, w2_hbm,
               o_ref,
               kbuf, vbuf, wqbuf, wobuf, w1buf, w3buf, w2buf,
               vx_ref, t0_ref, lhs_ref, s_ref, p_ref, p2_ref, pk_ref, lsum_ref, om_ref,
               ob_ref, mask_ref, cs_ref, qpk_ref, xn_ref, y_ref, xbuf, sem):
        def halves(src, dst):
            return [(src(par), dst(pl.ds(8 * par, 8))) for par in range(2)]

        def whole(src, dst):
            return halves(lambda p: src.at[:, p], lambda h: dst.at[:, :, h, :])

        def kv_group(g):
            kr = pl.ds(g * GP * PG, GP * PG)
            vr = pl.ds(g * GP * PG // 4, GP * PG // 4)
            return (halves(lambda p: k_hbm.at[kr, p, pl.ds(c0, nc)],
                           lambda h: kbuf.at[kr, :, h, :])
                    + halves(lambda p: v_hbm.at[vr, p, :, pl.ds(c0, nc)],
                             lambda h: vbuf.at[vr, :, :, h, :]))

        def w2_group(i):
            rows = pl.ds(W2_SPLIT[i], W2_SPLIT[i + 1] - W2_SPLIT[i])
            return halves(lambda p: w2_hbm.at[rows, p], lambda h: w2buf.at[rows, :, h, :])

        groups = ([whole(wq_hbm, wqbuf) + [(x_hbm, xbuf)]]
                  + [kv_group(NGRP - 1 - g) for g in range(NGRP)]
                  + [halves(lambda p: wo_hbm.at[:, p], lambda h: wobuf.at[:, :, :, h, :]),
                     whole(w1_hbm, w1buf) + whole(w3_hbm, w3buf)]
                  + [w2_group(i) for i in range(len(W2_SPLIT) - 1)])
        marker = len(groups)
        groups.append([(x_hbm, xbuf)])
        n_ring = len(groups)
        def k_rows(i, rows):
            return halves(lambda p: k_hbm.at[rows((NP - 2 + i) * PG), p, pl.ds(c0, nc)],
                          lambda h: kbuf.at[rows(i * PG), :, h, :])

        for i, n in enumerate((PG, RELOAD_ROWS)):
            groups.append([cp for g in range(n) for cp in k_rows(i, lambda r0: r0 + g)])
        late = n_ring + 1 + NSEM
        groups += [[]] * (late - len(groups))
        groups.append(k_rows(1, lambda r0: pl.ds(r0 + RELOAD_ROWS, PG - RELOAD_ROWS)))

        def copies(i):
            return [pltpu.make_async_copy(src, dst, sem.at[i % NSEM])
                    for src, dst in groups[i]]

        def start_dma(i):
            for cp in copies(i):
                cp.start()

        def wait(i):
            for cp in copies(i):
                cp.wait()
            if i + NSEM < n_ring:
                start_dma(i + NSEM)

        for i in range(NSEM):
            start_dma(i)

        k32 = kbuf.bitcast(U32)
        v32 = vbuf.bitcast(U32)
        wq32 = wqbuf.bitcast(U32)
        wo32 = wobuf.bitcast(U32)
        w13 = (w1buf.bitcast(U32), w3buf.bitcast(U32))
        w232 = w2buf.bitcast(U32)

        sub = lax.broadcasted_iota(jnp.int32, (8, LANES), 0)
        lane = lax.broadcasted_iota(jnp.int32, (8, LANES), 1)
        sub3 = lax.broadcasted_iota(jnp.int32, (8, PW), 0)
        lane3 = lax.broadcasted_iota(jnp.int32, (8, PW), 1)

        for r in range(4):
            half = U32(0x0000FFFF if r % 2 == 0 else 0xFFFF0000)
            lo = jnp.where(sub == r // 2, half, U32(0))
            hi = jnp.where(sub == 2 + r // 2, half, U32(0))
            mask_ref[r] = lo
            mask_ref[4 + r] = jnp.where(lane < DH - LANES, lo, hi)
            mask_ref[8 + r] = hi
            mask_ref[12 + r] = lo | hi
        p_refs = (p_ref, p2_ref)
        for pr in p_refs:
            pr[...] = jnp.zeros(pr.shape, F32)

        def dot(l32, r, free=True):
            del free
            return jnp.dot(pltpu.bitcast(l32, BF), r, preferred_element_type=F32)

        def tile_of(v, kk):
            return v[:, kk * LANES:(kk + 1) * LANES]

        def ln_stats(x):
            xb = x.astype(BF).astype(F32)
            m = jnp.mean(xb, axis=-1, keepdims=True)
            xc = xb - m
            v = jnp.mean(xc * xc, axis=-1, keepdims=True)
            return xb, m, lax.rsqrt(v + EPS)

        def raw_proj(xb, w32, c, mm=dot):
            lhs = _pack2(xb, jnp.ones_like(xb))
            acc = None
            for kk in range(DT):
                acc = _add(acc, mm(tile_of(lhs, kk), _rhs(w32, 8 * kk, c), False))
            return acc[0:8], acc[8:16]

        def col_bcast(v):
            return jnp.concatenate([v] * (LANES // 8), axis=0).T

        def vpu_fma(acc, w, xlo, xhi):
            w = pltpu.bitcast(w, BF).astype(F32)
            return _add(acc, w[0:8] * xlo + w[8:16] * xhi)

        def sub_sum(a):
            return jnp.broadcast_to(jnp.sum(a, axis=0, keepdims=True), a.shape)

        def expand_q(p, t, q):
            for r in range(4):
                lhs_ref[p % RING, 4 * t + r] = q & mask_ref[4 * t + r]

        def stage_q(p, mm=dot):
            acc = [None] * 3
            for kk in range(DT):
                for t in range(3):
                    acc[t] = _add(acc[t], mm(xn_ref[:, pl.ds(kk * LANES, LANES)],
                                             _rhs(wq32, 8 * kk, 3 * p + t))[0:8])
            for t in range(3):
                q = acc[t] * qscale
                expand_q(p, t, _pack2(q, q))

        def stage_qk(p, k, krow, mm=dot, scale=None):
            for j in range(2 * k, 2 * k + 2):
                acc = None
                for t in range(3):
                    for r in range(4):
                        acc = _add(acc, mm(lhs_ref[p % RING, 4 * t + r],
                                           _rhs(k32, krow + 8 * t, 4 * j + r))[0:8])
                s_ref[p % RING, j] = acc if scale is None else acc * scale

        def head_reduce(v, op, lane_op):
            for d in (1, 2):
                up = pltpu.roll(v, d, 0)
                down = pltpu.roll(v, 8 - d, 0)
                v = op(v, jnp.where(sub % (2 * d) >= d, up, down))
            return lane_op(v, axis=1, keepdims=True)

        def softmax(p, j0):
            s = s_ref[p % RING]
            m = head_reduce(jnp.max(s, axis=0), jnp.maximum, jnp.max)
            e = jnp.exp2(s - m)
            l = jnp.sum(e, axis=0)
            l = jnp.broadcast_to(head_reduce(l, jnp.add, jnp.sum), l.shape)
            lsum_ref[p, 0:8, :] = l
            for j in range(j0, nc // 4):
                pk_ref[p % RING, j] = _pack2(e[j], e[j])
            return e, l

        def widened(p):
            return XCOLS if p else XCOLS[:NVX]

        def vx_slot(p, g, e):
            return (NP - 2) * PG + 3 * p + g // 8, (e - NVX) * 8 + g % 8

        def t_slot(p, j, n):
            if p == 0:
                return t0_ref, pl.ds(j, n)
            row = (NP - 2) * PG if p == 1 else p * PG if p < NP - 2 else 2 * PG + 2
            return k32, (row + j // nc, pl.ds(j % nc, n))

        def pv_chain(p, g, gate, n=1, store=True):
            acc = None
            for c in range(nc - MC[p]):
                row = (p % PRING) * prow + 8 * (c // 4) + 4 * (g // HG) + c % 4
                pb = gate()[pl.ds(row, 16, stride=0), :]
                w = v32[p * (PG // 4) + g // 4, pl.ds(g % 4, n), c]
                if c in widened(p):
                    e = XCOLS.index(c)
                    if e < NVX:
                        hi = vx_ref[p, e, pl.ds(g, n)]
                    else:
                        r0, s0 = vx_slot(p, g, e)
                        hi = k32[r0, pl.ds(s0, n)]
                    w = pltpu.bitcast(jnp.concatenate([w, hi], axis=1), F32)
                else:
                    w = pltpu.bitcast(w, BF).astype(F32)
                acc = _add(acc, w * pb)
            acc = pltpu.bitcast(acc, U32).reshape(2 * n, 8, LANES)
            if store:
                ref, idx = t_slot(p, 2 * g, 2 * n)
                ref[idx] = acc
            return acc

        def pv_mxu(p, cols, transposed, mm=dot):
            acc = [None] * 3
            cols = list(cols)
            for i0 in range(0, len(cols), 4):
                ls = {c: pk_ref[p % RING, c // 4] & mask_ref[12 + c % 4]
                      for c in cols[i0:i0 + 4]}
                for t in range(3):
                    for c, l in ls.items():
                        tile = _rhs4(v32, 3 * p + t, c)
                        if transposed:
                            res = mm(l, tile)
                        else:
                            res = lax.dot_general(
                                pltpu.bitcast(l, BF), tile, (((1,), (1,)), ((), ())),
                                preferred_element_type=F32)
                        acc[t] = _add(acc[t], res[0:8])
            return jnp.concatenate(acc, axis=1)

        def own_head(o):
            return jnp.where((sub3 < 4) == (lane3 < DH), o, 0.0)

        def finish_o(p, o, nt=3):
            linv = 1.0 / lsum_ref[p, 0:8, :]
            la = jnp.broadcast_to(linv[0:1], linv.shape)
            lb = jnp.broadcast_to(linv[4:5], linv.shape)
            linv = [la, jnp.where(lane < DH - LANES, la, lb), lb]
            o = jnp.sum(o, axis=0, keepdims=True) * jnp.concatenate(linv[:nt], axis=1)
            ob_ref[p, :, 0:nt * LANES] = _pack2(o, o)

        def mxu_tiles(p):
            return TAIL_T if p == NP - 2 else 3

        def stage_reduce(p):
            o = None
            nt = mxu_tiles(p)
            if p < NP - 1:
                slots = [t_slot(p, 16 * t, 16) for t in range(nt)]
                tt = jnp.concatenate([ref[idx] for ref, idx in slots])
                tt = pltpu.bitcast(tt.reshape(nt * LANES, LANES), F32)
                o = jnp.sum(tt.T.reshape(LANES // 8, 8, nt * LANES), axis=0)
            if p == NP - 1 or MC[p]:
                o = _add(o, own_head(om_ref[p]))
            finish_o(p, o, nt)

        def stage_wo(tiles, mm=dot):
            for c in range(DT):
                acc = y_ref[:, pl.ds(c * LANES, LANES)]
                for p, t in tiles:
                    acc = acc + mm(ob_ref[p, :, pl.ds(t * LANES, LANES)],
                                   _rhs4(wo32, 3 * p + t, c))[0:8]
                y_ref[:, pl.ds(c * LANES, LANES)] = acc

        def begin_attention(x):
            y_ref[:, 0:D] = x
            xb, m, r = ln_stats(x)
            xn = (xb - m) * r
            xn_ref[:, 0:D] = _pack2(xn, xn)
            return xb, m, r

        wait(0)
        begin_attention(jnp.broadcast_to(xbuf[...].astype(F32), (8, D)))

        def pair1(i, carry):
            p = NP - 1 - i
            stage_q(p)
            for k in range(nk):
                stage_qk(p, k, p * PG)
            softmax(p, 0)
            finish_o(p, own_head(pv_mxu(p, range(nc), False)))
            om_ref[p] = jnp.zeros(om_ref.shape[1:], F32)
            qpk_ref[p] = jnp.zeros((8, LANES), U32)
            t0_ref[p] = jnp.zeros((8, LANES), U32)
            cs_ref[p] = jnp.zeros((8, LANES), F32)

            first = 0
            for pp in range(NP - 1):
                first = jnp.where(p == pp, nc - MC[pp], first)

            def transpose_v(c, carry2):
                for t in range(3):
                    tile = _rhs4(v32, 3 * p + t, c)
                    v32[pl.ds(2 * (3 * p + t), 2), :, c] = pltpu.bitcast(
                        tile.T, U32).reshape(2, 4, 8, LANES)
                return carry2

            lax.fori_loop(first, nc, transpose_v, 0)

            def widen(es):
                for g in range(0, PG, 4):
                    for e in es:
                        idx = (p * (PG // 4) + g // 4, slice(None), XCOLS[e])
                        w = pltpu.bitcast(pltpu.bitcast(v32[idx], BF).astype(F32), U32)
                        v32[idx] = w[:, 0:8]
                        if e < NVX:
                            vx_ref[p, e, pl.ds(g, 4)] = w[:, 8:16]
                        else:
                            r0, s0 = vx_slot(p, g, e)
                            k32[r0, pl.ds(s0, 4)] = w[:, 8:16]

            pl.when(p < NP - 1)(functools.partial(widen, range(NVX)))
            pl.when((p < NP - 1) & (p > 0))(
                functools.partial(widen, range(NVX, len(XCOLS))))
            return carry

        def group1(gi, row):
            for i in range(NGRP):
                pl.when(gi == i)(functools.partial(wait, 1 + i))
            lax.fori_loop(gi * GP, (gi + 1) * GP, pair1, 0)
            return row + PRING * prow // NGRP

        fence_row = pl.multiple_of(lax.fori_loop(0, NGRP, group1, 0), 8)
        wait(1 + NGRP)

        def woloop(p2, carry):
            stage_wo([(2 * p2 + i, t) for i in range(2) for t in range(3)])
            return carry

        lax.fori_loop(0, NP // 2, woloop, 0)

        x = y_ref[:, 0:D]
        xb, m, r = ln_stats(x)
        wait(2 + NGRP)
        gu = []
        for j in range(2 * FT):
            raw, cs = raw_proj(xb, w13[j % 2], j // 2)
            cs_ref[j] = cs
            gu.append((raw - m * cs) * r)
        hs = [_swiglu(g, u) for g, u in zip(gu[0::2], gu[1::2])]
        for kk in range(W2_MXU // 8, FT):
            p_ref[pl.ds(LANES * kk - 16 * W2_MXU, LANES), :] = col_bcast(
                hs[kk].astype(BF).astype(F32))
        hs = [_pack2(hh, hh) for hh in hs[:W2_MXU // 8]]
        cols = [tile_of(x, c) for c in range(DT)]
        part = [None] * DT
        for i in range(len(W2_SPLIT) - 1):
            wait(3 + NGRP + i)
            g0, g1 = W2_SPLIT[i], W2_SPLIT[i + 1]
            for c in range(DT):
                if g1 <= W2_MXU:
                    for kk in range(g0 // 8, g1 // 8):
                        cols[c] = cols[c] + dot(hs[kk], _rhs(w232, 8 * kk, c))[0:8]
                else:
                    for g in range(g0, g1):
                        row = 16 * (g - W2_MXU)
                        part[c] = vpu_fma(part[c], w232[g, c], p_ref[pl.ds(row, 8), :],
                                          p_ref[pl.ds(row + 8, 8), :])
        x = jnp.concatenate([cc + sub_sum(a) for cc, a in zip(cols, part)], axis=1)

        xb, m, r = begin_attention(x)
        rq = r * qscale

        def run_block(blk, chains, items, n_link, first, last_off, start, end):
            links = []
            y_vpu = None
            for j, (p, g) in enumerate(chains[:n_link]):
                tail = end and g >= 8 * TAIL_T
                acc = pv_chain(p, g, lambda: p_refs[g % 2], store=not tail)
                dep = acc[0] | acc[1]
                if tail:
                    linv = 1.0 / lsum_ref[p, pl.ds(4 * (g // HG), 8, stride=0), :]
                    oc = jnp.sum(pltpu.bitcast(acc, F32), axis=2, keepdims=True) * linv
                    oc = oc.astype(BF).astype(F32).reshape(16, LANES)
                    w = pltpu.bitcast(wo32[6 * p + g // 4, g % 4], BF).astype(F32) * oc
                    y_vpu = _add(y_vpu, w[:, 0:8] + w[:, 8:16])
                links.extend([(LINK0[blk] + LINKSTEP[blk] * j, dep)] * LINK_REP[blk])
            if start:
                xcol = [col_bcast(tile_of(xb, kk)) - m[0:1] for kk in range(DT)]
                links.extend([(XC_LINK, _bits_or(xc[LANES - 8:] for xc in xcol))] * 4)
            pops = []
            probs = {}
            busy = []

            def mm(l32, rr, free=True):
                links.sort(key=lambda lk: lk[0])
                if free and links and len(pops) >= links[0][0]:
                    l32 = jnp.where(sub < 4, l32, links.pop(0)[1])
                pops.append(dot(l32, rr))
                return pops[-1]

            for it in items:
                kind, p = it[0], it[1]
                if kind == 'fq':
                    for t in range(3):
                        raw, cs = raw_proj(xb, wq32, 3 * p + t, mm)
                        q = raw - m * cs
                        q = q if p == 0 else q * rq
                        expand_q(p, t, _pack2(q, q))
                elif kind == 'q':
                    stage_q(p, mm)
                    busy.append((len(pops) - Q_A[blk], len(pops) - Q_B[blk], Q_W[blk]))
                elif kind == 'qx':
                    for t in range(3):
                        expand_q(p, t, qpk_ref[3 * VQ.index(p) + t])
                elif kind == 'qk':
                    stage_qk(p, it[2], p % (NP - 2) * PG, mm, rq if p == 0 else None)
                elif kind == 'sm':
                    e, l = softmax(p, 0 if p == NP - 1 else (nc - MC[p]) // 4)
                    lag = SM_LAG0 if p == 0 else SM_LAG[blk]
                    pos = len(pops) + (lag if pops else lag - 14)
                    links.append((pos, pltpu.bitcast(l, U32)))
                    busy.append((pos - SM_A[blk], pos - SM_B[blk], SM_W[blk]))
                    if p < NP - 1:
                        probs[p] = e
                elif kind == 'pvm':
                    o = pv_mxu(p, range(it[2], it[3]), True, mm)
                    om_ref[p] = o + om_ref[p] if it[4] else o
                elif kind == 'reload':
                    start_dma(n_ring + p)
                elif kind == 'red':
                    stage_reduce(p)
                elif kind == 'wo':
                    busy.append((len(pops) - RED_A[blk], len(pops) - RED_B[blk], RED_W[blk]))
                    stage_wo([(pp, t) for pp in it[1:] for t in range(mxu_tiles(pp))], mm)

            def fence(buf, a):
                buf[pl.ds(fence_row, 8), :] = pops[a][0:8]

            if start:
                nkg = D // 16

                def xslot(kg):
                    u = kg // VQ_UNIT
                    return p_refs[u % 2], 16 * (u // 2 * VQ_UNIT + kg % VQ_UNIT)

                for kg in range(nkg):
                    buf, row = xslot(kg)
                    buf[pl.ds(row, 16), :] = xcol[kg // 8][16 * (kg % 8):16 * (kg % 8) + 16]
                for i, p in enumerate(VQ):
                    acc = None
                    for kg in range(nkg):
                        buf, row = xslot(kg)
                        if kg % VQ_UNIT == 0:
                            a = (i * nkg + kg) * (first - VQ_FIRST) // (len(VQ) * nkg)
                            fence(buf, VQ_FIRST + a // 2 * 2)
                        w = pltpu.bitcast(wq32[kg, pl.ds(3 * p, 3)], BF).astype(F32)
                        w = w * buf[pl.ds(row, 16), :]
                        acc = _add(acc, w[:, 0:8] + w[:, 8:16])
                    for t in range(3):
                        q = sub_sum(acc[t]) * rq
                        qpk_ref[3 * i + t] = _pack2(q, q)

            def store_probs(p):
                e = probs.pop(p)
                for pr in p_refs:
                    for j in range((nc - MC[p] + 3) // 4):
                        pr[pl.ds((p % PRING) * prow + 8 * j, 8), :] = e[j]

            rest = chains[n_link:]
            if rest:
                runs, i = [], 0
                while i < len(rest):
                    p, g = rest[i]
                    runs.append((p, g, min(GSHARE - g % GSHARE, len(rest) - i)))
                    i += runs[-1][2]
                cost = [n * (XCOST[blk] if c in widened(p) else 1.0)
                        for p, _, n in runs for c in range(nc - MC[p])]
                n_items = len(cost)
                n_units = (len(pops) - last_off - first) // FSTEP + 1
                less = [0.0] * n_units
                for lo, hi, w in busy:
                    us = [u for u in range(n_units) if lo <= first + u * FSTEP < hi]
                    for u in us:
                        less[u] += w / len(us)
                per = (sum(cost) + sum(less)) / n_units
                unit_of, total, used = [], 0.0, 0.0
                for u in range(n_units):
                    total += per - less[u]
                    while len(unit_of) < n_items and (
                            used + cost[len(unit_of)] / 2 < total or u + 1 == n_units):
                        used += cost[len(unit_of)]
                        unit_of.append(u)
                state = [0, -1, 1]

                def gate():
                    u = unit_of[state[0]]
                    state[0] += 1
                    if u != state[1]:
                        state[1] = u
                        state[2] += 1
                        fence(p_refs[state[2] % 2], first + u * FSTEP)
                    return p_refs[state[2] % 2]

            for p, g, n in runs if rest else []:
                if g == 0:
                    for i in range(state[0], n_items):
                        if unit_of[i] != state[1] or state[1] + 1 == n_units:
                            break
                        unit_of[i] += 1
                if p in probs:
                    store_probs(p)
                pv_chain(p, g, gate, n)
            for p in list(probs):
                store_probs(p)
            if end:
                x = y_ref[:, 0:D]
                if y_vpu is not None:
                    x = x + jnp.concatenate([sub_sum(y_vpu[c]) for c in range(DT)], axis=1)
                last_ffn(x, mm, len(pops), links)

        def last_ffn(x, mm, base, links):
            xb, m, r = ln_stats(x)
            lhs = _pack2(xb, xb)
            xcol = [col_bcast(tile_of(xb, kk)) for kk in range(UP_K)]
            links.extend([(base + UX_LINK, _bits_or(xc[LANES - 8:] for xc in xcol))] * 4)
            j0 = 2 * (FT - UP_COLS)
            part = {}
            order = ([8 * kk + i for i in range(8) for kk in range(UP_K)] if UP_IMAJ
                     else range(8 * UP_K))
            for j1 in range(j0, 2 * FT, UP_G):
                js = range(j1, min(j1 + UP_G, 2 * FT))
                acc = {j: None for j in js}
                for kg in order:
                    xc = xcol[kg // 8][16 * (kg % 8):16 * (kg % 8) + 16]
                    for j in js:
                        acc[j] = vpu_fma(acc[j], w13[j % 2][kg, j // 2], xc[0:8], xc[8:16])
                for j in js:
                    part[j] = sub_sum(acc[j])
                links.extend([(base + int(UP_LINK0 + UP_LINKSTEP * (js[-1] - j0)),
                               _bits_or(part[j] for j in js))] * UP_REP)
            work = [(j, kk) for kk in range(DT) for j in range(UP_KM)]
            work += [(j, kk) for j in range(UP_KM, 2 * FT)
                     for kk in range(UP_K if j in part else 0, DT)]
            for j, kk in work:
                part[j] = _add(part.get(j), mm(tile_of(lhs, kk),
                                               _rhs(w13[j % 2], 8 * kk, j // 2))[0:8])
            gu = [(part[j] - m * cs_ref[j]) * r for j in range(2 * FT)]
            hs = [_swiglu(g, u) for g, u in zip(gu[0::2], gu[1::2])]
            cols = [tile_of(x, c) for c in range(DT)]
            for kk in range(DOWN_K, FT):
                hh = _pack2(hs[kk], hs[kk])
                for c in range(DT):
                    cols[c] = cols[c] + mm(hh, _rhs(w232, 8 * kk, c))[0:8]
            hcol = [col_bcast(hs[kk].astype(BF).astype(F32)) for kk in range(DOWN_K)]
            if DN_MODE == 2:
                accs = [[None] * DT for _ in range(DOWN_K)]
            else:
                accs = [[None] * DT] * DOWN_K
            for kk, i in ([(kk, i) for i in range(8) for kk in range(DOWN_K)] if DN_MODE == 1
                          else [(kk, i) for kk in range(DOWN_K) for i in range(8)]):
                for c in range(DT):
                    accs[kk][c] = vpu_fma(accs[kk][c], w232[8 * kk + i, c],
                                          hcol[kk][16 * i:16 * i + 8],
                                          hcol[kk][16 * i + 8:16 * i + 16])
            acc = accs[0] if DN_MODE != 2 else [
                functools.reduce(_add, [a[c] for a in accs]) for c in range(DT)]
            cols = [cc + sub_sum(a) for cc, a in zip(cols, acc)]
            o_ref[...] = jnp.concatenate(cols, axis=1)[0:1].astype(o_ref.dtype)

        blocks = _plan(nc)
        for b, plan in enumerate(blocks):
            end = b == len(blocks) - 1
            if b > 0:
                wait(marker if end else n_ring + b - 1)
            if b == 1:
                start_dma(late)
            if b == 2:
                wait(late)
            run_block(b, *plan, b == 0, end)

    return kernel


@jax.jit
def pallas_interleave_layers__sliding_block_cached__glu_gated_swiglu__decode_kernel(
    A_x: jax.Array,
    A_k_cache: jax.Array,
    A_v_cache: jax.Array,
    A_wq: jax.Array,
    A_wo: jax.Array,
    B_x: jax.Array,
    B_w1: jax.Array,
    B_w3: jax.Array,
    B_w2: jax.Array,
):
    sk = A_k_cache.shape[2]
    win = min(4096, max(256, sk // 4))
    nt_total, nc = sk // LANES, win // LANES

    def kv_view(a):
        return _tile_view(jnp.swapaxes(a, 2, 3).reshape(H * DH, sk))

    def view4(t):
        return t.reshape(t.shape[0] // 4, 2, 4, t.shape[2], 8, LANES)

    def wbuf(r, c):
        return pltpu.VMEM((r // 16, c // LANES, 16, LANES), BF)

    def wbuf4(r, c):
        return pltpu.VMEM((r // 64, 4, c // LANES, 16, LANES), BF)

    any_spec = pl.BlockSpec(memory_space=pl.ANY)
    out = pl.pallas_call(
        _make_kernel(nt_total, nc),
        out_shape=jax.ShapeDtypeStruct((1, D), A_x.dtype),
        in_specs=[any_spec] * 8,
        out_specs=pl.BlockSpec(memory_space=pltpu.VMEM),
        scratch_shapes=[
            wbuf(H * DH, win), wbuf4(H * DH, win),
            wbuf(D, H * DH), wbuf4(H * DH, D),
            wbuf(D, F), wbuf(D, F), wbuf(F, D),
            pltpu.VMEM((NP - 1, NVX, PG, 8, LANES), U32),
            pltpu.VMEM((2 * PG, 8, LANES), U32),
            pltpu.VMEM((RING, 12, 8, LANES), U32),
            pltpu.VMEM((RING, nc // 4, 8, LANES), F32),
            pltpu.VMEM((PRING * 2 * nc + 32, LANES), F32),
            pltpu.VMEM((PRING * 2 * nc + 32, LANES), F32),
            pltpu.VMEM((RING, nc // 4, 8, LANES), U32),
            pltpu.VMEM((NP, 16, LANES), F32),
            pltpu.VMEM((NP, 8, PW), F32),
            pltpu.VMEM((NP, 8, PW), U32),
            pltpu.VMEM((16, 8, LANES), U32),
            pltpu.VMEM((2 * FT, 8, LANES), F32),
            pltpu.VMEM((16, 8, LANES), U32),
            pltpu.VMEM((8, 1024), U32),
            pltpu.VMEM((8, 1024), F32),
            pltpu.VMEM((1, D), BF),
            pltpu.SemaphoreType.DMA((NSEM,)),
        ],
        compiler_params=pltpu.CompilerParams(
            vmem_limit_bytes=128 * 1024 * 1024),
    )(A_x.reshape(1, D), kv_view(A_k_cache), view4(kv_view(A_v_cache)),
      _tile_view(A_wq), view4(_tile_view(A_wo)),
      _tile_view(B_w1), _tile_view(B_w3), _tile_view(B_w2))
    return out.reshape(A_x.shape)
```

```python
import functools
import math

import jax
import jax.numpy as jnp
from jax import lax
import jax.experimental.pallas as pl
import jax.experimental.pallas.tpu as pltpu

D = 640
H = 32
DH = 192
F = 1536
LANES = 128
EPS = 1e-5

NP = H // 2
PG = 2 * DH // 16
HG = DH // 16
PW = 2 * DH
DT = D // LANES
FT = F // LANES

GP = 4
NGRP = NP // GP
W2_SPLIT = (0, 56, 80, 92, 96)
W2_MXU = 80
RELOAD_ROWS = 8
NSEM = 3
RING = 4
PRING = 6

MC = (2, 2, 2, 2, 2, 2, 2, 2, 2, 2, 2, 2, 2, 0, 0)
XCOLS = (1, 7, 10, 16, 22, 25, 4, 13, 19, 28)
NVX = 6
VQ = (11, 12, 13, 14, 15)
V_END = (172, 297, 349)
TILES = (1060, 655, 291)
XCOST = (0.67, 0.77, 0.77, 0.67)
GSHARE = 2
PVM_AFTER = 2
WO_START = (0, 80, 65, 999)
WO_GAP = (0, 72, 60, 12)
WO_KEEP = 4
FSTEP = 2
FIRST = (160, 2, 0)
LAST_OFF = (8, 6, 6)
VQ_FIRST = 30
VQ_UNIT = 4
XC_LINK = 50
SM_LAG = (60, 64, 64, 64)
SM_LAG0 = 52
RED_W = (10, 10, 10, 10)
RED_A = (40, 40, 32, 40)
RED_B = (16, 24, 20, 16)
Q_W = (4, 4, 4, 4)
Q_A = (18, 12, 12, 12)
Q_B = (-4, -4, -4, -4)
SM_W = (4, 4, 7, 7)
SM_A = (56, 56, 56, 56)
SM_B = (30, 42, 30, 30)
NLINK = (0, 4, 3)
LINK0 = (8, 8, 8, 10)
LINKSTEP = (4, 5, 4, 7)
LINK_REP = (1, 1, 4, 1)
TAIL_T = 2
WO_JOINT = 2
UP_KM = 8
UP_K = 3
UP_COLS = 6
UP_LINK0 = 60
UP_LINKSTEP = 4.75
UX_LINK = 44
DOWN_K = 4

U32 = jnp.uint32
BF = jnp.bfloat16
F32 = jnp.float32


def _tile_view(w):
    r, c = w.shape
    return jnp.swapaxes(w.reshape(r // 16, 2, 8, c // LANES, LANES), 2, 3)


def _rhs(w32, g0, c):
    return pltpu.bitcast(w32[pl.ds(g0, 8), c].reshape(64, LANES), BF)


def _rhs4(w32, tile, c):
    return pltpu.bitcast(w32[pl.ds(2 * tile, 2), :, c].reshape(64, LANES), BF)


def _swiglu(g, u):
    hg = 0.5 * g
    return hg * (1.0 + jnp.tanh(hg)) * u


def _pack2(lo, hi):
    return pltpu.bitcast(jnp.concatenate([lo, hi], axis=0).astype(BF), U32)


def _add(a, b):
    return b if a is None else a + b


def _bits_or(vals):
    return functools.reduce(lambda a, b: a | b, [pltpu.bitcast(v, U32) for v in vals])


def _plan(nc):
    nk = nc // 8
    seq = [('fq', 0), ('fq', 1)]
    for p in range(NP):
        if 1 <= p < NP - 1:
            seq.append(('qx' if p + 1 in VQ else 'q', p + 1))
        for k in range(nk):
            if k == PVM_AFTER and p > 0 and MC[p - 1]:
                seq.append(('pvm', p - 1, nc - MC[p - 1], nc, False))
            seq.append(('qk', p, k))
        if p < 2:
            seq.append(('reload', p))
        seq.append(('sm', p))
    seq += [('pvm', NP - 1, c, c + 4, c > 0) for c in range(0, nc, 4)]
    last_pv = seq[-nc // 4]

    def tiles(it):
        if it[0] == 'pvm':
            return 3 * (it[3] - it[2])
        return dict(fq=15, q=15, wo=15, qk=24, sm=0, qx=0, reload=0)[it[0]]

    chains = [(p, g) for p in range(NP - 1) for g in range(PG)]
    blocks = []
    v0 = done = 0
    for b in range(len(V_END) + 1):
        final = b == len(V_END)
        v1 = len(chains) if final else V_END[b]
        todo = list(range(done, v0 // PG))
        done = v0 // PG
        budget = 10 ** 9 if final else TILES[b] - 15 * len(todo)
        body = []
        used = 0
        while seq and used + tiles(seq[0]) // 2 <= budget:
            body.append(seq.pop(0))
            used += tiles(body[-1])
        while body[-1][0] in ('sm', 'qx'):
            seq.insert(0, body.pop())
        assert b > 0 or not any(it[1] in VQ for it in body)
        keep = WO_KEEP if last_pv in body else 0
        items = [('red', p) for p in todo]
        used = 0
        nxt = WO_START[b]
        for it in body:
            if it == last_pv:
                while todo:
                    items.append(('wo', todo.pop(0)))
            if len(todo) > keep and used >= nxt:
                items.append(('wo', todo.pop(0)))
                nxt = used + WO_GAP[b]
            items.append(it)
            used += tiles(it)
        items += [('wo', p) for p in todo]
        if final:
            assert done == NP - 2
            assert TAIL_T == 3 or (MC[NP - 2] == 0 and v0 % PG <= 8 * TAIL_T)
            for p in (NP - 1, NP - 2):
                items += [('red', p), ('wo', p)]
            joint = [it for it in items if it[0] == 'wo'][-WO_JOINT:]
            items = [it for it in items if it not in joint]
            items.append(('wo', *[it[1] for it in joint]))
            blocks.append((chains[v0:v1], items, v1 - v0, 0, 0))
        else:
            blocks.append((chains[v0:v1], items, NLINK[b], FIRST[b], LAST_OFF[b]))
        v0 = v1
    seen = set()
    for b, (chs, items, n_link, _, _) in enumerate(blocks):
        assert all(it[1] - (NP - 2) < b for it in items if it[0] == 'qk')
        assert all(p in seen for p, _ in chs[:n_link])
        seen |= {it[1] for it in items if it[0] == 'sm'}
        assert all(p in seen for p, _ in chs)
        assert max(seen) - chs[-1][0] < PRING
    return blocks


def _make_kernel(n_tiles_total, nc):
    c0 = n_tiles_total - nc
    qscale = DH ** -0.5 * math.log2(math.e)
    prow = 2 * nc
    nk = nc // 8

    def kernel(x_hbm, k_hbm, v_hbm, wq_hbm, wo_hbm, w1_hbm, w3_hbm, w2_hbm,
               o_ref,
               kbuf, vbuf, wqbuf, wobuf, w1buf, w3buf, w2buf,
               vx_ref, t0_ref, lhs_ref, s_ref, p_ref, p2_ref, pk_ref, lsum_ref, om_ref,
               ob_ref, mask_ref, cs_ref, qpk_ref, xn_ref, y_ref, xbuf, sem):
        def halves(src, dst):
            return [(src(par), dst(pl.ds(8 * par, 8))) for par in range(2)]

        def whole(src, dst):
            return halves(lambda p: src.at[:, p], lambda h: dst.at[:, :, h, :])

        def kv_group(g):
            kr = pl.ds(g * GP * PG, GP * PG)
            vr = pl.ds(g * GP * PG // 4, GP * PG // 4)
            return (halves(lambda p: k_hbm.at[kr, p, pl.ds(c0, nc)],
                           lambda h: kbuf.at[kr, :, h, :])
                    + halves(lambda p: v_hbm.at[vr, p, :, pl.ds(c0, nc)],
                             lambda h: vbuf.at[vr, :, :, h, :]))

        def w2_group(i):
            rows = pl.ds(W2_SPLIT[i], W2_SPLIT[i + 1] - W2_SPLIT[i])
            return halves(lambda p: w2_hbm.at[rows, p], lambda h: w2buf.at[rows, :, h, :])

        groups = ([whole(wq_hbm, wqbuf) + [(x_hbm, xbuf)]]
                  + [kv_group(NGRP - 1 - g) for g in range(NGRP)]
                  + [halves(lambda p: wo_hbm.at[:, p], lambda h: wobuf.at[:, :, :, h, :]),
                     whole(w1_hbm, w1buf) + whole(w3_hbm, w3buf)]
                  + [w2_group(i) for i in range(len(W2_SPLIT) - 1)])
        marker = len(groups)
        groups.append([(x_hbm, xbuf)])
        n_ring = len(groups)
        def k_rows(i, rows):
            return halves(lambda p: k_hbm.at[rows((NP - 2 + i) * PG), p, pl.ds(c0, nc)],
                          lambda h: kbuf.at[rows(i * PG), :, h, :])

        for i, n in enumerate((PG, RELOAD_ROWS)):
            groups.append([cp for g in range(n) for cp in k_rows(i, lambda r0: r0 + g)])
        late = n_ring + 1 + NSEM
        groups += [[]] * (late - len(groups))
        groups.append(k_rows(1, lambda r0: pl.ds(r0 + RELOAD_ROWS, PG - RELOAD_ROWS)))

        def copies(i):
            return [pltpu.make_async_copy(src, dst, sem.at[i % NSEM])
                    for src, dst in groups[i]]

        def start_dma(i):
            for cp in copies(i):
                cp.start()

        def wait(i):
            for cp in copies(i):
                cp.wait()
            if i + NSEM < n_ring:
                start_dma(i + NSEM)

        for i in range(NSEM):
            start_dma(i)

        k32 = kbuf.bitcast(U32)
        v32 = vbuf.bitcast(U32)
        wq32 = wqbuf.bitcast(U32)
        wo32 = wobuf.bitcast(U32)
        w13 = (w1buf.bitcast(U32), w3buf.bitcast(U32))
        w232 = w2buf.bitcast(U32)

        sub = lax.broadcasted_iota(jnp.int32, (8, LANES), 0)
        lane = lax.broadcasted_iota(jnp.int32, (8, LANES), 1)
        sub3 = lax.broadcasted_iota(jnp.int32, (8, PW), 0)
        lane3 = lax.broadcasted_iota(jnp.int32, (8, PW), 1)

        for r in range(4):
            half = U32(0x0000FFFF if r % 2 == 0 else 0xFFFF0000)
            lo = jnp.where(sub == r // 2, half, U32(0))
            hi = jnp.where(sub == 2 + r // 2, half, U32(0))
            mask_ref[r] = lo
            mask_ref[4 + r] = jnp.where(lane < DH - LANES, lo, hi)
            mask_ref[8 + r] = hi
            mask_ref[12 + r] = lo | hi
        p_refs = (p_ref, p2_ref)
        for pr in p_refs:
            pr[...] = jnp.zeros(pr.shape, F32)

        def dot(l32, r, free=True):
            del free
            return jnp.dot(pltpu.bitcast(l32, BF), r, preferred_element_type=F32)

        def tile_of(v, kk):
            return v[:, kk * LANES:(kk + 1) * LANES]

        def ln_stats(x):
            xb = x.astype(BF).astype(F32)
            m = jnp.mean(xb, axis=-1, keepdims=True)
            xc = xb - m
            v = jnp.mean(xc * xc, axis=-1, keepdims=True)
            return xb, m, lax.rsqrt(v + EPS)

        def raw_proj(xb, w32, c, mm=dot):
            lhs = _pack2(xb, jnp.ones_like(xb))
            acc = None
            for kk in range(DT):
                acc = _add(acc, mm(tile_of(lhs, kk), _rhs(w32, 8 * kk, c), False))
            return acc[0:8], acc[8:16]

        def col_bcast(v):
            return jnp.concatenate([v] * (LANES // 8), axis=0).T

        def vpu_fma(acc, w, xlo, xhi):
            w = pltpu.bitcast(w, BF).astype(F32)
            return _add(acc, w[0:8] * xlo + w[8:16] * xhi)

        def sub_sum(a):
            return jnp.broadcast_to(jnp.sum(a, axis=0, keepdims=True), a.shape)

        def expand_q(p, t, q):
            for r in range(4):
                lhs_ref[p % RING, 4 * t + r] = q & mask_ref[4 * t + r]

        def stage_q(p, mm=dot):
            acc = [None] * 3
            for kk in range(DT):
                for t in range(3):
                    acc[t] = _add(acc[t], mm(xn_ref[:, pl.ds(kk * LANES, LANES)],
                                             _rhs(wq32, 8 * kk, 3 * p + t))[0:8])
            for t in range(3):
                q = acc[t] * qscale
                expand_q(p, t, _pack2(q, q))

        def stage_qk(p, k, krow, mm=dot, scale=None):
            for j in range(2 * k, 2 * k + 2):
                acc = None
                for t in range(3):
                    for r in range(4):
                        acc = _add(acc, mm(lhs_ref[p % RING, 4 * t + r],
                                           _rhs(k32, krow + 8 * t, 4 * j + r))[0:8])
                s_ref[p % RING, j] = acc if scale is None else acc * scale

        def head_reduce(v, op, lane_op):
            for d in (1, 2):
                up = pltpu.roll(v, d, 0)
                down = pltpu.roll(v, 8 - d, 0)
                v = op(v, jnp.where(sub % (2 * d) >= d, up, down))
            return lane_op(v, axis=1, keepdims=True)

        def softmax(p, j0):
            s = s_ref[p % RING]
            m = head_reduce(jnp.max(s, axis=0), jnp.maximum, jnp.max)
            e = jnp.exp2(s - m)
            l = jnp.sum(e, axis=0)
            l = jnp.broadcast_to(head_reduce(l, jnp.add, jnp.sum), l.shape)
            lsum_ref[p] = l
            for j in range(j0, nc // 4):
                pk_ref[p % RING, j] = _pack2(e[j], e[j])
            return e, l

        def widened(p):
            return XCOLS if p else XCOLS[:NVX]

        def vx_slot(p, g, e):
            return (NP - 2) * PG + 3 * p + g // 8, (e - NVX) * 8 + g % 8

        def t_slot(p, j, n):
            if p == 0:
                return t0_ref, pl.ds(j, n)
            row = (NP - 2) * PG if p == 1 else p * PG if p < NP - 2 else 2 * PG + 2
            return k32, (row + j // nc, pl.ds(j % nc, n))

        def pv_chain(p, g, gate, n=1, store=True):
            acc = None
            for c in range(nc - MC[p]):
                row = (p % PRING) * prow + 8 * (c // 4) + 4 * (g // HG) + c % 4
                pb = gate()[pl.ds(row, 16, stride=0), :]
                w = v32[p * (PG // 4) + g // 4, pl.ds(g % 4, n), c]
                if c in widened(p):
                    e = XCOLS.index(c)
                    if e < NVX:
                        hi = vx_ref[p, e, pl.ds(g, n)]
                    else:
                        r0, s0 = vx_slot(p, g, e)
                        hi = k32[r0, pl.ds(s0, n)]
                    w = pltpu.bitcast(jnp.concatenate([w, hi], axis=1), F32)
                else:
                    w = pltpu.bitcast(w, BF).astype(F32)
                acc = _add(acc, w * pb)
            acc = pltpu.bitcast(acc, U32).reshape(2 * n, 8, LANES)
            if store:
                ref, idx = t_slot(p, 2 * g, 2 * n)
                ref[idx] = acc
            return acc

        def pv_mxu(p, cols, transposed, mm=dot):
            acc = [None] * 3
            cols = list(cols)
            for i0 in range(0, len(cols), 4):
                ls = {c: pk_ref[p % RING, c // 4] & mask_ref[12 + c % 4]
                      for c in cols[i0:i0 + 4]}
                for t in range(3):
                    for c, l in ls.items():
                        tile = _rhs4(v32, 3 * p + t, c)
                        if transposed:
                            res = mm(l, tile)
                        else:
                            res = lax.dot_general(
                                pltpu.bitcast(l, BF), tile, (((1,), (1,)), ((), ())),
                                preferred_element_type=F32)
                        acc[t] = _add(acc[t], res[0:8])
            return jnp.concatenate(acc, axis=1)

        def own_head(o):
            return jnp.where((sub3 < 4) == (lane3 < DH), o, 0.0)

        def finish_o(p, o, nt=3):
            linv = 1.0 / lsum_ref[p]
            la = jnp.broadcast_to(linv[0:1], linv.shape)
            lb = jnp.broadcast_to(linv[4:5], linv.shape)
            linv = [la, jnp.where(lane < DH - LANES, la, lb), lb]
            o = jnp.sum(o, axis=0, keepdims=True) * jnp.concatenate(linv[:nt], axis=1)
            ob_ref[p, :, 0:nt * LANES] = _pack2(o, o)

        def mxu_tiles(p):
            return TAIL_T if p == NP - 2 else 3

        def stage_reduce(p):
            o = None
            nt = mxu_tiles(p)
            if p < NP - 1:
                slots = [t_slot(p, 16 * t, 16) for t in range(nt)]
                tt = jnp.concatenate([ref[idx] for ref, idx in slots])
                tt = pltpu.bitcast(tt.reshape(nt * LANES, LANES), F32)
                o = jnp.sum(tt.T.reshape(LANES // 8, 8, nt * LANES), axis=0)
            if p == NP - 1 or MC[p]:
                o = _add(o, own_head(om_ref[p]))
            finish_o(p, o, nt)

        def stage_wo(tiles, mm=dot):
            for c in range(DT):
                acc = y_ref[:, pl.ds(c * LANES, LANES)]
                for p, t in tiles:
                    acc = acc + mm(ob_ref[p, :, pl.ds(t * LANES, LANES)],
                                   _rhs4(wo32, 3 * p + t, c))[0:8]
                y_ref[:, pl.ds(c * LANES, LANES)] = acc

        def begin_attention(x):
            y_ref[:, 0:D] = x
            xb, m, r = ln_stats(x)
            xn = (xb - m) * r
            xn_ref[:, 0:D] = _pack2(xn, xn)
            return xb, m, r

        wait(0)
        begin_attention(jnp.broadcast_to(xbuf[...].astype(F32), (8, D)))

        def pair1(i, carry):
            p = NP - 1 - i
            stage_q(p)
            for k in range(nk):
                stage_qk(p, k, p * PG)
            softmax(p, 0)
            finish_o(p, own_head(pv_mxu(p, range(nc), False)))
            om_ref[p] = jnp.zeros(om_ref.shape[1:], F32)
            qpk_ref[p] = jnp.zeros((8, LANES), U32)
            t0_ref[p] = jnp.zeros((8, LANES), U32)
            cs_ref[p] = jnp.zeros((8, LANES), F32)

            first = 0
            for pp in range(NP - 1):
                first = jnp.where(p == pp, nc - MC[pp], first)

            def transpose_v(c, carry2):
                for t in range(3):
                    tile = _rhs4(v32, 3 * p + t, c)
                    v32[pl.ds(2 * (3 * p + t), 2), :, c] = pltpu.bitcast(
                        tile.T, U32).reshape(2, 4, 8, LANES)
                return carry2

            lax.fori_loop(first, nc, transpose_v, 0)

            def widen(es):
                for g in range(0, PG, 4):
                    for e in es:
                        idx = (p * (PG // 4) + g // 4, slice(None), XCOLS[e])
                        w = pltpu.bitcast(pltpu.bitcast(v32[idx], BF).astype(F32), U32)
                        v32[idx] = w[:, 0:8]
                        if e < NVX:
                            vx_ref[p, e, pl.ds(g, 4)] = w[:, 8:16]
                        else:
                            r0, s0 = vx_slot(p, g, e)
                            k32[r0, pl.ds(s0, 4)] = w[:, 8:16]

            pl.when(p < NP - 1)(functools.partial(widen, range(NVX)))
            pl.when((p < NP - 1) & (p > 0))(
                functools.partial(widen, range(NVX, len(XCOLS))))
            return carry

        def group1(gi, row):
            for i in range(NGRP):
                pl.when(gi == i)(functools.partial(wait, 1 + i))
            lax.fori_loop(gi * GP, (gi + 1) * GP, pair1, 0)
            return row + PRING * prow // NGRP

        fence_row = pl.multiple_of(lax.fori_loop(0, NGRP, group1, 0), 8)
        wait(1 + NGRP)

        def woloop(p2, carry):
            stage_wo([(2 * p2 + i, t) for i in range(2) for t in range(3)])
            return carry

        lax.fori_loop(0, NP // 2, woloop, 0)

        x = y_ref[:, 0:D]
        xb, m, r = ln_stats(x)
        wait(2 + NGRP)
        gu = []
        for j in range(2 * FT):
            raw, cs = raw_proj(xb, w13[j % 2], j // 2)
            cs_ref[j] = cs
            gu.append((raw - m * cs) * r)
        hs = [_swiglu(g, u) for g, u in zip(gu[0::2], gu[1::2])]
        for kk in range(W2_MXU // 8, FT):
            p_ref[pl.ds(LANES * kk - 16 * W2_MXU, LANES), :] = col_bcast(
                hs[kk].astype(BF).astype(F32))
        hs = [_pack2(hh, hh) for hh in hs[:W2_MXU // 8]]
        cols = [tile_of(x, c) for c in range(DT)]
        part = [None] * DT
        for i in range(len(W2_SPLIT) - 1):
            wait(3 + NGRP + i)
            g0, g1 = W2_SPLIT[i], W2_SPLIT[i + 1]
            for c in range(DT):
                if g1 <= W2_MXU:
                    for kk in range(g0 // 8, g1 // 8):
                        cols[c] = cols[c] + dot(hs[kk], _rhs(w232, 8 * kk, c))[0:8]
                else:
                    for g in range(g0, g1):
                        row = 16 * (g - W2_MXU)
                        part[c] = vpu_fma(part[c], w232[g, c], p_ref[pl.ds(row, 8), :],
                                          p_ref[pl.ds(row + 8, 8), :])
        x = jnp.concatenate([cc + sub_sum(a) for cc, a in zip(cols, part)], axis=1)

        xb, m, r = begin_attention(x)
        rq = r * qscale

        def run_block(blk, chains, items, n_link, first, last_off, start, end):
            links = []
            y_vpu = None
            for j, (p, g) in enumerate(chains[:n_link]):
                tail = end and g >= 8 * TAIL_T
                acc = pv_chain(p, g, lambda: p_refs[g % 2], store=not tail)
                dep = acc[0] | acc[1]
                if tail:
                    hd = 4 * (g // HG)
                    linv = jnp.broadcast_to((1.0 / lsum_ref[p])[hd:hd + 1], (8, LANES))
                    oc = jnp.sum(pltpu.bitcast(acc, F32), axis=2, keepdims=True) * linv
                    oc = oc.astype(BF).astype(F32).reshape(16, LANES)
                    w = pltpu.bitcast(wo32[6 * p + g // 4, g % 4], BF).astype(F32) * oc
                    y_vpu = _add(y_vpu, w[:, 0:8] + w[:, 8:16])
                links.extend([(LINK0[blk] + LINKSTEP[blk] * j, dep)] * LINK_REP[blk])
            if start:
                xcol = [col_bcast(tile_of(xb, kk)) - m[0:1] for kk in range(DT)]
                links.extend([(XC_LINK, _bits_or(xc[LANES - 8:] for xc in xcol))] * 4)
            pops = []
            probs = {}
            busy = []

            def mm(l32, rr, free=True):
                links.sort(key=lambda lk: lk[0])
                if free and links and len(pops) >= links[0][0]:
                    l32 = jnp.where(sub < 4, l32, links.pop(0)[1])
                pops.append(dot(l32, rr))
                return pops[-1]

            for it in items:
                kind, p = it[0], it[1]
                if kind == 'fq':
                    for t in range(3):
                        raw, cs = raw_proj(xb, wq32, 3 * p + t, mm)
                        q = raw - m * cs
                        q = q if p == 0 else q * rq
                        expand_q(p, t, _pack2(q, q))
                elif kind == 'q':
                    stage_q(p, mm)
                    busy.append((len(pops) - Q_A[blk], len(pops) - Q_B[blk], Q_W[blk]))
                elif kind == 'qx':
                    for t in range(3):
                        expand_q(p, t, qpk_ref[3 * VQ.index(p) + t])
                elif kind == 'qk':
                    stage_qk(p, it[2], p % (NP - 2) * PG, mm, rq if p == 0 else None)
                elif kind == 'sm':
                    e, l = softmax(p, 0 if p == NP - 1 else (nc - MC[p]) // 4)
                    lag = SM_LAG0 if p == 0 else SM_LAG[blk]
                    pos = len(pops) + (lag if pops else lag - 14)
                    links.append((pos, pltpu.bitcast(l, U32)))
                    busy.append((pos - SM_A[blk], pos - SM_B[blk], SM_W[blk]))
                    if p < NP - 1:
                        probs[p] = e
                elif kind == 'pvm':
                    o = pv_mxu(p, range(it[2], it[3]), True, mm)
                    om_ref[p] = o + om_ref[p] if it[4] else o
                elif kind == 'reload':
                    start_dma(n_ring + p)
                elif kind == 'red':
                    stage_reduce(p)
                elif kind == 'wo':
                    busy.append((len(pops) - RED_A[blk], len(pops) - RED_B[blk], RED_W[blk]))
                    stage_wo([(pp, t) for pp in it[1:] for t in range(mxu_tiles(pp))], mm)

            def fence(buf, a):
                buf[pl.ds(fence_row, 8), :] = pops[a][0:8]

            if start:
                nkg = D // 16

                def xslot(kg):
                    u = kg // VQ_UNIT
                    return p_refs[u % 2], 16 * (u // 2 * VQ_UNIT + kg % VQ_UNIT)

                for kg in range(nkg):
                    buf, row = xslot(kg)
                    buf[pl.ds(row, 16), :] = xcol[kg // 8][16 * (kg % 8):16 * (kg % 8) + 16]
                for i, p in enumerate(VQ):
                    acc = None
                    for kg in range(nkg):
                        buf, row = xslot(kg)
                        if kg % VQ_UNIT == 0:
                            a = (i * nkg + kg) * (first - VQ_FIRST) // (len(VQ) * nkg)
                            fence(buf, VQ_FIRST + a // 2 * 2)
                        w = pltpu.bitcast(wq32[kg, pl.ds(3 * p, 3)], BF).astype(F32)
                        w = w * buf[pl.ds(row, 16), :]
                        acc = _add(acc, w[:, 0:8] + w[:, 8:16])
                    for t in range(3):
                        q = sub_sum(acc[t]) * rq
                        qpk_ref[3 * i + t] = _pack2(q, q)

            def store_probs(p):
                e = probs.pop(p)
                for pr in p_refs:
                    for j in range((nc - MC[p] + 3) // 4):
                        pr[pl.ds((p % PRING) * prow + 8 * j, 8), :] = e[j]

            rest = chains[n_link:]
            if rest:
                runs, i = [], 0
                while i < len(rest):
                    p, g = rest[i]
                    runs.append((p, g, min(GSHARE - g % GSHARE, len(rest) - i)))
                    i += runs[-1][2]
                cost = [n * (XCOST[blk] if c in widened(p) else 1.0)
                        for p, _, n in runs for c in range(nc - MC[p])]
                n_items = len(cost)
                n_units = (len(pops) - last_off - first) // FSTEP + 1
                less = [0.0] * n_units
                for lo, hi, w in busy:
                    us = [u for u in range(n_units) if lo <= first + u * FSTEP < hi]
                    for u in us:
                        less[u] += w / len(us)
                per = (sum(cost) + sum(less)) / n_units
                unit_of, total, used = [], 0.0, 0.0
                for u in range(n_units):
                    total += per - less[u]
                    while len(unit_of) < n_items and (
                            used + cost[len(unit_of)] / 2 < total or u + 1 == n_units):
                        used += cost[len(unit_of)]
                        unit_of.append(u)
                state = [0, -1, 1]

                def gate():
                    u = unit_of[state[0]]
                    state[0] += 1
                    if u != state[1]:
                        state[1] = u
                        state[2] += 1
                        fence(p_refs[state[2] % 2], first + u * FSTEP)
                    return p_refs[state[2] % 2]

            for p, g, n in runs if rest else []:
                if g == 0:
                    for i in range(state[0], n_items):
                        if unit_of[i] != state[1] or state[1] + 1 == n_units:
                            break
                        unit_of[i] += 1
                if p in probs:
                    store_probs(p)
                pv_chain(p, g, gate, n)
            for p in list(probs):
                store_probs(p)
            if end:
                x = y_ref[:, 0:D]
                if y_vpu is not None:
                    x = x + jnp.concatenate([sub_sum(y_vpu[c]) for c in range(DT)], axis=1)
                last_ffn(x, mm, len(pops), links)

        def last_ffn(x, mm, base, links):
            xb, m, r = ln_stats(x)
            lhs = _pack2(xb, xb)
            xcol = [col_bcast(tile_of(xb, kk)) for kk in range(UP_K)]
            links.extend([(base + UX_LINK, _bits_or(xc[LANES - 8:] for xc in xcol))] * 4)
            j0 = 2 * (FT - UP_COLS)
            part = {}
            for j in range(j0, 2 * FT):
                acc = None
                for i in range(8):
                    for kk in range(UP_K):
                        xc = xcol[kk][16 * i:16 * i + 16]
                        acc = vpu_fma(acc, w13[j % 2][8 * kk + i, j // 2], xc[0:8], xc[8:16])
                part[j] = sub_sum(acc)
                links.append((base + int(UP_LINK0 + UP_LINKSTEP * (j - j0)),
                              pltpu.bitcast(part[j], U32)))
            work = [(j, kk) for kk in range(DT) for j in range(UP_KM)]
            work += [(j, kk) for j in range(UP_KM, 2 * FT)
                     for kk in range(UP_K if j in part else 0, DT)]
            for j, kk in work:
                part[j] = _add(part.get(j), mm(tile_of(lhs, kk),
                                               _rhs(w13[j % 2], 8 * kk, j // 2))[0:8])
            gu = [(part[j] - m * cs_ref[j]) * r for j in range(2 * FT)]
            hs = [_swiglu(g, u) for g, u in zip(gu[0::2], gu[1::2])]
            cols = [tile_of(x, c) for c in range(DT)]
            for kk in range(DOWN_K, FT):
                hh = _pack2(hs[kk], hs[kk])
                for c in range(DT):
                    cols[c] = cols[c] + mm(hh, _rhs(w232, 8 * kk, c))[0:8]
            hcol = [col_bcast(hs[kk].astype(BF).astype(F32)) for kk in range(DOWN_K)]
            acc = [None] * DT
            for i in range(8):
                for kk in range(DOWN_K):
                    for c in range(DT):
                        acc[c] = vpu_fma(acc[c], w232[8 * kk + i, c],
                                         hcol[kk][16 * i:16 * i + 8],
                                         hcol[kk][16 * i + 8:16 * i + 16])
            cols = [cc + sub_sum(a) for cc, a in zip(cols, acc)]
            o_ref[...] = jnp.concatenate(cols, axis=1)[0:1].astype(o_ref.dtype)

        blocks = _plan(nc)
        for b, plan in enumerate(blocks):
            end = b == len(blocks) - 1
            if b > 0:
                wait(marker if end else n_ring + b - 1)
            if b == 1:
                start_dma(late)
            if b == 2:
                wait(late)
            run_block(b, *plan, b == 0, end)

    return kernel


@jax.jit
def pallas_interleave_layers__sliding_block_cached__glu_gated_swiglu__decode_kernel(
    A_x: jax.Array,
    A_k_cache: jax.Array,
    A_v_cache: jax.Array,
    A_wq: jax.Array,
    A_wo: jax.Array,
    B_x: jax.Array,
    B_w1: jax.Array,
    B_w3: jax.Array,
    B_w2: jax.Array,
):
    sk = A_k_cache.shape[2]
    win = min(4096, max(256, sk // 4))
    nt_total, nc = sk // LANES, win // LANES

    def kv_view(a):
        return _tile_view(jnp.swapaxes(a, 2, 3).reshape(H * DH, sk))

    def view4(t):
        return t.reshape(t.shape[0] // 4, 2, 4, t.shape[2], 8, LANES)

    def wbuf(r, c):
        return pltpu.VMEM((r // 16, c // LANES, 16, LANES), BF)

    def wbuf4(r, c):
        return pltpu.VMEM((r // 64, 4, c // LANES, 16, LANES), BF)

    any_spec = pl.BlockSpec(memory_space=pl.ANY)
    out = pl.pallas_call(
        _make_kernel(nt_total, nc),
        out_shape=jax.ShapeDtypeStruct((1, D), A_x.dtype),
        in_specs=[any_spec] * 8,
        out_specs=pl.BlockSpec(memory_space=pltpu.VMEM),
        scratch_shapes=[
            wbuf(H * DH, win), wbuf4(H * DH, win),
            wbuf(D, H * DH), wbuf4(H * DH, D),
            wbuf(D, F), wbuf(D, F), wbuf(F, D),
            pltpu.VMEM((NP - 1, NVX, PG, 8, LANES), U32),
            pltpu.VMEM((2 * PG, 8, LANES), U32),
            pltpu.VMEM((RING, 12, 8, LANES), U32),
            pltpu.VMEM((RING, nc // 4, 8, LANES), F32),
            pltpu.VMEM((PRING * 2 * nc + 32, LANES), F32),
            pltpu.VMEM((PRING * 2 * nc + 32, LANES), F32),
            pltpu.VMEM((RING, nc // 4, 8, LANES), U32),
            pltpu.VMEM((NP, 8, LANES), F32),
            pltpu.VMEM((NP, 8, PW), F32),
            pltpu.VMEM((NP, 8, PW), U32),
            pltpu.VMEM((16, 8, LANES), U32),
            pltpu.VMEM((2 * FT, 8, LANES), F32),
            pltpu.VMEM((16, 8, LANES), U32),
            pltpu.VMEM((8, 1024), U32),
            pltpu.VMEM((8, 1024), F32),
            pltpu.VMEM((1, D), BF),
            pltpu.SemaphoreType.DMA((NSEM,)),
        ],
        compiler_params=pltpu.CompilerParams(
            vmem_limit_bytes=128 * 1024 * 1024),
    )(A_x.reshape(1, D), kv_view(A_k_cache), view4(kv_view(A_v_cache)),
      _tile_view(A_wq), view4(_tile_view(A_wo)),
      _tile_view(B_w1), _tile_view(B_w3), _tile_view(B_w2))
    return out.reshape(A_x.shape)
```

```python
import functools
import math

import jax
import jax.numpy as jnp
from jax import lax
import jax.experimental.pallas as pl
import jax.experimental.pallas.tpu as pltpu

D = 640
H = 32
DH = 192
F = 1536
LANES = 128
EPS = 1e-5

NP = H // 2
PG = 2 * DH // 16
HG = DH // 16
PW = 2 * DH
DT = D // LANES
FT = F // LANES

GP = 4
NGRP = NP // GP
W2_SPLIT = (0, 56, 80, 92, 96)
W2_MXU = 80
RELOAD_ROWS = 8
NSEM = 3
RING = 4
PRING = 6

MC = (2, 2, 2, 2, 2, 2, 2, 2, 3, 3, 2, 2, 2, 0, 0)
XCOLS = (1, 7, 10, 16, 22, 25, 4, 13, 19, 28)
NVX = 6
VQ = (11, 12, 13, 14, 15)
V_END = (172, 299, 349)
TILES = (1060, 661, 291)
XCOST = (0.67, 0.77, 0.67, 0.67)
GSHARE = 2
PVM_AFTER = 2
WO_START = (0, 80, 65, 999)
WO_GAP = (0, 72, 60, 12)
WO_KEEP = 4
FIRST = (160, 2, 0)
LAST_OFF = (8, 6, 6)
VQ_FIRST = 30
VQ_UNIT = 4
XC_LINK = 50
SM_LAG = (60, 64, 64, 64)
ANCH = ((0, 4), (0, 1, 4), (4, 1))
SM_MIN = 40
SM_LAG0 = 52
RED_W = (10, 10, 13, 10)
RED_A = (40, 40, 32, 40)
RED_B = (16, 28, 20, 16)
Q_W = (4, 4, 4, 4)
Q_A = (18, 12, 12, 12)
Q_B = (-4, -4, -4, -4)
SM_W = (4, 4, 7, 7)
SM_A = (56, 56, 64, 56)
SM_B = (30, 48, 36, 30)
NLINK = (0, 4, 3)
LINK0 = (8, 8, 8, 10)
LINKSTEP = (4, 5, 3, 7)
LINK_REP = (1, 1, 4, 1)
TAIL_T = 2
WO_JOINT = 2
UP_KM = 4
UP_K = 3
UP_COLS = 6
UP_LINK0 = 58
UP_LINKSTEP = 5.5
UX_LINK = 44
DOWN_K = 4

U32 = jnp.uint32
BF = jnp.bfloat16
F32 = jnp.float32


def _tile_view(w):
    r, c = w.shape
    return jnp.swapaxes(w.reshape(r // 16, 2, 8, c // LANES, LANES), 2, 3)


def _rhs(w32, g0, c):
    return pltpu.bitcast(w32[pl.ds(g0, 8), c].reshape(64, LANES), BF)


def _rhs4(w32, tile, c):
    return pltpu.bitcast(w32[pl.ds(2 * tile, 2), :, c].reshape(64, LANES), BF)


def _swiglu(g, u):
    hg = 0.5 * g
    return hg * (1.0 + jnp.tanh(hg)) * u


def _pack2(lo, hi):
    return pltpu.bitcast(jnp.concatenate([lo, hi], axis=0).astype(BF), U32)


def _add(a, b):
    return b if a is None else a + b


def _bits_or(vals):
    return functools.reduce(lambda a, b: a | b, [pltpu.bitcast(v, U32) for v in vals])


def _plan(nc):
    nk = nc // 8
    seq = [('fq', 0), ('fq', 1)]
    for p in range(NP):
        if 1 <= p < NP - 1:
            seq.append(('qx' if p + 1 in VQ else 'q', p + 1))
        for k in range(nk):
            if k == PVM_AFTER and p > 0 and MC[p - 1]:
                seq.append(('pvm', p - 1, nc - MC[p - 1], nc, False))
            seq.append(('qk', p, k))
        if p < 2:
            seq.append(('reload', p))
        seq.append(('sm', p))
    seq += [('pvm', NP - 1, c, c + 4, c > 0) for c in range(0, nc, 4)]
    last_pv = seq[-nc // 4]

    def tiles(it):
        if it[0] == 'pvm':
            return 3 * (it[3] - it[2])
        return dict(fq=15, q=15, wo=15, qk=24, sm=0, qx=0, reload=0)[it[0]]

    chains = [(p, g) for p in range(NP - 1) for g in range(PG)]
    blocks = []
    v0 = done = 0
    for b in range(len(V_END) + 1):
        final = b == len(V_END)
        v1 = len(chains) if final else V_END[b]
        todo = list(range(done, v0 // PG))
        done = v0 // PG
        budget = 10 ** 9 if final else TILES[b] - 15 * len(todo)
        body = []
        used = 0
        while seq and used + tiles(seq[0]) // 2 <= budget:
            body.append(seq.pop(0))
            used += tiles(body[-1])
        while body[-1][0] in ('sm', 'qx'):
            seq.insert(0, body.pop())
        left = 0
        for i in range(len(body) - 1, -1, -1):
            if body[i][0] == 'sm' and left < SM_MIN and not final:
                seq.insert(0, body.pop(i))
            else:
                left += tiles(body[i])
        assert b > 0 or not any(it[1] in VQ for it in body)
        keep = WO_KEEP if last_pv in body else 0
        items = [('red', p) for p in todo]
        used = 0
        nxt = WO_START[b]
        for it in body:
            if it == last_pv:
                while todo:
                    items.append(('wo', todo.pop(0)))
            if len(todo) > keep and used >= nxt:
                items.append(('wo', todo.pop(0)))
                nxt = used + WO_GAP[b]
            items.append(it)
            used += tiles(it)
        items += [('wo', p) for p in todo]
        if final:
            assert done == NP - 2
            assert TAIL_T == 3 or (MC[NP - 2] == 0 and v0 % PG <= 8 * TAIL_T)
            for p in (NP - 1, NP - 2):
                items += [('red', p), ('wo', p)]
            joint = [it for it in items if it[0] == 'wo'][-WO_JOINT:]
            items = [it for it in items if it not in joint]
            items.append(('wo', *[it[1] for it in joint]))
            blocks.append((chains[v0:v1], items, v1 - v0, 0, 0))
        else:
            blocks.append((chains[v0:v1], items, NLINK[b], FIRST[b], LAST_OFF[b]))
        v0 = v1
    seen = set()
    for b, (chs, items, n_link, _, _) in enumerate(blocks):
        assert all(it[1] - (NP - 2) < b for it in items if it[0] == 'qk')
        assert all(p in seen for p, _ in chs[:n_link])
        seen |= {it[1] for it in items if it[0] == 'sm'}
        assert all(p in seen for p, _ in chs)
        assert max(seen) - chs[-1][0] < PRING
    return blocks


def _make_kernel(n_tiles_total, nc):
    c0 = n_tiles_total - nc
    qscale = DH ** -0.5 * math.log2(math.e)
    prow = 2 * nc
    nk = nc // 8

    def kernel(x_hbm, k_hbm, v_hbm, wq_hbm, wo_hbm, w1_hbm, w3_hbm, w2_hbm,
               o_ref,
               kbuf, vbuf, wqbuf, wobuf, w1buf, w3buf, w2buf,
               vx_ref, t0_ref, lhs_ref, s_ref, p_ref, p2_ref, pk_ref, lsum_ref, om_ref,
               ob_ref, mask_ref, cs_ref, qpk_ref, xn_ref, y_ref, xbuf, sem):
        def halves(src, dst):
            return [(src(par), dst(pl.ds(8 * par, 8))) for par in range(2)]

        def whole(src, dst):
            return halves(lambda p: src.at[:, p], lambda h: dst.at[:, :, h, :])

        def kv_group(g):
            kr = pl.ds(g * GP * PG, GP * PG)
            vr = pl.ds(g * GP * PG // 4, GP * PG // 4)
            return (halves(lambda p: k_hbm.at[kr, p, pl.ds(c0, nc)],
                           lambda h: kbuf.at[kr, :, h, :])
                    + halves(lambda p: v_hbm.at[vr, p, :, pl.ds(c0, nc)],
                             lambda h: vbuf.at[vr, :, :, h, :]))

        def w2_group(i):
            rows = pl.ds(W2_SPLIT[i], W2_SPLIT[i + 1] - W2_SPLIT[i])
            return halves(lambda p: w2_hbm.at[rows, p], lambda h: w2buf.at[rows, :, h, :])

        groups = ([whole(wq_hbm, wqbuf) + [(x_hbm, xbuf)]]
                  + [kv_group(NGRP - 1 - g) for g in range(NGRP)]
                  + [halves(lambda p: wo_hbm.at[:, p], lambda h: wobuf.at[:, :, :, h, :]),
                     whole(w1_hbm, w1buf) + whole(w3_hbm, w3buf)]
                  + [w2_group(i) for i in range(len(W2_SPLIT) - 1)])
        marker = len(groups)
        groups.append([(x_hbm, xbuf)])
        n_ring = len(groups)
        def k_rows(i, rows):
            return halves(lambda p: k_hbm.at[rows((NP - 2 + i) * PG), p, pl.ds(c0, nc)],
                          lambda h: kbuf.at[rows(i * PG), :, h, :])

        for i, n in enumerate((PG, RELOAD_ROWS)):
            groups.append([cp for g in range(n) for cp in k_rows(i, lambda r0: r0 + g)])
        late = n_ring + 1 + NSEM
        groups += [[]] * (late - len(groups))
        groups.append(k_rows(1, lambda r0: pl.ds(r0 + RELOAD_ROWS, PG - RELOAD_ROWS)))

        def copies(i):
            return [pltpu.make_async_copy(src, dst, sem.at[i % NSEM])
                    for src, dst in groups[i]]

        def start_dma(i):
            for cp in copies(i):
                cp.start()

        def wait(i):
            for cp in copies(i):
                cp.wait()
            if i + NSEM < n_ring:
                start_dma(i + NSEM)

        for i in range(NSEM):
            start_dma(i)

        k32 = kbuf.bitcast(U32)
        v32 = vbuf.bitcast(U32)
        wq32 = wqbuf.bitcast(U32)
        wo32 = wobuf.bitcast(U32)
        w13 = (w1buf.bitcast(U32), w3buf.bitcast(U32))
        w232 = w2buf.bitcast(U32)

        sub = lax.broadcasted_iota(jnp.int32, (8, LANES), 0)
        lane = lax.broadcasted_iota(jnp.int32, (8, LANES), 1)
        sub3 = lax.broadcasted_iota(jnp.int32, (8, PW), 0)
        lane3 = lax.broadcasted_iota(jnp.int32, (8, PW), 1)

        for r in range(4):
            half = U32(0x0000FFFF if r % 2 == 0 else 0xFFFF0000)
            lo = jnp.where(sub == r // 2, half, U32(0))
            hi = jnp.where(sub == 2 + r // 2, half, U32(0))
            mask_ref[r] = lo
            mask_ref[4 + r] = jnp.where(lane < DH - LANES, lo, hi)
            mask_ref[8 + r] = hi
            mask_ref[12 + r] = lo | hi
        p_refs = (p_ref, p2_ref)
        for pr in p_refs:
            pr[...] = jnp.zeros(pr.shape, F32)

        def dot(l32, r, free=True):
            del free
            return jnp.dot(pltpu.bitcast(l32, BF), r, preferred_element_type=F32)

        def tile_of(v, kk):
            return v[:, kk * LANES:(kk + 1) * LANES]

        def ln_stats(x):
            xb = x.astype(BF).astype(F32)
            m = jnp.mean(xb, axis=-1, keepdims=True)
            xc = xb - m
            v = jnp.mean(xc * xc, axis=-1, keepdims=True)
            return xb, m, lax.rsqrt(v + EPS)

        def raw_proj(xb, w32, c, mm=dot):
            lhs = _pack2(xb, jnp.ones_like(xb))
            acc = None
            for kk in range(DT):
                acc = _add(acc, mm(tile_of(lhs, kk), _rhs(w32, 8 * kk, c), False))
            return acc[0:8], acc[8:16]

        def col_bcast(v):
            return jnp.concatenate([v] * (LANES // 8), axis=0).T

        def vpu_fma(acc, w, xlo, xhi):
            w = pltpu.bitcast(w, BF).astype(F32)
            return _add(acc, w[0:8] * xlo + w[8:16] * xhi)

        def sub_sum(a):
            return jnp.broadcast_to(jnp.sum(a, axis=0, keepdims=True), a.shape)

        def expand_q(p, t, q):
            for r in range(4):
                lhs_ref[p % RING, 4 * t + r] = q & mask_ref[4 * t + r]

        def stage_q(p, mm=dot):
            acc = [None] * 3
            for kk in range(DT):
                for t in range(3):
                    acc[t] = _add(acc[t], mm(xn_ref[:, pl.ds(kk * LANES, LANES)],
                                             _rhs(wq32, 8 * kk, 3 * p + t))[0:8])
            for t in range(3):
                q = acc[t] * qscale
                expand_q(p, t, _pack2(q, q))

        def stage_qk(p, k, krow, mm=dot, scale=None):
            for j in range(2 * k, 2 * k + 2):
                acc = None
                for t in range(3):
                    for r in range(4):
                        acc = _add(acc, mm(lhs_ref[p % RING, 4 * t + r],
                                           _rhs(k32, krow + 8 * t, 4 * j + r))[0:8])
                s_ref[p % RING, j] = acc if scale is None else acc * scale

        def head_reduce(v, op, lane_op):
            for d in (1, 2):
                up = pltpu.roll(v, d, 0)
                down = pltpu.roll(v, 8 - d, 0)
                v = op(v, jnp.where(sub % (2 * d) >= d, up, down))
            return lane_op(v, axis=1, keepdims=True)

        def softmax(p, j0):
            s = s_ref[p % RING]
            m = head_reduce(jnp.max(s, axis=0), jnp.maximum, jnp.max)
            e = jnp.exp2(s - m)
            l = jnp.sum(e, axis=0)
            l = jnp.broadcast_to(head_reduce(l, jnp.add, jnp.sum), l.shape)
            lsum_ref[p] = l
            for j in range(j0, nc // 4):
                pk_ref[p % RING, j] = _pack2(e[j], e[j])
            return e, l

        def widened(p):
            return XCOLS if p else XCOLS[:NVX]

        def vx_slot(p, g, e):
            return (NP - 2) * PG + 3 * p + g // 8, (e - NVX) * 8 + g % 8

        def t_slot(p, j, n):
            if p == 0:
                return t0_ref, pl.ds(j, n)
            row = (NP - 2) * PG if p == 1 else p * PG if p < NP - 2 else 2 * PG + 2
            return k32, (row + j // nc, pl.ds(j % nc, n))

        def pv_chain(p, g, gate, n=1, store=True):
            acc = None
            for c in range(nc - MC[p]):
                row = (p % PRING) * prow + 8 * (c // 4) + 4 * (g // HG) + c % 4
                pb = gate()[pl.ds(row, 16, stride=0), :]
                w = v32[p * (PG // 4) + g // 4, pl.ds(g % 4, n), c]
                if c in widened(p):
                    e = XCOLS.index(c)
                    if e < NVX:
                        hi = vx_ref[p, e, pl.ds(g, n)]
                    else:
                        r0, s0 = vx_slot(p, g, e)
                        hi = k32[r0, pl.ds(s0, n)]
                    w = pltpu.bitcast(jnp.concatenate([w, hi], axis=1), F32)
                else:
                    w = pltpu.bitcast(w, BF).astype(F32)
                acc = _add(acc, w * pb)
            acc = pltpu.bitcast(acc, U32).reshape(2 * n, 8, LANES)
            if store:
                ref, idx = t_slot(p, 2 * g, 2 * n)
                ref[idx] = acc
            return acc

        def pv_mxu(p, cols, transposed, mm=dot):
            acc = [None] * 3
            cols = list(cols)
            for i0 in range(0, len(cols), 4):
                ls = {c: pk_ref[p % RING, c // 4] & mask_ref[12 + c % 4]
                      for c in cols[i0:i0 + 4]}
                for t in range(3):
                    for c, l in ls.items():
                        tile = _rhs4(v32, 3 * p + t, c)
                        if transposed:
                            res = mm(l, tile)
                        else:
                            res = lax.dot_general(
                                pltpu.bitcast(l, BF), tile, (((1,), (1,)), ((), ())),
                                preferred_element_type=F32)
                        acc[t] = _add(acc[t], res[0:8])
            return jnp.concatenate(acc, axis=1)

        def own_head(o):
            return jnp.where((sub3 < 4) == (lane3 < DH), o, 0.0)

        def finish_o(p, o, nt=3):
            linv = 1.0 / lsum_ref[p]
            la = jnp.broadcast_to(linv[0:1], linv.shape)
            lb = jnp.broadcast_to(linv[4:5], linv.shape)
            linv = [la, jnp.where(lane < DH - LANES, la, lb), lb]
            o = jnp.sum(o, axis=0, keepdims=True) * jnp.concatenate(linv[:nt], axis=1)
            ob_ref[p, :, 0:nt * LANES] = _pack2(o, o)

        def mxu_tiles(p):
            return TAIL_T if p == NP - 2 else 3

        def stage_reduce(p):
            o = None
            nt = mxu_tiles(p)
            if p < NP - 1:
                slots = [t_slot(p, 16 * t, 16) for t in range(nt)]
                tt = jnp.concatenate([ref[idx] for ref, idx in slots])
                tt = pltpu.bitcast(tt.reshape(nt * LANES, LANES), F32)
                o = jnp.sum(tt.T.reshape(LANES // 8, 8, nt * LANES), axis=0)
            if p == NP - 1 or MC[p]:
                o = _add(o, own_head(om_ref[p]))
            finish_o(p, o, nt)

        def stage_wo(tiles, mm=dot):
            for c in range(DT):
                acc = y_ref[:, pl.ds(c * LANES, LANES)]
                for p, t in tiles:
                    acc = acc + mm(ob_ref[p, :, pl.ds(t * LANES, LANES)],
                                   _rhs4(wo32, 3 * p + t, c))[0:8]
                y_ref[:, pl.ds(c * LANES, LANES)] = acc

        def begin_attention(x):
            y_ref[:, 0:D] = x
            xb, m, r = ln_stats(x)
            xn = (xb - m) * r
            xn_ref[:, 0:D] = _pack2(xn, xn)
            return xb, m, r

        wait(0)
        begin_attention(jnp.broadcast_to(xbuf[...].astype(F32), (8, D)))

        def pair1(i, carry):
            p = NP - 1 - i
            stage_q(p)
            for k in range(nk):
                stage_qk(p, k, p * PG)
            softmax(p, 0)
            finish_o(p, own_head(pv_mxu(p, range(nc), False)))
            om_ref[p] = jnp.zeros(om_ref.shape[1:], F32)
            qpk_ref[p] = jnp.zeros((8, LANES), U32)
            t0_ref[p] = jnp.zeros((8, LANES), U32)
            cs_ref[p] = jnp.zeros((8, LANES), F32)

            first = 0
            for pp in range(NP - 1):
                first = jnp.where(p == pp, nc - MC[pp], first)

            def transpose_v(c, carry2):
                for t in range(3):
                    tile = _rhs4(v32, 3 * p + t, c)
                    v32[pl.ds(2 * (3 * p + t), 2), :, c] = pltpu.bitcast(
                        tile.T, U32).reshape(2, 4, 8, LANES)
                return carry2

            lax.fori_loop(first, nc, transpose_v, 0)

            def widen(es):
                for g in range(0, PG, 4):
                    for e in es:
                        idx = (p * (PG // 4) + g // 4, slice(None), XCOLS[e])
                        w = pltpu.bitcast(pltpu.bitcast(v32[idx], BF).astype(F32), U32)
                        v32[idx] = w[:, 0:8]
                        if e < NVX:
                            vx_ref[p, e, pl.ds(g, 4)] = w[:, 8:16]
                        else:
                            r0, s0 = vx_slot(p, g, e)
                            k32[r0, pl.ds(s0, 4)] = w[:, 8:16]

            pl.when(p < NP - 1)(functools.partial(widen, range(NVX)))
            pl.when((p < NP - 1) & (p > 0))(
                functools.partial(widen, range(NVX, len(XCOLS))))
            return carry

        def group1(gi, row):
            for i in range(NGRP):
                pl.when(gi == i)(functools.partial(wait, 1 + i))
            lax.fori_loop(gi * GP, (gi + 1) * GP, pair1, 0)
            return row + PRING * prow // NGRP

        fence_row = pl.multiple_of(lax.fori_loop(0, NGRP, group1, 0), 8)
        wait(1 + NGRP)

        def woloop(p2, carry):
            stage_wo([(2 * p2 + i, t) for i in range(2) for t in range(3)])
            return carry

        lax.fori_loop(0, NP // 2, woloop, 0)

        x = y_ref[:, 0:D]
        xb, m, r = ln_stats(x)
        wait(2 + NGRP)
        gu = []
        for j in range(2 * FT):
            raw, cs = raw_proj(xb, w13[j % 2], j // 2)
            cs_ref[j] = cs
            gu.append((raw - m * cs) * r)
        hs = [_swiglu(g, u) for g, u in zip(gu[0::2], gu[1::2])]
        for kk in range(W2_MXU // 8, FT):
            p_ref[pl.ds(LANES * kk - 16 * W2_MXU, LANES), :] = col_bcast(
                hs[kk].astype(BF).astype(F32))
        hs = [_pack2(hh, hh) for hh in hs[:W2_MXU // 8]]
        cols = [tile_of(x, c) for c in range(DT)]
        part = [None] * DT
        for i in range(len(W2_SPLIT) - 1):
            wait(3 + NGRP + i)
            g0, g1 = W2_SPLIT[i], W2_SPLIT[i + 1]
            for c in range(DT):
                if g1 <= W2_MXU:
                    for kk in range(g0 // 8, g1 // 8):
                        cols[c] = cols[c] + dot(hs[kk], _rhs(w232, 8 * kk, c))[0:8]
                else:
                    for g in range(g0, g1):
                        row = 16 * (g - W2_MXU)
                        part[c] = vpu_fma(part[c], w232[g, c], p_ref[pl.ds(row, 8), :],
                                          p_ref[pl.ds(row + 8, 8), :])
        x = jnp.concatenate([cc + sub_sum(a) for cc, a in zip(cols, part)], axis=1)

        xb, m, r = begin_attention(x)
        rq = r * qscale

        def run_block(blk, chains, items, n_link, first, last_off, start, end):
            links = []
            y_vpu = None
            for j, (p, g) in enumerate(chains[:n_link]):
                tail = end and g >= 8 * TAIL_T
                acc = pv_chain(p, g, lambda: p_refs[g % 2], store=not tail)
                dep = acc[0] | acc[1]
                if tail:
                    hd = 4 * (g // HG)
                    linv = jnp.broadcast_to((1.0 / lsum_ref[p])[hd:hd + 1], (8, LANES))
                    oc = jnp.sum(pltpu.bitcast(acc, F32), axis=2, keepdims=True) * linv
                    oc = oc.astype(BF).astype(F32).reshape(16, LANES)
                    w = pltpu.bitcast(wo32[6 * p + g // 4, g % 4], BF).astype(F32) * oc
                    y_vpu = _add(y_vpu, w[:, 0:8] + w[:, 8:16])
                links.extend([(LINK0[blk] + LINKSTEP[blk] * j, dep)] * LINK_REP[blk])
            if start:
                xcol = [col_bcast(tile_of(xb, kk)) - m[0:1] for kk in range(DT)]
                links.extend([(XC_LINK, _bits_or(xc[LANES - 8:] for xc in xcol))] * 4)
            pops = []
            probs = {}
            busy = []

            def mm(l32, rr, free=True):
                links.sort(key=lambda lk: lk[0])
                if free and links and len(pops) >= links[0][0]:
                    l32 = jnp.where(sub < 4, l32, links.pop(0)[1])
                pops.append(dot(l32, rr))
                return pops[-1]

            for it in items:
                kind, p = it[0], it[1]
                if kind == 'fq':
                    for t in range(3):
                        raw, cs = raw_proj(xb, wq32, 3 * p + t, mm)
                        q = raw - m * cs
                        q = q if p == 0 else q * rq
                        expand_q(p, t, _pack2(q, q))
                elif kind == 'q':
                    stage_q(p, mm)
                    busy.append((len(pops) - Q_A[blk], len(pops) - Q_B[blk], Q_W[blk]))
                elif kind == 'qx':
                    for t in range(3):
                        expand_q(p, t, qpk_ref[3 * VQ.index(p) + t])
                elif kind == 'qk':
                    stage_qk(p, it[2], p % (NP - 2) * PG, mm, rq if p == 0 else None)
                elif kind == 'sm':
                    e, l = softmax(p, 0 if p == NP - 1 else (nc - MC[p]) // 4)
                    lag = SM_LAG0 if p == 0 else SM_LAG[blk]
                    pos = len(pops) + (lag if pops else lag - 14)
                    links.append((pos, pltpu.bitcast(l, U32)))
                    busy.append((pos - SM_A[blk], pos - SM_B[blk], SM_W[blk]))
                    if p < NP - 1:
                        probs[p] = e
                elif kind == 'pvm':
                    o = pv_mxu(p, range(it[2], it[3]), True, mm)
                    om_ref[p] = o + om_ref[p] if it[4] else o
                elif kind == 'reload':
                    start_dma(n_ring + p)
                elif kind == 'red':
                    stage_reduce(p)
                elif kind == 'wo':
                    busy.append((len(pops) - RED_A[blk], len(pops) - RED_B[blk], RED_W[blk]))
                    stage_wo([(pp, t) for pp in it[1:] for t in range(mxu_tiles(pp))], mm)

            def fence(buf, a, h=0):
                buf[pl.ds(fence_row, 8), :] = pops[min(a, len(pops) - 1)][8 * h:8 * h + 8]

            if start:
                nkg = D // 16

                def xslot(kg):
                    u = kg // VQ_UNIT
                    return p_refs[u % 2], 16 * (u // 2 * VQ_UNIT + kg % VQ_UNIT)

                for kg in range(nkg):
                    buf, row = xslot(kg)
                    buf[pl.ds(row, 16), :] = xcol[kg // 8][16 * (kg % 8):16 * (kg % 8) + 16]
                for i, p in enumerate(VQ):
                    acc = None
                    for kg in range(nkg):
                        buf, row = xslot(kg)
                        if kg % VQ_UNIT == 0:
                            a = (i * nkg + kg) * (first - VQ_FIRST) // (len(VQ) * nkg)
                            fence(buf, VQ_FIRST + a // 2 * 2)
                        w = pltpu.bitcast(wq32[kg, pl.ds(3 * p, 3)], BF).astype(F32)
                        w = w * buf[pl.ds(row, 16), :]
                        acc = _add(acc, w[:, 0:8] + w[:, 8:16])
                    for t in range(3):
                        q = sub_sum(acc[t]) * rq
                        qpk_ref[3 * i + t] = _pack2(q, q)

            def store_probs(p):
                e = probs.pop(p)
                for pr in p_refs:
                    for j in range((nc - MC[p] + 3) // 4):
                        pr[pl.ds((p % PRING) * prow + 8 * j, 8), :] = e[j]

            rest = chains[n_link:]
            if rest:
                runs, i = [], 0
                while i < len(rest):
                    p, g = rest[i]
                    runs.append((p, g, min(GSHARE - g % GSHARE, len(rest) - i)))
                    i += runs[-1][2]
                cost = [n * (XCOST[blk] if c in widened(p) else 1.0)
                        for p, _, n in runs for c in range(nc - MC[p])]
                n_items = len(cost)
                anch = ANCH[blk]
                fstep = 4 / len(anch)
                n_units = int((len(pops) - last_off - first) / fstep) + 1
                less = [0.0] * n_units
                for lo, hi, w in busy:
                    us = [u for u in range(n_units) if lo <= first + u * fstep < hi]
                    for u in us:
                        less[u] += w / len(us)
                per = (sum(cost) + sum(less)) / n_units
                unit_of, total, used = [], 0.0, 0.0
                for u in range(n_units):
                    total += per - less[u]
                    while len(unit_of) < n_items and (
                            used + cost[len(unit_of)] / 2 < total or u + 1 == n_units):
                        used += cost[len(unit_of)]
                        unit_of.append(u)
                state = [0, -1, 1]

                def gate():
                    u = unit_of[state[0]]
                    state[0] += 1
                    if u != state[1]:
                        state[1] = u
                        state[2] += 1
                        a, h = divmod(anch[u % len(anch)], 2)
                        fence(p_refs[state[2] % 2], first + u // len(anch) * 4 + a, h)
                    return p_refs[state[2] % 2]

            for p, g, n in runs if rest else []:
                if g == 0:
                    for i in range(state[0], n_items):
                        if unit_of[i] != state[1] or state[1] + 1 == n_units:
                            break
                        unit_of[i] += 1
                if p in probs:
                    store_probs(p)
                pv_chain(p, g, gate, n)
            for p in list(probs):
                store_probs(p)
            if end:
                x = y_ref[:, 0:D]
                if y_vpu is not None:
                    x = x + jnp.concatenate([sub_sum(y_vpu[c]) for c in range(DT)], axis=1)
                last_ffn(x, mm, len(pops), links)

        def last_ffn(x, mm, base, links):
            xb, m, r = ln_stats(x)
            lhs = _pack2(xb, xb)
            xcol = [col_bcast(tile_of(xb, kk)) for kk in range(UP_K)]
            links.extend([(base + UX_LINK, _bits_or(xc[LANES - 8:] for xc in xcol))] * 4)
            j0 = 2 * (FT - UP_COLS)
            part = {}
            for j in range(j0, 2 * FT):
                acc = None
                for i in range(8):
                    for kk in range(UP_K):
                        xc = xcol[kk][16 * i:16 * i + 16]
                        acc = vpu_fma(acc, w13[j % 2][8 * kk + i, j // 2], xc[0:8], xc[8:16])
                part[j] = sub_sum(acc)
                links.append((base + int(UP_LINK0 + UP_LINKSTEP * (j - j0)),
                              pltpu.bitcast(part[j], U32)))
            work = [(j, kk) for kk in range(DT) for j in range(UP_KM)]
            work += [(j, kk) for j in range(UP_KM, 2 * FT)
                     for kk in range(UP_K if j in part else 0, DT)]
            for j, kk in work:
                part[j] = _add(part.get(j), mm(tile_of(lhs, kk),
                                               _rhs(w13[j % 2], 8 * kk, j // 2))[0:8])
            gu = [(part[j] - m * cs_ref[j]) * r for j in range(2 * FT)]
            hs = [_swiglu(g, u) for g, u in zip(gu[0::2], gu[1::2])]
            cols = [tile_of(x, c) for c in range(DT)]
            for kk in range(DOWN_K, FT):
                hh = _pack2(hs[kk], hs[kk])
                for c in range(DT):
                    cols[c] = cols[c] + mm(hh, _rhs(w232, 8 * kk, c))[0:8]
            hcol = [col_bcast(hs[kk].astype(BF).astype(F32)) for kk in range(DOWN_K)]
            acc = [None] * DT
            for i in range(8):
                for kk in range(DOWN_K):
                    for c in range(DT):
                        acc[c] = vpu_fma(acc[c], w232[8 * kk + i, c],
                                         hcol[kk][16 * i:16 * i + 8],
                                         hcol[kk][16 * i + 8:16 * i + 16])
            cols = [cc + sub_sum(a) for cc, a in zip(cols, acc)]
            o_ref[...] = jnp.concatenate(cols, axis=1)[0:1].astype(o_ref.dtype)

        blocks = _plan(nc)
        for b, plan in enumerate(blocks):
            end = b == len(blocks) - 1
            if b > 0:
                wait(marker if end else n_ring + b - 1)
            if b == 1:
                start_dma(late)
            if b == 2:
                wait(late)
            run_block(b, *plan, b == 0, end)

    return kernel


@jax.jit
def pallas_interleave_layers__sliding_block_cached__glu_gated_swiglu__decode_kernel(
    A_x: jax.Array,
    A_k_cache: jax.Array,
    A_v_cache: jax.Array,
    A_wq: jax.Array,
    A_wo: jax.Array,
    B_x: jax.Array,
    B_w1: jax.Array,
    B_w3: jax.Array,
    B_w2: jax.Array,
):
    sk = A_k_cache.shape[2]
    win = min(4096, max(256, sk // 4))
    nt_total, nc = sk // LANES, win // LANES

    def kv_view(a):
        return _tile_view(jnp.swapaxes(a, 2, 3).reshape(H * DH, sk))

    def view4(t):
        return t.reshape(t.shape[0] // 4, 2, 4, t.shape[2], 8, LANES)

    def wbuf(r, c):
        return pltpu.VMEM((r // 16, c // LANES, 16, LANES), BF)

    def wbuf4(r, c):
        return pltpu.VMEM((r // 64, 4, c // LANES, 16, LANES), BF)

    any_spec = pl.BlockSpec(memory_space=pl.ANY)
    out = pl.pallas_call(
        _make_kernel(nt_total, nc),
        out_shape=jax.ShapeDtypeStruct((1, D), A_x.dtype),
        in_specs=[any_spec] * 8,
        out_specs=pl.BlockSpec(memory_space=pltpu.VMEM),
        scratch_shapes=[
            wbuf(H * DH, win), wbuf4(H * DH, win),
            wbuf(D, H * DH), wbuf4(H * DH, D),
            wbuf(D, F), wbuf(D, F), wbuf(F, D),
            pltpu.VMEM((NP - 1, NVX, PG, 8, LANES), U32),
            pltpu.VMEM((2 * PG, 8, LANES), U32),
            pltpu.VMEM((RING, 12, 8, LANES), U32),
            pltpu.VMEM((RING, nc // 4, 8, LANES), F32),
            pltpu.VMEM((PRING * 2 * nc + 32, LANES), F32),
            pltpu.VMEM((PRING * 2 * nc + 32, LANES), F32),
            pltpu.VMEM((RING, nc // 4, 8, LANES), U32),
            pltpu.VMEM((NP, 8, LANES), F32),
            pltpu.VMEM((NP, 8, PW), F32),
            pltpu.VMEM((NP, 8, PW), U32),
            pltpu.VMEM((16, 8, LANES), U32),
            pltpu.VMEM((2 * FT, 8, LANES), F32),
            pltpu.VMEM((16, 8, LANES), U32),
            pltpu.VMEM((8, 1024), U32),
            pltpu.VMEM((8, 1024), F32),
            pltpu.VMEM((1, D), BF),
            pltpu.SemaphoreType.DMA((NSEM,)),
        ],
        compiler_params=pltpu.CompilerParams(
            vmem_limit_bytes=128 * 1024 * 1024),
    )(A_x.reshape(1, D), kv_view(A_k_cache), view4(kv_view(A_v_cache)),
      _tile_view(A_wq), view4(_tile_view(A_wo)),
      _tile_view(B_w1), _tile_view(B_w3), _tile_view(B_w2))
    return out.reshape(A_x.shape)
```

```python
import functools
import math

import jax
import jax.numpy as jnp
from jax import lax
import jax.experimental.pallas as pl
import jax.experimental.pallas.tpu as pltpu

D = 640
H = 32
DH = 192
F = 1536
LANES = 128
EPS = 1e-5

NP = H // 2
PG = 2 * DH // 16
HG = DH // 16
PW = 2 * DH
DT = D // LANES
FT = F // LANES

GP = 4
NGRP = NP // GP
W2_SPLIT = (0, 56, 80, 92, 96)
W2_MXU = 80
RELOAD_ROWS = 8
NSEM = 3
RING = 4
PRING = 6

MC = (2, 2, 2, 2, 2, 2, 2, 2, 2, 2, 2, 2, 2, 0, 0)
XCOLS = (1, 7, 10, 16, 22, 25, 4, 13, 19, 28)
NVX = 6
XMORE = ((1, 29), (2, 29), (3, 29), (4, 29),
         (0, 4), (0, 13), (0, 19), (0, 28), (5, 29), (8, 14), (10, 29))
VQ = (11, 12, 13, 14, 15)
V_END = (174, 299, 349)
TILES = (1060, 655, 291)
XCOST = (0.67, 0.77, 0.67, 0.67)
GSHARE = 2
PVM_AFTER = 2
WO_START = (0, 80, 80, 999)
WO_GAP = (0, 72, 60, 12)
WO_KEEP = 4
FIRST = (160, 2, 0)
LAST_OFF = (8, 6, 6)
VQ_FIRST = 30
VQ_UNIT = 4
XC_LINK = 50
SM_LAG = (60, 64, 64, 64)
ANCH = ((0, 4), (0, 1, 4), (6, 1))
SM_MIN = 40
SM_LAG0 = 52
RED_W = (10, 10, 10, 10)
RED_A = (40, 40, 32, 40)
RED_B = (16, 28, 20, 16)
Q_W = (4, 4, 4, 4)
Q_A = (18, 12, 12, 12)
Q_B = (-4, -4, -4, -4)
SM_W = (4, 4, 7, 7)
SM_A = (56, 56, 64, 56)
SM_B = (30, 48, 30, 30)
NLINK = (0, 4, 3)
LINK0 = (8, 10, 8, 10)
LINKSTEP = (4, 4, 2, 7)
LINK_REP = (1, 1, 4, 1)
TAIL_T = 2
WO_JOINT = 2
UP_KM = 4
UP_K = 3
UP_COLS = 6
UP_LINK0 = 58
UP_LINKSTEP = 5.5
UX_LINK = 44
DOWN_K = 4

U32 = jnp.uint32
BF = jnp.bfloat16
F32 = jnp.float32


def _tile_view(w):
    r, c = w.shape
    return jnp.swapaxes(w.reshape(r // 16, 2, 8, c // LANES, LANES), 2, 3)


def _rhs(w32, g0, c):
    return pltpu.bitcast(w32[pl.ds(g0, 8), c].reshape(64, LANES), BF)


def _rhs4(w32, tile, c):
    return pltpu.bitcast(w32[pl.ds(2 * tile, 2), :, c].reshape(64, LANES), BF)


def _swiglu(g, u):
    hg = 0.5 * g
    return hg * (1.0 + jnp.tanh(hg)) * u


def _pack2(lo, hi):
    return pltpu.bitcast(jnp.concatenate([lo, hi], axis=0).astype(BF), U32)


def _add(a, b):
    return b if a is None else a + b


def _bits_or(vals):
    return functools.reduce(lambda a, b: a | b, [pltpu.bitcast(v, U32) for v in vals])


def _plan(nc):
    nk = nc // 8
    seq = [('fq', 0), ('fq', 1)]
    for p in range(NP):
        if 1 <= p < NP - 1:
            seq.append(('qx' if p + 1 in VQ else 'q', p + 1))
        for k in range(nk):
            if k == PVM_AFTER and p > 0 and MC[p - 1]:
                seq.append(('pvm', p - 1, nc - MC[p - 1], nc, False))
            seq.append(('qk', p, k))
        if p < 2:
            seq.append(('reload', p))
        seq.append(('sm', p))
    seq += [('pvm', NP - 1, c, c + 4, c > 0) for c in range(0, nc, 4)]
    last_pv = seq[-nc // 4]

    def tiles(it):
        if it[0] == 'pvm':
            return 3 * (it[3] - it[2])
        return dict(fq=15, q=15, wo=15, qk=24, sm=0, qx=0, reload=0)[it[0]]

    chains = [(p, g) for p in range(NP - 1) for g in range(PG)]
    blocks = []
    v0 = done = 0
    for b in range(len(V_END) + 1):
        final = b == len(V_END)
        v1 = len(chains) if final else V_END[b]
        todo = list(range(done, v0 // PG))
        done = v0 // PG
        budget = 10 ** 9 if final else TILES[b] - 15 * len(todo)
        body = []
        used = 0
        while seq and used + tiles(seq[0]) // 2 <= budget:
            body.append(seq.pop(0))
            used += tiles(body[-1])
        while body[-1][0] in ('sm', 'qx'):
            seq.insert(0, body.pop())
        left = 0
        for i in range(len(body) - 1, -1, -1):
            if body[i][0] == 'sm' and left < SM_MIN and not final:
                seq.insert(0, body.pop(i))
            else:
                left += tiles(body[i])
        assert b > 0 or not any(it[1] in VQ for it in body)
        keep = WO_KEEP if last_pv in body else 0
        items = [('red', p) for p in todo]
        used = 0
        nxt = WO_START[b]
        for it in body:
            if it == last_pv:
                while todo:
                    items.append(('wo', todo.pop(0)))
            if len(todo) > keep and used >= nxt:
                items.append(('wo', todo.pop(0)))
                nxt = used + WO_GAP[b]
            items.append(it)
            used += tiles(it)
        items += [('wo', p) for p in todo]
        if final:
            assert done == NP - 2
            assert TAIL_T == 3 or (MC[NP - 2] == 0 and v0 % PG <= 8 * TAIL_T)
            for p in (NP - 1, NP - 2):
                items += [('red', p), ('wo', p)]
            joint = [it for it in items if it[0] == 'wo'][-WO_JOINT:]
            items = [it for it in items if it not in joint]
            items.append(('wo', *[it[1] for it in joint]))
            blocks.append((chains[v0:v1], items, v1 - v0, 0, 0))
        else:
            blocks.append((chains[v0:v1], items, NLINK[b], FIRST[b], LAST_OFF[b]))
        v0 = v1
    assert all(c < nc - MC[p] and (p > 0 or i >= 4) for i, (p, c) in enumerate(XMORE))
    seen = set()
    for b, (chs, items, n_link, _, _) in enumerate(blocks):
        assert all(it[1] - (NP - 2) < b for it in items if it[0] == 'qk')
        assert all(p in seen for p, _ in chs[:n_link])
        seen |= {it[1] for it in items if it[0] == 'sm'}
        assert all(p in seen for p, _ in chs)
        assert max(seen) - chs[-1][0] < PRING
    return blocks


def _make_kernel(n_tiles_total, nc):
    c0 = n_tiles_total - nc
    qscale = DH ** -0.5 * math.log2(math.e)
    prow = 2 * nc
    nk = nc // 8

    def kernel(x_hbm, k_hbm, v_hbm, wq_hbm, wo_hbm, w1_hbm, w3_hbm, w2_hbm,
               o_ref,
               kbuf, vbuf, wqbuf, wobuf, w1buf, w3buf, w2buf,
               vx_ref, vy_ref, t0_ref, lhs_ref, s_ref, p_ref, p2_ref, pk_ref, lsum_ref, om_ref,
               ob_ref, mask_ref, cs_ref, qpk_ref, xn_ref, y_ref, xbuf, sem):
        def halves(src, dst):
            return [(src(par), dst(pl.ds(8 * par, 8))) for par in range(2)]

        def whole(src, dst):
            return halves(lambda p: src.at[:, p], lambda h: dst.at[:, :, h, :])

        def kv_group(g):
            kr = pl.ds(g * GP * PG, GP * PG)
            vr = pl.ds(g * GP * PG // 4, GP * PG // 4)
            return (halves(lambda p: k_hbm.at[kr, p, pl.ds(c0, nc)],
                           lambda h: kbuf.at[kr, :, h, :])
                    + halves(lambda p: v_hbm.at[vr, p, :, pl.ds(c0, nc)],
                             lambda h: vbuf.at[vr, :, :, h, :]))

        def w2_group(i):
            rows = pl.ds(W2_SPLIT[i], W2_SPLIT[i + 1] - W2_SPLIT[i])
            return halves(lambda p: w2_hbm.at[rows, p], lambda h: w2buf.at[rows, :, h, :])

        groups = ([whole(wq_hbm, wqbuf) + [(x_hbm, xbuf)]]
                  + [kv_group(NGRP - 1 - g) for g in range(NGRP)]
                  + [halves(lambda p: wo_hbm.at[:, p], lambda h: wobuf.at[:, :, :, h, :]),
                     whole(w1_hbm, w1buf) + whole(w3_hbm, w3buf)]
                  + [w2_group(i) for i in range(len(W2_SPLIT) - 1)])
        marker = len(groups)
        groups.append([(x_hbm, xbuf)])
        n_ring = len(groups)
        def k_rows(i, rows):
            return halves(lambda p: k_hbm.at[rows((NP - 2 + i) * PG), p, pl.ds(c0, nc)],
                          lambda h: kbuf.at[rows(i * PG), :, h, :])

        for i, n in enumerate((PG, RELOAD_ROWS)):
            groups.append([cp for g in range(n) for cp in k_rows(i, lambda r0: r0 + g)])
        late = n_ring + 1 + NSEM
        groups += [[]] * (late - len(groups))
        groups.append(k_rows(1, lambda r0: pl.ds(r0 + RELOAD_ROWS, PG - RELOAD_ROWS)))

        def copies(i):
            return [pltpu.make_async_copy(src, dst, sem.at[i % NSEM])
                    for src, dst in groups[i]]

        def start_dma(i):
            for cp in copies(i):
                cp.start()

        def wait(i):
            for cp in copies(i):
                cp.wait()
            if i + NSEM < n_ring:
                start_dma(i + NSEM)

        for i in range(NSEM):
            start_dma(i)

        k32 = kbuf.bitcast(U32)
        v32 = vbuf.bitcast(U32)
        wq32 = wqbuf.bitcast(U32)
        wo32 = wobuf.bitcast(U32)
        w13 = (w1buf.bitcast(U32), w3buf.bitcast(U32))
        w232 = w2buf.bitcast(U32)

        sub = lax.broadcasted_iota(jnp.int32, (8, LANES), 0)
        lane = lax.broadcasted_iota(jnp.int32, (8, LANES), 1)
        sub3 = lax.broadcasted_iota(jnp.int32, (8, PW), 0)
        lane3 = lax.broadcasted_iota(jnp.int32, (8, PW), 1)

        for r in range(4):
            half = U32(0x0000FFFF if r % 2 == 0 else 0xFFFF0000)
            lo = jnp.where(sub == r // 2, half, U32(0))
            hi = jnp.where(sub == 2 + r // 2, half, U32(0))
            mask_ref[r] = lo
            mask_ref[4 + r] = jnp.where(lane < DH - LANES, lo, hi)
            mask_ref[8 + r] = hi
            mask_ref[12 + r] = lo | hi
        p_refs = (p_ref, p2_ref)
        for pr in p_refs:
            pr[...] = jnp.zeros(pr.shape, F32)

        def dot(l32, r, free=True):
            del free
            return jnp.dot(pltpu.bitcast(l32, BF), r, preferred_element_type=F32)

        def tile_of(v, kk):
            return v[:, kk * LANES:(kk + 1) * LANES]

        def ln_stats(x):
            xb = x.astype(BF).astype(F32)
            m = jnp.mean(xb, axis=-1, keepdims=True)
            xc = xb - m
            v = jnp.mean(xc * xc, axis=-1, keepdims=True)
            return xb, m, lax.rsqrt(v + EPS)

        def raw_proj(xb, w32, c, mm=dot):
            lhs = _pack2(xb, jnp.ones_like(xb))
            acc = None
            for kk in range(DT):
                acc = _add(acc, mm(tile_of(lhs, kk), _rhs(w32, 8 * kk, c), False))
            return acc[0:8], acc[8:16]

        def col_bcast(v):
            return jnp.concatenate([v] * (LANES // 8), axis=0).T

        def vpu_fma(acc, w, xlo, xhi):
            w = pltpu.bitcast(w, BF).astype(F32)
            return _add(acc, w[0:8] * xlo + w[8:16] * xhi)

        def sub_sum(a):
            return jnp.broadcast_to(jnp.sum(a, axis=0, keepdims=True), a.shape)

        def expand_q(p, t, q):
            for r in range(4):
                lhs_ref[p % RING, 4 * t + r] = q & mask_ref[4 * t + r]

        def stage_q(p, mm=dot):
            acc = [None] * 3
            for kk in range(DT):
                for t in range(3):
                    acc[t] = _add(acc[t], mm(xn_ref[:, pl.ds(kk * LANES, LANES)],
                                             _rhs(wq32, 8 * kk, 3 * p + t))[0:8])
            for t in range(3):
                q = acc[t] * qscale
                expand_q(p, t, _pack2(q, q))

        def stage_qk(p, k, krow, mm=dot, scale=None):
            for j in range(2 * k, 2 * k + 2):
                acc = None
                for t in range(3):
                    for r in range(4):
                        acc = _add(acc, mm(lhs_ref[p % RING, 4 * t + r],
                                           _rhs(k32, krow + 8 * t, 4 * j + r))[0:8])
                s_ref[p % RING, j] = acc if scale is None else acc * scale

        def head_reduce(v, op, lane_op):
            for d in (1, 2):
                up = pltpu.roll(v, d, 0)
                down = pltpu.roll(v, 8 - d, 0)
                v = op(v, jnp.where(sub % (2 * d) >= d, up, down))
            return lane_op(v, axis=1, keepdims=True)

        def softmax(p, j0):
            s = s_ref[p % RING]
            m = head_reduce(jnp.max(s, axis=0), jnp.maximum, jnp.max)
            e = jnp.exp2(s - m)
            l = jnp.sum(e, axis=0)
            l = jnp.broadcast_to(head_reduce(l, jnp.add, jnp.sum), l.shape)
            lsum_ref[p] = l
            for j in range(j0, nc // 4):
                pk_ref[p % RING, j] = _pack2(e[j], e[j])
            return e, l

        def widened(p):
            return (XCOLS if p else XCOLS[:NVX]) + tuple(c for pp, c in XMORE if pp == p)

        def hi_slot(p, g, n, c):
            if isinstance(p, int) and (p, c) in XMORE:
                i = XMORE.index((p, c))
                if i < 4:
                    return k32, (((NP - 2) * PG + 2, NP * PG - 3, NP * PG - 2,
                                  NP * PG - 1)[i], pl.ds(g, n))
                return vy_ref, (i - 4, pl.ds(g, n))
            e = XCOLS.index(c)
            if e < NVX:
                return vx_ref, (p, e, pl.ds(g, n))
            return k32, ((NP - 2) * PG + 3 * p + g // 8, pl.ds((e - NVX) * 8 + g % 8, n))

        def t_slot(p, j, n):
            if p == 0:
                return t0_ref, pl.ds(j, n)
            row = (NP - 2) * PG if p == 1 else p * PG if p < NP - 2 else 2 * PG + 2
            return k32, (row + j // nc, pl.ds(j % nc, n))

        def pv_chain(p, g, gate, n=1, store=True):
            acc = None
            for c in range(nc - MC[p]):
                row = (p % PRING) * prow + 8 * (c // 4) + 4 * (g // HG) + c % 4
                pb = gate()[pl.ds(row, 16, stride=0), :]
                w = v32[p * (PG // 4) + g // 4, pl.ds(g % 4, n), c]
                if c in widened(p):
                    ref, idx = hi_slot(p, g, n, c)
                    w = pltpu.bitcast(jnp.concatenate([w, ref[idx]], axis=1), F32)
                else:
                    w = pltpu.bitcast(w, BF).astype(F32)
                acc = _add(acc, w * pb)
            acc = pltpu.bitcast(acc, U32).reshape(2 * n, 8, LANES)
            if store:
                ref, idx = t_slot(p, 2 * g, 2 * n)
                ref[idx] = acc
            return acc

        def pv_mxu(p, cols, transposed, mm=dot):
            acc = [None] * 3
            cols = list(cols)
            for i0 in range(0, len(cols), 4):
                ls = {c: pk_ref[p % RING, c // 4] & mask_ref[12 + c % 4]
                      for c in cols[i0:i0 + 4]}
                for t in range(3):
                    for c, l in ls.items():
                        tile = _rhs4(v32, 3 * p + t, c)
                        if transposed:
                            res = mm(l, tile)
                        else:
                            res = lax.dot_general(
                                pltpu.bitcast(l, BF), tile, (((1,), (1,)), ((), ())),
                                preferred_element_type=F32)
                        acc[t] = _add(acc[t], res[0:8])
            return jnp.concatenate(acc, axis=1)

        def own_head(o):
            return jnp.where((sub3 < 4) == (lane3 < DH), o, 0.0)

        def finish_o(p, o, nt=3):
            linv = 1.0 / lsum_ref[p]
            la = jnp.broadcast_to(linv[0:1], linv.shape)
            lb = jnp.broadcast_to(linv[4:5], linv.shape)
            linv = [la, jnp.where(lane < DH - LANES, la, lb), lb]
            o = jnp.sum(o, axis=0, keepdims=True) * jnp.concatenate(linv[:nt], axis=1)
            ob_ref[p, :, 0:nt * LANES] = _pack2(o, o)

        def mxu_tiles(p):
            return TAIL_T if p == NP - 2 else 3

        def stage_reduce(p):
            o = None
            nt = mxu_tiles(p)
            if p < NP - 1:
                slots = [t_slot(p, 16 * t, 16) for t in range(nt)]
                tt = jnp.concatenate([ref[idx] for ref, idx in slots])
                tt = pltpu.bitcast(tt.reshape(nt * LANES, LANES), F32)
                o = jnp.sum(tt.T.reshape(LANES // 8, 8, nt * LANES), axis=0)
            if p == NP - 1 or MC[p]:
                o = _add(o, own_head(om_ref[p]))
            finish_o(p, o, nt)

        def stage_wo(tiles, mm=dot):
            for c in range(DT):
                acc = y_ref[:, pl.ds(c * LANES, LANES)]
                for p, t in tiles:
                    acc = acc + mm(ob_ref[p, :, pl.ds(t * LANES, LANES)],
                                   _rhs4(wo32, 3 * p + t, c))[0:8]
                y_ref[:, pl.ds(c * LANES, LANES)] = acc

        def begin_attention(x):
            y_ref[:, 0:D] = x
            xb, m, r = ln_stats(x)
            xn = (xb - m) * r
            xn_ref[:, 0:D] = _pack2(xn, xn)
            return xb, m, r

        wait(0)
        begin_attention(jnp.broadcast_to(xbuf[...].astype(F32), (8, D)))

        def pair1(i, carry):
            p = NP - 1 - i
            stage_q(p)
            for k in range(nk):
                stage_qk(p, k, p * PG)
            softmax(p, 0)
            finish_o(p, own_head(pv_mxu(p, range(nc), False)))
            om_ref[p] = jnp.zeros(om_ref.shape[1:], F32)
            qpk_ref[p] = jnp.zeros((8, LANES), U32)
            t0_ref[p] = jnp.zeros((8, LANES), U32)
            cs_ref[p] = jnp.zeros((8, LANES), F32)

            first = 0
            for pp in range(NP - 1):
                first = jnp.where(p == pp, nc - MC[pp], first)

            def transpose_v(c, carry2):
                for t in range(3):
                    tile = _rhs4(v32, 3 * p + t, c)
                    v32[pl.ds(2 * (3 * p + t), 2), :, c] = pltpu.bitcast(
                        tile.T, U32).reshape(2, 4, 8, LANES)
                return carry2

            lax.fori_loop(first, nc, transpose_v, 0)

            def widen(pp, cols):
                for g in range(0, PG, 4):
                    for c in cols:
                        idx = (pp * (PG // 4) + g // 4, slice(None), c)
                        w = pltpu.bitcast(pltpu.bitcast(v32[idx], BF).astype(F32), U32)
                        v32[idx] = w[:, 0:8]
                        ref, idx = hi_slot(pp, g, 4, c)
                        ref[idx] = w[:, 8:16]

            pl.when(p < NP - 1)(functools.partial(widen, p, XCOLS[:NVX]))
            pl.when((p < NP - 1) & (p > 0))(functools.partial(widen, p, XCOLS[NVX:]))
            for pp in sorted({pp for pp, _ in XMORE}):
                pl.when(p == pp)(functools.partial(
                    widen, pp, [c for p2, c in XMORE if p2 == pp]))
            return carry

        def group1(gi, row):
            for i in range(NGRP):
                pl.when(gi == i)(functools.partial(wait, 1 + i))
            lax.fori_loop(gi * GP, (gi + 1) * GP, pair1, 0)
            return row + PRING * prow // NGRP

        fence_row = pl.multiple_of(lax.fori_loop(0, NGRP, group1, 0), 8)
        wait(1 + NGRP)

        def woloop(p2, carry):
            stage_wo([(2 * p2 + i, t) for i in range(2) for t in range(3)])
            return carry

        lax.fori_loop(0, NP // 2, woloop, 0)

        x = y_ref[:, 0:D]
        xb, m, r = ln_stats(x)
        wait(2 + NGRP)
        gu = []
        for j in range(2 * FT):
            raw, cs = raw_proj(xb, w13[j % 2], j // 2)
            cs_ref[j] = cs
            gu.append((raw - m * cs) * r)
        hs = [_swiglu(g, u) for g, u in zip(gu[0::2], gu[1::2])]
        for kk in range(W2_MXU // 8, FT):
            p_ref[pl.ds(LANES * kk - 16 * W2_MXU, LANES), :] = col_bcast(
                hs[kk].astype(BF).astype(F32))
        hs = [_pack2(hh, hh) for hh in hs[:W2_MXU // 8]]
        cols = [tile_of(x, c) for c in range(DT)]
        part = [None] * DT
        for i in range(len(W2_SPLIT) - 1):
            wait(3 + NGRP + i)
            g0, g1 = W2_SPLIT[i], W2_SPLIT[i + 1]
            for c in range(DT):
                if g1 <= W2_MXU:
                    for kk in range(g0 // 8, g1 // 8):
                        cols[c] = cols[c] + dot(hs[kk], _rhs(w232, 8 * kk, c))[0:8]
                else:
                    for g in range(g0, g1):
                        row = 16 * (g - W2_MXU)
                        part[c] = vpu_fma(part[c], w232[g, c], p_ref[pl.ds(row, 8), :],
                                          p_ref[pl.ds(row + 8, 8), :])
        x = jnp.concatenate([cc + sub_sum(a) for cc, a in zip(cols, part)], axis=1)

        xb, m, r = begin_attention(x)
        rq = r * qscale

        def run_block(blk, chains, items, n_link, first, last_off, start, end):
            links = []
            y_vpu = None
            for j, (p, g) in enumerate(chains[:n_link]):
                tail = end and g >= 8 * TAIL_T
                acc = pv_chain(p, g, lambda: p_refs[g % 2], store=not tail)
                dep = acc[0] | acc[1]
                if tail:
                    hd = 4 * (g // HG)
                    linv = jnp.broadcast_to((1.0 / lsum_ref[p])[hd:hd + 1], (8, LANES))
                    oc = jnp.sum(pltpu.bitcast(acc, F32), axis=2, keepdims=True) * linv
                    oc = oc.astype(BF).astype(F32).reshape(16, LANES)
                    w = pltpu.bitcast(wo32[6 * p + g // 4, g % 4], BF).astype(F32) * oc
                    y_vpu = _add(y_vpu, w[:, 0:8] + w[:, 8:16])
                links.extend([(LINK0[blk] + LINKSTEP[blk] * j, dep)] * LINK_REP[blk])
            if start:
                xcol = [col_bcast(tile_of(xb, kk)) - m[0:1] for kk in range(DT)]
                links.extend([(XC_LINK, _bits_or(xc[LANES - 8:] for xc in xcol))] * 4)
            pops = []
            probs = {}
            busy = []

            def mm(l32, rr, free=True):
                links.sort(key=lambda lk: lk[0])
                if free and links and len(pops) >= links[0][0]:
                    l32 = jnp.where(sub < 4, l32, links.pop(0)[1])
                pops.append(dot(l32, rr))
                return pops[-1]

            for it in items:
                kind, p = it[0], it[1]
                if kind == 'fq':
                    for t in range(3):
                        raw, cs = raw_proj(xb, wq32, 3 * p + t, mm)
                        q = raw - m * cs
                        q = q if p == 0 else q * rq
                        expand_q(p, t, _pack2(q, q))
                elif kind == 'q':
                    stage_q(p, mm)
                    busy.append((len(pops) - Q_A[blk], len(pops) - Q_B[blk], Q_W[blk]))
                elif kind == 'qx':
                    for t in range(3):
                        expand_q(p, t, qpk_ref[3 * VQ.index(p) + t])
                elif kind == 'qk':
                    stage_qk(p, it[2], p % (NP - 2) * PG, mm, rq if p == 0 else None)
                elif kind == 'sm':
                    e, l = softmax(p, 0 if p == NP - 1 else (nc - MC[p]) // 4)
                    lag = SM_LAG0 if p == 0 else SM_LAG[blk]
                    pos = len(pops) + (lag if pops else lag - 14)
                    links.append((pos, pltpu.bitcast(l, U32)))
                    busy.append((pos - SM_A[blk], pos - SM_B[blk], SM_W[blk]))
                    if p < NP - 1:
                        probs[p] = e
                elif kind == 'pvm':
                    o = pv_mxu(p, range(it[2], it[3]), True, mm)
                    om_ref[p] = o + om_ref[p] if it[4] else o
                elif kind == 'reload':
                    start_dma(n_ring + p)
                elif kind == 'red':
                    stage_reduce(p)
                elif kind == 'wo':
                    busy.append((len(pops) - RED_A[blk], len(pops) - RED_B[blk], RED_W[blk]))
                    stage_wo([(pp, t) for pp in it[1:] for t in range(mxu_tiles(pp))], mm)

            def fence(buf, a, h=0):
                buf[pl.ds(fence_row, 8), :] = pops[min(a, len(pops) - 1)][8 * h:8 * h + 8]

            if start:
                nkg = D // 16

                def xslot(kg):
                    u = kg // VQ_UNIT
                    return p_refs[u % 2], 16 * (u // 2 * VQ_UNIT + kg % VQ_UNIT)

                for kg in range(nkg):
                    buf, row = xslot(kg)
                    buf[pl.ds(row, 16), :] = xcol[kg // 8][16 * (kg % 8):16 * (kg % 8) + 16]
                for i, p in enumerate(VQ):
                    acc = None
                    for kg in range(nkg):
                        buf, row = xslot(kg)
                        if kg % VQ_UNIT == 0:
                            a = (i * nkg + kg) * (first - VQ_FIRST) // (len(VQ) * nkg)
                            fence(buf, VQ_FIRST + a // 2 * 2)
                        w = pltpu.bitcast(wq32[kg, pl.ds(3 * p, 3)], BF).astype(F32)
                        w = w * buf[pl.ds(row, 16), :]
                        acc = _add(acc, w[:, 0:8] + w[:, 8:16])
                    for t in range(3):
                        q = sub_sum(acc[t]) * rq
                        qpk_ref[3 * i + t] = _pack2(q, q)

            def store_probs(p):
                e = probs.pop(p)
                for pr in p_refs:
                    for j in range((nc - MC[p] + 3) // 4):
                        pr[pl.ds((p % PRING) * prow + 8 * j, 8), :] = e[j]

            rest = chains[n_link:]
            if rest:
                runs, i = [], 0
                while i < len(rest):
                    p, g = rest[i]
                    runs.append((p, g, min(GSHARE - g % GSHARE, len(rest) - i)))
                    i += runs[-1][2]
                cost = [n * (XCOST[blk] if c in widened(p) else 1.0)
                        for p, _, n in runs for c in range(nc - MC[p])]
                n_items = len(cost)
                anch = ANCH[blk]
                fstep = 4 / len(anch)
                n_units = int((len(pops) - last_off - first) / fstep) + 1
                less = [0.0] * n_units
                for lo, hi, w in busy:
                    us = [u for u in range(n_units) if lo <= first + u * fstep < hi]
                    for u in us:
                        less[u] += w / len(us)
                per = (sum(cost) + sum(less)) / n_units
                unit_of, total, used = [], 0.0, 0.0
                for u in range(n_units):
                    total += per - less[u]
                    while len(unit_of) < n_items and (
                            used + cost[len(unit_of)] / 2 < total or u + 1 == n_units):
                        used += cost[len(unit_of)]
                        unit_of.append(u)
                state = [0, -1, 1]

                def gate():
                    u = unit_of[state[0]]
                    state[0] += 1
                    if u != state[1]:
                        state[1] = u
                        state[2] += 1
                        a, h = divmod(anch[u % len(anch)], 2)
                        fence(p_refs[state[2] % 2], first + u // len(anch) * 4 + a, h)
                    return p_refs[state[2] % 2]

            for p, g, n in runs if rest else []:
                if g == 0:
                    for i in range(state[0], n_items):
                        if unit_of[i] != state[1] or state[1] + 1 == n_units:
                            break
                        unit_of[i] += 1
                if p in probs:
                    store_probs(p)
                pv_chain(p, g, gate, n)
            for p in list(probs):
                store_probs(p)
            if end:
                x = y_ref[:, 0:D]
                if y_vpu is not None:
                    x = x + jnp.concatenate([sub_sum(y_vpu[c]) for c in range(DT)], axis=1)
                last_ffn(x, mm, len(pops), links)

        def last_ffn(x, mm, base, links):
            xb, m, r = ln_stats(x)
            lhs = _pack2(xb, xb)
            xcol = [col_bcast(tile_of(xb, kk)) for kk in range(UP_K)]
            links.extend([(base + UX_LINK, _bits_or(xc[LANES - 8:] for xc in xcol))] * 4)
            j0 = 2 * (FT - UP_COLS)
            part = {}
            for j in range(j0, 2 * FT):
                acc = None
                for i in range(8):
                    for kk in range(UP_K):
                        xc = xcol[kk][16 * i:16 * i + 16]
                        acc = vpu_fma(acc, w13[j % 2][8 * kk + i, j // 2], xc[0:8], xc[8:16])
                part[j] = sub_sum(acc)
                links.append((base + int(UP_LINK0 + UP_LINKSTEP * (j - j0)),
                              pltpu.bitcast(part[j], U32)))
            work = [(j, kk) for kk in range(DT) for j in range(UP_KM)]
            work += [(j, kk) for j in range(UP_KM, 2 * FT)
                     for kk in range(UP_K if j in part else 0, DT)]
            for j, kk in work:
                part[j] = _add(part.get(j), mm(tile_of(lhs, kk),
                                               _rhs(w13[j % 2], 8 * kk, j // 2))[0:8])
            gu = [(part[j] - m * cs_ref[j]) * r for j in range(2 * FT)]
            hs = [_swiglu(g, u) for g, u in zip(gu[0::2], gu[1::2])]
            cols = [tile_of(x, c) for c in range(DT)]
            for kk in range(DOWN_K, FT):
                hh = _pack2(hs[kk], hs[kk])
                for c in range(DT):
                    cols[c] = cols[c] + mm(hh, _rhs(w232, 8 * kk, c))[0:8]
            hcol = [col_bcast(hs[kk].astype(BF).astype(F32)) for kk in range(DOWN_K)]
            acc = [None] * DT
            for i in range(8):
                for kk in range(DOWN_K):
                    for c in range(DT):
                        acc[c] = vpu_fma(acc[c], w232[8 * kk + i, c],
                                         hcol[kk][16 * i:16 * i + 8],
                                         hcol[kk][16 * i + 8:16 * i + 16])
            cols = [cc + sub_sum(a) for cc, a in zip(cols, acc)]
            o_ref[...] = jnp.concatenate(cols, axis=1)[0:1].astype(o_ref.dtype)

        blocks = _plan(nc)
        for b, plan in enumerate(blocks):
            end = b == len(blocks) - 1
            if b > 0:
                wait(marker if end else n_ring + b - 1)
            if b == 1:
                start_dma(late)
            if b == 2:
                wait(late)
            run_block(b, *plan, b == 0, end)

    return kernel


@jax.jit
def pallas_interleave_layers__sliding_block_cached__glu_gated_swiglu__decode_kernel(
    A_x: jax.Array,
    A_k_cache: jax.Array,
    A_v_cache: jax.Array,
    A_wq: jax.Array,
    A_wo: jax.Array,
    B_x: jax.Array,
    B_w1: jax.Array,
    B_w3: jax.Array,
    B_w2: jax.Array,
):
    sk = A_k_cache.shape[2]
    win = min(4096, max(256, sk // 4))
    nt_total, nc = sk // LANES, win // LANES

    def kv_view(a):
        return _tile_view(jnp.swapaxes(a, 2, 3).reshape(H * DH, sk))

    def view4(t):
        return t.reshape(t.shape[0] // 4, 2, 4, t.shape[2], 8, LANES)

    def wbuf(r, c):
        return pltpu.VMEM((r // 16, c // LANES, 16, LANES), BF)

    def wbuf4(r, c):
        return pltpu.VMEM((r // 64, 4, c // LANES, 16, LANES), BF)

    any_spec = pl.BlockSpec(memory_space=pl.ANY)
    out = pl.pallas_call(
        _make_kernel(nt_total, nc),
        out_shape=jax.ShapeDtypeStruct((1, D), A_x.dtype),
        in_specs=[any_spec] * 8,
        out_specs=pl.BlockSpec(memory_space=pltpu.VMEM),
        scratch_shapes=[
            wbuf(H * DH, win), wbuf4(H * DH, win),
            wbuf(D, H * DH), wbuf4(H * DH, D),
            wbuf(D, F), wbuf(D, F), wbuf(F, D),
            pltpu.VMEM((NP - 1, NVX, PG, 8, LANES), U32),
            pltpu.VMEM((len(XMORE) - 4, PG, 8, LANES), U32),
            pltpu.VMEM((2 * PG, 8, LANES), U32),
            pltpu.VMEM((RING, 12, 8, LANES), U32),
            pltpu.VMEM((RING, nc // 4, 8, LANES), F32),
            pltpu.VMEM((PRING * 2 * nc + 32, LANES), F32),
            pltpu.VMEM((PRING * 2 * nc + 32, LANES), F32),
            pltpu.VMEM((RING, nc // 4, 8, LANES), U32),
            pltpu.VMEM((NP, 8, LANES), F32),
            pltpu.VMEM((NP, 8, PW), F32),
            pltpu.VMEM((NP, 8, PW), U32),
            pltpu.VMEM((16, 8, LANES), U32),
            pltpu.VMEM((2 * FT, 8, LANES), F32),
            pltpu.VMEM((16, 8, LANES), U32),
            pltpu.VMEM((8, 1024), U32),
            pltpu.VMEM((8, 1024), F32),
            pltpu.VMEM((1, D), BF),
            pltpu.SemaphoreType.DMA((NSEM,)),
        ],
        compiler_params=pltpu.CompilerParams(
            vmem_limit_bytes=128 * 1024 * 1024),
    )(A_x.reshape(1, D), kv_view(A_k_cache), view4(kv_view(A_v_cache)),
      _tile_view(A_wq), view4(_tile_view(A_wo)),
      _tile_view(B_w1), _tile_view(B_w3), _tile_view(B_w2))
    return out.reshape(A_x.shape)
```
